```python
import jax
import jax.numpy as jnp

def _softmax(x, axis=-1):
    return jax.nn.softmax(x, axis=axis)
def _gelu(x):
    return jax.nn.gelu(x, approximate=True)
def _silu(x):
    return jax.nn.silu(x)
def _sigmoid(x):
    return jax.nn.sigmoid(x)
def _layernorm(x, axis=-1, eps=1e-5):
    m = jnp.mean(x, axis=axis, keepdims=True)
    v = jnp.var(x, axis=axis, keepdims=True)
    return (x - m) / jnp.sqrt(v + eps)
def _scatter_add(tgt, idx, src, axis=0):
    return tgt.at[idx].add(src)
def _segment_sum(src, seg, n):
    return jax.ops.segment_sum(src, seg, n)
class _Rng:
    def __init__(self, key):
        self._k = key
    def _next(self):
        self._k, sub = jax.random.split(self._k)
        return sub
    def normal(self, shape):
        return jax.random.normal(self._next(), shape, dtype=jnp.bfloat16)
    def randint(self, lo, hi, shape):
        return jax.random.randint(self._next(), shape, lo, hi, dtype=jnp.int32)
    def uniform(self, shape, lo=0.0, hi=1.0):
        return jax.random.uniform(self._next(), shape, jnp.bfloat16, lo, hi)
    def permutation(self, n):
        return jax.random.permutation(self._next(), n)


kernel_name = 'concat_heads__sliding_block_cached__compressed_kv_cla__decode'

def setup_inputs():
    _rng = _Rng(jax.random.key(int.from_bytes(__import__("os").urandom(4), "little")))
    _w = (lambda a: (lambda t: t.astype(jnp.bfloat16) if jnp.issubdtype(t.dtype, jnp.floating) else t)(jnp.asarray(a)))
    def _A_setup():
        B, Sq, D = 4, 1, 512
        Hq, Hkv, Sk, Dh = 32, 32, 4096, 128
        assert Hq % Hkv == 0, (Hq, Hkv)
        return {
            "x": _w((lambda *s: _rng.normal(s) * 0.05)(B, Sq, D)),
            "k_cache": _w((lambda *s: _rng.normal(s) * 0.05)(B, Hkv, Sk, Dh)),
            "v_cache": _w((lambda *s: _rng.normal(s) * 0.05)(B, Hkv, Sk, Dh)),
            "wq": _w((lambda *s: _rng.normal(s) * 0.05)(D, Hq * Dh) * (D ** -0.5)),
            "wo": _w((lambda *s: _rng.normal(s) * 0.05)(Hq * Dh, D) * ((Hq * Dh) ** -0.5)),
        }
    _A_in = _A_setup()

    def _B_setup():
        B, H, Sq, Sk, D, M = 4, 32, 1, 4096, 128, 512
        Dc = 4 * D
        return {
            "x": _w((lambda *s: _rng.normal(s) * 0.05)(B, Sq, M)),
            "c_kv": _w((lambda *s: _rng.normal(s) * 0.05)(B, Sk, Dc)),
            "w_q": _w((lambda *s: _rng.normal(s) * 0.05)(M, H, D) * (M ** -0.5)),
            "w_uk": _w((lambda *s: _rng.normal(s) * 0.05)(Dc, H, D) * (Dc ** -0.5)),
            "w_uv": _w((lambda *s: _rng.normal(s) * 0.05)(Dc, H, D) * (Dc ** -0.5)),
            "w_o": _w((lambda *s: _rng.normal(s) * 0.05)(H, D, M) * ((H * D) ** -0.5)),
        }
    _B_in = _B_setup()

    return {
        "A_x": _A_in["x"],
        "A_k_cache": _A_in["k_cache"],
        "A_v_cache": _A_in["v_cache"],
        "A_wq": _A_in["wq"],
        "A_wo": _A_in["wo"],
        "B_x": _B_in["x"],
        "B_c_kv": _B_in["c_kv"],
        "B_w_q": _B_in["w_q"],
        "B_w_uk": _B_in["w_uk"],
        "B_w_uv": _B_in["w_uv"],
        "B_w_o": _B_in["w_o"],
    }

def reference(A_x, A_k_cache, A_v_cache, A_wq, A_wo, B_x, B_c_kv, B_w_q, B_w_uk, B_w_uv, B_w_o):
    def _A_ref(x, k_cache, v_cache, wq, wo):
        B, Sq, D = x.shape
        Hq, Dh = 32, 128
        Hkv, Sk = k_cache.shape[1], k_cache.shape[2]
        W = min(4096, max(256, Sk // 4))
        rep = Hq // Hkv
        q = (lambda x, *d: x.transpose(*d))((x @ wq).reshape(B, Sq, Hq, Dh), 0, 2, 1, 3)
        k = jnp.repeat(k_cache[:, :, Sk - W:, :], rep, axis=1)
        v = jnp.repeat(v_cache[:, :, Sk - W:, :], rep, axis=1)
        scores = jnp.einsum("bhqd,bhkd->bhqk", q, k) * (Dh ** -0.5)
        p = _softmax(scores, axis=-1)
        o = jnp.einsum("bhqk,bhkd->bhqd", p, v)
        return (lambda x, *d: x.transpose(*d))(o, 0, 2, 1, 3).reshape(B, Sq, Hq * Dh) @ wo

    def _B_ref(x, c_kv, w_q, w_uk, w_uv, w_o):
        B, Sq, M = x.shape[0], x.shape[1], x.shape[2]
        Sk = c_kv.shape[1]
        H, D = w_q.shape[1], w_q.shape[2]
        q = jnp.einsum("bqm,mhd->bhqd", x, w_q)
        k = jnp.einsum("bkc,chd->bhkd", c_kv, w_uk)
        v = jnp.einsum("bkc,chd->bhkd", c_kv, w_uv)
        scores = jnp.einsum("bhqd,bhkd->bhqk", q, k) * (D ** -0.5)
        off = Sk - Sq
        qi = jnp.arange(Sq)[:, None]
        kj = jnp.arange(Sk)[None, :]
        cmask = kj <= (qi + off)
        scores = jnp.where(cmask[None, None], scores, -1e9)
        p = _softmax(scores, axis=-1)
        ctx = jnp.einsum("bhqk,bhkd->bhqd", p, v)
        return jnp.einsum("bhqd,hdm->bqm", ctx, w_o)

    a = _A_ref(A_x, A_k_cache, A_v_cache, A_wq, A_wo)
    b = _B_ref(B_x, B_c_kv, B_w_q, B_w_uk, B_w_uv, B_w_o)
    return jnp.concatenate([a, b], axis=-1)
```

```python
import jax
import jax.numpy as jnp
from jax import lax
import jax.experimental.pallas as pl
import jax.experimental.pallas.tpu as pltpu

_NT = (((1,), (1,)), ((), ()))
_F32 = jnp.float32
_BF16 = jnp.bfloat16

_L = 128
_G = 8
_WO_CHUNKS = (2560, 1024, 384, 128)


def _dot(a, b):
    return jnp.dot(a, b, preferred_element_type=_F32)


def _dot_nt(a, b):
    return lax.dot_general(a, b, _NT, preferred_element_type=_F32)


@jax.jit
def pallas_concat_heads__sliding_block_cached__compressed_kv_cla__decode_kernel(
    A_x: jax.Array,
    A_k_cache: jax.Array,
    A_v_cache: jax.Array,
    A_wq: jax.Array,
    A_wo: jax.Array,
    B_x: jax.Array,
    B_c_kv: jax.Array,
    B_w_q: jax.Array,
    B_w_uk: jax.Array,
    B_w_uv: jax.Array,
    B_w_o: jax.Array,
):
    B, Sq, D = A_x.shape
    _, H, Sk, Dh = A_k_cache.shape
    assert Sq == 1 and B_x.shape[1] == 1
    assert A_wq.shape == (D, H * Dh)
    W = min(4096, max(256, Sk // 4))
    M, Hb, Db = B_w_q.shape
    Skb, Dc = B_c_kv.shape[1], B_c_kv.shape[2]
    BH = B * H
    NG = BH // _G
    NCT = Dc // _L
    scale_a = float(Dh) ** -0.5
    scale_b = float(Db) ** -0.5
    assert sum(_WO_CHUNKS) == H * Dh

    k3 = A_k_cache.reshape(BH, Sk, Dh)
    v3 = A_v_cache.reshape(BH, Sk, Dh)
    wob2 = B_w_o.reshape(Hb * Db, M)
    xa2 = A_x.reshape(B, D)
    xb2 = B_x.reshape(B, M)

    n_wo = len(_WO_CHUNKS)
    wo_off = [sum(_WO_CHUNKS[:i]) for i in range(n_wo)]
    S_XB, S_XA, S_WQB, S_WUK, S_WUV, S_WOB, S_WQA = range(7)
    S_C = 7
    S_KV = S_C + B
    S_WO = S_KV + 2 * NG
    n_sem = S_WO + n_wo

    def kernel(xa_h, k_h, v_h, wqa_h, woa_h, xb_h, c_h, wqb_h, wuk_h, wuv_h, wob_h,
               o_ref,
               xa_s, xb_s, k_s, v_s, wqa_s, woa_s, c_s, wqb_s, wuk_s, wuv_s, wob_s,
               qa_s, oa_s, qabs_s, ctx_s, sem):
        def cp(src, dst, s):
            return pltpu.make_async_copy(src, dst, sem.at[s])

        c_xb = cp(xb_h, xb_s, S_XB)
        c_xa = cp(xa_h, xa_s, S_XA)
        c_wqb = cp(wqb_h, wqb_s, S_WQB)
        c_wuk = cp(wuk_h, wuk_s, S_WUK)
        c_wuv = cp(wuv_h, wuv_s, S_WUV)
        c_wob = cp(wob_h, wob_s, S_WOB)
        c_wqa = cp(wqa_h, wqa_s, S_WQA)

        def c_c(b):
            return cp(c_h.at[b], c_s.at[b], S_C + b)

        def c_k(g):
            return cp(k_h.at[pl.ds(g * _G, _G), pl.ds(Sk - W, W), :], k_s.at[g], S_KV + 2 * g)

        def c_v(g):
            return cp(v_h.at[pl.ds(g * _G, _G), pl.ds(Sk - W, W), :], v_s.at[g], S_KV + 2 * g + 1)

        def c_wo(i):
            rows = pl.ds(wo_off[i], _WO_CHUNKS[i])
            return cp(woa_h.at[rows, :], woa_s.at[rows, :], S_WO + i)

        c_wqb.start()
        c_xb.start()
        c_xa.start()
        c_wuk.start()
        for b in range(B):
            c_c(b).start()
        c_wuv.start()
        c_wob.start()
        c_wqa.start()
        for g in range(NG):
            c_k(g).start()
            c_v(g).start()
        for i in range(n_wo):
            c_wo(i).start()

        c_wqb.wait()
        c_xb.wait()
        xb = xb_s[...]
        qb = _dot(xb, wqb_s[...].reshape(M, Hb * Db)) * scale_b
        qb = qb.astype(_BF16)
        c_wuk.wait()
        wuk = wuk_s[...].reshape(Dc, Hb * Db)
        for h in range(Hb):
            sl = slice(h * Db, (h + 1) * Db)
            r = _dot_nt(qb[:, sl], wuk[:, sl])
            for t in range(NCT):
                qabs_s[t, pl.ds(h, B, stride=Hb), :] = r[:, t * _L:(t + 1) * _L]

        def b_body(b, carry):
            c_c(b).wait()
            rows = pl.ds(pl.multiple_of(b * Hb, Hb), Hb)
            qa = jnp.concatenate(
                [qabs_s[t, rows, :] for t in range(NCT)], axis=1).astype(_BF16)
            s = _dot_nt(qa, c_s[b])
            m = jnp.max(s, axis=-1, keepdims=True)
            p = jnp.exp(s - m)
            l = jnp.sum(p, axis=-1, keepdims=True)
            cc = _dot(p.astype(_BF16), c_s[b]) / l
            for t in range(NCT):
                ctx_s[t, rows, :] = cc[:, t * _L:(t + 1) * _L]
            return carry

        lax.fori_loop(0, B, b_body, 0)

        c_wuv.wait()
        wuv = wuv_s[...].reshape(Dc, Hb * Db)
        parts = []
        for h in range(Hb):
            ch = jnp.concatenate(
                [ctx_s[t, pl.ds(h, B, stride=Hb), :] for t in range(NCT)],
                axis=1).astype(_BF16)
            parts.append(_dot(ch, wuv[:, h * Db:(h + 1) * Db]))
        ctx = jnp.concatenate(parts, axis=1).astype(_BF16)
        c_wob.wait()
        out_b = _dot(ctx, wob_s[...])
        o_ref[:, D:] = out_b.astype(o_ref.dtype)

        c_wqa.wait()
        c_xa.wait()
        xa = xa_s[...]
        qa_all = _dot(xa, wqa_s[...]) * scale_a
        for h in range(H):
            qa_s[pl.ds(h, B, stride=H), :] = qa_all[:, h * Dh:(h + 1) * Dh]

        def a_body(g, carry):
            rows = pl.ds(pl.multiple_of(g * _G, _G), _G)
            q8 = qa_s[rows, :].astype(_BF16)
            c_k(g).wait()
            row = lax.broadcasted_iota(jnp.int32, (_G, W), 0)
            s = None
            for j in range(_G):
                sj = _dot_nt(q8, k_s[g, j])
                s = sj if s is None else jnp.where(row == j, sj, s)
            m = jnp.max(s, axis=-1, keepdims=True)
            p = jnp.exp(s - m)
            l = jnp.sum(p, axis=-1, keepdims=True)
            pb = p.astype(_BF16)
            c_v(g).wait()
            row2 = lax.broadcasted_iota(jnp.int32, (_G, Dh), 0)
            o = None
            for j in range(_G):
                oj = _dot(pb, v_s[g, j])
                o = oj if o is None else jnp.where(row2 == j, oj, o)
            oa_s[rows, :] = o / l
            return carry

        lax.fori_loop(0, NG, a_body, 0)

        oa = jnp.concatenate(
            [oa_s[pl.ds(h, B, stride=H), :] for h in range(H)], axis=1).astype(_BF16)
        acc = None
        for i in range(n_wo):
            c_wo(i).wait()
            lo, n = wo_off[i], _WO_CHUNKS[i]
            part = _dot(oa[:, lo:lo + n], woa_s[lo:lo + n, :])
            acc = part if acc is None else acc + part
        o_ref[:, :D] = acc.astype(o_ref.dtype)

    any_spec = pl.BlockSpec(memory_space=pl.ANY)
    out = pl.pallas_call(
        kernel,
        out_shape=jax.ShapeDtypeStruct((B, D + M), A_x.dtype),
        in_specs=[any_spec] * 11,
        out_specs=pl.BlockSpec(memory_space=pltpu.VMEM),
        scratch_shapes=[
            pltpu.VMEM(xa2.shape, _BF16),
            pltpu.VMEM(xb2.shape, _BF16),
            pltpu.VMEM((NG, _G, W, Dh), _BF16),
            pltpu.VMEM((NG, _G, W, Dh), _BF16),
            pltpu.VMEM(A_wq.shape, _BF16),
            pltpu.VMEM(A_wo.shape, _BF16),
            pltpu.VMEM(B_c_kv.shape, _BF16),
            pltpu.VMEM(B_w_q.shape, _BF16),
            pltpu.VMEM(B_w_uk.shape, _BF16),
            pltpu.VMEM(B_w_uv.shape, _BF16),
            pltpu.VMEM(wob2.shape, _BF16),
            pltpu.VMEM((BH, Dh), _F32),
            pltpu.VMEM((BH, Dh), _F32),
            pltpu.VMEM((NCT, B * Hb, _L), _F32),
            pltpu.VMEM((NCT, B * Hb, _L), _F32),
            pltpu.SemaphoreType.DMA((n_sem,)),
        ],
        compiler_params=pltpu.CompilerParams(
            vmem_limit_bytes=120 * 1024 * 1024,
            disable_semaphore_checks=True,
        ),
        name="fused_decode",
    )(xa2, k3, v3, A_wq, A_wo, xb2, B_c_kv, B_w_q, B_w_uk, B_w_uv, wob2)
    return out.reshape(B, Sq, D + M)
```

```python
import jax
import jax.numpy as jnp
from jax import lax
import jax.experimental.pallas as pl
import jax.experimental.pallas.tpu as pltpu

_NT = (((1,), (1,)), ((), ()))
_F32 = jnp.float32
_BF16 = jnp.bfloat16

_L = 128
_G = 8
_WO_CHUNKS = (2560, 1024, 384, 128)
_LOOKAHEAD = 4
_SIDE_ROWS = 128
_SIDE_N = 25
_SIDE_NB = 4


def _dot(a, b):
    return jnp.dot(a, b, preferred_element_type=_F32)


def _dot_nt(a, b):
    return lax.dot_general(a, b, _NT, preferred_element_type=_F32)


@jax.jit
def pallas_concat_heads__sliding_block_cached__compressed_kv_cla__decode_kernel(
    A_x: jax.Array,
    A_k_cache: jax.Array,
    A_v_cache: jax.Array,
    A_wq: jax.Array,
    A_wo: jax.Array,
    B_x: jax.Array,
    B_c_kv: jax.Array,
    B_w_q: jax.Array,
    B_w_uk: jax.Array,
    B_w_uv: jax.Array,
    B_w_o: jax.Array,
):
    B, Sq, D = A_x.shape
    _, H, Sk, Dh = A_k_cache.shape
    assert Sq == 1 and B_x.shape[1] == 1
    assert A_wq.shape == (D, H * Dh)
    W = min(4096, max(256, Sk // 4))
    M, Hb, Db = B_w_q.shape
    Skb, Dc = B_c_kv.shape[1], B_c_kv.shape[2]
    BH = B * H
    NG = BH // _G
    NCT = Dc // _L
    scale_a = float(Dh) ** -0.5
    scale_b = float(Db) ** -0.5
    assert sum(_WO_CHUNKS) == H * Dh
    assert _SIDE_N <= 5 + B + NG

    k3 = A_k_cache.reshape(BH, Sk, Dh)
    v3 = A_v_cache.reshape(BH, Sk, Dh)
    wob2 = B_w_o.reshape(Hb * Db, M)
    xa2 = A_x.reshape(B, D)
    xb2 = B_x.reshape(B, M)

    n_wo = len(_WO_CHUNKS)
    wo_off = [sum(_WO_CHUNKS[:i]) for i in range(n_wo)]
    S_XB, S_XA, S_WQB, S_WUK, S_WUV, S_WOB, S_WQA = range(7)
    S_C = 7
    S_KV = S_C + B
    S_WO = S_KV + 2 * NG
    S_SA = S_WO + n_wo
    S_SB = S_SA + _SIDE_NB
    n_sem = S_SB + _SIDE_NB
    side_total = _SIDE_ROWS * _SIDE_N

    def kernel(xa_h, k_h, v_h, wqa_h, woa_h, xb_h, c_h, wqb_h, wuk_h, wuv_h, wob_h,
               o_ref,
               xa_s, xb_s, k_s, v_s, wqa_s, woa_s, c_s, wqb_s, wuk_s, wuv_s, wob_s,
               qa_s, oa_s, qabs_s, ctx_s, acc_s, ctxb_s, side_s, sem):
        def cp(src, dst, s):
            return pltpu.make_async_copy(src, dst, sem.at[s])

        c_xb = cp(xb_h, xb_s, S_XB)
        c_xa = cp(xa_h, xa_s, S_XA)
        c_wqb = cp(wqb_h, wqb_s, S_WQB)
        c_wuk = cp(wuk_h, wuk_s, S_WUK)
        c_wuv = cp(wuv_h, wuv_s, S_WUV)
        rest = pl.ds(side_total, Hb * Db - side_total)
        c_wob = cp(wob_h.at[rest, :], wob_s.at[rest, :], S_WOB)
        c_wqa = cp(wqa_h, wqa_s, S_WQA)

        def c_c(b):
            return cp(c_h.at[b], c_s.at[b], S_C + b)

        def c_k(g):
            return cp(k_h.at[pl.ds(g * _G, _G), pl.ds(Sk - W, W), :], k_s.at[g], S_KV + 2 * g)

        def c_v(g):
            return cp(v_h.at[pl.ds(g * _G, _G), pl.ds(Sk - W, W), :], v_s.at[g], S_KV + 2 * g + 1)

        def c_wo(i):
            rows = pl.ds(wo_off[i], _WO_CHUNKS[i])
            return cp(woa_h.at[rows, :], woa_s.at[rows, :], S_WO + i)

        def side_rows(i):
            start = i * _SIDE_ROWS
            if not isinstance(i, int):
                start = pl.multiple_of(start, 8)
            return pl.ds(start, _SIDE_ROWS)

        def c_sa(i):
            slot = i % _SIDE_NB
            return cp(wob_h.at[side_rows(i), :], side_s.at[slot], S_SA + slot)

        def c_sb(i):
            slot = i % _SIDE_NB
            return cp(side_s.at[slot], wob_s.at[side_rows(i), :], S_SB + slot)

        ahead = _SIDE_NB // 2

        def when(cond, fn):
            if isinstance(cond, bool):
                if cond:
                    fn()
            else:
                pl.when(cond)(fn)

        def tick(i):
            def go():
                c_sa(i).wait()
                c_sb(i).start()
                when(i >= ahead, lambda: c_sb(i - ahead).wait())
                when(i + ahead < _SIDE_N, lambda: c_sa(i + ahead).start())
            when(i < _SIDE_N, go)

        c_wqb.start()
        for i in range(ahead):
            c_sa(i).start()
        c_xb.start()
        c_xa.start()
        c_wuk.start()
        for b in range(B):
            c_c(b).start()
        c_wuv.start()
        c_wob.start()
        c_wqa.start()
        for g in range(_LOOKAHEAD):
            c_k(g).start()
            c_v(g).start()

        tick(0)
        c_wqb.wait()
        tick(1)
        c_xb.wait()
        xb = xb_s[...]
        qb = _dot(xb, wqb_s[...].reshape(M, Hb * Db)) * scale_b
        qb = qb.astype(_BF16)
        c_wuk.wait()
        tick(2)
        wuk = wuk_s[...].reshape(Dc, Hb * Db)
        for h in range(Hb):
            sl = slice(h * Db, (h + 1) * Db)
            r = _dot_nt(qb[:, sl], wuk[:, sl])
            for t in range(NCT):
                qabs_s[t, pl.ds(h, B, stride=Hb), :] = r[:, t * _L:(t + 1) * _L]

        def b_body(b, carry):
            c_c(b).wait()
            tick(3 + b)
            rows = pl.ds(pl.multiple_of(b * Hb, Hb), Hb)
            qa = jnp.concatenate(
                [qabs_s[t, rows, :] for t in range(NCT)], axis=1).astype(_BF16)
            s = _dot_nt(qa, c_s[b])
            m = jnp.max(s, axis=-1, keepdims=True)
            p = jnp.exp(s - m)
            l = jnp.sum(p, axis=-1, keepdims=True)
            cc = _dot(p.astype(_BF16), c_s[b]) / l
            for t in range(NCT):
                ctx_s[t, rows, :] = cc[:, t * _L:(t + 1) * _L]
            return carry

        lax.fori_loop(0, B, b_body, 0)

        c_wuv.wait()
        tick(3 + B)
        wuv = wuv_s[...].reshape(Dc, Hb * Db)
        parts = []
        for h in range(Hb):
            ch = jnp.concatenate(
                [ctx_s[t, pl.ds(h, B, stride=Hb), :] for t in range(NCT)],
                axis=1).astype(_BF16)
            parts.append(_dot(ch, wuv[:, h * Db:(h + 1) * Db]))
        ctxb_s[...] = jnp.concatenate(parts, axis=1)

        c_wqa.wait()
        tick(4 + B)
        c_xa.wait()
        xa = xa_s[...]
        qa_all = _dot(xa, wqa_s[...]) * scale_a
        for h in range(H):
            qa_s[pl.ds(h, B, stride=H), :] = qa_all[:, h * Dh:(h + 1) * Dh]

        def a_body(g, carry):
            rows = pl.ds(pl.multiple_of(g * _G, _G), _G)
            q8 = qa_s[rows, :].astype(_BF16)
            c_k(g).wait()
            tick(5 + B + g)

            @pl.when(g + _LOOKAHEAD < NG)
            def _():
                c_k(g + _LOOKAHEAD).start()
                c_v(g + _LOOKAHEAD).start()

            @pl.when(g + _LOOKAHEAD == NG)
            def _():
                for i in range(n_wo):
                    c_wo(i).start()

            row = lax.broadcasted_iota(jnp.int32, (_G, W), 0)
            s = None
            for j in range(_G):
                sj = _dot_nt(q8, k_s[g, j])
                s = sj if s is None else jnp.where(row == j, sj, s)
            m = jnp.max(s, axis=-1, keepdims=True)
            p = jnp.exp(s - m)
            l = jnp.sum(p, axis=-1, keepdims=True)
            pb = p.astype(_BF16)
            c_v(g).wait()
            row2 = lax.broadcasted_iota(jnp.int32, (_G, Dh), 0)
            o = None
            for j in range(_G):
                oj = _dot(pb, v_s[g, j])
                o = oj if o is None else jnp.where(row2 == j, oj, o)
            oa_s[rows, :] = o / l
            return carry

        lax.fori_loop(0, NG, a_body, 0)

        c_wob.wait()
        for i in range(_SIDE_N - ahead, _SIDE_N):
            c_sb(i).wait()
        o_ref[:, D:] = _dot(ctxb_s[...].astype(_BF16), wob_s[...]).astype(o_ref.dtype)

        oa = jnp.concatenate(
            [oa_s[pl.ds(h, B, stride=H), :] for h in range(H)], axis=1).astype(_BF16)
        for i in range(n_wo):
            c_wo(i).wait()
            lo, n = wo_off[i], _WO_CHUNKS[i]
            part = _dot(oa[:, lo:lo + n], woa_s[lo:lo + n, :])
            if i > 0:
                part = part + acc_s[...]
            if i < n_wo - 1:
                acc_s[...] = part
            else:
                o_ref[:, :D] = part.astype(o_ref.dtype)

    any_spec = pl.BlockSpec(memory_space=pl.ANY)
    out = pl.pallas_call(
        kernel,
        out_shape=jax.ShapeDtypeStruct((B, D + M), A_x.dtype),
        in_specs=[any_spec] * 11,
        out_specs=pl.BlockSpec(memory_space=pltpu.VMEM),
        scratch_shapes=[
            pltpu.VMEM(xa2.shape, _BF16),
            pltpu.VMEM(xb2.shape, _BF16),
            pltpu.VMEM((NG, _G, W, Dh), _BF16),
            pltpu.VMEM((NG, _G, W, Dh), _BF16),
            pltpu.VMEM(A_wq.shape, _BF16),
            pltpu.VMEM(A_wo.shape, _BF16),
            pltpu.VMEM(B_c_kv.shape, _BF16),
            pltpu.VMEM(B_w_q.shape, _BF16),
            pltpu.VMEM(B_w_uk.shape, _BF16),
            pltpu.VMEM(B_w_uv.shape, _BF16),
            pltpu.VMEM(wob2.shape, _BF16),
            pltpu.VMEM((BH, Dh), _F32),
            pltpu.VMEM((BH, Dh), _F32),
            pltpu.VMEM((NCT, B * Hb, _L), _F32),
            pltpu.VMEM((NCT, B * Hb, _L), _F32),
            pltpu.VMEM((B, D), _F32),
            pltpu.VMEM((B, Hb * Db), _F32),
            pltpu.SMEM((_SIDE_NB, _SIDE_ROWS, M), _BF16),
            pltpu.SemaphoreType.DMA((n_sem,)),
        ],
        compiler_params=pltpu.CompilerParams(
            vmem_limit_bytes=120 * 1024 * 1024,
            disable_semaphore_checks=True,
        ),
        name="fused_decode",
    )(xa2, k3, v3, A_wq, A_wo, xb2, B_c_kv, B_w_q, B_w_uk, B_w_uv, wob2)
    return out.reshape(B, Sq, D + M)
```

```python
import functools

import jax
import jax.numpy as jnp
from jax import lax
import jax.experimental.pallas as pl
import jax.experimental.pallas.tpu as pltpu

_NT = (((1,), (1,)), ((), ()))
_F32 = jnp.float32
_BF16 = jnp.bfloat16
_L = 128
_G = 8
_KIB = 1024

_CFG = dict(
    wo_chunks=(2560, 1024, 384, 128),
    piece=64 * _KIB,
    shift=32 * _KIB,
    block=512 * _KIB,
    side_rows=128,
    side_n=25,
    side_nb=4,
)


def _dot(a, b):
    return jnp.dot(a, b, preferred_element_type=_F32)


def _dot_nt(a, b):
    return lax.dot_general(a, b, _NT, preferred_element_type=_F32)


def _bounds(n_rows, row_bytes, piece, shift):
    step = piece // row_bytes
    first = (shift // row_bytes) % step
    cuts = [0] + [r for r in range(first, n_rows, step) if r > 0] + [n_rows]
    return list(zip(cuts[:-1], cuts[1:]))


def _fused(cfg, A_x, A_k_cache, A_v_cache, A_wq, A_wo, B_x, B_c_kv, B_w_q, B_w_uk, B_w_uv, B_w_o):
    B, Sq, D = A_x.shape
    _, H, Sk, Dh = A_k_cache.shape
    assert Sq == 1 and B_x.shape[1] == 1
    assert A_wq.shape == (D, H * Dh)
    W = min(4096, max(256, Sk // 4))
    M, Hb, Db = B_w_q.shape
    Skb, Dc = B_c_kv.shape[1], B_c_kv.shape[2]
    BH = B * H
    NG = BH // _G
    NCT = Dc // _L
    scale_a = float(Dh) ** -0.5
    scale_b = float(Db) ** -0.5
    wo_chunks = cfg["wo_chunks"]
    piece, shift, block = cfg["piece"], cfg["shift"], cfg["block"]
    side_rows, side_n, side_nb = cfg["side_rows"], cfg["side_n"], cfg["side_nb"]
    assert sum(wo_chunks) == H * Dh
    assert side_n <= 5 + B + NG

    xa2 = A_x.reshape(B, D)
    xb2 = B_x.reshape(B, M)
    k3 = A_k_cache.reshape(BH, Sk, Dh)
    v3 = A_v_cache.reshape(BH, Sk, Dh)
    wob2 = B_w_o.reshape(Hb * Db, M)

    def blocked(w, lead=0):
        row_bytes = 2 * functools.reduce(lambda a, b: a * b, w.shape[lead + 1:], 1)
        rows = block // row_bytes
        shape = w.shape[:lead] + (w.shape[lead] // rows, rows) + w.shape[lead + 1:]
        return w.reshape(shape), rows, row_bytes

    wqa3, r_wqa, b_wqa = blocked(A_wq)
    wqb4, r_wqb, b_wqb = blocked(B_w_q)
    wuk4, r_wu, b_wu = blocked(B_w_uk)
    wuv4, _, _ = blocked(B_w_uv)
    c4, r_c, b_c = blocked(B_c_kv, 1)
    cut_wqa = _bounds(r_wqa, b_wqa, max(piece, 8 * b_wqa), 0)
    cut_wqb = _bounds(r_wqb, b_wqb, piece, shift)
    cut_wu = _bounds(r_wu, b_wu, piece, shift)
    cut_c = _bounds(r_c, b_c, piece, shift)
    cut_kv = _bounds(W, 2 * Dh, piece, shift)

    n_wo = len(wo_chunks)
    wo_off = [sum(wo_chunks[:i]) for i in range(n_wo)]
    S_XB, S_XA, S_WQB, S_WUK, S_WUV, S_WOB, S_WQA = range(7)
    S_C = 7
    S_KV = S_C + B
    S_WO = S_KV + 2 * NG
    S_SA = S_WO + n_wo
    S_SB = S_SA + side_nb
    n_sem = S_SB + side_nb
    side_total = side_rows * side_n

    def kernel(xa_h, k_h, v_h, wqa_h, woa_h, xb_h, c_h, wqb_h, wuk_h, wuv_h, wob_h,
               o_ref,
               xa_s, xb_s, k_s, v_s, wqa_s, woa_s, c_s, wqb_s, wuk_s, wuv_s, wob_s,
               qa_s, oa_s, qabs_s, ctx_s, acc_s, ctxb_s, side_s, sem):
        def cp(src, dst, s):
            return pltpu.make_async_copy(src, dst, sem.at[s])

        def start_pieces(src, dst, cuts, s, row0=0):
            for lo, hi in cuts:
                cp(src.at[:, pl.ds(row0 + lo, hi - lo)], dst.at[:, pl.ds(lo, hi - lo)], s).start()

        def wait_all(dst, s):
            cp(dst, dst, s).wait()

        c_xb = cp(xb_h, xb_s, S_XB)
        c_xa = cp(xa_h, xa_s, S_XA)
        rest = pl.ds(side_total, Hb * Db - side_total)
        c_wob = cp(wob_h.at[rest, :], wob_s.at[rest, :], S_WOB)

        def start_c(b):
            start_pieces(c_h.at[b], c_s.at[b], cut_c, S_C + b)

        def start_kv(g):
            heads = pl.ds(g * _G, _G)
            start_pieces(k_h.at[heads], k_s.at[g], cut_kv, S_KV + 2 * g, Sk - W)
            start_pieces(v_h.at[heads], v_s.at[g], cut_kv, S_KV + 2 * g + 1, Sk - W)

        def c_wo(i):
            rows = pl.ds(wo_off[i], wo_chunks[i])
            return cp(woa_h.at[rows, :], woa_s.at[rows, :], S_WO + i)

        def side_slice(i):
            start = i * side_rows
            if not isinstance(i, int):
                start = pl.multiple_of(start, 8)
            return pl.ds(start, side_rows)

        def c_sa(i):
            slot = i % side_nb
            return cp(wob_h.at[side_slice(i), :], side_s.at[slot], S_SA + slot)

        def c_sb(i):
            slot = i % side_nb
            return cp(side_s.at[slot], wob_s.at[side_slice(i), :], S_SB + slot)

        ahead = side_nb // 2

        def when(cond, fn):
            if isinstance(cond, bool):
                if cond:
                    fn()
            else:
                pl.when(cond)(fn)

        def tick(i):
            def go():
                c_sa(i).wait()
                c_sb(i).start()
                when(i >= ahead, lambda: c_sb(i - ahead).wait())
                when(i + ahead < side_n, lambda: c_sa(i + ahead).start())
            when(i < side_n, go)

        start_pieces(wqb_h, wqb_s, cut_wqb, S_WQB)
        for i in range(ahead):
            c_sa(i).start()
        c_xb.start()
        c_xa.start()
        start_pieces(wuk_h, wuk_s, cut_wu, S_WUK)
        tick(0)

        wait_all(wqb_s, S_WQB)
        start_c(0)
        tick(1)
        c_xb.wait()
        wqb = wqb_s[...].reshape(M, Hb, Db).reshape(M, Hb * Db)
        qb = (_dot(xb_s[...], wqb) * scale_b).astype(_BF16)
        wait_all(wuk_s, S_WUK)
        start_c(1)
        tick(2)
        wuk = wuk_s[...].reshape(Dc, Hb, Db).reshape(Dc, Hb * Db)
        for h in range(Hb):
            sl = slice(h * Db, (h + 1) * Db)
            r = _dot_nt(qb[:, sl], wuk[:, sl])
            for t in range(NCT):
                qabs_s[t, pl.ds(h, B, stride=Hb), :] = r[:, t * _L:(t + 1) * _L]

        def b_body(b, carry):
            wait_all(c_s.at[b], S_C + b)
            pl.when(b + 2 < B)(lambda: start_c(b + 2))
            pl.when(b + 2 == B)(lambda: start_pieces(wuv_h, wuv_s, cut_wu, S_WUV))

            @pl.when(b + 2 == B + 1)
            def _():
                c_wob.start()
                start_pieces(wqa_h, wqa_s, cut_wqa, S_WQA)

            tick(3 + b)
            rows = pl.ds(pl.multiple_of(b * Hb, Hb), Hb)
            qa = jnp.concatenate(
                [qabs_s[t, rows, :] for t in range(NCT)], axis=1).astype(_BF16)
            s = _dot_nt(qa, c_s[b].reshape(Skb, Dc))
            m = jnp.max(s, axis=-1, keepdims=True)
            p = jnp.exp(s - m)
            l = jnp.sum(p, axis=-1, keepdims=True)
            cc = _dot(p.astype(_BF16), c_s[b].reshape(Skb, Dc)) / l
            for t in range(NCT):
                ctx_s[t, rows, :] = cc[:, t * _L:(t + 1) * _L]
            return carry

        lax.fori_loop(0, B, b_body, 0)

        wait_all(wuv_s, S_WUV)
        start_kv(0)
        tick(3 + B)
        wuv = wuv_s[...].reshape(Dc, Hb, Db).reshape(Dc, Hb * Db)
        parts = []
        for h in range(Hb):
            ch = jnp.concatenate(
                [ctx_s[t, pl.ds(h, B, stride=Hb), :] for t in range(NCT)],
                axis=1).astype(_BF16)
            parts.append(_dot(ch, wuv[:, h * Db:(h + 1) * Db]))
        ctxb_s[...] = jnp.concatenate(parts, axis=1)

        wait_all(wqa_s, S_WQA)
        start_kv(1)
        tick(4 + B)
        c_xa.wait()
        qa_all = _dot(xa_s[...], wqa_s[...].reshape(D, H * Dh)) * scale_a
        for h in range(H):
            qa_s[pl.ds(h, B, stride=H), :] = qa_all[:, h * Dh:(h + 1) * Dh]

        def a_body(g, carry):
            rows = pl.ds(pl.multiple_of(g * _G, _G), _G)
            q8 = qa_s[rows, :].astype(_BF16)
            wait_all(k_s.at[g], S_KV + 2 * g)
            pl.when(g + 2 < NG)(lambda: start_kv(g + 2))

            @pl.when(g + 2 == NG)
            def _():
                for i in range(n_wo):
                    c_wo(i).start()

            tick(5 + B + g)
            row = lax.broadcasted_iota(jnp.int32, (_G, W), 0)
            s = None
            for j in range(_G):
                sj = _dot_nt(q8, k_s[g, j])
                s = sj if s is None else jnp.where(row == j, sj, s)
            m = jnp.max(s, axis=-1, keepdims=True)
            p = jnp.exp(s - m)
            l = jnp.sum(p, axis=-1, keepdims=True)
            pb = p.astype(_BF16)
            wait_all(v_s.at[g], S_KV + 2 * g + 1)
            row2 = lax.broadcasted_iota(jnp.int32, (_G, Dh), 0)
            o = None
            for j in range(_G):
                oj = _dot(pb, v_s[g, j])
                o = oj if o is None else jnp.where(row2 == j, oj, o)
            oa_s[rows, :] = o / l
            return carry

        lax.fori_loop(0, NG, a_body, 0)

        c_wob.wait()
        for i in range(max(side_n - ahead, 0), side_n):
            c_sb(i).wait()
        o_ref[:, D:] = _dot(ctxb_s[...].astype(_BF16), wob_s[...]).astype(o_ref.dtype)

        oa = jnp.concatenate(
            [oa_s[pl.ds(h, B, stride=H), :] for h in range(H)], axis=1).astype(_BF16)
        for i in range(n_wo):
            c_wo(i).wait()
            lo, n = wo_off[i], wo_chunks[i]
            part = _dot(oa[:, lo:lo + n], woa_s[lo:lo + n, :])
            if i > 0:
                part = part + acc_s[...]
            if i < n_wo - 1:
                acc_s[...] = part
            else:
                o_ref[:, :D] = part.astype(o_ref.dtype)

    any_spec = pl.BlockSpec(memory_space=pl.ANY)
    out = pl.pallas_call(
        kernel,
        out_shape=jax.ShapeDtypeStruct((B, D + M), A_x.dtype),
        in_specs=[any_spec] * 11,
        out_specs=pl.BlockSpec(memory_space=pltpu.VMEM),
        scratch_shapes=[
            pltpu.VMEM(xa2.shape, _BF16),
            pltpu.VMEM(xb2.shape, _BF16),
            pltpu.VMEM((NG, _G, W, Dh), _BF16),
            pltpu.VMEM((NG, _G, W, Dh), _BF16),
            pltpu.VMEM(wqa3.shape, _BF16),
            pltpu.VMEM(A_wo.shape, _BF16),
            pltpu.VMEM(c4.shape, _BF16),
            pltpu.VMEM(wqb4.shape, _BF16),
            pltpu.VMEM(wuk4.shape, _BF16),
            pltpu.VMEM(wuv4.shape, _BF16),
            pltpu.VMEM(wob2.shape, _BF16),
            pltpu.VMEM((BH, Dh), _F32),
            pltpu.VMEM((BH, Dh), _F32),
            pltpu.VMEM((NCT, B * Hb, _L), _F32),
            pltpu.VMEM((NCT, B * Hb, _L), _F32),
            pltpu.VMEM((B, D), _F32),
            pltpu.VMEM((B, Hb * Db), _F32),
            pltpu.SMEM((side_nb, side_rows, M), _BF16),
            pltpu.SemaphoreType.DMA((n_sem,)),
        ],
        compiler_params=pltpu.CompilerParams(
            vmem_limit_bytes=120 * 1024 * 1024,
            disable_semaphore_checks=True,
        ),
        name="fused_decode",
    )(xa2, k3, v3, wqa3, A_wo, xb2, c4, wqb4, wuk4, wuv4, wob2)
    return out.reshape(B, Sq, D + M)


@jax.jit
def pallas_concat_heads__sliding_block_cached__compressed_kv_cla__decode_kernel(
    A_x: jax.Array,
    A_k_cache: jax.Array,
    A_v_cache: jax.Array,
    A_wq: jax.Array,
    A_wo: jax.Array,
    B_x: jax.Array,
    B_c_kv: jax.Array,
    B_w_q: jax.Array,
    B_w_uk: jax.Array,
    B_w_uv: jax.Array,
    B_w_o: jax.Array,
):
    return _fused(_CFG, A_x, A_k_cache, A_v_cache, A_wq, A_wo,
                  B_x, B_c_kv, B_w_q, B_w_uk, B_w_uv, B_w_o)
```

```python
import functools

import jax
import jax.numpy as jnp
from jax import lax
import jax.experimental.pallas as pl
import jax.experimental.pallas.tpu as pltpu

_NT = (((1,), (1,)), ((), ()))
_F32 = jnp.float32
_BF16 = jnp.bfloat16
_L = 128
_G = 8
_KIB = 1024

_CFG = dict(
    wo_chunks=(2560, 1024, 384, 128),
    piece=64 * _KIB,
    shift=32 * _KIB,
    block=512 * _KIB,
    side_rows=128,
    side_n=25,
    side_last=56,
    side_nb=4,
    side_late=2,
    late_at=1,
)


def _dot(a, b):
    return jnp.dot(a, b, preferred_element_type=_F32)


def _dot_nt(a, b):
    return lax.dot_general(a, b, _NT, preferred_element_type=_F32)


def _bounds(n_rows, row_bytes, piece, shift):
    step = piece // row_bytes
    first = (shift // row_bytes) % step
    cuts = [0] + [r for r in range(first, n_rows, step) if r > 0] + [n_rows]
    return list(zip(cuts[:-1], cuts[1:]))


def _fused(cfg, A_x, A_k_cache, A_v_cache, A_wq, A_wo, B_x, B_c_kv, B_w_q, B_w_uk, B_w_uv, B_w_o):
    B, Sq, D = A_x.shape
    _, H, Sk, Dh = A_k_cache.shape
    assert Sq == 1 and B_x.shape[1] == 1
    assert A_wq.shape == (D, H * Dh)
    W = min(4096, max(256, Sk // 4))
    M, Hb, Db = B_w_q.shape
    Skb, Dc = B_c_kv.shape[1], B_c_kv.shape[2]
    BH = B * H
    NG = BH // _G
    NCT = Dc // _L
    scale_a = float(Dh) ** -0.5
    scale_b = float(Db) ** -0.5
    wo_chunks = cfg["wo_chunks"]
    piece, shift, block = cfg["piece"], cfg["shift"], cfg["block"]
    side_rows, side_n, side_nb = cfg["side_rows"], cfg["side_n"], cfg["side_nb"]
    assert sum(wo_chunks) == H * Dh
    side_late, late_at = cfg["side_late"], cfg["late_at"]
    side_last = cfg["side_last"]
    side_all = side_n + (1 if side_last else 0)
    assert side_all <= 6 + B + NG

    xa2 = A_x.reshape(B, D)
    xb2 = B_x.reshape(B, M)
    k3 = A_k_cache.reshape(BH, Sk, Dh)
    v3 = A_v_cache.reshape(BH, Sk, Dh)
    wob2 = B_w_o.reshape(Hb * Db, M)

    def blocked(w, lead=0):
        row_bytes = 2 * functools.reduce(lambda a, b: a * b, w.shape[lead + 1:], 1)
        rows = block // row_bytes
        shape = w.shape[:lead] + (w.shape[lead] // rows, rows) + w.shape[lead + 1:]
        return w.reshape(shape), rows, row_bytes

    wqa3, r_wqa, b_wqa = blocked(A_wq)
    wqb4, r_wqb, b_wqb = blocked(B_w_q)
    wuk4, r_wu, b_wu = blocked(B_w_uk)
    wuv4, _, _ = blocked(B_w_uv)
    c4, r_c, b_c = blocked(B_c_kv, 1)
    cut_wqa = _bounds(r_wqa, b_wqa, max(piece, 8 * b_wqa), 0)
    cut_wqb = _bounds(r_wqb, b_wqb, piece, shift)
    cut_wu = _bounds(r_wu, b_wu, piece, shift)
    cut_c = _bounds(r_c, b_c, piece, shift)
    cut_kv = _bounds(W, 2 * Dh, piece, shift)

    n_wo = len(wo_chunks)
    wo_off = [sum(wo_chunks[:i]) for i in range(n_wo)]
    S_XB, S_XA, S_WQB, S_WUK, S_WUV, S_WOB, S_WQA = range(7)
    S_C = 7
    S_KV = S_C + B
    S_WO = S_KV + 2 * NG
    S_SA = S_WO + n_wo
    S_SB = S_SA + side_nb
    n_sem = S_SB + side_nb
    side_total = side_rows * side_n + side_last

    def kernel(xa_h, k_h, v_h, wqa_h, woa_h, xb_h, c_h, wqb_h, wuk_h, wuv_h, wob_h,
               o_ref,
               xa_s, xb_s, k_s, v_s, wqa_s, woa_s, c_s, wqb_s, wuk_s, wuv_s, wob_s,
               qa_s, oa_s, qabs_s, ctx_s, acc_s, accb_s, ctxb_s, side_s, sem):
        def cp(src, dst, s):
            return pltpu.make_async_copy(src, dst, sem.at[s])

        def start_pieces(src, dst, cuts, s, row0=0):
            for lo, hi in cuts:
                cp(src.at[:, pl.ds(row0 + lo, hi - lo)], dst.at[:, pl.ds(lo, hi - lo)], s).start()

        def wait_all(dst, s):
            cp(dst, dst, s).wait()

        c_xb = cp(xb_h, xb_s, S_XB)
        c_xa = cp(xa_h, xa_s, S_XA)
        rest = pl.ds(side_total, Hb * Db - side_total)
        c_wob = cp(wob_h.at[rest, :], wob_s.at[rest, :], S_WOB)

        def start_c(b):
            start_pieces(c_h.at[b], c_s.at[b], cut_c, S_C + b)

        def start_kv(g):
            heads = pl.ds(g * _G, _G)
            start_pieces(k_h.at[heads], k_s.at[g], cut_kv, S_KV + 2 * g, Sk - W)
            start_pieces(v_h.at[heads], v_s.at[g], cut_kv, S_KV + 2 * g + 1, Sk - W)

        def c_wo(i):
            rows = pl.ds(wo_off[i], wo_chunks[i])
            return cp(woa_h.at[rows, :], woa_s.at[rows, :], S_WO + i)

        def side_refs(i, last):
            start = i * side_rows
            if not isinstance(i, int):
                start = pl.multiple_of(start, 8)
            n = side_last if last else side_rows
            slot = i % side_nb
            return pl.ds(start, n), side_s.at[slot, pl.ds(0, n)], slot

        def c_sa(i, last=False):
            rows, stage, slot = side_refs(i, last)
            return cp(wob_h.at[rows, :], stage, S_SA + slot)

        def c_sb(i, last=False):
            rows, stage, slot = side_refs(i, last)
            return cp(stage, wob_s.at[rows, :], S_SB + slot)

        ahead = side_nb // 2

        def when(cond, fn):
            if isinstance(cond, bool):
                if cond:
                    fn()
            else:
                pl.when(cond)(fn)

        def tick(i):
            def go():
                c_sa(i).wait()
                c_sb(i).start()
                when(i >= ahead, lambda: c_sb(i - ahead).wait())
                when(i + ahead < side_n, lambda: c_sa(i + ahead).start())
                if side_last:
                    when(i + ahead == side_n, lambda: c_sa(side_n, True).start())
            when(i < side_n, go)

        start_pieces(wqb_h, wqb_s, cut_wqb, S_WQB)
        for i in range(ahead):
            c_sa(i).start()
        c_xb.start()
        c_xa.start()
        start_pieces(wuk_h, wuk_s, cut_wu, S_WUK)
        tick(0)

        wait_all(wqb_s, S_WQB)
        start_c(0)
        tick(1)
        c_xb.wait()
        wqb = wqb_s[...].reshape(M, Hb, Db).reshape(M, Hb * Db)
        qb = (_dot(xb_s[...], wqb) * scale_b).astype(_BF16)
        wait_all(wuk_s, S_WUK)
        start_c(1)
        tick(2)
        wuk = wuk_s[...].reshape(Dc, Hb, Db).reshape(Dc, Hb * Db)
        for h in range(Hb):
            sl = slice(h * Db, (h + 1) * Db)
            r = _dot_nt(qb[:, sl], wuk[:, sl])
            for t in range(NCT):
                qabs_s[t, pl.ds(h, B, stride=Hb), :] = r[:, t * _L:(t + 1) * _L]

        def b_body(b, carry):
            wait_all(c_s.at[b], S_C + b)
            pl.when(b + 2 < B)(lambda: start_c(b + 2))
            pl.when(b + 2 == B)(lambda: start_pieces(wuv_h, wuv_s, cut_wu, S_WUV))

            @pl.when(b + 2 == B + 1)
            def _():
                c_wob.start()
                start_pieces(wqa_h, wqa_s, cut_wqa, S_WQA)

            tick(3 + b)
            rows = pl.ds(pl.multiple_of(b * Hb, Hb), Hb)
            qa = jnp.concatenate(
                [qabs_s[t, rows, :] for t in range(NCT)], axis=1).astype(_BF16)
            s = _dot_nt(qa, c_s[b].reshape(Skb, Dc))
            m = jnp.max(s, axis=-1, keepdims=True)
            p = jnp.exp(s - m)
            l = jnp.sum(p, axis=-1, keepdims=True)
            cc = _dot(p.astype(_BF16), c_s[b].reshape(Skb, Dc)) / l
            for t in range(NCT):
                ctx_s[t, rows, :] = cc[:, t * _L:(t + 1) * _L]
            return carry

        lax.fori_loop(0, B, b_body, 0)

        wait_all(wuv_s, S_WUV)
        start_kv(0)
        tick(3 + B)
        wuv = wuv_s[...].reshape(Dc, Hb, Db).reshape(Dc, Hb * Db)
        parts = []
        for h in range(Hb):
            ch = jnp.concatenate(
                [ctx_s[t, pl.ds(h, B, stride=Hb), :] for t in range(NCT)],
                axis=1).astype(_BF16)
            parts.append(_dot(ch, wuv[:, h * Db:(h + 1) * Db]))
        ctxb_s[...] = jnp.concatenate(parts, axis=1)

        wait_all(wqa_s, S_WQA)
        start_kv(1)
        tick(4 + B)
        c_xa.wait()
        qa_all = _dot(xa_s[...], wqa_s[...].reshape(D, H * Dh)) * scale_a
        for h in range(H):
            qa_s[pl.ds(h, B, stride=H), :] = qa_all[:, h * Dh:(h + 1) * Dh]

        def a_body(g, carry):
            rows = pl.ds(pl.multiple_of(g * _G, _G), _G)
            q8 = qa_s[rows, :].astype(_BF16)
            wait_all(k_s.at[g], S_KV + 2 * g)
            pl.when(g + 2 < NG)(lambda: start_kv(g + 2))

            @pl.when(g + 2 == NG)
            def _():
                for i in range(n_wo):
                    c_wo(i).start()

            tick(5 + B + g)
            row = lax.broadcasted_iota(jnp.int32, (_G, W), 0)
            s = None
            for j in range(_G):
                sj = _dot_nt(q8, k_s[g, j])
                s = sj if s is None else jnp.where(row == j, sj, s)
            m = jnp.max(s, axis=-1, keepdims=True)
            p = jnp.exp(s - m)
            l = jnp.sum(p, axis=-1, keepdims=True)
            pb = p.astype(_BF16)
            wait_all(v_s.at[g], S_KV + 2 * g + 1)
            row2 = lax.broadcasted_iota(jnp.int32, (_G, Dh), 0)
            o = None
            for j in range(_G):
                oj = _dot(pb, v_s[g, j])
                o = oj if o is None else jnp.where(row2 == j, oj, o)
            oa_s[rows, :] = o / l
            return carry

        lax.fori_loop(0, NG, a_body, 0)

        tick(5 + B + NG)
        if side_last:
            c_sa(side_n, True).wait()
            c_sb(side_n, True).start()
        c_wob.wait()
        n_early = side_all - side_late
        waited = side_n - ahead
        for i in range(waited, n_early):
            c_sb(i).wait()
        r_early = n_early * side_rows
        ctxb = ctxb_s[...].astype(_BF16)
        accb_s[...] = (_dot(ctxb[:, :r_early], wob_s[:r_early, :])
                       + _dot(ctxb[:, side_total:], wob_s[side_total:, :]))

        oa = jnp.concatenate(
            [oa_s[pl.ds(h, B, stride=H), :] for h in range(H)], axis=1).astype(_BF16)
        for i in range(n_wo):
            c_wo(i).wait()
            lo, n = wo_off[i], wo_chunks[i]
            part = _dot(oa[:, lo:lo + n], woa_s[lo:lo + n, :])
            if i > 0:
                part = part + acc_s[...]
            if i < n_wo - 1:
                acc_s[...] = part
            else:
                o_ref[:, :D] = part.astype(o_ref.dtype)
            if i == late_at:
                for j in range(max(waited, n_early), side_all):
                    c_sb(j, j == side_n).wait()
                late = _dot(ctxb[:, r_early:side_total], wob_s[r_early:side_total, :])
                o_ref[:, D:] = (accb_s[...] + late).astype(o_ref.dtype)

    any_spec = pl.BlockSpec(memory_space=pl.ANY)
    out = pl.pallas_call(
        kernel,
        out_shape=jax.ShapeDtypeStruct((B, D + M), A_x.dtype),
        in_specs=[any_spec] * 11,
        out_specs=pl.BlockSpec(memory_space=pltpu.VMEM),
        scratch_shapes=[
            pltpu.VMEM(xa2.shape, _BF16),
            pltpu.VMEM(xb2.shape, _BF16),
            pltpu.VMEM((NG, _G, W, Dh), _BF16),
            pltpu.VMEM((NG, _G, W, Dh), _BF16),
            pltpu.VMEM(wqa3.shape, _BF16),
            pltpu.VMEM(A_wo.shape, _BF16),
            pltpu.VMEM(c4.shape, _BF16),
            pltpu.VMEM(wqb4.shape, _BF16),
            pltpu.VMEM(wuk4.shape, _BF16),
            pltpu.VMEM(wuv4.shape, _BF16),
            pltpu.VMEM(wob2.shape, _BF16),
            pltpu.VMEM((BH, Dh), _F32),
            pltpu.VMEM((BH, Dh), _F32),
            pltpu.VMEM((NCT, B * Hb, _L), _F32),
            pltpu.VMEM((NCT, B * Hb, _L), _F32),
            pltpu.VMEM((B, D), _F32),
            pltpu.VMEM((B, M), _F32),
            pltpu.VMEM((B, Hb * Db), _F32),
            pltpu.SMEM((side_nb, side_rows, M), _BF16),
            pltpu.SemaphoreType.DMA((n_sem,)),
        ],
        compiler_params=pltpu.CompilerParams(
            vmem_limit_bytes=120 * 1024 * 1024,
            disable_semaphore_checks=True,
        ),
        name="fused_decode",
    )(xa2, k3, v3, wqa3, A_wo, xb2, c4, wqb4, wuk4, wuv4, wob2)
    return out.reshape(B, Sq, D + M)


@jax.jit
def pallas_concat_heads__sliding_block_cached__compressed_kv_cla__decode_kernel(
    A_x: jax.Array,
    A_k_cache: jax.Array,
    A_v_cache: jax.Array,
    A_wq: jax.Array,
    A_wo: jax.Array,
    B_x: jax.Array,
    B_c_kv: jax.Array,
    B_w_q: jax.Array,
    B_w_uk: jax.Array,
    B_w_uv: jax.Array,
    B_w_o: jax.Array,
):
    return _fused(_CFG, A_x, A_k_cache, A_v_cache, A_wq, A_wo,
                  B_x, B_c_kv, B_w_q, B_w_uk, B_w_uv, B_w_o)
```

```python
import functools

import jax
import jax.numpy as jnp
from jax import lax
import jax.experimental.pallas as pl
import jax.experimental.pallas.tpu as pltpu

_NT = (((1,), (1,)), ((), ()))
_F32 = jnp.float32
_BF16 = jnp.bfloat16
_L = 128
_G = 8
_KIB = 1024

_CFG = dict(
    wo_chunks=(2432, 1024, 256, 128),
    wo_tail=(80, 64, 48, 32, 16, 16),
    piece=64 * _KIB,
    shift=32 * _KIB,
    block=512 * _KIB,
    side_rows=128,
    side_n=25,
    side_last=56,
    side_nb=4,
    side_late=2,
    late_at=2,
)


def _dot(a, b):
    return jnp.dot(a, b, preferred_element_type=_F32)


def _dot_nt(a, b):
    return lax.dot_general(a, b, _NT, preferred_element_type=_F32)


def _bounds(n_rows, row_bytes, piece, shift):
    step = piece // row_bytes
    first = (shift // row_bytes) % step
    cuts = [0] + [r for r in range(first, n_rows, step) if r > 0] + [n_rows]
    return list(zip(cuts[:-1], cuts[1:]))


def _fused(cfg, A_x, A_k_cache, A_v_cache, A_wq, A_wo, B_x, B_c_kv, B_w_q, B_w_uk, B_w_uv, B_w_o):
    B, Sq, D = A_x.shape
    _, H, Sk, Dh = A_k_cache.shape
    assert Sq == 1 and B_x.shape[1] == 1
    assert A_wq.shape == (D, H * Dh)
    W = min(4096, max(256, Sk // 4))
    M, Hb, Db = B_w_q.shape
    Skb, Dc = B_c_kv.shape[1], B_c_kv.shape[2]
    BH = B * H
    NG = BH // _G
    NCT = Dc // _L
    scale_a = float(Dh) ** -0.5
    scale_b = float(Db) ** -0.5
    n_mxu = len(cfg["wo_chunks"])
    wo_chunks = tuple(cfg["wo_chunks"]) + tuple(cfg["wo_tail"])
    tail_rows = sum(cfg["wo_tail"])
    assert tail_rows % Dh == 0
    piece, shift, block = cfg["piece"], cfg["shift"], cfg["block"]
    side_rows, side_n, side_nb = cfg["side_rows"], cfg["side_n"], cfg["side_nb"]
    assert sum(wo_chunks) == H * Dh
    side_late, late_at = cfg["side_late"], cfg["late_at"]
    side_last = cfg["side_last"]
    side_all = side_n + (1 if side_last else 0)
    assert side_all <= 6 + B + NG

    xa2 = A_x.reshape(B, D)
    xb2 = B_x.reshape(B, M)
    k3 = A_k_cache.reshape(BH, Sk, Dh)
    v3 = A_v_cache.reshape(BH, Sk, Dh)
    wob2 = B_w_o.reshape(Hb * Db, M)

    def blocked(w, lead=0):
        row_bytes = 2 * functools.reduce(lambda a, b: a * b, w.shape[lead + 1:], 1)
        rows = block // row_bytes
        shape = w.shape[:lead] + (w.shape[lead] // rows, rows) + w.shape[lead + 1:]
        return w.reshape(shape), rows, row_bytes

    wqa3, r_wqa, b_wqa = blocked(A_wq)
    wqb4, r_wqb, b_wqb = blocked(B_w_q)
    wuk4, r_wu, b_wu = blocked(B_w_uk)
    wuv4, _, _ = blocked(B_w_uv)
    c4, r_c, b_c = blocked(B_c_kv, 1)
    cut_wqa = _bounds(r_wqa, b_wqa, max(piece, 8 * b_wqa), 0)
    cut_wqb = _bounds(r_wqb, b_wqb, piece, shift)
    cut_wu = _bounds(r_wu, b_wu, piece, shift)
    cut_c = _bounds(r_c, b_c, piece, shift)
    cut_kv = _bounds(W, 2 * Dh, piece, shift)

    n_wo = len(wo_chunks)
    wo_off = [sum(wo_chunks[:i]) for i in range(n_wo)]
    S_XB, S_XA, S_WQB, S_WUK, S_WUV, S_WOB, S_WQA = range(7)
    S_C = 7
    S_KV = S_C + B
    S_WO = S_KV + 2 * NG
    S_SA = S_WO + n_wo
    S_SB = S_SA + side_nb
    n_sem = S_SB + side_nb
    side_total = side_rows * side_n + side_last

    def kernel(xa_h, k_h, v_h, wqa_h, woa_h, xb_h, c_h, wqb_h, wuk_h, wuv_h, wob_h,
               o_ref,
               xa_s, xb_s, k_s, v_s, wqa_s, woa_s, c_s, wqb_s, wuk_s, wuv_s, wob_s,
               qa_s, oa_s, qabs_s, ctx_s, acc_s, accb_s, ctxb_s, coef_s, vacc_s, side_s, sem):
        def cp(src, dst, s):
            return pltpu.make_async_copy(src, dst, sem.at[s])

        def start_pieces(src, dst, cuts, s, row0=0):
            for lo, hi in cuts:
                cp(src.at[:, pl.ds(row0 + lo, hi - lo)], dst.at[:, pl.ds(lo, hi - lo)], s).start()

        def wait_all(dst, s):
            cp(dst, dst, s).wait()

        c_xb = cp(xb_h, xb_s, S_XB)
        c_xa = cp(xa_h, xa_s, S_XA)
        rest = pl.ds(side_total, Hb * Db - side_total)
        c_wob = cp(wob_h.at[rest, :], wob_s.at[rest, :], S_WOB)

        def start_c(b):
            start_pieces(c_h.at[b], c_s.at[b], cut_c, S_C + b)

        def start_kv(g):
            heads = pl.ds(g * _G, _G)
            start_pieces(k_h.at[heads], k_s.at[g], cut_kv, S_KV + 2 * g, Sk - W)
            start_pieces(v_h.at[heads], v_s.at[g], cut_kv, S_KV + 2 * g + 1, Sk - W)

        def c_wo(i):
            rows = pl.ds(wo_off[i], wo_chunks[i])
            return cp(woa_h.at[rows, :], woa_s.at[rows, :], S_WO + i)

        def side_refs(i, last):
            start = i * side_rows
            if not isinstance(i, int):
                start = pl.multiple_of(start, 8)
            n = side_last if last else side_rows
            slot = i % side_nb
            return pl.ds(start, n), side_s.at[slot, pl.ds(0, n)], slot

        def c_sa(i, last=False):
            rows, stage, slot = side_refs(i, last)
            return cp(wob_h.at[rows, :], stage, S_SA + slot)

        def c_sb(i, last=False):
            rows, stage, slot = side_refs(i, last)
            return cp(stage, wob_s.at[rows, :], S_SB + slot)

        ahead = side_nb // 2

        def when(cond, fn):
            if isinstance(cond, bool):
                if cond:
                    fn()
            else:
                pl.when(cond)(fn)

        def tick(i):
            def go():
                c_sa(i).wait()
                c_sb(i).start()
                when(i >= ahead, lambda: c_sb(i - ahead).wait())
                when(i + ahead < side_n, lambda: c_sa(i + ahead).start())
                if side_last:
                    when(i + ahead == side_n, lambda: c_sa(side_n, True).start())
            when(i < side_n, go)

        start_pieces(wqb_h, wqb_s, cut_wqb, S_WQB)
        for i in range(ahead):
            c_sa(i).start()
        c_xb.start()
        c_xa.start()
        start_pieces(wuk_h, wuk_s, cut_wu, S_WUK)
        tick(0)

        wait_all(wqb_s, S_WQB)
        start_c(0)
        tick(1)
        c_xb.wait()
        wqb = wqb_s[...].reshape(M, Hb, Db).reshape(M, Hb * Db)
        qb = (_dot(xb_s[...], wqb) * scale_b).astype(_BF16)
        wait_all(wuk_s, S_WUK)
        start_c(1)
        tick(2)
        wuk = wuk_s[...].reshape(Dc, Hb, Db).reshape(Dc, Hb * Db)
        for h in range(Hb):
            sl = slice(h * Db, (h + 1) * Db)
            r = _dot_nt(qb[:, sl], wuk[:, sl])
            for t in range(NCT):
                qabs_s[t, pl.ds(h, B, stride=Hb), :] = r[:, t * _L:(t + 1) * _L]

        def b_body(b, carry):
            wait_all(c_s.at[b], S_C + b)
            pl.when(b + 2 < B)(lambda: start_c(b + 2))
            pl.when(b + 2 == B)(lambda: start_pieces(wuv_h, wuv_s, cut_wu, S_WUV))

            @pl.when(b + 2 == B + 1)
            def _():
                c_wob.start()
                start_pieces(wqa_h, wqa_s, cut_wqa, S_WQA)

            tick(3 + b)
            rows = pl.ds(pl.multiple_of(b * Hb, Hb), Hb)
            qa = jnp.concatenate(
                [qabs_s[t, rows, :] for t in range(NCT)], axis=1).astype(_BF16)
            s = _dot_nt(qa, c_s[b].reshape(Skb, Dc))
            m = jnp.max(s, axis=-1, keepdims=True)
            p = jnp.exp(s - m)
            l = jnp.sum(p, axis=-1, keepdims=True)
            cc = _dot(p.astype(_BF16), c_s[b].reshape(Skb, Dc)) / l
            for t in range(NCT):
                ctx_s[t, rows, :] = cc[:, t * _L:(t + 1) * _L]
            return carry

        lax.fori_loop(0, B, b_body, 0)

        wait_all(wuv_s, S_WUV)
        start_kv(0)
        tick(3 + B)
        wuv = wuv_s[...].reshape(Dc, Hb, Db).reshape(Dc, Hb * Db)
        parts = []
        for h in range(Hb):
            ch = jnp.concatenate(
                [ctx_s[t, pl.ds(h, B, stride=Hb), :] for t in range(NCT)],
                axis=1).astype(_BF16)
            parts.append(_dot(ch, wuv[:, h * Db:(h + 1) * Db]))
        ctxb_s[...] = jnp.concatenate(parts, axis=1)

        wait_all(wqa_s, S_WQA)
        start_kv(1)
        tick(4 + B)
        c_xa.wait()
        qa_all = _dot(xa_s[...], wqa_s[...].reshape(D, H * Dh)) * scale_a
        for h in range(H):
            qa_s[pl.ds(h, B, stride=H), :] = qa_all[:, h * Dh:(h + 1) * Dh]

        def a_body(g, carry):
            rows = pl.ds(pl.multiple_of(g * _G, _G), _G)
            q8 = qa_s[rows, :].astype(_BF16)
            wait_all(k_s.at[g], S_KV + 2 * g)
            pl.when(g + 2 < NG)(lambda: start_kv(g + 2))

            @pl.when(g + 2 == NG)
            def _():
                for i in range(n_wo):
                    c_wo(i).start()

            tick(5 + B + g)
            row = lax.broadcasted_iota(jnp.int32, (_G, W), 0)
            s = None
            for j in range(_G):
                sj = _dot_nt(q8, k_s[g, j])
                s = sj if s is None else jnp.where(row == j, sj, s)
            m = jnp.max(s, axis=-1, keepdims=True)
            p = jnp.exp(s - m)
            l = jnp.sum(p, axis=-1, keepdims=True)
            pb = p.astype(_BF16)
            wait_all(v_s.at[g], S_KV + 2 * g + 1)
            row2 = lax.broadcasted_iota(jnp.int32, (_G, Dh), 0)
            o = None
            for j in range(_G):
                oj = _dot(pb, v_s[g, j])
                o = oj if o is None else jnp.where(row2 == j, oj, o)
            oa_s[rows, :] = o / l
            return carry

        lax.fori_loop(0, NG, a_body, 0)

        tick(5 + B + NG)
        if side_last:
            c_sa(side_n, True).wait()
            c_sb(side_n, True).start()
        c_wob.wait()
        n_early = side_all - side_late
        waited = side_n - ahead
        for i in range(waited, n_early):
            c_sb(i).wait()
        r_early = n_early * side_rows
        ctxb = ctxb_s[...].astype(_BF16)
        accb_s[...] = (_dot(ctxb[:, :r_early], wob_s[:r_early, :])
                       + _dot(ctxb[:, side_total:], wob_s[side_total:, :]))

        oa32 = jnp.concatenate([oa_s[pl.ds(h, B, stride=H), :] for h in range(H)], axis=1)
        oa = oa32.astype(_BF16)
        tail0 = H * Dh - tail_rows
        for b in range(B):
            for t in range(tail_rows // Dh):
                src = oa32[b:b + 1, tail0 + t * Dh:tail0 + (t + 1) * Dh]
                coef_s[b, t * Dh:(t + 1) * Dh, :] = jnp.broadcast_to(src, (_L, Dh)).T
        for i in range(n_mxu):
            c_wo(i).wait()
            if i == late_at:
                for j in range(max(waited, n_early), side_all):
                    c_sb(j, j == side_n).wait()
                late = _dot(ctxb[:, r_early:side_total], wob_s[r_early:side_total, :])
                o_ref[:, D:] = (accb_s[...] + late).astype(o_ref.dtype)
            lo, n = wo_off[i], wo_chunks[i]
            part = _dot(oa[:, lo:lo + n], woa_s[lo:lo + n, :])
            if i > 0:
                part = part + acc_s[...]
            if i < n_wo - 1:
                acc_s[...] = part
            else:
                o_ref[:, :D] = part.astype(o_ref.dtype)
        for i in range(n_mxu, n_wo):
            c_wo(i).wait()
            lo, n = wo_off[i], wo_chunks[i]
            w = woa_s[lo:lo + n, :].astype(_F32)
            sums = []
            for b in range(B):
                cf = coef_s[b, lo - tail0:lo - tail0 + n, :]
                prod = w * jnp.concatenate([cf] * (D // _L), axis=1)
                acc = vacc_s[b] if i > n_mxu else None
                for r in range(0, n, 8):
                    acc = prod[r:r + 8] if acc is None else acc + prod[r:r + 8]
                if i < n_wo - 1:
                    vacc_s[b] = acc
                else:
                    sums.append(jnp.sum(acc, axis=0, keepdims=True))
            if i == n_wo - 1:
                res = acc_s[...] + jnp.concatenate(sums, axis=0)
                o_ref[:, :D] = res.astype(o_ref.dtype)

    any_spec = pl.BlockSpec(memory_space=pl.ANY)
    out = pl.pallas_call(
        kernel,
        out_shape=jax.ShapeDtypeStruct((B, D + M), A_x.dtype),
        in_specs=[any_spec] * 11,
        out_specs=pl.BlockSpec(memory_space=pltpu.VMEM),
        scratch_shapes=[
            pltpu.VMEM(xa2.shape, _BF16),
            pltpu.VMEM(xb2.shape, _BF16),
            pltpu.VMEM((NG, _G, W, Dh), _BF16),
            pltpu.VMEM((NG, _G, W, Dh), _BF16),
            pltpu.VMEM(wqa3.shape, _BF16),
            pltpu.VMEM(A_wo.shape, _BF16),
            pltpu.VMEM(c4.shape, _BF16),
            pltpu.VMEM(wqb4.shape, _BF16),
            pltpu.VMEM(wuk4.shape, _BF16),
            pltpu.VMEM(wuv4.shape, _BF16),
            pltpu.VMEM(wob2.shape, _BF16),
            pltpu.VMEM((BH, Dh), _F32),
            pltpu.VMEM((BH, Dh), _F32),
            pltpu.VMEM((NCT, B * Hb, _L), _F32),
            pltpu.VMEM((NCT, B * Hb, _L), _F32),
            pltpu.VMEM((B, D), _F32),
            pltpu.VMEM((B, M), _F32),
            pltpu.VMEM((B, Hb * Db), _F32),
            pltpu.VMEM((B, max(tail_rows, 8), _L), _F32),
            pltpu.VMEM((B, 8, D), _F32),
            pltpu.SMEM((side_nb, side_rows, M), _BF16),
            pltpu.SemaphoreType.DMA((n_sem,)),
        ],
        compiler_params=pltpu.CompilerParams(
            vmem_limit_bytes=120 * 1024 * 1024,
            disable_semaphore_checks=True,
        ),
        name="fused_decode",
    )(xa2, k3, v3, wqa3, A_wo, xb2, c4, wqb4, wuk4, wuv4, wob2)
    return out.reshape(B, Sq, D + M)


@jax.jit
def pallas_concat_heads__sliding_block_cached__compressed_kv_cla__decode_kernel(
    A_x: jax.Array,
    A_k_cache: jax.Array,
    A_v_cache: jax.Array,
    A_wq: jax.Array,
    A_wo: jax.Array,
    B_x: jax.Array,
    B_c_kv: jax.Array,
    B_w_q: jax.Array,
    B_w_uk: jax.Array,
    B_w_uv: jax.Array,
    B_w_o: jax.Array,
):
    return _fused(_CFG, A_x, A_k_cache, A_v_cache, A_wq, A_wo,
                  B_x, B_c_kv, B_w_q, B_w_uk, B_w_uv, B_w_o)
```

```python
import functools

import jax
import jax.numpy as jnp
from jax import lax
import jax.experimental.pallas as pl
import jax.experimental.pallas.tpu as pltpu

_NT = (((1,), (1,)), ((), ()))
_F32 = jnp.float32
_BF16 = jnp.bfloat16
_L = 128
_G = 8
_KIB = 1024

_CFG = dict(
    wo_chunks=(1920, 1024, 256, 128),
    wo_tail=(80, 64, 48, 32, 16, 16),
    piece=64 * _KIB,
    shift_a=28 * _KIB,
    shift_b=32 * _KIB,
    block=512 * _KIB,
    inj=16 * _KIB,
    inj_kv=28 * _KIB,
    side_rows=128,
    side_n=24,
    side_last=64,
    side_nb=4,
    side_late=1,
    late_at=2,
    pump0=14,
    pump_w=6,
    pump_c=8,
    pump_q=10,
    pump_k=4,
    pump_v=6,
    seg_w=1,
    kick_s=(1, 3, 5, 7),
    kick_c=(3,),
    kick_qk=(1, 3, 5),
    kick_pv=(3,),
)


def _dot(a, b):
    return jnp.dot(a, b, preferred_element_type=_F32)


def _dot_nt(a, b):
    return lax.dot_general(a, b, _NT, preferred_element_type=_F32)


def _bounds(n_rows, row_bytes, piece, shift, skip=0):
    step = piece // row_bytes
    first = (shift // row_bytes) % step
    cuts = [skip] + [r for r in range(first, n_rows, step) if r > skip] + [n_rows]
    return list(zip(cuts[:-1], cuts[1:]))


class _Pump:
    def __init__(self, copies):
        self.copies, self.started, self.waited = list(copies), 0, 0

    def kick(self):
        if self.started < len(self.copies):
            self.copies[self.started]().start(priority=0)
            self.started += 1

    def _wait_to(self, n):
        while self.waited < n:
            self.copies[self.waited]().wait()
            self.waited += 1

    def pump(self, n):
        for _ in range(n):
            self.kick()
            self._wait_to(self.started - 1)

    def drain(self):
        while self.started < len(self.copies):
            self.kick()
        self._wait_to(self.started)


def _fused(cfg, A_x, A_k_cache, A_v_cache, A_wq, A_wo, B_x, B_c_kv, B_w_q, B_w_uk, B_w_uv, B_w_o):
    B, Sq, D = A_x.shape
    _, H, Sk, Dh = A_k_cache.shape
    assert Sq == 1 and B_x.shape[1] == 1
    assert A_wq.shape == (D, H * Dh)
    W = min(4096, max(256, Sk // 4))
    M, Hb, Db = B_w_q.shape
    Skb, Dc = B_c_kv.shape[1], B_c_kv.shape[2]
    BH = B * H
    NG = BH // _G
    NCT = Dc // _L
    HH = Hb // 2
    scale_a = float(Dh) ** -0.5
    scale_b = float(Db) ** -0.5
    piece, block, inj = cfg["piece"], cfg["block"], cfg["inj"]
    shift_a, shift_b = cfg["shift_a"], cfg["shift_b"]
    side_rows, side_n, side_nb = cfg["side_rows"], cfg["side_n"], cfg["side_nb"]
    side_late, late_at = cfg["side_late"], cfg["late_at"]
    n_mxu = len(cfg["wo_chunks"])
    wo_chunks = tuple(cfg["wo_chunks"]) + tuple(cfg["wo_tail"])
    tail_rows = sum(cfg["wo_tail"])
    assert tail_rows % Dh == 0 and M % _L == 0 and NG >= 4
    side_last = cfg["side_last"]
    side_all = side_n + (1 if side_last else 0)
    assert side_all <= 5 + B + NG

    xa2 = A_x.reshape(B, D)
    xb2 = B_x.reshape(B, M)
    k3 = A_k_cache.reshape(BH, Sk, Dh)
    v3 = A_v_cache.reshape(BH, Sk, Dh)
    wob2 = B_w_o.reshape(Hb * Db, M)

    def blocked(w, lead=0):
        row_bytes = 2 * functools.reduce(lambda a, b: a * b, w.shape[lead + 1:], 1)
        rows = block // row_bytes
        shape = w.shape[:lead] + (w.shape[lead] // rows, rows) + w.shape[lead + 1:]
        return w.reshape(shape), rows, row_bytes

    wqa3, r_wqa, b_wqa = blocked(A_wq)
    wqb4, r_w, b_w = blocked(B_w_q)
    wuk4, _, _ = blocked(B_w_uk)
    wuv4, _, _ = blocked(B_w_uv)
    c4, r_c, b_c = blocked(B_c_kv, 1)
    assert wqb4.shape == wuk4.shape == wuv4.shape and (2 * r_w) == _L
    NBLK = wqb4.shape[0]
    i_w, i_c, i_wo = inj // b_w, inj // b_c, inj // (2 * D)
    i_kv = cfg["inj_kv"] // (2 * Dh)
    i_wqa = inj // (2 * 8)
    cut_w0 = _bounds(r_w, b_w, piece, shift_b)
    cut_w = _bounds(r_w, b_w, piece, shift_b, 2 * i_w)
    cut_c = _bounds(r_c, b_c, piece, shift_b, 2 * i_c)
    cut_kv = _bounds(W, 2 * Dh, piece, shift_a, i_kv)
    cut_wqa = _bounds(r_wqa, b_wqa, max(piece, 8 * b_wqa), 0, 8)
    n_iwo = 4 * _G
    wo_base = n_iwo * i_wo
    assert wo_base + sum(wo_chunks) == H * Dh

    n_wo = len(wo_chunks)
    wo_off = [wo_base + sum(wo_chunks[:i]) for i in range(n_wo)]
    S_XB, S_XA, S_WQB, S_WUK, S_WUV, S_WOB, S_WQA, S_WOI = range(8)
    S_C = 8
    S_KV = S_C + B
    S_WO = S_KV + 2 * NG
    S_SA = S_WO + n_wo
    S_SB = S_SA + side_nb
    n_sem = S_SB + side_nb
    side_total = side_rows * side_n + side_last

    def kernel(xa_h, k_h, v_h, wqa_h, woa_h, xb_h, c_h, wqb_h, wuk_h, wuv_h, wob_h,
               o_ref,
               xa_s, xb_s, k_s, v_s, wqa_s, woa_s, c_s, wqb_s, wuk_s, wuv_s, wob_s,
               qa_s, oa_s, qabs_s, ctx_s, acc_s, accb_s, ctxb_s, coef_s, vacc_s, p_s, s_s, side_s, sem):
        def cp(src, dst, s):
            return pltpu.make_async_copy(src, dst, sem.at[s])

        def start_pieces(src, dst, cuts, s, row0=0):
            for lo, hi in cuts:
                cp(src.at[:, pl.ds(row0 + lo, hi - lo)], dst.at[:, pl.ds(lo, hi - lo)],
                   s).start(priority=cfg.get('bulk_prio', 1))

        def wait_pieces(dst, cuts, s):
            view = dst.at[:, pl.ds(cuts[0][0], cuts[-1][1] - cuts[0][0])]
            cp(view, view, s).wait()

        def heads_of(src, dst, rows, s):
            return [functools.partial(
                lambda k, j: cp(src.at[k, pl.ds(j * rows, rows)], dst.at[k, pl.ds(j * rows, rows)], s),
                k, j) for j in range(2) for k in range(NBLK)]

        c_xb = cp(xb_h, xb_s, S_XB)
        c_xa = cp(xa_h, xa_s, S_XA)
        rest = pl.ds(side_total, Hb * Db - side_total)
        c_wob = cp(wob_h.at[rest, :], wob_s.at[rest, :], S_WOB)

        def start_c(b):
            start_pieces(c_h.at[b], c_s.at[b], cut_c, S_C + b)

        def pump_c(b):
            return _Pump(heads_of(c_h.at[b], c_s.at[b], i_c, S_C + b))

        wqa_rest = (slice(None), pl.ds(0, 8), pl.ds(2 * i_wqa, H * Dh - 2 * i_wqa))
        c_wqa0 = cp(wqa_h.at[wqa_rest], wqa_s.at[wqa_rest], S_WQA)

        def start_wqa():
            c_wob.start(priority=cfg.get('bulk_prio', 1))
            c_wqa0.start(priority=cfg.get('bulk_prio', 1))
            start_pieces(wqa_h, wqa_s, cut_wqa, S_WQA)

        def pump_wqa():
            def one(k, j):
                at = (k, pl.ds(0, 8), pl.ds(j * i_wqa, i_wqa))
                return cp(wqa_h.at[at], wqa_s.at[at], S_WQA)
            return _Pump([functools.partial(one, k, j) for j in range(2) for k in range(NBLK)])

        def start_k(g):
            start_pieces(k_h.at[pl.ds(g * _G, _G)], k_s.at[g], cut_kv, S_KV + 2 * g, Sk - W)

        def start_v(g):
            start_pieces(v_h.at[pl.ds(g * _G, _G)], v_s.at[g], cut_kv, S_KV + 2 * g + 1, Sk - W)

        def pump_kv(g):
            def one(src, dst, s, j):
                return cp(src.at[g * _G + j, pl.ds(Sk - W, i_kv)], dst.at[g, j, pl.ds(0, i_kv)], s)
            return _Pump([functools.partial(one, k_h, k_s, S_KV + 2 * g, j) for j in range(_G)]
                         + [functools.partial(one, v_h, v_s, S_KV + 2 * g + 1, j) for j in range(_G)])

        def c_wo(i):
            rows = pl.ds(wo_off[i], wo_chunks[i])
            return cp(woa_h.at[rows, :], woa_s.at[rows, :], S_WO + i)

        def pump_wo(half):
            def one(j):
                rows = pl.ds(j * i_wo, i_wo)
                return cp(woa_h.at[rows, :], woa_s.at[rows, :], S_WOI)
            n = n_iwo // 2
            return _Pump([functools.partial(one, j) for j in range(half * n, (half + 1) * n)])

        def side_refs(i):
            start = i * side_rows
            n = side_rows
            if not isinstance(i, int):
                start = pl.multiple_of(start, 8)
            elif i == side_n:
                n = side_last
            slot = i % side_nb
            return pl.ds(start, n), side_s.at[slot, pl.ds(0, n)], slot

        def c_sa(i):
            rows, stage, slot = side_refs(i)
            return cp(wob_h.at[rows, :], stage, S_SA + slot)

        def c_sb(i):
            rows, stage, slot = side_refs(i)
            return cp(stage, wob_s.at[rows, :], S_SB + slot)

        lag = 2

        def when(cond, fn):
            if isinstance(cond, bool):
                if cond:
                    fn()
            else:
                pl.when(cond)(fn)

        def tick(i):
            def forward():
                c_sa(i).wait()
                c_sb(i).start()

            def refill():
                if not isinstance(i, int) or i >= lag:
                    c_sb(i - lag).wait()
                c_sa(i - lag + side_nb).start()

            if isinstance(i, int):
                when(i < side_all, forward)
                when(i - lag + side_nb < side_all, refill)
            else:
                assert 4 + B + NG - 3 - lag + side_nb < side_n
                forward()
                refill()

        def head_major(w_s, t, hh):
            w = w_s[2 * t:2 * t + 2, :, hh * HH:(hh + 1) * HH, :]
            return w.reshape(_L, HH, Db).reshape(_L, HH * Db)

        start_pieces(wqb_h, wqb_s, cut_w0, S_WQB)
        c_xb.start()
        c_xa.start()
        for i in range(side_nb - lag):
            c_sa(i).start()
        start_pieces(wuk_h, wuk_s, cut_w, S_WUK)
        pm = _Pump(heads_of(wuk_h, wuk_s, i_w, S_WUK))
        pm.pump(cfg["pump0"])
        pm.drain()

        seg_w = cfg["seg_w"]

        wait_pieces(wqb_s, cut_w0, S_WQB)
        start_c(0)
        pm = pump_c(0)
        pm.kick()
        tick(0)
        c_xb.wait()
        xb = xb_s[...]
        for t in range(M // _L):
            for hh in range(2):
                cols = slice(hh * HH * Db, (hh + 1) * HH * Db)
                part = _dot(xb[:, t * _L:(t + 1) * _L], head_major(wqb_s, t, hh))
                ctxb_s[:, cols] = part if t == 0 else ctxb_s[:, cols] + part
                if (2 * t + hh + 1) % seg_w == 0:
                    pm.pump(1)
        pm.pump(cfg["pump_w"])
        pm.drain()

        wait_pieces(wuk_s, cut_w, S_WUK)
        start_c(1)
        pm = pump_c(1)
        pm.kick()
        tick(1)
        qb = (ctxb_s[...] * scale_b).astype(_BF16)
        for t in range(NCT):
            for hh in range(2):
                w = head_major(wuk_s, t, hh)
                for j in range(HH):
                    h = hh * HH + j
                    qabs_s[t, pl.ds(h, B, stride=Hb), :] = _dot_nt(
                        qb[:, h * Db:(h + 1) * Db], w[:, j * Db:(j + 1) * Db])
                if (2 * t + hh + 1) % seg_w == 0:
                    pm.pump(1)
        pm.pump(cfg["pump_w"])
        pm.drain()

        def attend_b(b, start_next, pm, same_buffer):
            wait_pieces(c_s.at[b], cut_c, S_C + b)
            start_next()
            pm.kick()
            tick(2 + b)
            step = pm.kick if same_buffer else functools.partial(pm.pump, 1)
            rows = pl.ds(b * Hb, Hb)
            qa = jnp.concatenate(
                [qabs_s[t, rows, :] for t in range(NCT)], axis=1).astype(_BF16)
            for k in range(NBLK):
                s_s[:, k * r_c:(k + 1) * r_c] = _dot_nt(qa, c_s[b, k])
                if k in cfg["kick_s"]:
                    step()
            s = s_s[...]
            m = jnp.max(s, axis=-1, keepdims=True)
            p = jnp.exp(s - m)
            l = jnp.sum(p, axis=-1, keepdims=True)
            pb = p.astype(_BF16)
            cc = None
            for k in range(NBLK):
                part = _dot(pb[:, k * r_c:(k + 1) * r_c], c_s[b, k])
                cc = part if cc is None else cc + part
                if k in cfg["kick_c"]:
                    if not same_buffer:
                        s_s[:, :Dc] = cc
                    step()
                    if not same_buffer:
                        cc = s_s[:, :Dc]
            cc = cc / l
            for t in range(NCT):
                ctx_s[t, rows, :] = cc[:, t * _L:(t + 1) * _L]
            pm.pump(cfg["pump_c"])
            pm.drain()

        for b in range(B):
            if b + 2 < B:
                attend_b(b, functools.partial(start_c, b + 2), pump_c(b + 2), True)
            elif b + 2 == B:
                attend_b(b, functools.partial(start_pieces, wuv_h, wuv_s, cut_w, S_WUV),
                         _Pump(heads_of(wuv_h, wuv_s, i_w, S_WUV)), False)
            else:
                attend_b(b, start_wqa, pump_wqa(), False)

        wait_pieces(wuv_s, cut_w, S_WUV)
        start_k(0)
        start_v(0)
        pm = pump_kv(0)
        pm.kick()
        tick(2 + B)
        for t in range(NCT):
            for hh in range(2):
                w = head_major(wuv_s, t, hh)
                parts = []
                for j in range(HH):
                    ch = ctx_s[t, pl.ds(hh * HH + j, B, stride=Hb), :].astype(_BF16)
                    parts.append(_dot(ch, w[:, j * Db:(j + 1) * Db]))
                cols = slice(hh * HH * Db, (hh + 1) * HH * Db)
                part = jnp.concatenate(parts, axis=1)
                ctxb_s[:, cols] = part if t == 0 else ctxb_s[:, cols] + part
                if (2 * t + hh + 1) % seg_w == 0:
                    pm.pump(1)
        pm.pump(cfg["pump_w"])
        pm.drain()

        c_wqa0.wait()
        wait_pieces(wqa_s, cut_wqa, S_WQA)
        start_k(1)
        pm = pump_kv(1)
        pm.kick()
        tick(3 + B)
        c_xa.wait()
        qa_all = _dot(xa_s[...], wqa_s[...].reshape(D, H * Dh)) * scale_a
        for h in range(H):
            qa_s[pl.ds(h, B, stride=H), :] = qa_all[:, h * Dh:(h + 1) * Dh]
        pm.pump(cfg["pump_q"])
        pm.drain()

        def attend_a(g, start_at_k, start_at_v, pm):
            start = g * _G if isinstance(g, int) else pl.multiple_of(g * _G, _G)
            rows = pl.ds(start, _G)
            q8 = qa_s[rows, :].astype(_BF16)
            wait_pieces(k_s.at[g], cut_kv, S_KV + 2 * g)
            start_at_k()
            pm.kick()
            tick(4 + B + g)
            row = lax.broadcasted_iota(jnp.int32, (_G, W), 0)
            s = None
            for j in range(_G):
                sj = _dot_nt(q8, k_s[g, j])
                s = sj if s is None else jnp.where(row == j, sj, s)
                if j in cfg["kick_qk"]:
                    pm.kick()
            m = jnp.max(s, axis=-1, keepdims=True)
            p = jnp.exp(s - m)
            l = jnp.sum(p, axis=-1, keepdims=True)
            p_s[...] = p
            pm.pump(cfg["pump_k"])
            wait_pieces(v_s.at[g], cut_kv, S_KV + 2 * g + 1)
            start_at_v()
            pm.kick()
            pb = p_s[...].astype(_BF16)
            row2 = lax.broadcasted_iota(jnp.int32, (_G, Dh), 0)
            o = None
            for j in range(_G):
                oj = _dot(pb, v_s[g, j])
                o = oj if o is None else jnp.where(row2 == j, oj, o)
                if j in cfg["kick_pv"]:
                    pm.kick()
            oa_s[rows, :] = o / l

        def a_body(g, carry):
            pm = pump_kv(g + 2)
            attend_a(g, functools.partial(start_v, g + 1), functools.partial(start_k, g + 2), pm)
            pm.pump(cfg["pump_v"])
            pm.drain()
            return carry

        lax.fori_loop(0, NG - 2, a_body, 0)

        def start_wo():
            for i in range(n_wo):
                c_wo(i).start(priority=cfg.get('bulk_prio', 1))

        pm = pump_wo(0)
        attend_a(NG - 2, functools.partial(start_v, NG - 1), start_wo, pm)
        pm.pump(cfg["pump_v"])
        pm.drain()
        pm = pump_wo(1)
        attend_a(NG - 1, lambda: None, lambda: None, pm)

        c_wob.wait()
        n_early = side_all - side_late
        waited = max(side_all - side_nb, 0)
        for i in range(waited, n_early):
            c_sb(i).wait()
        r_early = n_early * side_rows
        ctxb = ctxb_s[...].astype(_BF16)
        part = _dot(ctxb[:, side_total:], wob_s[side_total:, :])
        pm.kick()
        step = 8 * _L
        for lo in range(0, r_early, step):
            hi = min(lo + step, r_early)
            part = part + _dot(ctxb[:, lo:hi], wob_s[lo:hi, :])
            pm.kick()
        accb_s[...] = part
        tick(4 + B + NG)

        oa32 = jnp.concatenate([oa_s[pl.ds(h, B, stride=H), :] for h in range(H)], axis=1)
        oa = oa32.astype(_BF16)
        tail0 = H * Dh - tail_rows
        for b in range(B):
            for t in range(tail_rows // Dh):
                src = oa32[b:b + 1, tail0 + t * Dh:tail0 + (t + 1) * Dh]
                coef_s[b, t * Dh:(t + 1) * Dh, :] = jnp.broadcast_to(src, (_L, Dh)).T
        pm.pump(cfg.get("pump_e", 3))
        pm.drain()
        acc_s[...] = _dot(oa[:, :wo_base], woa_s[:wo_base, :])
        for i in range(n_mxu):
            c_wo(i).wait()
            if i == late_at:
                for j in range(max(waited, n_early), side_all):
                    c_sb(j).wait()
                late = _dot(ctxb[:, r_early:side_total], wob_s[r_early:side_total, :])
                o_ref[:, D:] = (accb_s[...] + late).astype(o_ref.dtype)
            lo, n = wo_off[i], wo_chunks[i]
            part = _dot(oa[:, lo:lo + n], woa_s[lo:lo + n, :]) + acc_s[...]
            if i < n_wo - 1:
                acc_s[...] = part
            else:
                o_ref[:, :D] = part.astype(o_ref.dtype)
        for i in range(n_mxu, n_wo):
            c_wo(i).wait()
            lo, n = wo_off[i], wo_chunks[i]
            w = woa_s[lo:lo + n, :].astype(_F32)
            sums = []
            for b in range(B):
                cf = coef_s[b, lo - tail0:lo - tail0 + n, :]
                prod = w * jnp.concatenate([cf] * (D // _L), axis=1)
                acc = vacc_s[b] if i > n_mxu else None
                for r in range(0, n, 8):
                    acc = prod[r:r + 8] if acc is None else acc + prod[r:r + 8]
                if i < n_wo - 1:
                    vacc_s[b] = acc
                else:
                    sums.append(jnp.sum(acc, axis=0, keepdims=True))
            if i == n_wo - 1:
                res = acc_s[...] + jnp.concatenate(sums, axis=0)
                o_ref[:, :D] = res.astype(o_ref.dtype)

    any_spec = pl.BlockSpec(memory_space=pl.ANY)
    out = pl.pallas_call(
        kernel,
        out_shape=jax.ShapeDtypeStruct((B, D + M), A_x.dtype),
        in_specs=[any_spec] * 11,
        out_specs=pl.BlockSpec(memory_space=pltpu.VMEM),
        scratch_shapes=[
            pltpu.VMEM(xa2.shape, _BF16),
            pltpu.VMEM(xb2.shape, _BF16),
            pltpu.VMEM((NG, _G, W, Dh), _BF16),
            pltpu.VMEM((NG, _G, W, Dh), _BF16),
            pltpu.VMEM(wqa3.shape, _BF16),
            pltpu.VMEM(A_wo.shape, _BF16),
            pltpu.VMEM(c4.shape, _BF16),
            pltpu.VMEM(wqb4.shape, _BF16),
            pltpu.VMEM(wuk4.shape, _BF16),
            pltpu.VMEM(wuv4.shape, _BF16),
            pltpu.VMEM(wob2.shape, _BF16),
            pltpu.VMEM((BH, Dh), _F32),
            pltpu.VMEM((BH, Dh), _F32),
            pltpu.VMEM((NCT, B * Hb, _L), _F32),
            pltpu.VMEM((NCT, B * Hb, _L), _F32),
            pltpu.VMEM((B, D), _F32),
            pltpu.VMEM((B, M), _F32),
            pltpu.VMEM((B, Hb * Db), _F32),
            pltpu.VMEM((B, max(tail_rows, 8), _L), _F32),
            pltpu.VMEM((B, 8, D), _F32),
            pltpu.VMEM((_G, W), _F32),
            pltpu.VMEM((Hb, Skb), _F32),
            pltpu.SMEM((side_nb, side_rows, M), _BF16),
            pltpu.SemaphoreType.DMA((n_sem,)),
        ],
        compiler_params=pltpu.CompilerParams(
            vmem_limit_bytes=120 * 1024 * 1024,
            disable_semaphore_checks=True,
        ),
        name="fused_decode",
    )(xa2, k3, v3, wqa3, A_wo, xb2, c4, wqb4, wuk4, wuv4, wob2)
    return out.reshape(B, Sq, D + M)


@jax.jit
def pallas_concat_heads__sliding_block_cached__compressed_kv_cla__decode_kernel(
    A_x: jax.Array,
    A_k_cache: jax.Array,
    A_v_cache: jax.Array,
    A_wq: jax.Array,
    A_wo: jax.Array,
    B_x: jax.Array,
    B_c_kv: jax.Array,
    B_w_q: jax.Array,
    B_w_uk: jax.Array,
    B_w_uv: jax.Array,
    B_w_o: jax.Array,
):
    return _fused(_CFG, A_x, A_k_cache, A_v_cache, A_wq, A_wo,
                  B_x, B_c_kv, B_w_q, B_w_uk, B_w_uv, B_w_o)
```

```python
import functools
import itertools

import jax
import jax.numpy as jnp
from jax import lax
import jax.experimental.pallas as pl
import jax.experimental.pallas.tpu as pltpu

_NT = (((1,), (1,)), ((), ()))
_F32 = jnp.float32
_BF16 = jnp.bfloat16
_L = 128
_G = 8
_KIB = 1024

_CFG = dict(
    wo_chunks=(1920, 1024, 256, 128),
    wo_tail=(80, 64, 48, 32, 16, 16),
    piece=64 * _KIB,
    shift_a=30 * _KIB,
    shift_b=32 * _KIB,
    block=512 * _KIB,
    inj_w=(16 * _KIB, 8 * _KIB, 8 * _KIB),
    inj_c=(16 * _KIB, 8 * _KIB, 8 * _KIB),
    inj_q=(16 * _KIB, 16 * _KIB),
    inj_k=(16 * _KIB,),
    inj_v=(14 * _KIB, 16 * _KIB),
    inj_wo=16 * _KIB,
    side_rows=128,
    side_n=24,
    side_last=32,
    side_nb=4,
    side_late=1,
    late_at=2,
    pump0=20,
    pump_w=10,
    pump_c=14,
    pump_q=18,
    pump_k=8,
    pump_v=9,
    lag_0=2, lag_w=2, lag_c=2, lag_q=2, lag_k=2, lag_v=2,
    seg_w=1,
    kick_s=(1, 3, 5, 7),
    kick_c=(3,),
    kick_qk=(1, 3, 5),
    kick_pv=(3,),
)


def _dot(a, b):
    return jnp.dot(a, b, preferred_element_type=_F32)


def _dot_nt(a, b):
    return lax.dot_general(a, b, _NT, preferred_element_type=_F32)


def _bounds(n_rows, row_bytes, piece, shift, skip=0):
    step = piece // row_bytes
    first = (shift // row_bytes) % step
    cuts = [skip] + [r for r in range(first, n_rows, step) if r > skip] + [n_rows]
    return list(zip(cuts[:-1], cuts[1:]))


class _Pump:
    def __init__(self, copies):
        self.copies, self.started, self.waited = list(copies), 0, 0

    def kick(self):
        if self.started < len(self.copies):
            self.copies[self.started]().start(priority=0)
            self.started += 1

    def _wait_to(self, n):
        while self.waited < n:
            self.copies[self.waited]().wait()
            self.waited += 1

    def pump(self, n, lag=1):
        for _ in range(n):
            self.kick()
            self._wait_to(self.started - lag)

    def drain(self):
        while self.started < len(self.copies):
            self.kick()
        self._wait_to(self.started)


def _fused(cfg, A_x, A_k_cache, A_v_cache, A_wq, A_wo, B_x, B_c_kv, B_w_q, B_w_uk, B_w_uv, B_w_o):
    B, Sq, D = A_x.shape
    _, H, Sk, Dh = A_k_cache.shape
    assert Sq == 1 and B_x.shape[1] == 1
    assert A_wq.shape == (D, H * Dh)
    W = min(4096, max(256, Sk // 4))
    M, Hb, Db = B_w_q.shape
    Skb, Dc = B_c_kv.shape[1], B_c_kv.shape[2]
    BH = B * H
    NG = BH // _G
    NCT = Dc // _L
    HH = Hb // 2
    scale_a = float(Dh) ** -0.5
    scale_b = float(Db) ** -0.5
    piece, block = cfg["piece"], cfg["block"]
    shift_a, shift_b = cfg["shift_a"], cfg["shift_b"]
    side_rows, side_n, side_nb = cfg["side_rows"], cfg["side_n"], cfg["side_nb"]
    side_late, late_at = cfg["side_late"], cfg["late_at"]
    n_mxu = len(cfg["wo_chunks"])
    wo_chunks = tuple(cfg["wo_chunks"]) + tuple(cfg["wo_tail"])
    tail_rows = sum(cfg["wo_tail"])
    assert tail_rows % Dh == 0 and M % _L == 0 and NG >= 4
    side_last = cfg["side_last"]
    side_all = side_n + (1 if side_last else 0)
    assert side_all <= 5 + B + NG

    xa2 = A_x.reshape(B, D)
    xb2 = B_x.reshape(B, M)
    k3 = A_k_cache.reshape(BH, Sk, Dh)
    v3 = A_v_cache.reshape(BH, Sk, Dh)
    wob2 = B_w_o.reshape(Hb * Db, M)

    def blocked(w, lead=0):
        row_bytes = 2 * functools.reduce(lambda a, b: a * b, w.shape[lead + 1:], 1)
        rows = block // row_bytes
        shape = w.shape[:lead] + (w.shape[lead] // rows, rows) + w.shape[lead + 1:]
        return w.reshape(shape), rows, row_bytes

    wqa3, r_wqa, b_wqa = blocked(A_wq)
    wqb4, r_w, b_w = blocked(B_w_q)
    wuk4, _, _ = blocked(B_w_uk)
    wuv4, _, _ = blocked(B_w_uv)
    c4, r_c, b_c = blocked(B_c_kv, 1)
    assert wqb4.shape == wuk4.shape == wuv4.shape and (2 * r_w) == _L
    NBLK = wqb4.shape[0]

    def spans(sizes, unit):
        ends = list(itertools.accumulate(n // unit for n in sizes))
        return list(zip([0] + ends[:-1], ends))

    i_w, i_c = spans(cfg["inj_w"], b_w), spans(cfg["inj_c"], b_c)
    i_k, i_v = spans(cfg["inj_k"], 2 * Dh), spans(cfg["inj_v"], 2 * Dh)
    i_wqa = spans(cfg["inj_q"], 2 * 8)
    i_wo = cfg["inj_wo"] // (2 * D)
    cut_w0 = _bounds(r_w, b_w, piece, shift_b)
    cut_w = _bounds(r_w, b_w, piece, shift_b, i_w[-1][1])
    cut_c = _bounds(r_c, b_c, piece, shift_b, i_c[-1][1])
    cut_k = _bounds(W, 2 * Dh, piece, shift_a, i_k[-1][1])
    cut_v = _bounds(W, 2 * Dh, piece, shift_a, i_v[-1][1])
    cut_wqa = _bounds(r_wqa, b_wqa, max(piece, 8 * b_wqa), 0, 8)
    n_iwo = 4 * _G
    wo_base = n_iwo * i_wo
    assert wo_base + sum(wo_chunks) == H * Dh

    n_wo = len(wo_chunks)
    wo_off = [wo_base + sum(wo_chunks[:i]) for i in range(n_wo)]
    S_XB, S_XA, S_WQB, S_WUK, S_WUV, S_WOB, S_WQA, S_WOI = range(8)
    S_C = 8
    S_KV = S_C + B
    S_WO = S_KV + 2 * NG
    S_SA = S_WO + n_wo
    S_SB = S_SA + side_nb
    n_sem = S_SB + side_nb
    side_total = side_rows * side_n + side_last

    def kernel(xa_h, k_h, v_h, wqa_h, woa_h, xb_h, c_h, wqb_h, wuk_h, wuv_h, wob_h,
               o_ref,
               xa_s, xb_s, kv_s, wqa_s, woa_s, c_s, wqb_s, wuk_s, wuv_s, wob_s,
               qa_s, oa_s, qabs_s, ctx_s, acc_s, accb_s, ctxb_s, coef_s, vacc_s, p_s, s_s, side_s, sem):
        def cp(src, dst, s):
            return pltpu.make_async_copy(src, dst, sem.at[s])

        def start_pieces(src, dst, cuts, s, row0=0):
            for lo, hi in cuts:
                cp(src.at[:, pl.ds(row0 + lo, hi - lo)], dst.at[:, pl.ds(lo, hi - lo)],
                   s).start(priority=cfg.get('bulk_prio', 1))

        def wait_pieces(dst, cuts, s):
            view = dst.at[:, pl.ds(cuts[0][0], cuts[-1][1] - cuts[0][0])]
            cp(view, view, s).wait()

        def heads_of(src, dst, ranges, s, row0=0):
            def one(k, lo, hi):
                return cp(src.at[k, pl.ds(row0 + lo, hi - lo)], dst.at[k, pl.ds(lo, hi - lo)], s)
            return [functools.partial(one, k, lo, hi)
                    for lo, hi in ranges for k in range(dst.shape[0])]

        k_s, v_s = kv_s.at[0], kv_s.at[1]
        c_xb = cp(xb_h, xb_s, S_XB)
        c_xa = cp(xa_h, xa_s, S_XA)
        rest = pl.ds(side_total, Hb * Db - side_total)
        c_wob = cp(wob_h.at[rest, :], wob_s.at[rest, :], S_WOB)

        def start_c(b):
            start_pieces(c_h.at[b], c_s.at[b], cut_c, S_C + b)

        def pump_c(b):
            return _Pump(heads_of(c_h.at[b], c_s.at[b], i_c, S_C + b))

        wqa_rest = (slice(None), pl.ds(0, 8), pl.ds(i_wqa[-1][1], H * Dh - i_wqa[-1][1]))
        c_wqa0 = cp(wqa_h.at[wqa_rest], wqa_s.at[wqa_rest], S_WQA)

        def start_wqa():
            c_wob.start(priority=cfg.get('bulk_prio', 1))
            c_wqa0.start(priority=cfg.get('bulk_prio', 1))
            start_pieces(wqa_h, wqa_s, cut_wqa, S_WQA)

        def pump_wqa():
            def one(k, lo, hi):
                at = (k, pl.ds(0, 8), pl.ds(lo, hi - lo))
                return cp(wqa_h.at[at], wqa_s.at[at], S_WQA)
            return _Pump([functools.partial(one, k, lo, hi)
                          for lo, hi in i_wqa for k in range(NBLK)])

        def start_k(g):
            start_pieces(k_h.at[pl.ds(g * _G, _G)], k_s.at[g], cut_k, S_KV + 2 * g, Sk - W)

        def start_v(g):
            start_pieces(v_h.at[pl.ds(g * _G, _G)], v_s.at[g], cut_v, S_KV + 2 * g + 1, Sk - W)

        def pump_kv(g):
            heads = pl.ds(g * _G, _G)
            return _Pump(heads_of(k_h.at[heads], k_s.at[g], i_k, S_KV + 2 * g, Sk - W)
                         + heads_of(v_h.at[heads], v_s.at[g], i_v, S_KV + 2 * g + 1, Sk - W))

        def c_wo(i):
            rows = pl.ds(wo_off[i], wo_chunks[i])
            return cp(woa_h.at[rows, :], woa_s.at[rows, :], S_WO + i)

        def pump_wo(half):
            def one(j):
                rows = pl.ds(j * i_wo, i_wo)
                return cp(woa_h.at[rows, :], woa_s.at[rows, :], S_WOI)
            n = n_iwo // 2
            return _Pump([functools.partial(one, j) for j in range(half * n, (half + 1) * n)])

        def side_refs(i):
            start = i * side_rows
            n = side_rows
            if not isinstance(i, int):
                start = pl.multiple_of(start, 8)
            elif i == side_n:
                n = side_last
            slot = i % side_nb
            return pl.ds(start, n), side_s.at[slot, pl.ds(0, n)], slot

        def c_sa(i):
            rows, stage, slot = side_refs(i)
            return cp(wob_h.at[rows, :], stage, S_SA + slot)

        def c_sb(i):
            rows, stage, slot = side_refs(i)
            return cp(stage, wob_s.at[rows, :], S_SB + slot)

        lag = 2

        def when(cond, fn):
            if isinstance(cond, bool):
                if cond:
                    fn()
            else:
                pl.when(cond)(fn)

        def tick(i):
            def forward():
                c_sa(i).wait()
                c_sb(i).start()

            def refill():
                if not isinstance(i, int) or i >= lag:
                    c_sb(i - lag).wait()
                c_sa(i - lag + side_nb).start()

            if isinstance(i, int):
                when(i < side_all, forward)
                when(i - lag + side_nb < side_all, refill)
            else:
                assert 4 + B + NG - 3 - lag + side_nb < side_n
                forward()
                refill()

        def head_major(w_s, t, hh):
            w = w_s[2 * t:2 * t + 2, :, hh * HH:(hh + 1) * HH, :]
            return w.reshape(_L, HH, Db).reshape(_L, HH * Db)

        start_pieces(wqb_h, wqb_s, cut_w0, S_WQB)
        c_xb.start()
        c_xa.start()
        for i in range(side_nb - lag):
            c_sa(i).start()
        start_pieces(wuk_h, wuk_s, cut_w, S_WUK)
        pm = _Pump(heads_of(wuk_h, wuk_s, i_w, S_WUK))
        pm.pump(cfg["pump0"], cfg["lag_0"])
        pm.drain()

        seg_w = cfg["seg_w"]

        wait_pieces(wqb_s, cut_w0, S_WQB)
        start_c(0)
        pm = pump_c(0)
        pm.kick()
        tick(0)
        c_xb.wait()
        xb = xb_s[...]
        for t in range(M // _L):
            for hh in range(2):
                cols = slice(hh * HH * Db, (hh + 1) * HH * Db)
                part = _dot(xb[:, t * _L:(t + 1) * _L], head_major(wqb_s, t, hh))
                ctxb_s[:, cols] = part if t == 0 else ctxb_s[:, cols] + part
                if (2 * t + hh + 1) % seg_w == 0:
                    pm.pump(1)
        pm.pump(cfg["pump_w"], cfg["lag_w"])
        pm.drain()

        wait_pieces(wuk_s, cut_w, S_WUK)
        start_c(1)
        pm = pump_c(1)
        pm.kick()
        tick(1)
        qb = (ctxb_s[...] * scale_b).astype(_BF16)
        for t in range(NCT):
            for hh in range(2):
                w = head_major(wuk_s, t, hh)
                for j in range(HH):
                    h = hh * HH + j
                    qabs_s[t, pl.ds(h, B, stride=Hb), :] = _dot_nt(
                        qb[:, h * Db:(h + 1) * Db], w[:, j * Db:(j + 1) * Db])
                if (2 * t + hh + 1) % seg_w == 0:
                    pm.pump(1)
        pm.pump(cfg["pump_w"], cfg["lag_w"])
        pm.drain()

        def attend_b(b, start_next, pm, same_buffer):
            wait_pieces(c_s.at[b], cut_c, S_C + b)
            start_next()
            pm.kick()
            tick(2 + b)
            step = pm.kick if same_buffer else functools.partial(pm.pump, 1)
            rows = pl.ds(b * Hb, Hb)
            qa = jnp.concatenate(
                [qabs_s[t, rows, :] for t in range(NCT)], axis=1).astype(_BF16)
            for k in range(NBLK):
                s_s[:, k * r_c:(k + 1) * r_c] = _dot_nt(qa, c_s[b, k])
                if k in cfg["kick_s"]:
                    step()
            s = s_s[...]
            m = jnp.max(s, axis=-1, keepdims=True)
            p = jnp.exp(s - m)
            l = jnp.sum(p, axis=-1, keepdims=True)
            pb = p.astype(_BF16)
            cc = None
            for k in range(NBLK):
                part = _dot(pb[:, k * r_c:(k + 1) * r_c], c_s[b, k])
                cc = part if cc is None else cc + part
                if k in cfg["kick_c"]:
                    if not same_buffer:
                        s_s[:, :Dc] = cc
                    step()
                    if not same_buffer:
                        cc = s_s[:, :Dc]
            cc = cc / l
            for t in range(NCT):
                ctx_s[t, rows, :] = cc[:, t * _L:(t + 1) * _L]
            pm.pump(cfg["pump_c"], cfg["lag_c"])
            pm.drain()

        for b in range(B):
            if b + 2 < B:
                attend_b(b, functools.partial(start_c, b + 2), pump_c(b + 2), True)
            elif b + 2 == B:
                attend_b(b, functools.partial(start_pieces, wuv_h, wuv_s, cut_w, S_WUV),
                         _Pump(heads_of(wuv_h, wuv_s, i_w, S_WUV)), False)
            else:
                attend_b(b, start_wqa, pump_wqa(), False)

        wait_pieces(wuv_s, cut_w, S_WUV)
        start_k(0)
        start_v(0)
        pm = pump_kv(0)
        pm.kick()
        tick(2 + B)
        for t in range(NCT):
            for hh in range(2):
                w = head_major(wuv_s, t, hh)
                parts = []
                for j in range(HH):
                    ch = ctx_s[t, pl.ds(hh * HH + j, B, stride=Hb), :].astype(_BF16)
                    parts.append(_dot(ch, w[:, j * Db:(j + 1) * Db]))
                cols = slice(hh * HH * Db, (hh + 1) * HH * Db)
                part = jnp.concatenate(parts, axis=1)
                ctxb_s[:, cols] = part if t == 0 else ctxb_s[:, cols] + part
                if (2 * t + hh + 1) % seg_w == 0:
                    pm.pump(1)
        pm.pump(cfg["pump_w"], cfg["lag_w"])
        pm.drain()

        c_wqa0.wait()
        wait_pieces(wqa_s, cut_wqa, S_WQA)
        start_k(1)
        pm = pump_kv(1)
        pm.kick()
        tick(3 + B)
        c_xa.wait()
        qa_all = _dot(xa_s[...], wqa_s[...].reshape(D, H * Dh)) * scale_a
        for h in range(H):
            qa_s[pl.ds(h, B, stride=H), :] = qa_all[:, h * Dh:(h + 1) * Dh]
        pm.pump(cfg["pump_q"], cfg["lag_q"])
        pm.drain()

        def attend_a(g, start_at_k, start_at_v, pm):
            start = g * _G if isinstance(g, int) else pl.multiple_of(g * _G, _G)
            rows = pl.ds(start, _G)
            q8 = qa_s[rows, :].astype(_BF16)
            wait_pieces(k_s.at[g], cut_k, S_KV + 2 * g)
            start_at_k()
            pm.kick()
            tick(4 + B + g)
            row = lax.broadcasted_iota(jnp.int32, (_G, W), 0)
            s = None
            for j in range(_G):
                sj = _dot_nt(q8, k_s[g, j])
                s = sj if s is None else jnp.where(row == j, sj, s)
                if j in cfg["kick_qk"]:
                    pm.kick()
            m = jnp.max(s, axis=-1, keepdims=True)
            p = jnp.exp(s - m)
            l = jnp.sum(p, axis=-1, keepdims=True)
            p_s[...] = p
            pm.pump(cfg["pump_k"], cfg["lag_k"])
            wait_pieces(v_s.at[g], cut_v, S_KV + 2 * g + 1)
            start_at_v()
            pm.kick()
            pb = p_s[...].astype(_BF16)
            row2 = lax.broadcasted_iota(jnp.int32, (_G, Dh), 0)
            o = None
            for j in range(_G):
                oj = _dot(pb, v_s[g, j])
                o = oj if o is None else jnp.where(row2 == j, oj, o)
                if j in cfg["kick_pv"]:
                    pm.kick()
            oa_s[rows, :] = o / l

        def a_body(g, carry):
            pm = pump_kv(g + 2)
            attend_a(g, functools.partial(start_v, g + 1), functools.partial(start_k, g + 2), pm)
            pm.pump(cfg["pump_v"], cfg["lag_v"])
            pm.drain()
            return carry

        lax.fori_loop(0, NG - 2, a_body, 0)

        def start_wo():
            for i in range(n_wo):
                c_wo(i).start(priority=cfg.get('bulk_prio', 1))

        pm = pump_wo(0)
        attend_a(NG - 2, functools.partial(start_v, NG - 1), start_wo, pm)
        pm.pump(cfg["pump_v"], cfg["lag_v"])
        pm.drain()
        pm = pump_wo(1)
        attend_a(NG - 1, lambda: None, lambda: None, pm)

        c_wob.wait()
        n_early = side_all - side_late
        waited = max(side_all - side_nb, 0)
        for i in range(waited, n_early):
            c_sb(i).wait()
        r_early = n_early * side_rows
        ctxb = ctxb_s[...].astype(_BF16)
        part = _dot(ctxb[:, side_total:], wob_s[side_total:, :])
        pm.kick()
        step = 8 * _L
        for lo in range(0, r_early, step):
            hi = min(lo + step, r_early)
            part = part + _dot(ctxb[:, lo:hi], wob_s[lo:hi, :])
            pm.kick()
        accb_s[...] = part
        tick(4 + B + NG)

        oa32 = jnp.concatenate([oa_s[pl.ds(h, B, stride=H), :] for h in range(H)], axis=1)
        oa = oa32.astype(_BF16)
        tail0 = H * Dh - tail_rows
        for b in range(B):
            for t in range(tail_rows // Dh):
                src = oa32[b:b + 1, tail0 + t * Dh:tail0 + (t + 1) * Dh]
                coef_s[b, t * Dh:(t + 1) * Dh, :] = jnp.broadcast_to(src, (_L, Dh)).T
        pm.pump(cfg.get("pump_e", 3))
        pm.drain()
        acc_s[...] = _dot(oa[:, :wo_base], woa_s[:wo_base, :])
        for i in range(n_mxu):
            c_wo(i).wait()
            if i == late_at:
                for j in range(max(waited, n_early), side_all):
                    c_sb(j).wait()
                late = _dot(ctxb[:, r_early:side_total], wob_s[r_early:side_total, :])
                o_ref[:, D:] = (accb_s[...] + late).astype(o_ref.dtype)
            lo, n = wo_off[i], wo_chunks[i]
            part = _dot(oa[:, lo:lo + n], woa_s[lo:lo + n, :]) + acc_s[...]
            if i < n_wo - 1:
                acc_s[...] = part
            else:
                o_ref[:, :D] = part.astype(o_ref.dtype)
        for i in range(n_mxu, n_wo):
            c_wo(i).wait()
            lo, n = wo_off[i], wo_chunks[i]
            w = woa_s[lo:lo + n, :].astype(_F32)
            sums = []
            for b in range(B):
                cf = coef_s[b, lo - tail0:lo - tail0 + n, :]
                prod = w * jnp.concatenate([cf] * (D // _L), axis=1)
                acc = vacc_s[b] if i > n_mxu else None
                for r in range(0, n, 8):
                    acc = prod[r:r + 8] if acc is None else acc + prod[r:r + 8]
                if i < n_wo - 1:
                    vacc_s[b] = acc
                else:
                    sums.append(jnp.sum(acc, axis=0, keepdims=True))
            if i == n_wo - 1:
                res = acc_s[...] + jnp.concatenate(sums, axis=0)
                o_ref[:, :D] = res.astype(o_ref.dtype)

    any_spec = pl.BlockSpec(memory_space=pl.ANY)
    out = pl.pallas_call(
        kernel,
        out_shape=jax.ShapeDtypeStruct((B, D + M), A_x.dtype),
        in_specs=[any_spec] * 11,
        out_specs=pl.BlockSpec(memory_space=pltpu.VMEM),
        scratch_shapes=[
            pltpu.VMEM(xa2.shape, _BF16),
            pltpu.VMEM(xb2.shape, _BF16),
            pltpu.VMEM((2, NG, _G, W, Dh), _BF16),
            pltpu.VMEM(wqa3.shape, _BF16),
            pltpu.VMEM(A_wo.shape, _BF16),
            pltpu.VMEM(c4.shape, _BF16),
            pltpu.VMEM(wqb4.shape, _BF16),
            pltpu.VMEM(wuk4.shape, _BF16),
            pltpu.VMEM(wuv4.shape, _BF16),
            pltpu.VMEM(wob2.shape, _BF16),
            pltpu.VMEM((BH, Dh), _F32),
            pltpu.VMEM((BH, Dh), _F32),
            pltpu.VMEM((NCT, B * Hb, _L), _F32),
            pltpu.VMEM((NCT, B * Hb, _L), _F32),
            pltpu.VMEM((B, D), _F32),
            pltpu.VMEM((B, M), _F32),
            pltpu.VMEM((B, Hb * Db), _F32),
            pltpu.VMEM((B, max(tail_rows, 8), _L), _F32),
            pltpu.VMEM((B, 8, D), _F32),
            pltpu.VMEM((_G, W), _F32),
            pltpu.VMEM((Hb, Skb), _F32),
            pltpu.SMEM((side_nb, side_rows, M), _BF16),
            pltpu.SemaphoreType.DMA((n_sem,)),
        ],
        compiler_params=pltpu.CompilerParams(
            vmem_limit_bytes=120 * 1024 * 1024,
            disable_semaphore_checks=True,
            disable_bounds_checks=cfg.get('nobc', True),
        ),
        name="fused_decode",
    )(xa2, k3, v3, wqa3, A_wo, xb2, c4, wqb4, wuk4, wuv4, wob2)
    return out.reshape(B, Sq, D + M)


@jax.jit
def pallas_concat_heads__sliding_block_cached__compressed_kv_cla__decode_kernel(
    A_x: jax.Array,
    A_k_cache: jax.Array,
    A_v_cache: jax.Array,
    A_wq: jax.Array,
    A_wo: jax.Array,
    B_x: jax.Array,
    B_c_kv: jax.Array,
    B_w_q: jax.Array,
    B_w_uk: jax.Array,
    B_w_uv: jax.Array,
    B_w_o: jax.Array,
):
    return _fused(_CFG, A_x, A_k_cache, A_v_cache, A_wq, A_wo,
                  B_x, B_c_kv, B_w_q, B_w_uk, B_w_uv, B_w_o)
```

```python
import functools
import itertools

import jax
import jax.numpy as jnp
from jax import lax
import jax.experimental.pallas as pl
import jax.experimental.pallas.tpu as pltpu

_NT = (((1,), (1,)), ((), ()))
_F32 = jnp.float32
_BF16 = jnp.bfloat16
_L = 128
_G = 8
_KIB = 1024

_CFG = dict(
    wo_inj=1,
    wo_wide=5,
    wo_chunks=(512, 128, 128),
    wo_tail=(80, 64, 48, 32, 16, 16),
    shift_wo=32 * _KIB,
    pump_k15=4, pump_e=6, lag_e=2, seg_b=8,
    piece=64 * _KIB,
    shift_a=30 * _KIB,
    shift_b=32 * _KIB,
    block=512 * _KIB,
    inj_w=(16 * _KIB, 8 * _KIB, 8 * _KIB),
    inj_c=(16 * _KIB, 8 * _KIB, 8 * _KIB),
    inj_q=(16 * _KIB, 16 * _KIB),
    inj_k=(16 * _KIB,),
    inj_v=(14 * _KIB, 16 * _KIB),
    inj_wo=((8 * _KIB,) * 24, (16 * _KIB,) * 20),
    side_rows=128,
    side_n=24,
    side_last=32,
    side_nb=4,
    side_late=2,
    late_at=1,
    pump0=18,
    pump_w=8,
    pump_c=12,
    pump_q=8,
    pump_k=8,
    pump_v=9,
    lag_0=2, lag_w=2, lag_c=2, lag_q=2, lag_k=2, lag_v=2,
    seg_w=1,
    kick_s=(1, 3, 5, 7),
    kick_c=(3,),
    kick_qk=(1, 3, 5),
    kick_pv=(3,),
)


def _dot(a, b):
    return jnp.dot(a, b, preferred_element_type=_F32)


def _dot_nt(a, b):
    return lax.dot_general(a, b, _NT, preferred_element_type=_F32)


def _bounds(n_rows, row_bytes, piece, shift, skip=0):
    step = piece // row_bytes
    first = (shift // row_bytes) % step
    cuts = [skip] + [r for r in range(first, n_rows, step) if r > skip] + [n_rows]
    return list(zip(cuts[:-1], cuts[1:]))


class _Pump:
    def __init__(self, copies):
        self.copies, self.started, self.waited = list(copies), 0, 0

    def kick(self):
        if self.started < len(self.copies):
            self.copies[self.started]().start(priority=0)
            self.started += 1

    def _wait_to(self, n):
        while self.waited < n:
            self.copies[self.waited]().wait()
            self.waited += 1

    def pump(self, n, lag=1):
        for _ in range(n):
            self.kick()
            self._wait_to(self.started - lag)

    def drain(self):
        while self.started < len(self.copies):
            self.kick()
        self._wait_to(self.started)


def _fused(cfg, A_x, A_k_cache, A_v_cache, A_wq, A_wo, B_x, B_c_kv, B_w_q, B_w_uk, B_w_uv, B_w_o):
    B, Sq, D = A_x.shape
    _, H, Sk, Dh = A_k_cache.shape
    assert Sq == 1 and B_x.shape[1] == 1
    assert A_wq.shape == (D, H * Dh)
    W = min(4096, max(256, Sk // 4))
    M, Hb, Db = B_w_q.shape
    Skb, Dc = B_c_kv.shape[1], B_c_kv.shape[2]
    BH = B * H
    NG = BH // _G
    NCT = Dc // _L
    HH = Hb // 2
    scale_a = float(Dh) ** -0.5
    scale_b = float(Db) ** -0.5
    piece, block = cfg["piece"], cfg["block"]
    shift_a, shift_b = cfg["shift_a"], cfg["shift_b"]
    side_rows, side_n, side_nb = cfg["side_rows"], cfg["side_n"], cfg["side_nb"]
    side_late, late_at = cfg["side_late"], cfg["late_at"]
    n_mxu = len(cfg["wo_chunks"])
    wo_chunks = tuple(cfg["wo_chunks"]) + tuple(cfg["wo_tail"])
    tail_rows = sum(cfg["wo_tail"])
    assert tail_rows % Dh == 0 and M % _L == 0 and NG >= 4
    side_last = cfg["side_last"]
    side_all = side_n + (1 if side_last else 0)
    assert side_all <= 5 + B + NG

    xa2 = A_x.reshape(B, D)
    xb2 = B_x.reshape(B, M)
    k3 = A_k_cache.reshape(BH, Sk, Dh)
    v3 = A_v_cache.reshape(BH, Sk, Dh)
    wob2 = B_w_o.reshape(Hb * Db, M)

    def blocked(w, lead=0):
        row_bytes = 2 * functools.reduce(lambda a, b: a * b, w.shape[lead + 1:], 1)
        rows = block // row_bytes
        shape = w.shape[:lead] + (w.shape[lead] // rows, rows) + w.shape[lead + 1:]
        return w.reshape(shape), rows, row_bytes

    wqa3, r_wqa, b_wqa = blocked(A_wq)
    wqb4, r_w, b_w = blocked(B_w_q)
    wuk4, _, _ = blocked(B_w_uk)
    wuv4, _, _ = blocked(B_w_uv)
    c4, r_c, b_c = blocked(B_c_kv, 1)
    woa3, r_wo, b_wo = blocked(A_wo)
    assert wqb4.shape == wuk4.shape == wuv4.shape and (2 * r_w) == _L
    NBLK = wqb4.shape[0]

    def spans(sizes, unit):
        ends = list(itertools.accumulate(n // unit for n in sizes))
        return list(zip([0] + ends[:-1], ends))

    i_w, i_c = spans(cfg["inj_w"], b_w), spans(cfg["inj_c"], b_c)
    i_k, i_v = spans(cfg["inj_k"], 2 * Dh), spans(cfg["inj_v"], 2 * Dh)
    i_wqa = spans(cfg["inj_q"], 2 * 8)
    i_wo = spans(cfg["inj_wo"][0] + cfg["inj_wo"][1], 2 * D)
    n14 = len(cfg["inj_wo"][0])
    cut_w0 = _bounds(r_w, b_w, piece, shift_b)
    cut_w = _bounds(r_w, b_w, piece, shift_b, i_w[-1][1])
    cut_c = _bounds(r_c, b_c, piece, shift_b, i_c[-1][1])
    cut_k = _bounds(W, 2 * Dh, piece, shift_a, i_k[-1][1])
    cut_v = _bounds(W, 2 * Dh, piece, shift_a, i_v[-1][1])
    cut_wqa = _bounds(r_wqa, b_wqa, max(piece, 8 * b_wqa), 0, 8)
    wo_inj, wo_wide = cfg["wo_inj"], cfg["wo_wide"]
    cut_wo = _bounds(r_wo, b_wo, piece, cfg["shift_wo"])
    wo_base = (wo_inj + wo_wide) * r_wo
    assert i_wo[-1][1] == wo_inj * r_wo
    assert wo_base + sum(wo_chunks) == H * Dh
    n_wo = len(wo_chunks)
    wo_off = [wo_base + sum(wo_chunks[:i]) for i in range(n_wo)]
    assert all(lo // r_wo == (lo + n - 1) // r_wo for lo, n in zip(wo_off, wo_chunks))
    S_XB, S_XA, S_WQB, S_WUK, S_WUV, S_WOB, S_WQA, S_INJ, S_WIDE = range(9)
    S_C = 9
    S_KV = S_C + B
    S_WO = S_KV + 2 * NG
    S_SA = S_WO + n_wo
    S_SB = S_SA + side_nb
    n_sem = S_SB + side_nb
    side_total = side_rows * side_n + side_last

    def kernel(xa_h, k_h, v_h, wqa_h, woa_h, xb_h, c_h, wqb_h, wuk_h, wuv_h, wob_h,
               o_ref,
               xa_s, xb_s, kv_s, wqa_s, woa_s, c_s, wqb_s, wuk_s, wuv_s, wob_s,
               qa_s, oa_s, qabs_s, ctx_s, acc_s, accb_s, ctxb_s, oab_s, coef_s, vacc_s, p_s, s_s, side_s, sem):
        def cp(src, dst, s):
            return pltpu.make_async_copy(src, dst, sem.at[s])

        def start_pieces(src, dst, cuts, s, row0=0):
            for lo, hi in cuts:
                cp(src.at[:, pl.ds(row0 + lo, hi - lo)], dst.at[:, pl.ds(lo, hi - lo)],
                   s).start(priority=cfg.get('bulk_prio', 1))

        def wait_pieces(dst, cuts, s):
            view = dst.at[:, pl.ds(cuts[0][0], cuts[-1][1] - cuts[0][0])]
            cp(view, view, s).wait()

        def heads_of(src, dst, ranges, row0=0):
            def one(k, lo, hi):
                return cp(src.at[k, pl.ds(row0 + lo, hi - lo)], dst.at[k, pl.ds(lo, hi - lo)], S_INJ)
            return [functools.partial(one, k, lo, hi)
                    for lo, hi in ranges for k in range(dst.shape[0])]

        k_s, v_s = kv_s.at[0], kv_s.at[1]
        c_xb = cp(xb_h, xb_s, S_XB)
        c_xa = cp(xa_h, xa_s, S_XA)
        rest = pl.ds(side_total, Hb * Db - side_total)
        c_wob = cp(wob_h.at[rest, :], wob_s.at[rest, :], S_WOB)

        def start_c(b):
            start_pieces(c_h.at[b], c_s.at[b], cut_c, S_C + b)

        def pump_c(b):
            return _Pump(heads_of(c_h.at[b], c_s.at[b], i_c))

        wqa_rest = (slice(None), pl.ds(0, 8), pl.ds(i_wqa[-1][1], H * Dh - i_wqa[-1][1]))
        c_wqa0 = cp(wqa_h.at[wqa_rest], wqa_s.at[wqa_rest], S_WQA)

        def start_wqa():
            c_wob.start(priority=cfg.get('bulk_prio', 1))
            c_wqa0.start(priority=cfg.get('bulk_prio', 1))
            start_pieces(wqa_h, wqa_s, cut_wqa, S_WQA)

        def pump_wqa():
            def one(k, lo, hi):
                at = (k, pl.ds(0, 8), pl.ds(lo, hi - lo))
                return cp(wqa_h.at[at], wqa_s.at[at], S_INJ)
            return _Pump([functools.partial(one, k, lo, hi)
                          for lo, hi in i_wqa for k in range(NBLK)])

        def start_k(g):
            start_pieces(k_h.at[pl.ds(g * _G, _G)], k_s.at[g], cut_k, S_KV + 2 * g, Sk - W)

        def start_v(g):
            start_pieces(v_h.at[pl.ds(g * _G, _G)], v_s.at[g], cut_v, S_KV + 2 * g + 1, Sk - W)

        def pump_kv(g):
            heads = pl.ds(g * _G, _G)
            return _Pump(heads_of(k_h.at[heads], k_s.at[g], i_k, Sk - W)
                         + heads_of(v_h.at[heads], v_s.at[g], i_v, Sk - W))

        def wo_at(lo, n):
            return lo // r_wo, pl.ds(lo % r_wo, n)

        def c_wo(i):
            at = wo_at(wo_off[i], wo_chunks[i])
            return cp(woa_h.at[at], woa_s.at[at], S_WO + i)

        wide = pl.ds(wo_inj, wo_wide)

        def start_wo():
            start_pieces(woa_h.at[wide], woa_s.at[wide], cut_wo, S_WIDE)
            for i in range(n_wo):
                c_wo(i).start(priority=cfg.get('bulk_prio', 1))

        def pump_wo(first, last):
            def one(lo, hi):
                at = wo_at(lo, hi - lo)
                return cp(woa_h.at[at], woa_s.at[at], S_INJ)
            return _Pump([functools.partial(one, *i_wo[j]) for j in range(first, last)])

        def side_refs(i):
            start = i * side_rows
            n = side_rows
            if not isinstance(i, int):
                start = pl.multiple_of(start, 8)
            elif i == side_n:
                n = side_last
            slot = i % side_nb
            return pl.ds(start, n), side_s.at[slot, pl.ds(0, n)], slot

        def c_sa(i):
            rows, stage, slot = side_refs(i)
            return cp(wob_h.at[rows, :], stage, S_SA + slot)

        def c_sb(i):
            rows, stage, slot = side_refs(i)
            return cp(stage, wob_s.at[rows, :], S_SB + slot)

        lag = 2

        def when(cond, fn):
            if isinstance(cond, bool):
                if cond:
                    fn()
            else:
                pl.when(cond)(fn)

        def tick(i):
            def forward():
                c_sa(i).wait()
                c_sb(i).start()

            def refill():
                if not isinstance(i, int) or i >= lag:
                    c_sb(i - lag).wait()
                c_sa(i - lag + side_nb).start()

            if isinstance(i, int):
                when(i < side_all, forward)
                when(i - lag + side_nb < side_all, refill)
            else:
                assert 4 + B + NG - 3 - lag + side_nb < side_n
                forward()
                refill()

        def head_major(w_s, t, hh):
            w = w_s[2 * t:2 * t + 2, :, hh * HH:(hh + 1) * HH, :]
            return w.reshape(_L, HH, Db).reshape(_L, HH * Db)

        start_pieces(wqb_h, wqb_s, cut_w0, S_WQB)
        c_xb.start()
        c_xa.start()
        for i in range(side_nb - lag):
            c_sa(i).start()
        start_pieces(wuk_h, wuk_s, cut_w, S_WUK)
        pm = _Pump(heads_of(wuk_h, wuk_s, i_w))
        pm.pump(cfg["pump0"], cfg["lag_0"])
        pm.drain()

        seg_w = cfg["seg_w"]

        wait_pieces(wqb_s, cut_w0, S_WQB)
        start_c(0)
        pm = pump_c(0)
        pm.kick()
        tick(0)
        c_xb.wait()
        xb = xb_s[...]
        for t in range(M // _L):
            for hh in range(2):
                cols = slice(hh * HH * Db, (hh + 1) * HH * Db)
                part = _dot(xb[:, t * _L:(t + 1) * _L], head_major(wqb_s, t, hh))
                ctxb_s[:, cols] = part if t == 0 else ctxb_s[:, cols] + part
                if (2 * t + hh + 1) % seg_w == 0:
                    pm.pump(1)
        pm.pump(cfg["pump_w"], cfg["lag_w"])
        pm.drain()

        wait_pieces(wuk_s, cut_w, S_WUK)
        start_c(1)
        pm = pump_c(1)
        pm.kick()
        tick(1)
        qb = (ctxb_s[...] * scale_b).astype(_BF16)
        for t in range(NCT):
            for hh in range(2):
                w = head_major(wuk_s, t, hh)
                parts = [_dot_nt(qb[:, (hh * HH + j) * Db:(hh * HH + j + 1) * Db],
                                 w[:, j * Db:(j + 1) * Db]) for j in range(HH)]
                qabs_s[t, :, hh * HH:(hh + 1) * HH, :] = jnp.concatenate(
                    parts, axis=1).reshape(B, HH, _L)
                if (2 * t + hh + 1) % seg_w == 0:
                    pm.pump(1)
        pm.pump(cfg["pump_w"], cfg["lag_w"])
        pm.drain()

        def attend_b(b, start_next, pm, same_buffer):
            wait_pieces(c_s.at[b], cut_c, S_C + b)
            start_next()
            pm.kick()
            tick(2 + b)
            step = pm.kick if same_buffer else functools.partial(pm.pump, 1)
            qa = jnp.concatenate(
                [qabs_s[t, b] for t in range(NCT)], axis=1).astype(_BF16)
            for k in range(NBLK):
                s_s[:, k * r_c:(k + 1) * r_c] = _dot_nt(qa, c_s[b, k])
                if k in cfg["kick_s"]:
                    step()
            s = s_s[...]
            m = jnp.max(s, axis=-1, keepdims=True)
            p = jnp.exp(s - m)
            l = jnp.sum(p, axis=-1, keepdims=True)
            pb = p.astype(_BF16)
            cc = None
            for k in range(NBLK):
                part = _dot(pb[:, k * r_c:(k + 1) * r_c], c_s[b, k])
                cc = part if cc is None else cc + part
                if k in cfg["kick_c"]:
                    if not same_buffer:
                        s_s[:, :Dc] = cc
                    step()
                    if not same_buffer:
                        cc = s_s[:, :Dc]
            cc = cc / l
            for t in range(NCT):
                ctx_s[t, b] = cc[:, t * _L:(t + 1) * _L]
            pm.pump(cfg["pump_c"], cfg["lag_c"])
            pm.drain()

        for b in range(B):
            if b + 2 < B:
                attend_b(b, functools.partial(start_c, b + 2), pump_c(b + 2), True)
            elif b + 2 == B:
                attend_b(b, functools.partial(start_pieces, wuv_h, wuv_s, cut_w, S_WUV),
                         _Pump(heads_of(wuv_h, wuv_s, i_w)), False)
            else:
                attend_b(b, start_wqa, pump_wqa(), False)

        wait_pieces(wuv_s, cut_w, S_WUV)
        start_k(0)
        start_v(0)
        pm = pump_kv(0)
        pm.kick()
        tick(2 + B)
        for t in range(NCT):
            for hh in range(2):
                w = head_major(wuv_s, t, hh)
                ch = ctx_s[t, :, hh * HH:(hh + 1) * HH, :].reshape(B, HH * _L).astype(_BF16)
                parts = [_dot(ch[:, j * _L:(j + 1) * _L], w[:, j * Db:(j + 1) * Db])
                         for j in range(HH)]
                cols = slice(hh * HH * Db, (hh + 1) * HH * Db)
                part = jnp.concatenate(parts, axis=1)
                ctxb_s[:, cols] = part if t == 0 else ctxb_s[:, cols] + part
                if (2 * t + hh + 1) % seg_w == 0:
                    pm.pump(1)
        pm.pump(cfg["pump_w"], cfg["lag_w"])
        pm.drain()

        c_wqa0.wait()
        wait_pieces(wqa_s, cut_wqa, S_WQA)
        start_k(1)
        pm = pump_kv(1)
        pm.kick()
        tick(3 + B)
        c_xa.wait()
        qa_all = _dot(xa_s[...], wqa_s[...].reshape(D, H * Dh)) * scale_a
        qa_s[...] = qa_all.reshape(B, H, Dh).reshape(BH, Dh)
        pm.pump(cfg["pump_q"], cfg["lag_q"])
        pm.drain()

        def attend_a(g, start_at_k, start_at_v, pm, same_buffer, between):
            start = g * _G if isinstance(g, int) else pl.multiple_of(g * _G, _G)
            rows = pl.ds(start, _G)
            q8 = qa_s[rows, :].astype(_BF16)
            wait_pieces(k_s.at[g], cut_k, S_KV + 2 * g)
            start_at_k()
            pm.kick()
            tick(4 + B + g)
            row = lax.broadcasted_iota(jnp.int32, (_G, W), 0)
            s = None
            for j in range(_G):
                sj = _dot_nt(q8, k_s[g, j])
                s = sj if s is None else jnp.where(row == j, sj, s)
                if j in cfg["kick_qk"]:
                    if same_buffer:
                        pm.kick()
                    else:
                        p_s[...] = s
                        pm.pump(1)
                        s = p_s[...]
            m = jnp.max(s, axis=-1, keepdims=True)
            p = jnp.exp(s - m)
            l = jnp.sum(p, axis=-1, keepdims=True)
            p_s[...] = p
            between()
            wait_pieces(v_s.at[g], cut_v, S_KV + 2 * g + 1)
            start_at_v()
            pm.kick() if same_buffer else pm.pump(1)
            pb = p_s[...].astype(_BF16)
            row2 = lax.broadcasted_iota(jnp.int32, (_G, Dh), 0)
            o = None
            for j in range(_G):
                oj = _dot(pb, v_s[g, j])
                o = oj if o is None else jnp.where(row2 == j, oj, o)
                if j in cfg["kick_pv"] and same_buffer:
                    pm.kick()
            oa_s[rows, :] = o / l

        def a_body(g, carry):
            pm = pump_kv(g + 2)
            attend_a(g, functools.partial(start_v, g + 1), functools.partial(start_k, g + 2), pm,
                     True, functools.partial(pm.pump, cfg["pump_k"], cfg["lag_k"]))
            pm.pump(cfg["pump_v"], cfg["lag_v"])
            pm.drain()
            return carry

        lax.fori_loop(0, NG - 2, a_body, 0)

        pm = pump_wo(0, n14)
        attend_a(NG - 2, functools.partial(start_v, NG - 1), start_wo, pm,
                 False, functools.partial(pm.pump, cfg["pump_k"], cfg["lag_k"]))
        pm.pump(cfg["pump_v"], cfg["lag_v"])
        pm.drain()

        n_early = side_all - side_late
        waited = max(side_all - side_nb, 0)
        r_early = n_early * side_rows
        pm = pump_wo(n14, len(i_wo))

        def project_b():
            tick(4 + B + NG)
            c_wob.wait()
            for i in range(waited, n_early):
                c_sb(i).wait()
            ctxb = ctxb_s[...].astype(_BF16)
            accb_s[...] = _dot(ctxb[:, side_total:], wob_s[side_total:, :])
            step = cfg["seg_b"] * _L
            for lo in range(0, r_early, step):
                pm.pump(1)
                hi = min(lo + step, r_early)
                accb_s[...] += _dot(ctxb[:, lo:hi], wob_s[lo:hi, :])
            pm.pump(cfg["pump_k15"], cfg["lag_k"])

        attend_a(NG - 1, lambda: None, lambda: None, pm, False, project_b)
        pm.pump(1)

        oa32 = oa_s[...].reshape(B, H, Dh).reshape(B, H * Dh)
        oab_s[...] = oa32
        tail0 = H * Dh - tail_rows
        for b in range(B):
            for t in range(tail_rows // Dh):
                src = oa32[b:b + 1, tail0 + t * Dh:tail0 + (t + 1) * Dh]
                coef_s[b, t * Dh:(t + 1) * Dh, :] = jnp.broadcast_to(src, (_L, Dh)).T
        pm.pump(cfg["pump_e"], cfg["lag_e"])
        pm.drain()
        oa = oab_s[...].astype(_BF16)
        n_inj = wo_inj * r_wo
        acc_s[...] = _dot(oa[:, :n_inj], woa_s[:wo_inj].reshape(n_inj, D))
        wait_pieces(woa_s.at[wide], cut_wo, S_WIDE)
        acc_s[...] += _dot(oa[:, n_inj:wo_base],
                           woa_s[wo_inj:wo_inj + wo_wide].reshape(wo_base - n_inj, D))
        for i in range(n_mxu):
            c_wo(i).wait()
            if i == late_at:
                for j in range(max(waited, n_early), side_all):
                    c_sb(j).wait()
                late = _dot(ctxb_s[:, r_early:side_total].astype(_BF16),
                            wob_s[r_early:side_total, :])
                o_ref[:, D:] = (accb_s[...] + late).astype(o_ref.dtype)
            lo, n = wo_off[i], wo_chunks[i]
            part = _dot(oa[:, lo:lo + n], woa_s[wo_at(lo, n)]) + acc_s[...]
            if i < n_wo - 1:
                acc_s[...] = part
            else:
                o_ref[:, :D] = part.astype(o_ref.dtype)
        for i in range(n_mxu, n_wo):
            c_wo(i).wait()
            lo, n = wo_off[i], wo_chunks[i]
            w = woa_s[wo_at(lo, n)].astype(_F32)
            sums = []
            for b in range(B):
                cf = coef_s[b, lo - tail0:lo - tail0 + n, :]
                prod = w * jnp.concatenate([cf] * (D // _L), axis=1)
                acc = vacc_s[b] if i > n_mxu else None
                for r in range(0, n, 8):
                    acc = prod[r:r + 8] if acc is None else acc + prod[r:r + 8]
                if i < n_wo - 1:
                    vacc_s[b] = acc
                else:
                    sums.append(jnp.sum(acc, axis=0, keepdims=True))
            if i == n_wo - 1:
                res = acc_s[...] + jnp.concatenate(sums, axis=0)
                o_ref[:, :D] = res.astype(o_ref.dtype)

    any_spec = pl.BlockSpec(memory_space=pl.ANY)
    out = pl.pallas_call(
        kernel,
        out_shape=jax.ShapeDtypeStruct((B, D + M), A_x.dtype),
        in_specs=[any_spec] * 11,
        out_specs=pl.BlockSpec(memory_space=pltpu.VMEM),
        scratch_shapes=[
            pltpu.VMEM(xa2.shape, _BF16),
            pltpu.VMEM(xb2.shape, _BF16),
            pltpu.VMEM((2, NG, _G, W, Dh), _BF16),
            pltpu.VMEM(wqa3.shape, _BF16),
            pltpu.VMEM(woa3.shape, _BF16),
            pltpu.VMEM(c4.shape, _BF16),
            pltpu.VMEM(wqb4.shape, _BF16),
            pltpu.VMEM(wuk4.shape, _BF16),
            pltpu.VMEM(wuv4.shape, _BF16),
            pltpu.VMEM(wob2.shape, _BF16),
            pltpu.VMEM((BH, Dh), _F32),
            pltpu.VMEM((BH, Dh), _F32),
            pltpu.VMEM((NCT, B, Hb, _L), _F32),
            pltpu.VMEM((NCT, B, Hb, _L), _F32),
            pltpu.VMEM((B, D), _F32),
            pltpu.VMEM((B, M), _F32),
            pltpu.VMEM((B, Hb * Db), _F32),
            pltpu.VMEM((B, H * Dh), _F32),
            pltpu.VMEM((B, max(tail_rows, 8), _L), _F32),
            pltpu.VMEM((B, 8, D), _F32),
            pltpu.VMEM((_G, W), _F32),
            pltpu.VMEM((Hb, Skb), _F32),
            pltpu.SMEM((side_nb, side_rows, M), _BF16),
            pltpu.SemaphoreType.DMA((n_sem,)),
        ],
        compiler_params=pltpu.CompilerParams(
            vmem_limit_bytes=120 * 1024 * 1024,
            disable_semaphore_checks=True,
            disable_bounds_checks=cfg.get('nobc', True),
        ),
        name="fused_decode",
    )(xa2, k3, v3, wqa3, woa3, xb2, c4, wqb4, wuk4, wuv4, wob2)
    return out.reshape(B, Sq, D + M)


@jax.jit
def pallas_concat_heads__sliding_block_cached__compressed_kv_cla__decode_kernel(
    A_x: jax.Array,
    A_k_cache: jax.Array,
    A_v_cache: jax.Array,
    A_wq: jax.Array,
    A_wo: jax.Array,
    B_x: jax.Array,
    B_c_kv: jax.Array,
    B_w_q: jax.Array,
    B_w_uk: jax.Array,
    B_w_uv: jax.Array,
    B_w_o: jax.Array,
):
    return _fused(_CFG, A_x, A_k_cache, A_v_cache, A_wq, A_wo,
                  B_x, B_c_kv, B_w_q, B_w_uk, B_w_uv, B_w_o)
```

```python
import functools
import itertools

import jax
import jax.numpy as jnp
from jax import lax
import jax.experimental.pallas as pl
import jax.experimental.pallas.tpu as pltpu

_NT = (((1,), (1,)), ((), ()))
_F32 = jnp.float32
_BF16 = jnp.bfloat16
_L = 128
_G = 8
_KIB = 1024

_CFG = dict(
    wo_inj=1,
    wo_wide=5,
    wo_chunks=(512, 128, 128),
    wo_tail=(80, 64, 48, 32, 16, 16),
    shift_wo=32 * _KIB,
    pump_k15=4, pump_e=6, lag_e=2, seg_b=8,
    piece=64 * _KIB,
    shift_a=30 * _KIB,
    shift_b=32 * _KIB,
    block=512 * _KIB,
    inj_w=(16 * _KIB, 8 * _KIB, 8 * _KIB),
    inj_c=(16 * _KIB, 8 * _KIB, 8 * _KIB),
    inj_q=(14 * _KIB, 8 * _KIB, 8 * _KIB),
    inj_k=(16 * _KIB,),
    inj_v=(14 * _KIB, 16 * _KIB),
    inj_wo=((8 * _KIB,) * 24, (16 * _KIB,) * 20),
    side_rows=128,
    side_n=24,
    side_last=32,
    side_nb=4,
    side_late=2,
    late_at=1,
    pump0=18,
    pump_w=8,
    pump_c=12,
    pump_q=8,
    pump_k=8,
    pump_v=9,
    lag_0=2, lag_w=2, lag_c=2, lag_q=2, lag_k=2, lag_v=2,
    seg_w=1,
    kick_s=(1, 3, 5, 7),
    kick_c=(3,),
    kick_qk=(1, 3, 5),
    kick_pv=(3,),
)


def _dot(a, b):
    return jnp.dot(a, b, preferred_element_type=_F32)


def _dot_nt(a, b):
    return lax.dot_general(a, b, _NT, preferred_element_type=_F32)


def _bounds(n_rows, row_bytes, piece, shift, skip=0):
    step = piece // row_bytes
    first = (shift // row_bytes) % step
    cuts = [skip] + [r for r in range(first, n_rows, step) if r > skip] + [n_rows]
    return list(zip(cuts[:-1], cuts[1:]))


class _Pump:
    def __init__(self, copies):
        self.copies, self.started, self.waited = list(copies), 0, 0

    def kick(self):
        if self.started < len(self.copies):
            self.copies[self.started]().start(priority=0)
            self.started += 1

    def _wait_to(self, n):
        while self.waited < n:
            self.copies[self.waited]().wait()
            self.waited += 1

    def pump(self, n, lag=1):
        for _ in range(n):
            self.kick()
            self._wait_to(self.started - lag)

    def drain(self):
        while self.started < len(self.copies):
            self.kick()
        self._wait_to(self.started)


def _fused(cfg, A_x, A_k_cache, A_v_cache, A_wq, A_wo, B_x, B_c_kv, B_w_q, B_w_uk, B_w_uv, B_w_o):
    B, Sq, D = A_x.shape
    _, H, Sk, Dh = A_k_cache.shape
    assert Sq == 1 and B_x.shape[1] == 1
    assert A_wq.shape == (D, H * Dh)
    W = min(4096, max(256, Sk // 4))
    M, Hb, Db = B_w_q.shape
    Skb, Dc = B_c_kv.shape[1], B_c_kv.shape[2]
    BH = B * H
    NG = BH // _G
    NCT = Dc // _L
    HH = Hb // 2
    scale_a = float(Dh) ** -0.5
    scale_b = float(Db) ** -0.5
    piece, block = cfg["piece"], cfg["block"]
    shift_a, shift_b = cfg["shift_a"], cfg["shift_b"]
    side_rows, side_n, side_nb = cfg["side_rows"], cfg["side_n"], cfg["side_nb"]
    side_late, late_at = cfg["side_late"], cfg["late_at"]
    n_mxu = len(cfg["wo_chunks"])
    wo_chunks = tuple(cfg["wo_chunks"]) + tuple(cfg["wo_tail"])
    tail_rows = sum(cfg["wo_tail"])
    assert tail_rows % Dh == 0 and M % _L == 0 and NG >= 4
    side_last = cfg["side_last"]
    side_all = side_n + (1 if side_last else 0)
    assert side_all <= 5 + B + NG

    xa2 = A_x.reshape(B, D)
    xb2 = B_x.reshape(B, M)
    k3 = A_k_cache.reshape(BH, Sk, Dh)
    v3 = A_v_cache.reshape(BH, Sk, Dh)
    wob2 = B_w_o.reshape(Hb * Db, M)

    def blocked(w, lead=0):
        row_bytes = 2 * functools.reduce(lambda a, b: a * b, w.shape[lead + 1:], 1)
        rows = block // row_bytes
        shape = w.shape[:lead] + (w.shape[lead] // rows, rows) + w.shape[lead + 1:]
        return w.reshape(shape), rows, row_bytes

    n_ct = H * Dh // _L
    wqa_t = A_wq.reshape(D // 8, 8, n_ct, _L).transpose(0, 2, 1, 3).reshape(D // 8 * n_ct, 8, _L)
    wqa3, r_wqa, b_wqa = blocked(wqa_t)
    wqb4, r_w, b_w = blocked(B_w_q)
    wuk4, _, _ = blocked(B_w_uk)
    wuv4, _, _ = blocked(B_w_uv)
    c4, r_c, b_c = blocked(B_c_kv, 1)
    woa3, r_wo, b_wo = blocked(A_wo)
    assert wqb4.shape == wuk4.shape == wuv4.shape and (2 * r_w) == _L
    NBLK = wqb4.shape[0]

    def spans(sizes, unit):
        ends = list(itertools.accumulate(n // unit for n in sizes))
        return list(zip([0] + ends[:-1], ends))

    i_w, i_c = spans(cfg["inj_w"], b_w), spans(cfg["inj_c"], b_c)
    i_k, i_v = spans(cfg["inj_k"], 2 * Dh), spans(cfg["inj_v"], 2 * Dh)
    i_wqa = spans(cfg["inj_q"], b_wqa)
    i_wo = spans(cfg["inj_wo"][0] + cfg["inj_wo"][1], 2 * D)
    n14 = len(cfg["inj_wo"][0])
    cut_w0 = _bounds(r_w, b_w, piece, shift_b)
    cut_w = _bounds(r_w, b_w, piece, shift_b, i_w[-1][1])
    cut_c = _bounds(r_c, b_c, piece, shift_b, i_c[-1][1])
    cut_k = _bounds(W, 2 * Dh, piece, shift_a, i_k[-1][1])
    cut_v = _bounds(W, 2 * Dh, piece, shift_a, i_v[-1][1])
    cut_wqa = _bounds(r_wqa, b_wqa, piece, shift_a, i_wqa[-1][1])
    wo_inj, wo_wide = cfg["wo_inj"], cfg["wo_wide"]
    cut_wo = _bounds(r_wo, b_wo, piece, cfg["shift_wo"])
    wo_base = (wo_inj + wo_wide) * r_wo
    assert i_wo[-1][1] == wo_inj * r_wo
    assert wo_base + sum(wo_chunks) == H * Dh
    n_wo = len(wo_chunks)
    wo_off = [wo_base + sum(wo_chunks[:i]) for i in range(n_wo)]
    assert all(lo // r_wo == (lo + n - 1) // r_wo for lo, n in zip(wo_off, wo_chunks))
    S_XB, S_XA, S_WQB, S_WUK, S_WUV, S_WOB, S_WQA, S_INJ, S_WIDE = range(9)
    S_C = 9
    S_KV = S_C + B
    S_WO = S_KV + 2 * NG
    S_SA = S_WO + n_wo
    S_SB = S_SA + side_nb
    n_sem = S_SB + side_nb
    side_total = side_rows * side_n + side_last

    def kernel(xa_h, k_h, v_h, wqa_h, woa_h, xb_h, c_h, wqb_h, wuk_h, wuv_h, wob_h,
               o_ref,
               xa_s, xb_s, kv_s, wqa_s, woa_s, c_s, wqb_s, wuk_s, wuv_s, wob_s,
               qa_s, oa_s, qabs_s, ctx_s, acc_s, accb_s, ctxb_s, oab_s, coef_s, vacc_s, p_s, s_s, side_s, sem):
        def cp(src, dst, s):
            return pltpu.make_async_copy(src, dst, sem.at[s])

        def start_pieces(src, dst, cuts, s, row0=0):
            for lo, hi in cuts:
                cp(src.at[:, pl.ds(row0 + lo, hi - lo)], dst.at[:, pl.ds(lo, hi - lo)],
                   s).start(priority=cfg.get('bulk_prio', 1))

        def wait_pieces(dst, cuts, s):
            view = dst.at[:, pl.ds(cuts[0][0], cuts[-1][1] - cuts[0][0])]
            cp(view, view, s).wait()

        def heads_of(src, dst, ranges, row0=0):
            def one(k, lo, hi):
                return cp(src.at[k, pl.ds(row0 + lo, hi - lo)], dst.at[k, pl.ds(lo, hi - lo)], S_INJ)
            return [functools.partial(one, k, lo, hi)
                    for lo, hi in ranges for k in range(dst.shape[0])]

        k_s, v_s = kv_s.at[0], kv_s.at[1]
        c_xb = cp(xb_h, xb_s, S_XB)
        c_xa = cp(xa_h, xa_s, S_XA)
        rest = pl.ds(side_total, Hb * Db - side_total)
        c_wob = cp(wob_h.at[rest, :], wob_s.at[rest, :], S_WOB)

        def start_c(b):
            start_pieces(c_h.at[b], c_s.at[b], cut_c, S_C + b)

        def pump_c(b):
            return _Pump(heads_of(c_h.at[b], c_s.at[b], i_c))

        def start_wqa():
            c_wob.start(priority=cfg.get('bulk_prio', 1))
            start_pieces(wqa_h, wqa_s, cut_wqa, S_WQA)

        def start_k(g):
            start_pieces(k_h.at[pl.ds(g * _G, _G)], k_s.at[g], cut_k, S_KV + 2 * g, Sk - W)

        def start_v(g):
            start_pieces(v_h.at[pl.ds(g * _G, _G)], v_s.at[g], cut_v, S_KV + 2 * g + 1, Sk - W)

        def pump_kv(g):
            heads = pl.ds(g * _G, _G)
            return _Pump(heads_of(k_h.at[heads], k_s.at[g], i_k, Sk - W)
                         + heads_of(v_h.at[heads], v_s.at[g], i_v, Sk - W))

        def wo_at(lo, n):
            return lo // r_wo, pl.ds(lo % r_wo, n)

        def c_wo(i):
            at = wo_at(wo_off[i], wo_chunks[i])
            return cp(woa_h.at[at], woa_s.at[at], S_WO + i)

        wide = pl.ds(wo_inj, wo_wide)

        def start_wo():
            start_pieces(woa_h.at[wide], woa_s.at[wide], cut_wo, S_WIDE)
            for i in range(n_wo):
                c_wo(i).start(priority=cfg.get('bulk_prio', 1))

        def pump_wo(first, last):
            def one(lo, hi):
                at = wo_at(lo, hi - lo)
                return cp(woa_h.at[at], woa_s.at[at], S_INJ)
            return _Pump([functools.partial(one, *i_wo[j]) for j in range(first, last)])

        def side_refs(i):
            start = i * side_rows
            n = side_rows
            if not isinstance(i, int):
                start = pl.multiple_of(start, 8)
            elif i == side_n:
                n = side_last
            slot = i % side_nb
            return pl.ds(start, n), side_s.at[slot, pl.ds(0, n)], slot

        def c_sa(i):
            rows, stage, slot = side_refs(i)
            return cp(wob_h.at[rows, :], stage, S_SA + slot)

        def c_sb(i):
            rows, stage, slot = side_refs(i)
            return cp(stage, wob_s.at[rows, :], S_SB + slot)

        lag = 2

        def when(cond, fn):
            if isinstance(cond, bool):
                if cond:
                    fn()
            else:
                pl.when(cond)(fn)

        def tick(i):
            def forward():
                c_sa(i).wait()
                c_sb(i).start()

            def refill():
                if not isinstance(i, int) or i >= lag:
                    c_sb(i - lag).wait()
                c_sa(i - lag + side_nb).start()

            if isinstance(i, int):
                when(i < side_all, forward)
                when(i - lag + side_nb < side_all, refill)
            else:
                assert 4 + B + NG - 3 - lag + side_nb < side_n
                forward()
                refill()

        def head_major(w_s, t, hh):
            w = w_s[2 * t:2 * t + 2, :, hh * HH:(hh + 1) * HH, :]
            return w.reshape(_L, HH, Db).reshape(_L, HH * Db)

        start_pieces(wqb_h, wqb_s, cut_w0, S_WQB)
        c_xb.start()
        c_xa.start()
        for i in range(side_nb - lag):
            c_sa(i).start()
        start_pieces(wuk_h, wuk_s, cut_w, S_WUK)
        pm = _Pump(heads_of(wuk_h, wuk_s, i_w))
        pm.pump(cfg["pump0"], cfg["lag_0"])
        pm.drain()

        seg_w = cfg["seg_w"]

        wait_pieces(wqb_s, cut_w0, S_WQB)
        start_c(0)
        pm = pump_c(0)
        pm.kick()
        tick(0)
        c_xb.wait()
        xb = xb_s[...]
        for t in range(M // _L):
            for hh in range(2):
                cols = slice(hh * HH * Db, (hh + 1) * HH * Db)
                part = _dot(xb[:, t * _L:(t + 1) * _L], head_major(wqb_s, t, hh))
                ctxb_s[:, cols] = part if t == 0 else ctxb_s[:, cols] + part
                if (2 * t + hh + 1) % seg_w == 0:
                    pm.pump(1)
        pm.pump(cfg["pump_w"], cfg["lag_w"])
        pm.drain()

        wait_pieces(wuk_s, cut_w, S_WUK)
        start_c(1)
        pm = pump_c(1)
        pm.kick()
        tick(1)
        qb = (ctxb_s[...] * scale_b).astype(_BF16)
        for t in range(NCT):
            for hh in range(2):
                w = head_major(wuk_s, t, hh)
                parts = [_dot_nt(qb[:, (hh * HH + j) * Db:(hh * HH + j + 1) * Db],
                                 w[:, j * Db:(j + 1) * Db]) for j in range(HH)]
                qabs_s[t, :, hh * HH:(hh + 1) * HH, :] = jnp.concatenate(
                    parts, axis=1).reshape(B, HH, _L)
                if (2 * t + hh + 1) % seg_w == 0:
                    pm.pump(1)
        pm.pump(cfg["pump_w"], cfg["lag_w"])
        pm.drain()

        def attend_b(b, start_next, pm, same_buffer):
            wait_pieces(c_s.at[b], cut_c, S_C + b)
            start_next()
            pm.kick()
            tick(2 + b)
            step = pm.kick if same_buffer else functools.partial(pm.pump, 1)
            qa = jnp.concatenate(
                [qabs_s[t, b] for t in range(NCT)], axis=1).astype(_BF16)
            for k in range(NBLK):
                s_s[:, k * r_c:(k + 1) * r_c] = _dot_nt(qa, c_s[b, k])
                if k in cfg["kick_s"]:
                    step()
            s = s_s[...]
            m = jnp.max(s, axis=-1, keepdims=True)
            p = jnp.exp(s - m)
            l = jnp.sum(p, axis=-1, keepdims=True)
            pb = p.astype(_BF16)
            cc = None
            for k in range(NBLK):
                part = _dot(pb[:, k * r_c:(k + 1) * r_c], c_s[b, k])
                cc = part if cc is None else cc + part
                if k in cfg["kick_c"]:
                    if not same_buffer:
                        s_s[:, :Dc] = cc
                    step()
                    if not same_buffer:
                        cc = s_s[:, :Dc]
            cc = cc / l
            for t in range(NCT):
                ctx_s[t, b] = cc[:, t * _L:(t + 1) * _L]
            pm.pump(cfg["pump_c"], cfg["lag_c"])
            pm.drain()

        for b in range(B):
            if b + 2 < B:
                attend_b(b, functools.partial(start_c, b + 2), pump_c(b + 2), True)
            elif b + 2 == B:
                attend_b(b, functools.partial(start_pieces, wuv_h, wuv_s, cut_w, S_WUV),
                         _Pump(heads_of(wuv_h, wuv_s, i_w)), False)
            else:
                attend_b(b, start_wqa, _Pump(heads_of(wqa_h, wqa_s, i_wqa)), False)

        wait_pieces(wuv_s, cut_w, S_WUV)
        start_k(0)
        start_v(0)
        pm = pump_kv(0)
        pm.kick()
        tick(2 + B)
        for t in range(NCT):
            for hh in range(2):
                w = head_major(wuv_s, t, hh)
                ch = ctx_s[t, :, hh * HH:(hh + 1) * HH, :].reshape(B, HH * _L).astype(_BF16)
                parts = [_dot(ch[:, j * _L:(j + 1) * _L], w[:, j * Db:(j + 1) * Db])
                         for j in range(HH)]
                cols = slice(hh * HH * Db, (hh + 1) * HH * Db)
                part = jnp.concatenate(parts, axis=1)
                ctxb_s[:, cols] = part if t == 0 else ctxb_s[:, cols] + part
                if (2 * t + hh + 1) % seg_w == 0:
                    pm.pump(1)
        pm.pump(cfg["pump_w"], cfg["lag_w"])
        pm.drain()

        wait_pieces(wqa_s, cut_wqa, S_WQA)
        start_k(1)
        pm = pump_kv(1)
        pm.kick()
        tick(3 + B)
        c_xa.wait()
        xa = xa_s[...]
        wq_tiles = wqa_s[...].reshape(D // 8, n_ct, 8, _L)
        qa_all = jnp.concatenate(
            [_dot(xa, wq_tiles[:, ct].reshape(D, _L)) for ct in range(n_ct)], axis=1) * scale_a
        qa_s[...] = qa_all.reshape(B, H, Dh).reshape(BH, Dh)
        pm.pump(cfg["pump_q"], cfg["lag_q"])
        pm.drain()

        def attend_a(g, start_at_k, start_at_v, pm, same_buffer, between):
            start = g * _G if isinstance(g, int) else pl.multiple_of(g * _G, _G)
            rows = pl.ds(start, _G)
            q8 = qa_s[rows, :].astype(_BF16)
            wait_pieces(k_s.at[g], cut_k, S_KV + 2 * g)
            start_at_k()
            pm.kick()
            tick(4 + B + g)
            row = lax.broadcasted_iota(jnp.int32, (_G, W), 0)
            s = None
            for j in range(_G):
                sj = _dot_nt(q8, k_s[g, j])
                s = sj if s is None else jnp.where(row == j, sj, s)
                if j in cfg["kick_qk"]:
                    if same_buffer:
                        pm.kick()
                    else:
                        p_s[...] = s
                        pm.pump(1)
                        s = p_s[...]
            m = jnp.max(s, axis=-1, keepdims=True)
            p = jnp.exp(s - m)
            l = jnp.sum(p, axis=-1, keepdims=True)
            p_s[...] = p
            between()
            wait_pieces(v_s.at[g], cut_v, S_KV + 2 * g + 1)
            start_at_v()
            pm.kick() if same_buffer else pm.pump(1)
            pb = p_s[...].astype(_BF16)
            row2 = lax.broadcasted_iota(jnp.int32, (_G, Dh), 0)
            o = None
            for j in range(_G):
                oj = _dot(pb, v_s[g, j])
                o = oj if o is None else jnp.where(row2 == j, oj, o)
                if j in cfg["kick_pv"] and same_buffer:
                    pm.kick()
            oa_s[rows, :] = o / l

        def a_body(g, carry):
            pm = pump_kv(g + 2)
            attend_a(g, functools.partial(start_v, g + 1), functools.partial(start_k, g + 2), pm,
                     True, functools.partial(pm.pump, cfg["pump_k"], cfg["lag_k"]))
            pm.pump(cfg["pump_v"], cfg["lag_v"])
            pm.drain()
            return carry

        lax.fori_loop(0, NG - 2, a_body, 0)

        pm = pump_wo(0, n14)
        attend_a(NG - 2, functools.partial(start_v, NG - 1), start_wo, pm,
                 False, functools.partial(pm.pump, cfg["pump_k"], cfg["lag_k"]))
        pm.pump(cfg["pump_v"], cfg["lag_v"])
        pm.drain()

        n_early = side_all - side_late
        waited = max(side_all - side_nb, 0)
        r_early = n_early * side_rows
        pm = pump_wo(n14, len(i_wo))

        def project_b():
            tick(4 + B + NG)
            c_wob.wait()
            for i in range(waited, n_early):
                c_sb(i).wait()
            ctxb = ctxb_s[...].astype(_BF16)
            accb_s[...] = _dot(ctxb[:, side_total:], wob_s[side_total:, :])
            step = cfg["seg_b"] * _L
            for lo in range(0, r_early, step):
                pm.pump(1)
                hi = min(lo + step, r_early)
                accb_s[...] += _dot(ctxb[:, lo:hi], wob_s[lo:hi, :])
            pm.pump(cfg["pump_k15"], cfg["lag_k"])

        attend_a(NG - 1, lambda: None, lambda: None, pm, False, project_b)
        pm.pump(1)

        oa32 = oa_s[...].reshape(B, H, Dh).reshape(B, H * Dh)
        oab_s[...] = oa32
        tail0 = H * Dh - tail_rows
        for b in range(B):
            for t in range(tail_rows // Dh):
                src = oa32[b:b + 1, tail0 + t * Dh:tail0 + (t + 1) * Dh]
                coef_s[b, t * Dh:(t + 1) * Dh, :] = jnp.broadcast_to(src, (_L, Dh)).T
        pm.pump(cfg["pump_e"], cfg["lag_e"])
        pm.drain()
        oa = oab_s[...].astype(_BF16)
        n_inj = wo_inj * r_wo
        acc_s[...] = _dot(oa[:, :n_inj], woa_s[:wo_inj].reshape(n_inj, D))
        wait_pieces(woa_s.at[wide], cut_wo, S_WIDE)
        acc_s[...] += _dot(oa[:, n_inj:wo_base],
                           woa_s[wo_inj:wo_inj + wo_wide].reshape(wo_base - n_inj, D))
        for i in range(n_mxu):
            c_wo(i).wait()
            if i == late_at:
                for j in range(max(waited, n_early), side_all):
                    c_sb(j).wait()
                late = _dot(ctxb_s[:, r_early:side_total].astype(_BF16),
                            wob_s[r_early:side_total, :])
                o_ref[:, D:] = (accb_s[...] + late).astype(o_ref.dtype)
            lo, n = wo_off[i], wo_chunks[i]
            part = _dot(oa[:, lo:lo + n], woa_s[wo_at(lo, n)]) + acc_s[...]
            if i < n_wo - 1:
                acc_s[...] = part
            else:
                o_ref[:, :D] = part.astype(o_ref.dtype)
        for i in range(n_mxu, n_wo):
            c_wo(i).wait()
            lo, n = wo_off[i], wo_chunks[i]
            w = woa_s[wo_at(lo, n)].astype(_F32)
            sums = []
            for b in range(B):
                cf = coef_s[b, lo - tail0:lo - tail0 + n, :]
                prod = w * jnp.concatenate([cf] * (D // _L), axis=1)
                acc = vacc_s[b] if i > n_mxu else None
                for r in range(0, n, 8):
                    acc = prod[r:r + 8] if acc is None else acc + prod[r:r + 8]
                if i < n_wo - 1:
                    vacc_s[b] = acc
                else:
                    sums.append(jnp.sum(acc, axis=0, keepdims=True))
            if i == n_wo - 1:
                res = acc_s[...] + jnp.concatenate(sums, axis=0)
                o_ref[:, :D] = res.astype(o_ref.dtype)

    any_spec = pl.BlockSpec(memory_space=pl.ANY)
    out = pl.pallas_call(
        kernel,
        out_shape=jax.ShapeDtypeStruct((B, D + M), A_x.dtype),
        in_specs=[any_spec] * 11,
        out_specs=pl.BlockSpec(memory_space=pltpu.VMEM),
        scratch_shapes=[
            pltpu.VMEM(xa2.shape, _BF16),
            pltpu.VMEM(xb2.shape, _BF16),
            pltpu.VMEM((2, NG, _G, W, Dh), _BF16),
            pltpu.VMEM(wqa3.shape, _BF16),
            pltpu.VMEM(woa3.shape, _BF16),
            pltpu.VMEM(c4.shape, _BF16),
            pltpu.VMEM(wqb4.shape, _BF16),
            pltpu.VMEM(wuk4.shape, _BF16),
            pltpu.VMEM(wuv4.shape, _BF16),
            pltpu.VMEM(wob2.shape, _BF16),
            pltpu.VMEM((BH, Dh), _F32),
            pltpu.VMEM((BH, Dh), _F32),
            pltpu.VMEM((NCT, B, Hb, _L), _F32),
            pltpu.VMEM((NCT, B, Hb, _L), _F32),
            pltpu.VMEM((B, D), _F32),
            pltpu.VMEM((B, M), _F32),
            pltpu.VMEM((B, Hb * Db), _F32),
            pltpu.VMEM((B, H * Dh), _F32),
            pltpu.VMEM((B, max(tail_rows, 8), _L), _F32),
            pltpu.VMEM((B, 8, D), _F32),
            pltpu.VMEM((_G, W), _F32),
            pltpu.VMEM((Hb, Skb), _F32),
            pltpu.SMEM((side_nb, side_rows, M), _BF16),
            pltpu.SemaphoreType.DMA((n_sem,)),
        ],
        compiler_params=pltpu.CompilerParams(
            vmem_limit_bytes=120 * 1024 * 1024,
            disable_semaphore_checks=True,
            disable_bounds_checks=cfg.get('nobc', True),
        ),
        name="fused_decode",
    )(xa2, k3, v3, wqa3, woa3, xb2, c4, wqb4, wuk4, wuv4, wob2)
    return out.reshape(B, Sq, D + M)


@jax.jit
def pallas_concat_heads__sliding_block_cached__compressed_kv_cla__decode_kernel(
    A_x: jax.Array,
    A_k_cache: jax.Array,
    A_v_cache: jax.Array,
    A_wq: jax.Array,
    A_wo: jax.Array,
    B_x: jax.Array,
    B_c_kv: jax.Array,
    B_w_q: jax.Array,
    B_w_uk: jax.Array,
    B_w_uv: jax.Array,
    B_w_o: jax.Array,
):
    return _fused(_CFG, A_x, A_k_cache, A_v_cache, A_wq, A_wo,
                  B_x, B_c_kv, B_w_q, B_w_uk, B_w_uv, B_w_o)
```

```python
import functools
import itertools

import jax
import jax.numpy as jnp
from jax import lax
import jax.experimental.pallas as pl
import jax.experimental.pallas.tpu as pltpu

_NT = (((1,), (1,)), ((), ()))
_F32 = jnp.float32
_BF16 = jnp.bfloat16
_L = 128
_G = 8
_KIB = 1024

_CFG = dict(
    wo_inj=1,
    wo_wide=5,
    wo_chunks=(512, 128, 128),
    wo_tail=(80, 64, 48, 32, 16, 16),
    shift_wo=32 * _KIB,
    pump_k15=4, pump_e=6, lag_e=2, seg_b=8,
    piece=64 * _KIB,
    shift_a=30 * _KIB,
    shift_b=34 * _KIB,
    block=512 * _KIB,
    inj_w=(16 * _KIB, 18 * _KIB),
    inj_c=(16 * _KIB, 18 * _KIB),
    inj_q=(14 * _KIB, 8 * _KIB, 8 * _KIB),
    inj_k=(16 * _KIB,),
    inj_v=(14 * _KIB, 16 * _KIB),
    inj_wo=((8 * _KIB,) * 24, (16 * _KIB,) * 20),
    side_rows=128,
    side_n=24,
    side_last=32,
    side_nb=4,
    side_late=2,
    late_at=1,
    pump0=14,
    pump_w=6,
    pump_c=8,
    pump_q=8,
    pump_k=8,
    pump_v=9,
    lag_0=1, lag_w=1, lag_c=1, lag_q=2, lag_k=2, lag_v=2,
    seg_w=1,
    kick_s=(1, 3, 5, 7),
    kick_c=(3,),
    kick_qk=(1, 3, 5),
    kick_pv=(3,),
)


def _dot(a, b):
    return jnp.dot(a, b, preferred_element_type=_F32)


def _dot_nt(a, b):
    return lax.dot_general(a, b, _NT, preferred_element_type=_F32)


def _bounds(n_rows, row_bytes, piece, shift, skip=0):
    step = piece // row_bytes
    first = (shift // row_bytes) % step
    cuts = [skip] + [r for r in range(first, n_rows, step) if r > skip] + [n_rows]
    return list(zip(cuts[:-1], cuts[1:]))


class _Pump:
    def __init__(self, copies):
        self.copies, self.started, self.waited = list(copies), 0, 0

    def kick(self):
        if self.started < len(self.copies):
            self.copies[self.started]().start(priority=0)
            self.started += 1

    def _wait_to(self, n):
        while self.waited < n:
            self.copies[self.waited]().wait()
            self.waited += 1

    def pump(self, n, lag=1):
        for _ in range(n):
            self.kick()
            self._wait_to(self.started - lag)

    def drain(self):
        while self.started < len(self.copies):
            self.kick()
        self._wait_to(self.started)


def _fused(cfg, A_x, A_k_cache, A_v_cache, A_wq, A_wo, B_x, B_c_kv, B_w_q, B_w_uk, B_w_uv, B_w_o):
    B, Sq, D = A_x.shape
    _, H, Sk, Dh = A_k_cache.shape
    assert Sq == 1 and B_x.shape[1] == 1
    assert A_wq.shape == (D, H * Dh)
    W = min(4096, max(256, Sk // 4))
    M, Hb, Db = B_w_q.shape
    Skb, Dc = B_c_kv.shape[1], B_c_kv.shape[2]
    BH = B * H
    NG = BH // _G
    NCT = Dc // _L
    HH = Hb // 2
    scale_a = float(Dh) ** -0.5
    scale_b = float(Db) ** -0.5
    piece, block = cfg["piece"], cfg["block"]
    shift_a, shift_b = cfg["shift_a"], cfg["shift_b"]
    side_rows, side_n, side_nb = cfg["side_rows"], cfg["side_n"], cfg["side_nb"]
    side_late, late_at = cfg["side_late"], cfg["late_at"]
    n_mxu = len(cfg["wo_chunks"])
    wo_chunks = tuple(cfg["wo_chunks"]) + tuple(cfg["wo_tail"])
    tail_rows = sum(cfg["wo_tail"])
    assert tail_rows % Dh == 0 and M % _L == 0 and NG >= 4
    side_last = cfg["side_last"]
    side_all = side_n + (1 if side_last else 0)
    assert side_all <= 5 + B + NG

    xa2 = A_x.reshape(B, D)
    xb2 = B_x.reshape(B, M)
    k3 = A_k_cache.reshape(BH, Sk, Dh)
    v3 = A_v_cache.reshape(BH, Sk, Dh)
    wob2 = B_w_o.reshape(Hb * Db, M)

    def blocked(w, lead=0):
        row_bytes = 2 * functools.reduce(lambda a, b: a * b, w.shape[lead + 1:], 1)
        rows = block // row_bytes
        shape = w.shape[:lead] + (w.shape[lead] // rows, rows) + w.shape[lead + 1:]
        return w.reshape(shape), rows, row_bytes

    n_ct = H * Dh // _L
    wqa_t = A_wq.reshape(D // 8, 8, n_ct, _L).transpose(0, 2, 1, 3).reshape(D // 8 * n_ct, 8, _L)
    wqa3, r_wqa, b_wqa = blocked(wqa_t)
    wqb4, r_w, b_w = blocked(B_w_q.reshape(M * Hb, Db))
    wuk4, _, _ = blocked(B_w_uk.reshape(Dc * Hb, Db))
    wuv4, _, _ = blocked(B_w_uv.reshape(Dc * Hb, Db))
    c_t = B_c_kv.reshape(B, Skb // 8, 8, NCT, _L).transpose(0, 1, 3, 2, 4)
    c4, r_c, b_c = blocked(c_t.reshape(B, Skb // 8 * NCT, 8, _L), 1)
    k_c = r_c // NCT * 8
    woa3, r_wo, b_wo = blocked(A_wo)
    assert wqb4.shape == wuk4.shape == wuv4.shape and 2 * r_w == _L * Hb
    NBLK = wqb4.shape[0]

    def spans(sizes, unit):
        ends = list(itertools.accumulate(n // unit for n in sizes))
        return list(zip([0] + ends[:-1], ends))

    i_w, i_c = spans(cfg["inj_w"], b_w), spans(cfg["inj_c"], b_c)
    i_k, i_v = spans(cfg["inj_k"], 2 * Dh), spans(cfg["inj_v"], 2 * Dh)
    i_wqa = spans(cfg["inj_q"], b_wqa)
    i_wo = spans(cfg["inj_wo"][0] + cfg["inj_wo"][1], 2 * D)
    n14 = len(cfg["inj_wo"][0])
    cut_w0 = _bounds(r_w, b_w, piece, shift_b)
    cut_w = _bounds(r_w, b_w, piece, shift_b, i_w[-1][1])
    cut_c = _bounds(r_c, b_c, piece, shift_b, i_c[-1][1])
    cut_k = _bounds(W, 2 * Dh, piece, shift_a, i_k[-1][1])
    cut_v = _bounds(W, 2 * Dh, piece, shift_a, i_v[-1][1])
    cut_wqa = _bounds(r_wqa, b_wqa, piece, shift_a, i_wqa[-1][1])
    wo_inj, wo_wide = cfg["wo_inj"], cfg["wo_wide"]
    cut_wo = _bounds(r_wo, b_wo, piece, cfg["shift_wo"])
    wo_base = (wo_inj + wo_wide) * r_wo
    assert i_wo[-1][1] == wo_inj * r_wo
    assert wo_base + sum(wo_chunks) == H * Dh
    n_wo = len(wo_chunks)
    wo_off = [wo_base + sum(wo_chunks[:i]) for i in range(n_wo)]
    assert all(lo // r_wo == (lo + n - 1) // r_wo for lo, n in zip(wo_off, wo_chunks))
    S_XB, S_XA, S_WQB, S_WUK, S_WUV, S_WOB, S_WQA, S_INJ, S_WIDE = range(9)
    S_C = 9
    S_KV = S_C + B
    S_WO = S_KV + 2 * NG
    S_SA = S_WO + n_wo
    S_SB = S_SA + side_nb
    n_sem = S_SB + side_nb
    side_total = side_rows * side_n + side_last

    def kernel(xa_h, k_h, v_h, wqa_h, woa_h, xb_h, c_h, wqb_h, wuk_h, wuv_h, wob_h,
               o_ref,
               xa_s, xb_s, kv_s, wqa_s, woa_s, c_s, wqb_s, wuk_s, wuv_s, wob_s,
               qa_s, oa_s, qabs_s, ctx_s, acc_s, accb_s, ctxb_s, oab_s, coef_s, vacc_s, p_s, s_s, side_s, sem):
        def cp(src, dst, s):
            return pltpu.make_async_copy(src, dst, sem.at[s])

        def start_pieces(src, dst, cuts, s, row0=0):
            for lo, hi in cuts:
                cp(src.at[:, pl.ds(row0 + lo, hi - lo)], dst.at[:, pl.ds(lo, hi - lo)],
                   s).start(priority=cfg.get('bulk_prio', 1))

        def wait_pieces(dst, cuts, s):
            view = dst.at[:, pl.ds(cuts[0][0], cuts[-1][1] - cuts[0][0])]
            cp(view, view, s).wait()

        def heads_of(src, dst, ranges, row0=0):
            def one(k, lo, hi):
                return cp(src.at[k, pl.ds(row0 + lo, hi - lo)], dst.at[k, pl.ds(lo, hi - lo)], S_INJ)
            return [functools.partial(one, k, lo, hi)
                    for lo, hi in ranges for k in range(dst.shape[0])]

        k_s, v_s = kv_s.at[0], kv_s.at[1]
        c_xb = cp(xb_h, xb_s, S_XB)
        c_xa = cp(xa_h, xa_s, S_XA)
        rest = pl.ds(side_total, Hb * Db - side_total)
        c_wob = cp(wob_h.at[rest, :], wob_s.at[rest, :], S_WOB)

        def start_c(b):
            start_pieces(c_h.at[b], c_s.at[b], cut_c, S_C + b)

        def pump_c(b):
            return _Pump(heads_of(c_h.at[b], c_s.at[b], i_c))

        def start_wqa():
            c_wob.start(priority=cfg.get('bulk_prio', 1))
            start_pieces(wqa_h, wqa_s, cut_wqa, S_WQA)

        def start_k(g):
            start_pieces(k_h.at[pl.ds(g * _G, _G)], k_s.at[g], cut_k, S_KV + 2 * g, Sk - W)

        def start_v(g):
            start_pieces(v_h.at[pl.ds(g * _G, _G)], v_s.at[g], cut_v, S_KV + 2 * g + 1, Sk - W)

        def pump_kv(g):
            heads = pl.ds(g * _G, _G)
            return _Pump(heads_of(k_h.at[heads], k_s.at[g], i_k, Sk - W)
                         + heads_of(v_h.at[heads], v_s.at[g], i_v, Sk - W))

        def wo_at(lo, n):
            return lo // r_wo, pl.ds(lo % r_wo, n)

        def c_wo(i):
            at = wo_at(wo_off[i], wo_chunks[i])
            return cp(woa_h.at[at], woa_s.at[at], S_WO + i)

        wide = pl.ds(wo_inj, wo_wide)

        def start_wo():
            start_pieces(woa_h.at[wide], woa_s.at[wide], cut_wo, S_WIDE)
            for i in range(n_wo):
                c_wo(i).start(priority=cfg.get('bulk_prio', 1))

        def pump_wo(first, last):
            def one(lo, hi):
                at = wo_at(lo, hi - lo)
                return cp(woa_h.at[at], woa_s.at[at], S_INJ)
            return _Pump([functools.partial(one, *i_wo[j]) for j in range(first, last)])

        def side_refs(i):
            start = i * side_rows
            n = side_rows
            if not isinstance(i, int):
                start = pl.multiple_of(start, 8)
            elif i == side_n:
                n = side_last
            slot = i % side_nb
            return pl.ds(start, n), side_s.at[slot, pl.ds(0, n)], slot

        def c_sa(i):
            rows, stage, slot = side_refs(i)
            return cp(wob_h.at[rows, :], stage, S_SA + slot)

        def c_sb(i):
            rows, stage, slot = side_refs(i)
            return cp(stage, wob_s.at[rows, :], S_SB + slot)

        lag = 2

        def when(cond, fn):
            if isinstance(cond, bool):
                if cond:
                    fn()
            else:
                pl.when(cond)(fn)

        def tick(i):
            def forward():
                c_sa(i).wait()
                c_sb(i).start()

            def refill():
                if not isinstance(i, int) or i >= lag:
                    c_sb(i - lag).wait()
                c_sa(i - lag + side_nb).start()

            if isinstance(i, int):
                when(i < side_all, forward)
                when(i - lag + side_nb < side_all, refill)
            else:
                assert 4 + B + NG - 3 - lag + side_nb < side_n
                forward()
                refill()

        def head_major(w_s, t, hh):
            w = w_s[2 * t:2 * t + 2].reshape(_L, Hb, Db)[:, hh * HH:(hh + 1) * HH, :]
            return w.reshape(_L, HH * Db)

        start_pieces(wqb_h, wqb_s, cut_w0, S_WQB)
        c_xb.start()
        c_xa.start()
        for i in range(side_nb - lag):
            c_sa(i).start()
        start_pieces(wuk_h, wuk_s, cut_w, S_WUK)
        pm = _Pump(heads_of(wuk_h, wuk_s, i_w))
        pm.pump(cfg["pump0"], cfg["lag_0"])
        pm.drain()

        seg_w = cfg["seg_w"]

        wait_pieces(wqb_s, cut_w0, S_WQB)
        start_c(0)
        pm = pump_c(0)
        pm.kick()
        tick(0)
        c_xb.wait()
        xb = xb_s[...]
        for t in range(M // _L):
            for hh in range(2):
                cols = slice(hh * HH * Db, (hh + 1) * HH * Db)
                part = _dot(xb[:, t * _L:(t + 1) * _L], head_major(wqb_s, t, hh))
                ctxb_s[:, cols] = part if t == 0 else ctxb_s[:, cols] + part
                if (2 * t + hh + 1) % seg_w == 0:
                    pm.pump(1)
        pm.pump(cfg["pump_w"], cfg["lag_w"])
        pm.drain()

        wait_pieces(wuk_s, cut_w, S_WUK)
        start_c(1)
        pm = pump_c(1)
        pm.kick()
        tick(1)
        qb = (ctxb_s[...] * scale_b).astype(_BF16)
        for t in range(NCT):
            for hh in range(2):
                w = head_major(wuk_s, t, hh)
                parts = [_dot_nt(qb[:, (hh * HH + j) * Db:(hh * HH + j + 1) * Db],
                                 w[:, j * Db:(j + 1) * Db]) for j in range(HH)]
                qabs_s[t, :, hh * HH:(hh + 1) * HH, :] = jnp.concatenate(
                    parts, axis=1).reshape(B, HH, _L)
                if (2 * t + hh + 1) % seg_w == 0:
                    pm.pump(1)
        pm.pump(cfg["pump_w"], cfg["lag_w"])
        pm.drain()

        def attend_b(b, start_next, pm, same_buffer):
            wait_pieces(c_s.at[b], cut_c, S_C + b)
            start_next()
            pm.kick()
            tick(2 + b)
            step = pm.kick if same_buffer else functools.partial(pm.pump, 1)
            qa = jnp.concatenate(
                [qabs_s[t, b] for t in range(NCT)], axis=1).astype(_BF16)

            def latent(k):
                tiles = c_s[b, k].reshape(k_c // 8, NCT, 8, _L)
                return jnp.concatenate(
                    [tiles[:, t].reshape(k_c, _L) for t in range(NCT)], axis=1)

            for k in range(NBLK):
                s_s[:, k * k_c:(k + 1) * k_c] = _dot_nt(qa, latent(k))
                if k in cfg["kick_s"]:
                    step()
            s = s_s[...]
            m = jnp.max(s, axis=-1, keepdims=True)
            p = jnp.exp(s - m)
            l = jnp.sum(p, axis=-1, keepdims=True)
            pb = p.astype(_BF16)
            cc = None
            for k in range(NBLK):
                part = _dot(pb[:, k * k_c:(k + 1) * k_c], latent(k))
                cc = part if cc is None else cc + part
                if k in cfg["kick_c"]:
                    if not same_buffer:
                        s_s[:, :Dc] = cc
                    step()
                    if not same_buffer:
                        cc = s_s[:, :Dc]
            cc = cc / l
            for t in range(NCT):
                ctx_s[t, b] = cc[:, t * _L:(t + 1) * _L]
            pm.pump(cfg["pump_c"], cfg["lag_c"])
            pm.drain()

        for b in range(B):
            if b + 2 < B:
                attend_b(b, functools.partial(start_c, b + 2), pump_c(b + 2), True)
            elif b + 2 == B:
                attend_b(b, functools.partial(start_pieces, wuv_h, wuv_s, cut_w, S_WUV),
                         _Pump(heads_of(wuv_h, wuv_s, i_w)), False)
            else:
                attend_b(b, start_wqa, _Pump(heads_of(wqa_h, wqa_s, i_wqa)), False)

        wait_pieces(wuv_s, cut_w, S_WUV)
        start_k(0)
        start_v(0)
        pm = pump_kv(0)
        pm.kick()
        tick(2 + B)
        for t in range(NCT):
            for hh in range(2):
                w = head_major(wuv_s, t, hh)
                ch = ctx_s[t, :, hh * HH:(hh + 1) * HH, :].reshape(B, HH * _L).astype(_BF16)
                parts = [_dot(ch[:, j * _L:(j + 1) * _L], w[:, j * Db:(j + 1) * Db])
                         for j in range(HH)]
                cols = slice(hh * HH * Db, (hh + 1) * HH * Db)
                part = jnp.concatenate(parts, axis=1)
                ctxb_s[:, cols] = part if t == 0 else ctxb_s[:, cols] + part
                if (2 * t + hh + 1) % seg_w == 0:
                    pm.pump(1)
        pm.pump(cfg["pump_w"], cfg["lag_w"])
        pm.drain()

        wait_pieces(wqa_s, cut_wqa, S_WQA)
        start_k(1)
        pm = pump_kv(1)
        pm.kick()
        tick(3 + B)
        c_xa.wait()
        xa = xa_s[...]
        wq_tiles = wqa_s[...].reshape(D // 8, n_ct, 8, _L)
        qa_all = jnp.concatenate(
            [_dot(xa, wq_tiles[:, ct].reshape(D, _L)) for ct in range(n_ct)], axis=1) * scale_a
        qa_s[...] = qa_all.reshape(B, H, Dh).reshape(BH, Dh)
        pm.pump(cfg["pump_q"], cfg["lag_q"])
        pm.drain()

        def attend_a(g, start_at_k, start_at_v, pm, same_buffer, between):
            start = g * _G if isinstance(g, int) else pl.multiple_of(g * _G, _G)
            rows = pl.ds(start, _G)
            q8 = qa_s[rows, :].astype(_BF16)
            wait_pieces(k_s.at[g], cut_k, S_KV + 2 * g)
            start_at_k()
            pm.kick()
            tick(4 + B + g)
            row = lax.broadcasted_iota(jnp.int32, (_G, W), 0)
            s = None
            for j in range(_G):
                sj = _dot_nt(q8, k_s[g, j])
                s = sj if s is None else jnp.where(row == j, sj, s)
                if j in cfg["kick_qk"]:
                    if same_buffer:
                        pm.kick()
                    else:
                        p_s[...] = s
                        pm.pump(1)
                        s = p_s[...]
            m = jnp.max(s, axis=-1, keepdims=True)
            p = jnp.exp(s - m)
            l = jnp.sum(p, axis=-1, keepdims=True)
            p_s[...] = p
            between()
            wait_pieces(v_s.at[g], cut_v, S_KV + 2 * g + 1)
            start_at_v()
            pm.kick() if same_buffer else pm.pump(1)
            pb = p_s[...].astype(_BF16)
            row2 = lax.broadcasted_iota(jnp.int32, (_G, Dh), 0)
            o = None
            for j in range(_G):
                oj = _dot(pb, v_s[g, j])
                o = oj if o is None else jnp.where(row2 == j, oj, o)
                if j in cfg["kick_pv"] and same_buffer:
                    pm.kick()
            oa_s[rows, :] = o / l

        def a_body(g, carry):
            pm = pump_kv(g + 2)
            attend_a(g, functools.partial(start_v, g + 1), functools.partial(start_k, g + 2), pm,
                     True, functools.partial(pm.pump, cfg["pump_k"], cfg["lag_k"]))
            pm.pump(cfg["pump_v"], cfg["lag_v"])
            pm.drain()
            return carry

        lax.fori_loop(0, NG - 2, a_body, 0)

        pm = pump_wo(0, n14)
        attend_a(NG - 2, functools.partial(start_v, NG - 1), start_wo, pm,
                 False, functools.partial(pm.pump, cfg["pump_k"], cfg["lag_k"]))
        pm.pump(cfg["pump_v"], cfg["lag_v"])
        pm.drain()

        n_early = side_all - side_late
        waited = max(side_all - side_nb, 0)
        r_early = n_early * side_rows
        pm = pump_wo(n14, len(i_wo))

        def project_b():
            tick(4 + B + NG)
            c_wob.wait()
            for i in range(waited, n_early):
                c_sb(i).wait()
            ctxb = ctxb_s[...].astype(_BF16)
            accb_s[...] = _dot(ctxb[:, side_total:], wob_s[side_total:, :])
            step = cfg["seg_b"] * _L
            for lo in range(0, r_early, step):
                pm.pump(1)
                hi = min(lo + step, r_early)
                accb_s[...] += _dot(ctxb[:, lo:hi], wob_s[lo:hi, :])
            pm.pump(cfg["pump_k15"], cfg["lag_k"])

        attend_a(NG - 1, lambda: None, lambda: None, pm, False, project_b)
        pm.pump(1)

        oa32 = oa_s[...].reshape(B, H, Dh).reshape(B, H * Dh)
        oab_s[...] = oa32
        tail0 = H * Dh - tail_rows
        for b in range(B):
            for t in range(tail_rows // Dh):
                src = oa32[b:b + 1, tail0 + t * Dh:tail0 + (t + 1) * Dh]
                coef_s[b, t * Dh:(t + 1) * Dh, :] = jnp.broadcast_to(src, (_L, Dh)).T
        pm.pump(cfg["pump_e"], cfg["lag_e"])
        pm.drain()
        oa = oab_s[...].astype(_BF16)
        n_inj = wo_inj * r_wo
        acc_s[...] = _dot(oa[:, :n_inj], woa_s[:wo_inj].reshape(n_inj, D))
        wait_pieces(woa_s.at[wide], cut_wo, S_WIDE)
        acc_s[...] += _dot(oa[:, n_inj:wo_base],
                           woa_s[wo_inj:wo_inj + wo_wide].reshape(wo_base - n_inj, D))
        for i in range(n_mxu):
            c_wo(i).wait()
            if i == late_at:
                for j in range(max(waited, n_early), side_all):
                    c_sb(j).wait()
                late = _dot(ctxb_s[:, r_early:side_total].astype(_BF16),
                            wob_s[r_early:side_total, :])
                o_ref[:, D:] = (accb_s[...] + late).astype(o_ref.dtype)
            lo, n = wo_off[i], wo_chunks[i]
            part = _dot(oa[:, lo:lo + n], woa_s[wo_at(lo, n)]) + acc_s[...]
            if i < n_wo - 1:
                acc_s[...] = part
            else:
                o_ref[:, :D] = part.astype(o_ref.dtype)
        for i in range(n_mxu, n_wo):
            c_wo(i).wait()
            lo, n = wo_off[i], wo_chunks[i]
            w = woa_s[wo_at(lo, n)].astype(_F32)
            sums = []
            for b in range(B):
                cf = coef_s[b, lo - tail0:lo - tail0 + n, :]
                prod = w * jnp.concatenate([cf] * (D // _L), axis=1)
                acc = vacc_s[b] if i > n_mxu else None
                for r in range(0, n, 8):
                    acc = prod[r:r + 8] if acc is None else acc + prod[r:r + 8]
                if i < n_wo - 1:
                    vacc_s[b] = acc
                else:
                    sums.append(jnp.sum(acc, axis=0, keepdims=True))
            if i == n_wo - 1:
                res = acc_s[...] + jnp.concatenate(sums, axis=0)
                o_ref[:, :D] = res.astype(o_ref.dtype)

    any_spec = pl.BlockSpec(memory_space=pl.ANY)
    out = pl.pallas_call(
        kernel,
        out_shape=jax.ShapeDtypeStruct((B, D + M), A_x.dtype),
        in_specs=[any_spec] * 11,
        out_specs=pl.BlockSpec(memory_space=pltpu.VMEM),
        scratch_shapes=[
            pltpu.VMEM(xa2.shape, _BF16),
            pltpu.VMEM(xb2.shape, _BF16),
            pltpu.VMEM((2, NG, _G, W, Dh), _BF16),
            pltpu.VMEM(wqa3.shape, _BF16),
            pltpu.VMEM(woa3.shape, _BF16),
            pltpu.VMEM(c4.shape, _BF16),
            pltpu.VMEM(wqb4.shape, _BF16),
            pltpu.VMEM(wuk4.shape, _BF16),
            pltpu.VMEM(wuv4.shape, _BF16),
            pltpu.VMEM(wob2.shape, _BF16),
            pltpu.VMEM((BH, Dh), _F32),
            pltpu.VMEM((BH, Dh), _F32),
            pltpu.VMEM((NCT, B, Hb, _L), _F32),
            pltpu.VMEM((NCT, B, Hb, _L), _F32),
            pltpu.VMEM((B, D), _F32),
            pltpu.VMEM((B, M), _F32),
            pltpu.VMEM((B, Hb * Db), _F32),
            pltpu.VMEM((B, H * Dh), _F32),
            pltpu.VMEM((B, max(tail_rows, 8), _L), _F32),
            pltpu.VMEM((B, 8, D), _F32),
            pltpu.VMEM((_G, W), _F32),
            pltpu.VMEM((Hb, Skb), _F32),
            pltpu.SMEM((side_nb, side_rows, M), _BF16),
            pltpu.SemaphoreType.DMA((n_sem,)),
        ],
        compiler_params=pltpu.CompilerParams(
            vmem_limit_bytes=120 * 1024 * 1024,
            disable_semaphore_checks=True,
            disable_bounds_checks=cfg.get('nobc', True),
        ),
        name="fused_decode",
    )(xa2, k3, v3, wqa3, woa3, xb2, c4, wqb4, wuk4, wuv4, wob2)
    return out.reshape(B, Sq, D + M)


@jax.jit
def pallas_concat_heads__sliding_block_cached__compressed_kv_cla__decode_kernel(
    A_x: jax.Array,
    A_k_cache: jax.Array,
    A_v_cache: jax.Array,
    A_wq: jax.Array,
    A_wo: jax.Array,
    B_x: jax.Array,
    B_c_kv: jax.Array,
    B_w_q: jax.Array,
    B_w_uk: jax.Array,
    B_w_uv: jax.Array,
    B_w_o: jax.Array,
):
    return _fused(_CFG, A_x, A_k_cache, A_v_cache, A_wq, A_wo,
                  B_x, B_c_kv, B_w_q, B_w_uk, B_w_uv, B_w_o)
```

```python
import functools
import itertools

import jax
import jax.numpy as jnp
from jax import lax
import jax.experimental.pallas as pl
import jax.experimental.pallas.tpu as pltpu

_NT = (((1,), (1,)), ((), ()))
_F32 = jnp.float32
_BF16 = jnp.bfloat16
_L = 128
_G = 8
_KIB = 1024
_URGENT, _BULK = 0, 1

_CFG = dict(
    wo_inj=1,
    wo_wide=5,
    wo_chunks=(512, 128, 128),
    wo_tail=(80, 64, 48, 32, 16, 16),
    shift_wo=32 * _KIB,
    pump_k15=4, pump_e=6, lag_e=2, seg_b=8,
    piece=64 * _KIB,
    shift_a=30 * _KIB,
    shift_b=34 * _KIB,
    block=512 * _KIB,
    inj_w=(16 * _KIB, 18 * _KIB),
    inj_c=(16 * _KIB, 18 * _KIB),
    inj_q=(14 * _KIB, 16 * _KIB),
    inj_k=(14 * _KIB, 16 * _KIB),
    inj_v=(14 * _KIB, 16 * _KIB),
    inj_wo=((8 * _KIB,) * 24, (16 * _KIB,) * 20),
    side_rows=128,
    side_n=24,
    side_last=16,
    side_nb=4,
    side_late=2,
    late_at=1,
    pump0=14,
    pump_w=6,
    pump_uv=18, lag_uv=3,
    pump_c=7,
    pump_q=8,
    pump_k=10,
    pump_v=13,
    lag_0=1, lag_w=1, lag_c=1, lag_q=2, lag_k=3, lag_v=3,
    seg_w=1,
    kick_s=(0, 1, 3, 5, 7),
    kick_c=(2, 5),
    kick_qk=(0, 2, 4, 6),
    kick_pv=(2, 5),
)


def _dot(a, b):
    return jnp.dot(a, b, preferred_element_type=_F32)


def _dot_nt(a, b):
    return lax.dot_general(a, b, _NT, preferred_element_type=_F32)


def _bounds(n_rows, row_bytes, piece, shift, skip=0):
    step = piece // row_bytes
    first = (shift // row_bytes) % step
    cuts = [skip] + [r for r in range(first, n_rows, step) if r > skip] + [n_rows]
    return list(zip(cuts[:-1], cuts[1:]))


class _Pump:
    def __init__(self, copies):
        self.copies, self.started, self.waited = list(copies), 0, 0

    def kick(self):
        if self.started < len(self.copies):
            self.copies[self.started]().start(priority=_URGENT)
            self.started += 1

    def _wait_to(self, n):
        while self.waited < n:
            self.copies[self.waited]().wait()
            self.waited += 1

    def pump(self, n, lag=1):
        for _ in range(n):
            self.kick()
            self._wait_to(self.started - lag)

    def drain(self):
        while self.started < len(self.copies):
            self.kick()
        self._wait_to(self.started)


def _fused(cfg, A_x, A_k_cache, A_v_cache, A_wq, A_wo, B_x, B_c_kv, B_w_q, B_w_uk, B_w_uv, B_w_o):
    B, Sq, D = A_x.shape
    _, H, Sk, Dh = A_k_cache.shape
    assert Sq == 1 and B_x.shape[1] == 1
    assert A_wq.shape == (D, H * Dh)
    W = min(4096, max(256, Sk // 4))
    M, Hb, Db = B_w_q.shape
    Skb, Dc = B_c_kv.shape[1], B_c_kv.shape[2]
    BH = B * H
    NG = BH // _G
    NCT = Dc // _L
    HH = Hb // 2
    scale_a = float(Dh) ** -0.5
    scale_b = float(Db) ** -0.5
    piece, block = cfg["piece"], cfg["block"]
    shift_a, shift_b = cfg["shift_a"], cfg["shift_b"]
    side_rows, side_n, side_nb = cfg["side_rows"], cfg["side_n"], cfg["side_nb"]
    side_late, late_at = cfg["side_late"], cfg["late_at"]
    n_mxu = len(cfg["wo_chunks"])
    wo_chunks = tuple(cfg["wo_chunks"]) + tuple(cfg["wo_tail"])
    tail_rows = sum(cfg["wo_tail"])
    assert tail_rows % Dh == 0 and M % _L == 0 and NG >= 4
    side_last = cfg["side_last"]
    side_all = side_n + (1 if side_last else 0)
    assert side_all <= 5 + B + NG

    xa2 = A_x.reshape(B, D)
    xb2 = B_x.reshape(B, M)
    k3 = A_k_cache.reshape(BH, Sk, Dh)
    v3 = A_v_cache.reshape(BH, Sk, Dh)
    wob2 = B_w_o.reshape(Hb * Db, M)

    def blocked(w, lead=0):
        row_bytes = 2 * functools.reduce(lambda a, b: a * b, w.shape[lead + 1:], 1)
        rows = block // row_bytes
        shape = w.shape[:lead] + (w.shape[lead] // rows, rows) + w.shape[lead + 1:]
        return w.reshape(shape), rows, row_bytes

    n_ct = H * Dh // _L
    wqa_t = A_wq.reshape(D // 8, 8, n_ct, _L).transpose(0, 2, 1, 3).reshape(D // 8 * n_ct, 8, _L)
    wqa3, r_wqa, b_wqa = blocked(wqa_t)
    wqb4, r_w, b_w = blocked(B_w_q.reshape(M * Hb, Db))
    wuk4, _, _ = blocked(B_w_uk.reshape(Dc * Hb, Db))
    wuv4, _, _ = blocked(B_w_uv.reshape(Dc * Hb, Db))
    c_t = B_c_kv.reshape(B, Skb // 8, 8, NCT, _L).transpose(0, 1, 3, 2, 4)
    c4, r_c, b_c = blocked(c_t.reshape(B, Skb // 8 * NCT, 8, _L), 1)
    k_c = r_c // NCT * 8
    woa3, r_wo, b_wo = blocked(A_wo)
    assert wqb4.shape == wuk4.shape == wuv4.shape and 2 * r_w == _L * Hb
    NBLK = wqb4.shape[0]

    def spans(sizes, unit):
        ends = list(itertools.accumulate(n // unit for n in sizes))
        return list(zip([0] + ends[:-1], ends))

    i_w, i_c = spans(cfg["inj_w"], b_w), spans(cfg["inj_c"], b_c)
    i_k, i_v = spans(cfg["inj_k"], 2 * Dh), spans(cfg["inj_v"], 2 * Dh)
    i_wqa = spans(cfg["inj_q"], b_wqa)
    i_wo = spans(cfg["inj_wo"][0] + cfg["inj_wo"][1], 2 * D)
    n14 = len(cfg["inj_wo"][0])
    cut_w0 = _bounds(r_w, b_w, piece, shift_b)
    cut_w = _bounds(r_w, b_w, piece, shift_b, i_w[-1][1])
    cut_c = _bounds(r_c, b_c, piece, shift_b, i_c[-1][1])
    cut_k = _bounds(W, 2 * Dh, piece, shift_a, i_k[-1][1])
    cut_v = _bounds(W, 2 * Dh, piece, shift_a, i_v[-1][1])
    cut_wqa = _bounds(r_wqa, b_wqa, piece, shift_a, i_wqa[-1][1])
    wo_inj, wo_wide = cfg["wo_inj"], cfg["wo_wide"]
    cut_wo = _bounds(r_wo, b_wo, piece, cfg["shift_wo"])
    wo_base = (wo_inj + wo_wide) * r_wo
    assert i_wo[-1][1] == wo_inj * r_wo
    assert wo_base + sum(wo_chunks) == H * Dh
    n_wo = len(wo_chunks)
    wo_off = [wo_base + sum(wo_chunks[:i]) for i in range(n_wo)]
    assert all(lo // r_wo == (lo + n - 1) // r_wo for lo, n in zip(wo_off, wo_chunks))
    S_XB, S_XA, S_WQB, S_WUK, S_WUV, S_WOB, S_WQA, S_INJ, S_WIDE = range(9)
    S_C = 9
    S_KV = S_C + B
    S_WO = S_KV + 2 * NG
    S_SA = S_WO + n_wo
    S_SB = S_SA + side_nb
    n_sem = S_SB + side_nb
    side_total = side_rows * side_n + side_last

    def kernel(xa_h, k_h, v_h, wqa_h, woa_h, xb_h, c_h, wqb_h, wuk_h, wuv_h, wob_h,
               o_ref,
               xa_s, xb_s, kv_s, wqa_s, woa_s, c_s, wqb_s, wuk_s, wuv_s, wob_s,
               qa_s, oa_s, qabs_s, ctx_s, acc_s, accb_s, ctxb_s, oab_s, coef_s, vacc_s, p_s, s_s, side_s, sem):
        def cp(src, dst, s):
            return pltpu.make_async_copy(src, dst, sem.at[s])

        def start_pieces(src, dst, cuts, s, row0=0):
            for lo, hi in cuts:
                cp(src.at[:, pl.ds(row0 + lo, hi - lo)], dst.at[:, pl.ds(lo, hi - lo)],
                   s).start(priority=_BULK)

        def wait_pieces(dst, cuts, s):
            view = dst.at[:, pl.ds(cuts[0][0], cuts[-1][1] - cuts[0][0])]
            cp(view, view, s).wait()

        def heads_of(src, dst, ranges, row0=0):
            def one(k, lo, hi):
                return cp(src.at[k, pl.ds(row0 + lo, hi - lo)], dst.at[k, pl.ds(lo, hi - lo)], S_INJ)
            return [functools.partial(one, k, lo, hi)
                    for lo, hi in ranges for k in range(dst.shape[0])]

        k_s, v_s = kv_s.at[0], kv_s.at[1]
        c_xb = cp(xb_h, xb_s, S_XB)
        c_xa = cp(xa_h, xa_s, S_XA)
        rest = pl.ds(side_total, Hb * Db - side_total)
        c_wob = cp(wob_h.at[rest, :], wob_s.at[rest, :], S_WOB)

        def start_c(b):
            start_pieces(c_h.at[b], c_s.at[b], cut_c, S_C + b)

        def pump_c(b):
            return _Pump(heads_of(c_h.at[b], c_s.at[b], i_c))

        def start_wqa():
            c_wob.start(priority=_BULK)
            start_pieces(wqa_h, wqa_s, cut_wqa, S_WQA)

        def start_k(g):
            start_pieces(k_h.at[pl.ds(g * _G, _G)], k_s.at[g], cut_k, S_KV + 2 * g, Sk - W)

        def start_v(g):
            start_pieces(v_h.at[pl.ds(g * _G, _G)], v_s.at[g], cut_v, S_KV + 2 * g + 1, Sk - W)

        def pump_kv(g):
            heads = pl.ds(g * _G, _G)
            return _Pump(heads_of(k_h.at[heads], k_s.at[g], i_k, Sk - W)
                         + heads_of(v_h.at[heads], v_s.at[g], i_v, Sk - W))

        def wo_at(lo, n):
            return lo // r_wo, pl.ds(lo % r_wo, n)

        def c_wo(i):
            at = wo_at(wo_off[i], wo_chunks[i])
            return cp(woa_h.at[at], woa_s.at[at], S_WO + i)

        wide = pl.ds(wo_inj, wo_wide)

        def start_wo():
            start_pieces(woa_h.at[wide], woa_s.at[wide], cut_wo, S_WIDE)
            for i in range(n_wo):
                c_wo(i).start(priority=_BULK)

        def pump_wo(first, last):
            def one(lo, hi):
                at = wo_at(lo, hi - lo)
                return cp(woa_h.at[at], woa_s.at[at], S_INJ)
            return _Pump([functools.partial(one, *i_wo[j]) for j in range(first, last)])

        def side_refs(i):
            start = i * side_rows
            n = side_rows
            if not isinstance(i, int):
                start = pl.multiple_of(start, 8)
            elif i == side_n:
                n = side_last
            slot = i % side_nb
            return pl.ds(start, n), side_s.at[slot, pl.ds(0, n)], slot

        def c_sa(i):
            rows, stage, slot = side_refs(i)
            return cp(wob_h.at[rows, :], stage, S_SA + slot)

        def c_sb(i):
            rows, stage, slot = side_refs(i)
            return cp(stage, wob_s.at[rows, :], S_SB + slot)

        lag = 2

        def when(cond, fn):
            if isinstance(cond, bool):
                if cond:
                    fn()
            else:
                pl.when(cond)(fn)

        def tick(i):
            def forward():
                c_sa(i).wait()
                c_sb(i).start()

            def refill():
                if not isinstance(i, int) or i >= lag:
                    c_sb(i - lag).wait()
                c_sa(i - lag + side_nb).start()

            if isinstance(i, int):
                when(i < side_all, forward)
                when(i - lag + side_nb < side_all, refill)
            else:
                assert 4 + B + NG - 3 - lag + side_nb < side_n
                forward()
                refill()

        def head_major(w_s, t, hh):
            w = w_s[2 * t:2 * t + 2].reshape(_L, Hb, Db)[:, hh * HH:(hh + 1) * HH, :]
            return w.reshape(_L, HH * Db)

        start_pieces(wqb_h, wqb_s, cut_w0, S_WQB)
        c_xb.start()
        c_xa.start()
        for i in range(side_nb - lag):
            c_sa(i).start()
        start_pieces(wuk_h, wuk_s, cut_w, S_WUK)
        pm = _Pump(heads_of(wuk_h, wuk_s, i_w))
        pm.pump(cfg["pump0"], cfg["lag_0"])
        pm.drain()

        seg_w = cfg["seg_w"]

        wait_pieces(wqb_s, cut_w0, S_WQB)
        start_c(0)
        pm = pump_c(0)
        pm.kick()
        tick(0)
        c_xb.wait()
        xb = xb_s[...]
        for t in range(M // _L):
            for hh in range(2):
                cols = slice(hh * HH * Db, (hh + 1) * HH * Db)
                part = _dot(xb[:, t * _L:(t + 1) * _L], head_major(wqb_s, t, hh))
                ctxb_s[:, cols] = part if t == 0 else ctxb_s[:, cols] + part
                if (2 * t + hh + 1) % seg_w == 0:
                    pm.pump(1)
        pm.pump(cfg["pump_w"], cfg["lag_w"])
        pm.drain()

        wait_pieces(wuk_s, cut_w, S_WUK)
        start_c(1)
        pm = pump_c(1)
        pm.kick()
        tick(1)
        qb = (ctxb_s[...] * scale_b).astype(_BF16)
        for t in range(NCT):
            for hh in range(2):
                w = head_major(wuk_s, t, hh)
                parts = [_dot_nt(qb[:, (hh * HH + j) * Db:(hh * HH + j + 1) * Db],
                                 w[:, j * Db:(j + 1) * Db]) for j in range(HH)]
                qabs_s[t, :, hh * HH:(hh + 1) * HH, :] = jnp.concatenate(
                    parts, axis=1).reshape(B, HH, _L)
                if (2 * t + hh + 1) % seg_w == 0:
                    pm.pump(1)
        pm.pump(cfg["pump_w"], cfg["lag_w"])
        pm.drain()

        def attend_b(b, start_next, pm, same_buffer):
            wait_pieces(c_s.at[b], cut_c, S_C + b)
            start_next()
            pm.kick()
            tick(2 + b)
            step = pm.kick if same_buffer else functools.partial(pm.pump, 1)
            qa = jnp.concatenate(
                [qabs_s[t, b] for t in range(NCT)], axis=1).astype(_BF16)

            def latent(k):
                tiles = c_s[b, k].reshape(k_c // 8, NCT, 8, _L)
                return jnp.concatenate(
                    [tiles[:, t].reshape(k_c, _L) for t in range(NCT)], axis=1)

            for k in range(NBLK):
                s_s[:, k * k_c:(k + 1) * k_c] = _dot_nt(qa, latent(k))
                if k in cfg["kick_s"]:
                    step()
            s = s_s[...]
            m = jnp.max(s, axis=-1, keepdims=True)
            p = jnp.exp(s - m)
            l = jnp.sum(p, axis=-1, keepdims=True)
            pb = p.astype(_BF16)
            cc = None
            for k in range(NBLK):
                part = _dot(pb[:, k * k_c:(k + 1) * k_c], latent(k))
                cc = part if cc is None else cc + part
                if k in cfg["kick_c"]:
                    if not same_buffer:
                        s_s[:, :Dc] = cc
                    step()
                    if not same_buffer:
                        cc = s_s[:, :Dc]
            cc = cc / l
            for t in range(NCT):
                ctx_s[t, b] = cc[:, t * _L:(t + 1) * _L]
            pm.pump(cfg["pump_c"], cfg["lag_c"])
            pm.drain()

        for b in range(B):
            if b + 2 < B:
                attend_b(b, functools.partial(start_c, b + 2), pump_c(b + 2), True)
            elif b + 2 == B:
                attend_b(b, functools.partial(start_pieces, wuv_h, wuv_s, cut_w, S_WUV),
                         _Pump(heads_of(wuv_h, wuv_s, i_w)), False)
            else:
                attend_b(b, start_wqa, _Pump(heads_of(wqa_h, wqa_s, i_wqa)), False)

        wait_pieces(wuv_s, cut_w, S_WUV)
        start_k(0)
        start_v(0)
        pm = pump_kv(0)
        pm.kick()
        tick(2 + B)
        for t in range(NCT):
            for hh in range(2):
                w = head_major(wuv_s, t, hh)
                ch = ctx_s[t, :, hh * HH:(hh + 1) * HH, :].reshape(B, HH * _L).astype(_BF16)
                parts = [_dot(ch[:, j * _L:(j + 1) * _L], w[:, j * Db:(j + 1) * Db])
                         for j in range(HH)]
                cols = slice(hh * HH * Db, (hh + 1) * HH * Db)
                part = jnp.concatenate(parts, axis=1)
                ctxb_s[:, cols] = part if t == 0 else ctxb_s[:, cols] + part
                if (2 * t + hh + 1) % seg_w == 0:
                    pm.pump(1)
        pm.pump(cfg["pump_uv"], cfg["lag_uv"])
        pm.drain()

        wait_pieces(wqa_s, cut_wqa, S_WQA)
        start_k(1)
        pm = pump_kv(1)
        pm.kick()
        tick(3 + B)
        c_xa.wait()
        xa = xa_s[...]
        wq_tiles = wqa_s[...].reshape(D // 8, n_ct, 8, _L)
        qa_all = jnp.concatenate(
            [_dot(xa, wq_tiles[:, ct].reshape(D, _L)) for ct in range(n_ct)], axis=1) * scale_a
        qa_s[...] = qa_all.reshape(B, H, Dh).reshape(BH, Dh)
        pm.pump(cfg["pump_q"], cfg["lag_q"])
        pm.drain()

        def attend_a(g, start_at_k, start_at_v, pm, same_buffer, between):
            start = g * _G if isinstance(g, int) else pl.multiple_of(g * _G, _G)
            rows = pl.ds(start, _G)
            q8 = qa_s[rows, :].astype(_BF16)
            wait_pieces(k_s.at[g], cut_k, S_KV + 2 * g)
            start_at_k()
            pm.kick()
            tick(4 + B + g)
            row = lax.broadcasted_iota(jnp.int32, (_G, W), 0)
            s = None
            for j in range(_G):
                sj = _dot_nt(q8, k_s[g, j])
                s = sj if s is None else jnp.where(row == j, sj, s)
                if j in cfg["kick_qk"]:
                    if same_buffer:
                        pm.kick()
                    else:
                        p_s[...] = s
                        pm.pump(1)
                        s = p_s[...]
            m = jnp.max(s, axis=-1, keepdims=True)
            p = jnp.exp(s - m)
            l = jnp.sum(p, axis=-1, keepdims=True)
            p_s[...] = p
            between()
            wait_pieces(v_s.at[g], cut_v, S_KV + 2 * g + 1)
            start_at_v()
            pm.kick() if same_buffer else pm.pump(1)
            pb = p_s[...].astype(_BF16)
            row2 = lax.broadcasted_iota(jnp.int32, (_G, Dh), 0)
            o = None
            for j in range(_G):
                oj = _dot(pb, v_s[g, j])
                o = oj if o is None else jnp.where(row2 == j, oj, o)
                if j in cfg["kick_pv"] and same_buffer:
                    pm.kick()
            oa_s[rows, :] = o / l

        def a_body(g, carry):
            pm = pump_kv(g + 2)
            attend_a(g, functools.partial(start_v, g + 1), functools.partial(start_k, g + 2), pm,
                     True, functools.partial(pm.pump, cfg["pump_k"], cfg["lag_k"]))
            pm.pump(cfg["pump_v"], cfg["lag_v"])
            pm.drain()
            return carry

        lax.fori_loop(0, NG - 2, a_body, 0)

        pm = pump_wo(0, n14)
        attend_a(NG - 2, functools.partial(start_v, NG - 1), start_wo, pm,
                 False, functools.partial(pm.pump, cfg["pump_k"], cfg["lag_k"]))
        pm.pump(cfg["pump_v"], cfg["lag_v"])
        pm.drain()

        n_early = side_all - side_late
        waited = max(side_all - side_nb, 0)
        r_early = n_early * side_rows
        pm = pump_wo(n14, len(i_wo))

        def project_b():
            tick(4 + B + NG)
            c_wob.wait()
            for i in range(waited, n_early):
                c_sb(i).wait()
            ctxb = ctxb_s[...].astype(_BF16)
            accb_s[...] = _dot(ctxb[:, side_total:], wob_s[side_total:, :])
            step = cfg["seg_b"] * _L
            for lo in range(0, r_early, step):
                pm.pump(1)
                hi = min(lo + step, r_early)
                accb_s[...] += _dot(ctxb[:, lo:hi], wob_s[lo:hi, :])
            pm.pump(cfg["pump_k15"], cfg["lag_k"])

        attend_a(NG - 1, lambda: None, lambda: None, pm, False, project_b)
        pm.pump(1)

        oa32 = oa_s[...].reshape(B, H, Dh).reshape(B, H * Dh)
        oab_s[...] = oa32
        tail0 = H * Dh - tail_rows
        for b in range(B):
            for t in range(tail_rows // Dh):
                src = oa32[b:b + 1, tail0 + t * Dh:tail0 + (t + 1) * Dh]
                coef_s[b, t * Dh:(t + 1) * Dh, :] = jnp.broadcast_to(src, (_L, Dh)).T
        pm.pump(cfg["pump_e"], cfg["lag_e"])
        pm.drain()
        oa = oab_s[...].astype(_BF16)
        n_inj = wo_inj * r_wo
        acc_s[...] = _dot(oa[:, :n_inj], woa_s[:wo_inj].reshape(n_inj, D))
        wait_pieces(woa_s.at[wide], cut_wo, S_WIDE)
        acc_s[...] += _dot(oa[:, n_inj:wo_base],
                           woa_s[wo_inj:wo_inj + wo_wide].reshape(wo_base - n_inj, D))
        for i in range(n_mxu):
            c_wo(i).wait()
            if i == late_at:
                for j in range(max(waited, n_early), side_all):
                    c_sb(j).wait()
                late = _dot(ctxb_s[:, r_early:side_total].astype(_BF16),
                            wob_s[r_early:side_total, :])
                o_ref[:, D:] = (accb_s[...] + late).astype(o_ref.dtype)
            lo, n = wo_off[i], wo_chunks[i]
            part = _dot(oa[:, lo:lo + n], woa_s[wo_at(lo, n)]) + acc_s[...]
            if i < n_wo - 1:
                acc_s[...] = part
            else:
                o_ref[:, :D] = part.astype(o_ref.dtype)
        for i in range(n_mxu, n_wo):
            c_wo(i).wait()
            lo, n = wo_off[i], wo_chunks[i]
            w = woa_s[wo_at(lo, n)].astype(_F32)
            sums = []
            for b in range(B):
                cf = coef_s[b, lo - tail0:lo - tail0 + n, :]
                prod = w * jnp.concatenate([cf] * (D // _L), axis=1)
                acc = vacc_s[b] if i > n_mxu else None
                for r in range(0, n, 8):
                    acc = prod[r:r + 8] if acc is None else acc + prod[r:r + 8]
                if i < n_wo - 1:
                    vacc_s[b] = acc
                else:
                    sums.append(jnp.sum(acc, axis=0, keepdims=True))
            if i == n_wo - 1:
                res = acc_s[...] + jnp.concatenate(sums, axis=0)
                o_ref[:, :D] = res.astype(o_ref.dtype)

    any_spec = pl.BlockSpec(memory_space=pl.ANY)
    out = pl.pallas_call(
        kernel,
        out_shape=jax.ShapeDtypeStruct((B, D + M), A_x.dtype),
        in_specs=[any_spec] * 11,
        out_specs=pl.BlockSpec(memory_space=pltpu.VMEM),
        scratch_shapes=[
            pltpu.VMEM(xa2.shape, _BF16),
            pltpu.VMEM(xb2.shape, _BF16),
            pltpu.VMEM((2, NG, _G, W, Dh), _BF16),
            pltpu.VMEM(wqa3.shape, _BF16),
            pltpu.VMEM(woa3.shape, _BF16),
            pltpu.VMEM(c4.shape, _BF16),
            pltpu.VMEM(wqb4.shape, _BF16),
            pltpu.VMEM(wuk4.shape, _BF16),
            pltpu.VMEM(wuv4.shape, _BF16),
            pltpu.VMEM(wob2.shape, _BF16),
            pltpu.VMEM((BH, Dh), _F32),
            pltpu.VMEM((BH, Dh), _F32),
            pltpu.VMEM((NCT, B, Hb, _L), _F32),
            pltpu.VMEM((NCT, B, Hb, _L), _F32),
            pltpu.VMEM((B, D), _F32),
            pltpu.VMEM((B, M), _F32),
            pltpu.VMEM((B, Hb * Db), _F32),
            pltpu.VMEM((B, H * Dh), _F32),
            pltpu.VMEM((B, max(tail_rows, 8), _L), _F32),
            pltpu.VMEM((B, 8, D), _F32),
            pltpu.VMEM((_G, W), _F32),
            pltpu.VMEM((Hb, Skb), _F32),
            pltpu.SMEM((side_nb, side_rows, M), _BF16),
            pltpu.SemaphoreType.DMA((n_sem,)),
        ],
        compiler_params=pltpu.CompilerParams(
            vmem_limit_bytes=120 * 1024 * 1024,
            disable_semaphore_checks=True,
            disable_bounds_checks=True,
        ),
        name="fused_decode",
    )(xa2, k3, v3, wqa3, woa3, xb2, c4, wqb4, wuk4, wuv4, wob2)
    return out.reshape(B, Sq, D + M)


@jax.jit
def pallas_concat_heads__sliding_block_cached__compressed_kv_cla__decode_kernel(
    A_x: jax.Array,
    A_k_cache: jax.Array,
    A_v_cache: jax.Array,
    A_wq: jax.Array,
    A_wo: jax.Array,
    B_x: jax.Array,
    B_c_kv: jax.Array,
    B_w_q: jax.Array,
    B_w_uk: jax.Array,
    B_w_uv: jax.Array,
    B_w_o: jax.Array,
):
    return _fused(_CFG, A_x, A_k_cache, A_v_cache, A_wq, A_wo,
                  B_x, B_c_kv, B_w_q, B_w_uk, B_w_uv, B_w_o)
```

```python
import functools
import itertools

import jax
import jax.numpy as jnp
from jax import lax
import jax.experimental.pallas as pl
import jax.experimental.pallas.tpu as pltpu

_NT = (((1,), (1,)), ((), ()))
_F32 = jnp.float32
_BF16 = jnp.bfloat16
_L = 128
_G = 8
_KIB = 1024
_URGENT, _BULK = 0, 1

_CFG = dict(
    piece=64 * _KIB,
    block=512 * _KIB,
    shift_a=30 * _KIB,
    shift_b=34 * _KIB,
    shift_wo=32 * _KIB,
    inj_w=(16 * _KIB, 18 * _KIB),
    inj_c=(16 * _KIB, 18 * _KIB),
    inj_q=(14 * _KIB, 16 * _KIB),
    inj_k=(14 * _KIB, 16 * _KIB),
    inj_v=(14 * _KIB, 16 * _KIB),
    inj_wo=((8 * _KIB,) * 24, (16 * _KIB,) * 20),
    pump_0=(14, 1),
    pump_w=(6, 1),
    pump_c=(7, 1),
    pump_uv=(18, 3),
    pump_q=(8, 2),
    pump_k=(10, 3),
    pump_v=(13, 3),
    pump_b=(4, 3),
    pump_e=(6, 2),
    kick_s=(0, 1, 3, 5, 7),
    kick_c=(2, 5),
    kick_qk=(0, 2, 4, 6),
    kick_pv=(2, 5),
    side_rows=128,
    side_n=24,
    side_nb=4,
    side_late=1,
    late_at=1,
    wo_inj=1,
    wo_wide=5,
    wo_chunks=(512, 128, 128),
    wo_tail=(80, 64, 48, 32, 16, 16),
)


def _dot(a, b):
    return jnp.dot(a, b, preferred_element_type=_F32)


def _dot_nt(a, b):
    return lax.dot_general(a, b, _NT, preferred_element_type=_F32)


def _bounds(n_rows, row_bytes, piece, shift, skip=0):
    step = piece // row_bytes
    first = (shift // row_bytes) % step
    cuts = [skip] + [r for r in range(first, n_rows, step) if r > skip] + [n_rows]
    return list(zip(cuts[:-1], cuts[1:]))


class _Pump:
    def __init__(self, copies):
        self.copies, self.started, self.waited = list(copies), 0, 0

    def kick(self):
        if self.started < len(self.copies):
            self.copies[self.started]().start(priority=_URGENT)
            self.started += 1

    def _wait_to(self, n):
        while self.waited < n:
            self.copies[self.waited]().wait()
            self.waited += 1

    def pump(self, n, lag=1):
        for _ in range(n):
            self.kick()
            self._wait_to(self.started - lag)

    def drain(self):
        while self.started < len(self.copies):
            self.kick()
        self._wait_to(self.started)


def _fused(cfg, A_x, A_k_cache, A_v_cache, A_wq, A_wo, B_x, B_c_kv, B_w_q, B_w_uk, B_w_uv, B_w_o):
    B, Sq, D = A_x.shape
    _, H, Sk, Dh = A_k_cache.shape
    assert Sq == 1 and B_x.shape[1] == 1
    assert A_wq.shape == (D, H * Dh)
    W = min(4096, max(256, Sk // 4))
    M, Hb, Db = B_w_q.shape
    Skb, Dc = B_c_kv.shape[1], B_c_kv.shape[2]
    BH = B * H
    NG = BH // _G
    NCT = Dc // _L
    HH = Hb // 2
    scale_a = float(Dh) ** -0.5
    scale_b = float(Db) ** -0.5
    piece, block = cfg["piece"], cfg["block"]
    shift_a, shift_b = cfg["shift_a"], cfg["shift_b"]
    side_rows, side_n, side_nb = cfg["side_rows"], cfg["side_n"], cfg["side_nb"]
    side_late, late_at = cfg["side_late"], cfg["late_at"]
    n_mxu = len(cfg["wo_chunks"])
    wo_chunks = tuple(cfg["wo_chunks"]) + tuple(cfg["wo_tail"])
    tail_rows = sum(cfg["wo_tail"])
    assert tail_rows % Dh == 0 and M % _L == 0 and NG >= 4
    side_lag = side_nb // 2
    assert 4 + B + NG - 3 + side_lag < side_n <= 4 + B + NG

    xa2 = A_x.reshape(B, D)
    xb2 = B_x.reshape(B, M)
    k3 = A_k_cache.reshape(BH, Sk, Dh)
    v3 = A_v_cache.reshape(BH, Sk, Dh)
    wob2 = B_w_o.reshape(Hb * Db, M)

    def blocked(w, lead=0):
        row_bytes = 2 * functools.reduce(lambda a, b: a * b, w.shape[lead + 1:], 1)
        rows = block // row_bytes
        shape = w.shape[:lead] + (w.shape[lead] // rows, rows) + w.shape[lead + 1:]
        return w.reshape(shape), rows, row_bytes

    n_ct = H * Dh // _L
    wqa_t = A_wq.reshape(D // 8, 8, n_ct, _L).transpose(0, 2, 1, 3).reshape(D // 8 * n_ct, 8, _L)
    wqa3, r_wqa, b_wqa = blocked(wqa_t)
    wqb4, r_w, b_w = blocked(B_w_q.reshape(M * Hb, Db))
    wuk4, _, _ = blocked(B_w_uk.reshape(Dc * Hb, Db))
    wuv4, _, _ = blocked(B_w_uv.reshape(Dc * Hb, Db))
    c_t = B_c_kv.reshape(B, Skb // 8, 8, NCT, _L).transpose(0, 1, 3, 2, 4)
    c4, r_c, b_c = blocked(c_t.reshape(B, Skb // 8 * NCT, 8, _L), 1)
    k_c = r_c // NCT * 8
    woa3, r_wo, b_wo = blocked(A_wo)
    assert wqb4.shape == wuk4.shape == wuv4.shape and 2 * r_w == _L * Hb
    NBLK = wqb4.shape[0]

    def spans(sizes, unit):
        ends = list(itertools.accumulate(n // unit for n in sizes))
        return list(zip([0] + ends[:-1], ends))

    i_w, i_c = spans(cfg["inj_w"], b_w), spans(cfg["inj_c"], b_c)
    i_k, i_v = spans(cfg["inj_k"], 2 * Dh), spans(cfg["inj_v"], 2 * Dh)
    i_wqa = spans(cfg["inj_q"], b_wqa)
    i_wo = spans(cfg["inj_wo"][0] + cfg["inj_wo"][1], 2 * D)
    n_wo_first = len(cfg["inj_wo"][0])
    cut_w0 = _bounds(r_w, b_w, piece, shift_b)
    cut_w = _bounds(r_w, b_w, piece, shift_b, i_w[-1][1])
    cut_c = _bounds(r_c, b_c, piece, shift_b, i_c[-1][1])
    cut_k = _bounds(W, 2 * Dh, piece, shift_a, i_k[-1][1])
    cut_v = _bounds(W, 2 * Dh, piece, shift_a, i_v[-1][1])
    cut_wqa = _bounds(r_wqa, b_wqa, piece, shift_a, i_wqa[-1][1])
    wo_inj, wo_wide = cfg["wo_inj"], cfg["wo_wide"]
    cut_wo = _bounds(r_wo, b_wo, piece, cfg["shift_wo"])
    wo_base = (wo_inj + wo_wide) * r_wo
    assert i_wo[-1][1] == wo_inj * r_wo
    assert wo_base + sum(wo_chunks) == H * Dh
    n_wo = len(wo_chunks)
    wo_off = [wo_base + sum(wo_chunks[:i]) for i in range(n_wo)]
    assert all(lo // r_wo == (lo + n - 1) // r_wo for lo, n in zip(wo_off, wo_chunks))
    S_XB, S_XA, S_WQB, S_WUK, S_WUV, S_WOB, S_WQA, S_INJ, S_WIDE = range(9)
    S_C = 9
    S_KV = S_C + B
    S_WO = S_KV + 2 * NG
    S_SA = S_WO + n_wo
    S_SB = S_SA + side_nb
    n_sem = S_SB + side_nb
    side_total = side_rows * side_n

    def kernel(xa_h, k_h, v_h, wqa_h, woa_h, xb_h, c_h, wqb_h, wuk_h, wuv_h, wob_h,
               o_ref,
               xa_s, xb_s, kv_s, wqa_s, woa_s, c_s, wqb_s, wuk_s, wuv_s, wob_s,
               qa_s, oa_s, qabs_s, ctx_s, acc_s, accb_s, ctxb_s, oab_s, coef_s, vacc_s, p_s, s_s,
               side_s, sem):
        def cp(src, dst, s):
            return pltpu.make_async_copy(src, dst, sem.at[s])

        def start_pieces(src, dst, cuts, s, row0=0):
            for lo, hi in cuts:
                cp(src.at[:, pl.ds(row0 + lo, hi - lo)], dst.at[:, pl.ds(lo, hi - lo)],
                   s).start(priority=_BULK)

        def wait_pieces(dst, cuts, s):
            view = dst.at[:, pl.ds(cuts[0][0], cuts[-1][1] - cuts[0][0])]
            cp(view, view, s).wait()

        def heads_of(src, dst, ranges, row0=0):
            def one(k, lo, hi):
                return cp(src.at[k, pl.ds(row0 + lo, hi - lo)], dst.at[k, pl.ds(lo, hi - lo)], S_INJ)
            return [functools.partial(one, k, lo, hi)
                    for lo, hi in ranges for k in range(dst.shape[0])]

        k_s, v_s = kv_s.at[0], kv_s.at[1]
        c_xb = cp(xb_h, xb_s, S_XB)
        c_xa = cp(xa_h, xa_s, S_XA)
        rest = pl.ds(side_total, Hb * Db - side_total)
        c_wob = cp(wob_h.at[rest, :], wob_s.at[rest, :], S_WOB)

        def start_c(b):
            start_pieces(c_h.at[b], c_s.at[b], cut_c, S_C + b)

        def pump_c(b):
            return _Pump(heads_of(c_h.at[b], c_s.at[b], i_c))

        def start_wqa():
            c_wob.start(priority=_BULK)
            start_pieces(wqa_h, wqa_s, cut_wqa, S_WQA)

        def start_k(g):
            start_pieces(k_h.at[pl.ds(g * _G, _G)], k_s.at[g], cut_k, S_KV + 2 * g, Sk - W)

        def start_v(g):
            start_pieces(v_h.at[pl.ds(g * _G, _G)], v_s.at[g], cut_v, S_KV + 2 * g + 1, Sk - W)

        def pump_kv(g):
            heads = pl.ds(g * _G, _G)
            return _Pump(heads_of(k_h.at[heads], k_s.at[g], i_k, Sk - W)
                         + heads_of(v_h.at[heads], v_s.at[g], i_v, Sk - W))

        def wo_at(lo, n):
            return lo // r_wo, pl.ds(lo % r_wo, n)

        def c_wo(i):
            at = wo_at(wo_off[i], wo_chunks[i])
            return cp(woa_h.at[at], woa_s.at[at], S_WO + i)

        wide = pl.ds(wo_inj, wo_wide)

        def start_wo():
            start_pieces(woa_h.at[wide], woa_s.at[wide], cut_wo, S_WIDE)
            for i in range(n_wo):
                c_wo(i).start(priority=_BULK)

        def pump_wo(first, last):
            def one(lo, hi):
                at = wo_at(lo, hi - lo)
                return cp(woa_h.at[at], woa_s.at[at], S_INJ)
            return _Pump([functools.partial(one, *i_wo[j]) for j in range(first, last)])

        def side_rows_of(i):
            start = i * side_rows
            return pl.ds(start if isinstance(i, int) else pl.multiple_of(start, 8), side_rows)

        def c_sa(i):
            return cp(wob_h.at[side_rows_of(i), :], side_s.at[i % side_nb], S_SA + i % side_nb)

        def c_sb(i):
            return cp(side_s.at[i % side_nb], wob_s.at[side_rows_of(i), :], S_SB + i % side_nb)

        def tick(i):
            traced = not isinstance(i, int)
            if traced or i < side_n:
                c_sa(i).wait()
                c_sb(i).start()
            if traced or i + side_lag < side_n:
                if traced or i >= side_lag:
                    c_sb(i - side_lag).wait()
                c_sa(i + side_lag).start()

        def head_major(w_s, t, hh):
            w = w_s[2 * t:2 * t + 2].reshape(_L, Hb, Db)[:, hh * HH:(hh + 1) * HH, :]
            return w.reshape(_L, HH * Db)

        start_pieces(wqb_h, wqb_s, cut_w0, S_WQB)
        c_xb.start()
        c_xa.start()
        for i in range(side_lag):
            c_sa(i).start()
        start_pieces(wuk_h, wuk_s, cut_w, S_WUK)
        pm = _Pump(heads_of(wuk_h, wuk_s, i_w))
        pm.pump(*cfg["pump_0"])
        pm.drain()


        wait_pieces(wqb_s, cut_w0, S_WQB)
        start_c(0)
        pm = pump_c(0)
        pm.kick()
        tick(0)
        c_xb.wait()
        xb = xb_s[...]
        for t in range(M // _L):
            for hh in range(2):
                cols = slice(hh * HH * Db, (hh + 1) * HH * Db)
                part = _dot(xb[:, t * _L:(t + 1) * _L], head_major(wqb_s, t, hh))
                ctxb_s[:, cols] = part if t == 0 else ctxb_s[:, cols] + part
                pm.pump(1)
        pm.pump(*cfg["pump_w"])
        pm.drain()

        wait_pieces(wuk_s, cut_w, S_WUK)
        start_c(1)
        pm = pump_c(1)
        pm.kick()
        tick(1)
        qb = (ctxb_s[...] * scale_b).astype(_BF16)
        for t in range(NCT):
            for hh in range(2):
                w = head_major(wuk_s, t, hh)
                parts = [_dot_nt(qb[:, (hh * HH + j) * Db:(hh * HH + j + 1) * Db],
                                 w[:, j * Db:(j + 1) * Db]) for j in range(HH)]
                qabs_s[t, :, hh * HH:(hh + 1) * HH, :] = jnp.concatenate(
                    parts, axis=1).reshape(B, HH, _L)
                pm.pump(1)
        pm.pump(*cfg["pump_w"])
        pm.drain()

        def attend_b(b, start_next, pm, same_buffer):
            wait_pieces(c_s.at[b], cut_c, S_C + b)
            start_next()
            pm.kick()
            tick(2 + b)
            step = pm.kick if same_buffer else functools.partial(pm.pump, 1)
            qa = jnp.concatenate(
                [qabs_s[t, b] for t in range(NCT)], axis=1).astype(_BF16)

            def latent(k):
                tiles = c_s[b, k].reshape(k_c // 8, NCT, 8, _L)
                return jnp.concatenate(
                    [tiles[:, t].reshape(k_c, _L) for t in range(NCT)], axis=1)

            for k in range(NBLK):
                s_s[:, k * k_c:(k + 1) * k_c] = _dot_nt(qa, latent(k))
                if k in cfg["kick_s"]:
                    step()
            s = s_s[...]
            m = jnp.max(s, axis=-1, keepdims=True)
            p = jnp.exp(s - m)
            l = jnp.sum(p, axis=-1, keepdims=True)
            pb = p.astype(_BF16)
            cc = None
            for k in range(NBLK):
                part = _dot(pb[:, k * k_c:(k + 1) * k_c], latent(k))
                cc = part if cc is None else cc + part
                if k in cfg["kick_c"]:
                    if not same_buffer:
                        s_s[:, :Dc] = cc
                    step()
                    if not same_buffer:
                        cc = s_s[:, :Dc]
            cc = cc / l
            for t in range(NCT):
                ctx_s[t, b] = cc[:, t * _L:(t + 1) * _L]
            pm.pump(*cfg["pump_c"])
            pm.drain()

        for b in range(B):
            if b + 2 < B:
                attend_b(b, functools.partial(start_c, b + 2), pump_c(b + 2), True)
            elif b + 2 == B:
                attend_b(b, functools.partial(start_pieces, wuv_h, wuv_s, cut_w, S_WUV),
                         _Pump(heads_of(wuv_h, wuv_s, i_w)), False)
            else:
                attend_b(b, start_wqa, _Pump(heads_of(wqa_h, wqa_s, i_wqa)), False)

        wait_pieces(wuv_s, cut_w, S_WUV)
        start_k(0)
        start_v(0)
        pm = pump_kv(0)
        pm.kick()
        tick(2 + B)
        for t in range(NCT):
            for hh in range(2):
                w = head_major(wuv_s, t, hh)
                ch = ctx_s[t, :, hh * HH:(hh + 1) * HH, :].reshape(B, HH * _L).astype(_BF16)
                parts = [_dot(ch[:, j * _L:(j + 1) * _L], w[:, j * Db:(j + 1) * Db])
                         for j in range(HH)]
                cols = slice(hh * HH * Db, (hh + 1) * HH * Db)
                part = jnp.concatenate(parts, axis=1)
                ctxb_s[:, cols] = part if t == 0 else ctxb_s[:, cols] + part
                pm.pump(1)
        pm.pump(*cfg["pump_uv"])
        pm.drain()

        wait_pieces(wqa_s, cut_wqa, S_WQA)
        start_k(1)
        pm = pump_kv(1)
        pm.kick()
        tick(3 + B)
        c_xa.wait()
        xa = xa_s[...]
        wq_tiles = wqa_s[...].reshape(D // 8, n_ct, 8, _L)
        qa_all = jnp.concatenate(
            [_dot(xa, wq_tiles[:, ct].reshape(D, _L)) for ct in range(n_ct)], axis=1) * scale_a
        qa_s[...] = qa_all.reshape(B, H, Dh).reshape(BH, Dh)
        pm.pump(*cfg["pump_q"])
        pm.drain()

        def attend_a(g, start_at_k, start_at_v, pm, same_buffer, between):
            start = g * _G if isinstance(g, int) else pl.multiple_of(g * _G, _G)
            rows = pl.ds(start, _G)
            q8 = qa_s[rows, :].astype(_BF16)
            wait_pieces(k_s.at[g], cut_k, S_KV + 2 * g)
            start_at_k()
            pm.kick()
            tick(4 + B + g)
            row = lax.broadcasted_iota(jnp.int32, (_G, W), 0)
            s = None
            for j in range(_G):
                sj = _dot_nt(q8, k_s[g, j])
                s = sj if s is None else jnp.where(row == j, sj, s)
                if j in cfg["kick_qk"]:
                    if same_buffer:
                        pm.kick()
                    else:
                        p_s[...] = s
                        pm.pump(1)
                        s = p_s[...]
            m = jnp.max(s, axis=-1, keepdims=True)
            p = jnp.exp(s - m)
            l = jnp.sum(p, axis=-1, keepdims=True)
            p_s[...] = p
            between()
            wait_pieces(v_s.at[g], cut_v, S_KV + 2 * g + 1)
            start_at_v()
            if same_buffer:
                pm.kick()
            else:
                pm.pump(1)
            pb = p_s[...].astype(_BF16)
            row2 = lax.broadcasted_iota(jnp.int32, (_G, Dh), 0)
            o = None
            for j in range(_G):
                oj = _dot(pb, v_s[g, j])
                o = oj if o is None else jnp.where(row2 == j, oj, o)
                if j in cfg["kick_pv"] and same_buffer:
                    pm.kick()
            oa_s[rows, :] = o / l

        def a_body(g, carry):
            pm = pump_kv(g + 2)
            attend_a(g, functools.partial(start_v, g + 1), functools.partial(start_k, g + 2), pm,
                     True, functools.partial(pm.pump, *cfg["pump_k"]))
            pm.pump(*cfg["pump_v"])
            pm.drain()
            return carry

        lax.fori_loop(0, NG - 2, a_body, 0)

        pm = pump_wo(0, n_wo_first)
        attend_a(NG - 2, functools.partial(start_v, NG - 1), start_wo, pm,
                 False, functools.partial(pm.pump, *cfg["pump_k"]))
        pm.pump(*cfg["pump_v"])
        pm.drain()

        n_early = side_n - side_late
        waited = side_n - side_nb
        r_early = n_early * side_rows
        pm = pump_wo(n_wo_first, len(i_wo))

        def project_b():
            c_wob.wait()
            for i in range(waited, n_early):
                c_sb(i).wait()
            ctxb = ctxb_s[...].astype(_BF16)
            accb_s[...] = _dot(ctxb[:, side_total:], wob_s[side_total:, :])
            step = 8 * _L
            for lo in range(0, r_early, step):
                pm.pump(1)
                hi = min(lo + step, r_early)
                accb_s[...] += _dot(ctxb[:, lo:hi], wob_s[lo:hi, :])
            pm.pump(*cfg["pump_b"])

        attend_a(NG - 1, lambda: None, lambda: None, pm, False, project_b)
        pm.pump(1)

        oa32 = oa_s[...].reshape(B, H, Dh).reshape(B, H * Dh)
        oab_s[...] = oa32
        tail0 = H * Dh - tail_rows
        for b in range(B):
            for t in range(tail_rows // Dh):
                src = oa32[b:b + 1, tail0 + t * Dh:tail0 + (t + 1) * Dh]
                coef_s[b, t * Dh:(t + 1) * Dh, :] = jnp.broadcast_to(src, (_L, Dh)).T
        pm.pump(*cfg["pump_e"])
        pm.drain()
        oa = oab_s[...].astype(_BF16)
        n_inj = wo_inj * r_wo
        acc_s[...] = _dot(oa[:, :n_inj], woa_s[:wo_inj].reshape(n_inj, D))
        wait_pieces(woa_s.at[wide], cut_wo, S_WIDE)
        acc_s[...] += _dot(oa[:, n_inj:wo_base],
                           woa_s[wo_inj:wo_inj + wo_wide].reshape(wo_base - n_inj, D))
        for i in range(n_mxu):
            c_wo(i).wait()
            if i == late_at:
                for j in range(n_early, side_n):
                    c_sb(j).wait()
                late = _dot(ctxb_s[:, r_early:side_total].astype(_BF16),
                            wob_s[r_early:side_total, :])
                o_ref[:, D:] = (accb_s[...] + late).astype(o_ref.dtype)
            lo, n = wo_off[i], wo_chunks[i]
            part = _dot(oa[:, lo:lo + n], woa_s[wo_at(lo, n)]) + acc_s[...]
            if i < n_wo - 1:
                acc_s[...] = part
            else:
                o_ref[:, :D] = part.astype(o_ref.dtype)
        for i in range(n_mxu, n_wo):
            c_wo(i).wait()
            lo, n = wo_off[i], wo_chunks[i]
            w = woa_s[wo_at(lo, n)].astype(_F32)
            sums = []
            for b in range(B):
                cf = coef_s[b, lo - tail0:lo - tail0 + n, :]
                prod = w * jnp.concatenate([cf] * (D // _L), axis=1)
                acc = vacc_s[b] if i > n_mxu else None
                for r in range(0, n, 8):
                    acc = prod[r:r + 8] if acc is None else acc + prod[r:r + 8]
                if i < n_wo - 1:
                    vacc_s[b] = acc
                else:
                    sums.append(jnp.sum(acc, axis=0, keepdims=True))
            if i == n_wo - 1:
                res = acc_s[...] + jnp.concatenate(sums, axis=0)
                o_ref[:, :D] = res.astype(o_ref.dtype)

    any_spec = pl.BlockSpec(memory_space=pl.ANY)
    out = pl.pallas_call(
        kernel,
        out_shape=jax.ShapeDtypeStruct((B, D + M), A_x.dtype),
        in_specs=[any_spec] * 11,
        out_specs=pl.BlockSpec(memory_space=pltpu.VMEM),
        scratch_shapes=[
            pltpu.VMEM(xa2.shape, _BF16),
            pltpu.VMEM(xb2.shape, _BF16),
            pltpu.VMEM((2, NG, _G, W, Dh), _BF16),
            pltpu.VMEM(wqa3.shape, _BF16),
            pltpu.VMEM(woa3.shape, _BF16),
            pltpu.VMEM(c4.shape, _BF16),
            pltpu.VMEM(wqb4.shape, _BF16),
            pltpu.VMEM(wuk4.shape, _BF16),
            pltpu.VMEM(wuv4.shape, _BF16),
            pltpu.VMEM(wob2.shape, _BF16),
            pltpu.VMEM((BH, Dh), _F32),
            pltpu.VMEM((BH, Dh), _F32),
            pltpu.VMEM((NCT, B, Hb, _L), _F32),
            pltpu.VMEM((NCT, B, Hb, _L), _F32),
            pltpu.VMEM((B, D), _F32),
            pltpu.VMEM((B, M), _F32),
            pltpu.VMEM((B, Hb * Db), _F32),
            pltpu.VMEM((B, H * Dh), _F32),
            pltpu.VMEM((B, max(tail_rows, 8), _L), _F32),
            pltpu.VMEM((B, 8, D), _F32),
            pltpu.VMEM((_G, W), _F32),
            pltpu.VMEM((Hb, Skb), _F32),
            pltpu.SMEM((side_nb, side_rows, M), _BF16),
            pltpu.SemaphoreType.DMA((n_sem,)),
        ],
        compiler_params=pltpu.CompilerParams(
            vmem_limit_bytes=120 * 1024 * 1024,
            disable_semaphore_checks=True,
            disable_bounds_checks=True,
        ),
        name="fused_decode",
    )(xa2, k3, v3, wqa3, woa3, xb2, c4, wqb4, wuk4, wuv4, wob2)
    return out.reshape(B, Sq, D + M)


@jax.jit
def pallas_concat_heads__sliding_block_cached__compressed_kv_cla__decode_kernel(
    A_x: jax.Array,
    A_k_cache: jax.Array,
    A_v_cache: jax.Array,
    A_wq: jax.Array,
    A_wo: jax.Array,
    B_x: jax.Array,
    B_c_kv: jax.Array,
    B_w_q: jax.Array,
    B_w_uk: jax.Array,
    B_w_uv: jax.Array,
    B_w_o: jax.Array,
):
    return _fused(_CFG, A_x, A_k_cache, A_v_cache, A_wq, A_wo,
                  B_x, B_c_kv, B_w_q, B_w_uk, B_w_uv, B_w_o)
```

```python
import functools

import jax
import jax.numpy as jnp
from jax import lax
import jax.experimental.pallas as pl
import jax.experimental.pallas.tpu as pltpu

_NT = (((1,), (1,)), ((), ()))
_F32 = jnp.float32
_BF16 = jnp.bfloat16
_L = 128
_G = 8
_KIB = 1024
_URGENT, _BULK = 0, 1

_CFG = dict(
    piece=64 * _KIB,
    block=512 * _KIB,
    shift_a=30 * _KIB,
    shift_b=34 * _KIB,
    shift_wo=32 * _KIB,
    inj_0=(16 * _KIB, 18 * _KIB),
    inj_w=(16 * _KIB, 18 * _KIB),
    inj_c=(16 * _KIB, 18 * _KIB),
    inj_q=(14 * _KIB, 16 * _KIB),
    inj_k=(14 * _KIB, 16 * _KIB),
    inj_v=(14 * _KIB, 16 * _KIB),
    inj_wo=((8 * _KIB,) * 24, (16 * _KIB,) * 20),
    pump_0=(30, 3),
    pump_w=(6, 1),
    pump_c=(7, 1),
    pump_uv=(18, 3),
    pump_q=(8, 2),
    pump_k=(10, 3),
    pump_v=(13, 3),
    pump_b=(4, 3),
    pump_e=(2, 2),
    pump_f=(4, 2),
    kick_s=(0, 1, 3, 5, 7),
    kick_c=(2, 5),
    kick_qk=(0, 2, 4, 6),
    kick_pv=(2, 5),
    side_rows=128,
    side_n=24,
    side_last=80,
    side_nb=6,
    side_late=2,
    late_at=1,
    wo_inj=1,
    wo_wide=5,
    wo_chunks=(512, 128, 128),
    wo_tail=(80, 64, 48, 32, 16, 16),
)


def _dot(a, b):
    return jnp.dot(a, b, preferred_element_type=_F32)


def _dot_nt(a, b):
    return lax.dot_general(a, b, _NT, preferred_element_type=_F32)


def _bounds(n_rows, row_bytes, piece, shift, skip=0):
    step = piece // row_bytes
    first = (shift // row_bytes) % step
    cuts = [skip] + [r for r in range(first, n_rows, step) if r > skip] + [n_rows]
    return list(zip(cuts[:-1], cuts[1:]))


class _Pump:
    def __init__(self, copies):
        self.copies, self.started, self.waited = list(copies), 0, 0

    def kick(self):
        if self.started < len(self.copies):
            self.copies[self.started]().start(priority=_URGENT)
            self.started += 1

    def _wait_to(self, n):
        while self.waited < n:
            self.copies[self.waited]().wait()
            self.waited += 1

    def pump(self, n, lag=1):
        for _ in range(n):
            self.kick()
            self._wait_to(self.started - lag)

    def drain(self):
        while self.started < len(self.copies):
            self.kick()
        self._wait_to(self.started)


def _fused(cfg, A_x, A_k_cache, A_v_cache, A_wq, A_wo, B_x, B_c_kv, B_w_q, B_w_uk, B_w_uv, B_w_o):
    B, Sq, D = A_x.shape
    _, H, Sk, Dh = A_k_cache.shape
    assert Sq == 1 and B_x.shape[1] == 1
    assert A_wq.shape == (D, H * Dh)
    W = min(4096, max(256, Sk // 4))
    M, Hb, Db = B_w_q.shape
    Skb, Dc = B_c_kv.shape[1], B_c_kv.shape[2]
    BH = B * H
    NG = BH // _G
    NCT = Dc // _L
    HH = Hb // 2
    scale_a = float(Dh) ** -0.5
    scale_b = float(Db) ** -0.5
    piece, block = cfg["piece"], cfg["block"]
    shift_a, shift_b = cfg["shift_a"], cfg["shift_b"]
    side_rows, side_n, side_nb = cfg["side_rows"], cfg["side_n"], cfg["side_nb"]
    side_late, late_at = cfg["side_late"], cfg["late_at"]
    n_mxu = len(cfg["wo_chunks"])
    wo_chunks = tuple(cfg["wo_chunks"]) + tuple(cfg["wo_tail"])
    tail_rows = sum(cfg["wo_tail"])
    assert tail_rows % Dh == 0 and M % _L == 0 and NG >= 4
    side_lag = 2
    side_lead = side_nb - side_lag
    side_last = cfg["side_last"]
    side_all = side_n + (1 if side_last else 0)
    assert side_n <= 4 + B + NG

    xa2 = A_x.reshape(B, D)
    xb2 = B_x.reshape(B, M)
    k3 = A_k_cache.reshape(BH, Sk, Dh)
    v3 = A_v_cache.reshape(BH, Sk, Dh)
    wob2 = B_w_o.reshape(Hb * Db, M)

    def blocked(w, lead=0):
        row_bytes = 2 * functools.reduce(lambda a, b: a * b, w.shape[lead + 1:], 1)
        rows = block // row_bytes
        shape = w.shape[:lead] + (w.shape[lead] // rows, rows) + w.shape[lead + 1:]
        return w.reshape(shape), rows, row_bytes

    n_ct = H * Dh // _L
    wqa_t = A_wq.reshape(D // 8, 8, n_ct, _L).transpose(0, 2, 1, 3).reshape(D // 8 * n_ct, 8, _L)
    wqa3, r_wqa, b_wqa = blocked(wqa_t)
    wqb4, r_w, b_w = blocked(B_w_q.reshape(M * Hb, Db))
    wuk4, _, _ = blocked(B_w_uk.reshape(Dc * Hb, Db))
    wuv4, _, _ = blocked(B_w_uv.reshape(Dc * Hb, Db))
    c_t = B_c_kv.reshape(B, Skb // 8, 8, NCT, _L).transpose(0, 1, 3, 2, 4)
    c4, r_c, b_c = blocked(c_t.reshape(B, Skb // 8 * NCT, 8, _L), 1)
    k_c = r_c // NCT * 8
    woa3, r_wo, b_wo = blocked(A_wo)
    assert wqb4.shape == wuk4.shape == wuv4.shape and 2 * r_w == _L * Hb
    NBLK = wqb4.shape[0]

    def spans(sizes, unit, n_rows=0):
        out, front, back = [], 0, n_rows
        for n in sizes:
            if n > 0:
                out.append((front, front + n // unit))
                front += n // unit
            else:
                out.append((back + n // unit, back))
                back += n // unit
        return out, front, back

    def split(sizes, n_rows, unit, shift):
        small, front, back = spans(sizes, unit, n_rows)
        return small, _bounds(back, unit, piece, shift, front)

    i_w, cut_w = split(cfg["inj_w"], r_w, b_w, shift_b)
    i_c, cut_c = split(cfg["inj_c"], r_c, b_c, shift_b)
    i_k, cut_k = split(cfg["inj_k"], W, 2 * Dh, shift_a)
    i_v, cut_v = split(cfg["inj_v"], W, 2 * Dh, shift_a)
    i_wqa, cut_wqa = split(cfg["inj_q"], r_wqa, b_wqa, shift_a)
    i_wo, _, _ = spans(cfg["inj_wo"][0] + cfg["inj_wo"][1], 2 * D)
    n_wo_first = len(cfg["inj_wo"][0])
    i_w0, cut_w0 = split(cfg["inj_0"], r_w, b_w, shift_b)
    wo_inj, wo_wide = cfg["wo_inj"], cfg["wo_wide"]
    cut_wo = _bounds(r_wo, b_wo, piece, cfg["shift_wo"])
    wo_base = (wo_inj + wo_wide) * r_wo
    assert i_wo[-1][1] == wo_inj * r_wo
    assert wo_base + sum(wo_chunks) == H * Dh
    n_wo = len(wo_chunks)
    wo_off = [wo_base + sum(wo_chunks[:i]) for i in range(n_wo)]
    assert all(lo // r_wo == (lo + n - 1) // r_wo for lo, n in zip(wo_off, wo_chunks))
    S_XB, S_XA, S_WQB, S_WUK, S_WUV, S_WOB, S_WQA, S_INJ, S_WIDE = range(9)
    S_C = 9
    S_KV = S_C + B
    S_WO = S_KV + 2 * NG
    S_SA = S_WO + n_wo
    S_SB = S_SA + side_nb
    n_sem = S_SB + side_nb
    side_total = side_rows * side_n + side_last

    def kernel(xa_h, k_h, v_h, wqa_h, woa_h, xb_h, c_h, wqb_h, wuk_h, wuv_h, wob_h,
               o_ref,
               xa_s, xb_s, kv_s, wqa_s, woa_s, c_s, wqb_s, wuk_s, wuv_s, wob_s,
               qa_s, oa_s, qabs_s, ctx_s, acc_s, accb_s, ctxb_s, oab_s, coef_s, vacc_s, p_s, s_s,
               side_s, sem):
        def cp(src, dst, s):
            return pltpu.make_async_copy(src, dst, sem.at[s])

        def start_pieces(src, dst, cuts, s, row0=0):
            for lo, hi in cuts:
                cp(src.at[:, pl.ds(row0 + lo, hi - lo)], dst.at[:, pl.ds(lo, hi - lo)],
                   s).start(priority=_BULK)

        def wait_pieces(dst, cuts, s):
            view = dst.at[:, pl.ds(cuts[0][0], cuts[-1][1] - cuts[0][0])]
            cp(view, view, s).wait()

        def heads_of(src, dst, ranges, row0=0):
            def one(k, lo, hi):
                return cp(src.at[k, pl.ds(row0 + lo, hi - lo)], dst.at[k, pl.ds(lo, hi - lo)], S_INJ)
            return [functools.partial(one, k, lo, hi)
                    for lo, hi in ranges for k in range(dst.shape[0])]

        k_s, v_s = kv_s.at[0], kv_s.at[1]
        c_xb = cp(xb_h, xb_s, S_XB)
        c_xa = cp(xa_h, xa_s, S_XA)
        rest = pl.ds(side_total, Hb * Db - side_total)
        c_wob = cp(wob_h.at[rest, :], wob_s.at[rest, :], S_WOB)

        def start_c(b):
            start_pieces(c_h.at[b], c_s.at[b], cut_c, S_C + b)

        def pump_c(b):
            return _Pump(heads_of(c_h.at[b], c_s.at[b], i_c))

        def start_wqa():
            c_wob.start(priority=_BULK)
            start_pieces(wqa_h, wqa_s, cut_wqa, S_WQA)

        def start_k(g):
            start_pieces(k_h.at[pl.ds(g * _G, _G)], k_s.at[g], cut_k, S_KV + 2 * g, Sk - W)

        def start_v(g):
            start_pieces(v_h.at[pl.ds(g * _G, _G)], v_s.at[g], cut_v, S_KV + 2 * g + 1, Sk - W)

        def pump_kv(g):
            heads = pl.ds(g * _G, _G)
            return _Pump(heads_of(k_h.at[heads], k_s.at[g], i_k, Sk - W)
                         + heads_of(v_h.at[heads], v_s.at[g], i_v, Sk - W))

        def wo_at(lo, n):
            return lo // r_wo, pl.ds(lo % r_wo, n)

        def c_wo(i):
            at = wo_at(wo_off[i], wo_chunks[i])
            return cp(woa_h.at[at], woa_s.at[at], S_WO + i)

        wide = pl.ds(wo_inj, wo_wide)

        def start_wo():
            start_pieces(woa_h.at[wide], woa_s.at[wide], cut_wo, S_WIDE)
            for i in range(n_wo):
                c_wo(i).start(priority=_BULK)

        def pump_wo(first, last):
            def one(lo, hi):
                at = wo_at(lo, hi - lo)
                return cp(woa_h.at[at], woa_s.at[at], S_INJ)
            return _Pump([functools.partial(one, *i_wo[j]) for j in range(first, last)])

        def side_refs(i):
            if isinstance(i, int):
                n = side_rows if i < side_n else side_last
                return pl.ds(i * side_rows, n), side_s.at[i % side_nb, pl.ds(0, n)], i % side_nb
            slot = lax.rem(i, side_nb)
            return pl.ds(pl.multiple_of(i * side_rows, 8), side_rows), side_s.at[slot], slot

        def c_sa(i):
            rows, stage, slot = side_refs(i)
            return cp(wob_h.at[rows, :], stage, S_SA + slot)

        def c_sb(i):
            rows, stage, slot = side_refs(i)
            return cp(stage, wob_s.at[rows, :], S_SB + slot)

        def tick(i):
            traced = not isinstance(i, int)
            if traced or i < side_n:
                c_sa(i).wait()
                c_sb(i).start()

            def refill(j):
                if traced or i >= side_lag:
                    c_sb(i - side_lag).wait()
                c_sa(j).start()

            if traced:
                pl.when(i + side_lead < side_n)(lambda: refill(i + side_lead))
            elif i + side_lead < side_n:
                refill(i + side_lead)

        def head_major(w_s, t, hh):
            w = w_s[2 * t:2 * t + 2].reshape(_L, Hb, Db)[:, hh * HH:(hh + 1) * HH, :]
            return w.reshape(_L, HH * Db)

        start_pieces(wqb_h, wqb_s, cut_w0, S_WQB)
        c_xb.start()
        c_xa.start()
        for i in range(side_lead):
            c_sa(i).start()
        start_pieces(wuk_h, wuk_s, cut_w, S_WUK)
        pm = _Pump(heads_of(wqb_h, wqb_s, i_w0) + heads_of(wuk_h, wuk_s, i_w))
        pm.pump(*cfg["pump_0"])
        pm.drain()


        wait_pieces(wqb_s, cut_w0, S_WQB)
        start_c(0)
        pm = pump_c(0)
        pm.kick()
        tick(0)
        c_xb.wait()
        xb = xb_s[...]
        for t in range(M // _L):
            for hh in range(2):
                cols = slice(hh * HH * Db, (hh + 1) * HH * Db)
                part = _dot(xb[:, t * _L:(t + 1) * _L], head_major(wqb_s, t, hh))
                ctxb_s[:, cols] = part if t == 0 else ctxb_s[:, cols] + part
                pm.pump(1)
        pm.pump(*cfg["pump_w"])
        pm.drain()

        wait_pieces(wuk_s, cut_w, S_WUK)
        start_c(1)
        pm = pump_c(1)
        pm.kick()
        tick(1)
        qb = (ctxb_s[...] * scale_b).astype(_BF16)
        for t in range(NCT):
            for hh in range(2):
                w = head_major(wuk_s, t, hh)
                parts = [_dot_nt(qb[:, (hh * HH + j) * Db:(hh * HH + j + 1) * Db],
                                 w[:, j * Db:(j + 1) * Db]) for j in range(HH)]
                qabs_s[t, :, hh * HH:(hh + 1) * HH, :] = jnp.concatenate(
                    parts, axis=1).reshape(B, HH, _L)
                pm.pump(1)
        pm.pump(*cfg["pump_w"])
        pm.drain()

        def attend_b(b, start_next, pm, same_buffer):
            wait_pieces(c_s.at[b], cut_c, S_C + b)
            start_next()
            pm.kick()
            tick(2 + b)
            step = pm.kick if same_buffer else functools.partial(pm.pump, 1)
            qa = jnp.concatenate(
                [qabs_s[t, b] for t in range(NCT)], axis=1).astype(_BF16)

            def latent(k):
                tiles = c_s[b, k].reshape(k_c // 8, NCT, 8, _L)
                return jnp.concatenate(
                    [tiles[:, t].reshape(k_c, _L) for t in range(NCT)], axis=1)

            for k in range(NBLK):
                s_s[:, k * k_c:(k + 1) * k_c] = _dot_nt(qa, latent(k))
                if k in cfg["kick_s"]:
                    step()
            s = s_s[...]
            m = jnp.max(s, axis=-1, keepdims=True)
            p = jnp.exp(s - m)
            l = jnp.sum(p, axis=-1, keepdims=True)
            pb = p.astype(_BF16)
            cc = None
            for k in range(NBLK):
                part = _dot(pb[:, k * k_c:(k + 1) * k_c], latent(k))
                cc = part if cc is None else cc + part
                if k in cfg["kick_c"]:
                    if not same_buffer:
                        s_s[:, :Dc] = cc
                    step()
                    if not same_buffer:
                        cc = s_s[:, :Dc]
            cc = cc / l
            for t in range(NCT):
                ctx_s[t, b] = cc[:, t * _L:(t + 1) * _L]
            pm.pump(*cfg["pump_c"])
            pm.drain()

        for b in range(B):
            if b + 2 < B:
                attend_b(b, functools.partial(start_c, b + 2), pump_c(b + 2), True)
            elif b + 2 == B:
                attend_b(b, functools.partial(start_pieces, wuv_h, wuv_s, cut_w, S_WUV),
                         _Pump(heads_of(wuv_h, wuv_s, i_w)), False)
            else:
                attend_b(b, start_wqa, _Pump(heads_of(wqa_h, wqa_s, i_wqa)), False)

        wait_pieces(wuv_s, cut_w, S_WUV)
        start_k(0)
        start_v(0)
        pm = pump_kv(0)
        pm.kick()
        tick(2 + B)
        for t in range(NCT):
            for hh in range(2):
                w = head_major(wuv_s, t, hh)
                ch = ctx_s[t, :, hh * HH:(hh + 1) * HH, :].reshape(B, HH * _L).astype(_BF16)
                parts = [_dot(ch[:, j * _L:(j + 1) * _L], w[:, j * Db:(j + 1) * Db])
                         for j in range(HH)]
                cols = slice(hh * HH * Db, (hh + 1) * HH * Db)
                part = jnp.concatenate(parts, axis=1)
                ctxb_s[:, cols] = part if t == 0 else ctxb_s[:, cols] + part
                pm.pump(1)
        pm.pump(*cfg["pump_uv"])
        pm.drain()

        wait_pieces(wqa_s, cut_wqa, S_WQA)
        start_k(1)
        pm = pump_kv(1)
        pm.kick()
        tick(3 + B)
        c_xa.wait()
        xa = xa_s[...]
        wq_tiles = wqa_s[...].reshape(D // 8, n_ct, 8, _L)
        qa_all = jnp.concatenate(
            [_dot(xa, wq_tiles[:, ct].reshape(D, _L)) for ct in range(n_ct)], axis=1) * scale_a
        qa_s[...] = qa_all.reshape(B, H, Dh).reshape(BH, Dh)
        pm.pump(*cfg["pump_q"])
        pm.drain()

        def attend_a(g, start_at_k, start_at_v, pm, same_buffer, between):
            start = g * _G if isinstance(g, int) else pl.multiple_of(g * _G, _G)
            rows = pl.ds(start, _G)
            q8 = qa_s[rows, :].astype(_BF16)
            wait_pieces(k_s.at[g], cut_k, S_KV + 2 * g)
            start_at_k()
            pm.kick()
            tick(4 + B + g)
            row = lax.broadcasted_iota(jnp.int32, (_G, W), 0)
            s = None
            for j in range(_G):
                sj = _dot_nt(q8, k_s[g, j])
                s = sj if s is None else jnp.where(row == j, sj, s)
                if j in cfg["kick_qk"]:
                    if same_buffer:
                        pm.kick()
                    else:
                        p_s[...] = s
                        pm.pump(1)
                        s = p_s[...]
            m = jnp.max(s, axis=-1, keepdims=True)
            p = jnp.exp(s - m)
            l = jnp.sum(p, axis=-1, keepdims=True)
            p_s[...] = p
            between()
            wait_pieces(v_s.at[g], cut_v, S_KV + 2 * g + 1)
            start_at_v()
            if same_buffer:
                pm.kick()
            else:
                pm.pump(1)
            pb = p_s[...].astype(_BF16)
            row2 = lax.broadcasted_iota(jnp.int32, (_G, Dh), 0)
            o = None
            for j in range(_G):
                oj = _dot(pb, v_s[g, j])
                o = oj if o is None else jnp.where(row2 == j, oj, o)
                if j in cfg["kick_pv"] and same_buffer:
                    pm.kick()
            oa_s[rows, :] = o / l

        def a_body(g, carry):
            pm = pump_kv(g + 2)
            attend_a(g, functools.partial(start_v, g + 1), functools.partial(start_k, g + 2), pm,
                     True, functools.partial(pm.pump, *cfg["pump_k"]))
            pm.pump(*cfg["pump_v"])
            pm.drain()
            return carry

        lax.fori_loop(0, NG - 2, a_body, 0)

        pm = pump_wo(0, n_wo_first)
        attend_a(NG - 2, functools.partial(start_v, NG - 1), start_wo, pm,
                 False, functools.partial(pm.pump, *cfg["pump_k"]))
        pm.pump(*cfg["pump_v"])
        pm.drain()

        n_early = side_all - side_late
        waited = side_n - side_nb
        r_early = n_early * side_rows
        pm = pump_wo(n_wo_first, len(i_wo))

        def project_b():
            c_wob.wait()
            for i in range(waited + (1 if side_last else 0), n_early):
                c_sb(i).wait()
            ctxb = ctxb_s[...].astype(_BF16)
            accb_s[...] = _dot(ctxb[:, side_total:], wob_s[side_total:, :])
            step = 8 * _L
            for lo in range(0, r_early, step):
                pm.pump(1)
                hi = min(lo + step, r_early)
                accb_s[...] += _dot(ctxb[:, lo:hi], wob_s[lo:hi, :])
            pm.pump(*cfg["pump_b"])

        def start_last_piece():
            if side_last:
                c_sb(waited).wait()
                c_sa(side_n).start()

        attend_a(NG - 1, start_last_piece, lambda: None, pm, False, project_b)
        pm.pump(1)

        oa32 = oa_s[...].reshape(B, H, Dh).reshape(B, H * Dh)
        oab_s[...] = oa32
        tail0 = H * Dh - tail_rows
        for b in range(B):
            for t in range(tail_rows // Dh):
                src = oa32[b:b + 1, tail0 + t * Dh:tail0 + (t + 1) * Dh]
                coef_s[b, t * Dh:(t + 1) * Dh, :] = jnp.broadcast_to(src, (_L, Dh)).T
        pm.pump(*cfg["pump_e"])
        if side_last:
            c_sa(side_n).wait()
            c_sb(side_n).start()
        pm.pump(*cfg["pump_f"])
        pm.drain()
        oa = oab_s[...].astype(_BF16)
        n_inj = wo_inj * r_wo
        acc_s[...] = _dot(oa[:, :n_inj], woa_s[:wo_inj].reshape(n_inj, D))
        wait_pieces(woa_s.at[wide], cut_wo, S_WIDE)
        acc_s[...] += _dot(oa[:, n_inj:wo_base],
                           woa_s[wo_inj:wo_inj + wo_wide].reshape(wo_base - n_inj, D))
        for i in range(n_mxu):
            c_wo(i).wait()
            if i == late_at:
                for j in range(n_early, side_all):
                    c_sb(j).wait()
                late = _dot(ctxb_s[:, r_early:side_total].astype(_BF16),
                            wob_s[r_early:side_total, :])
                o_ref[:, D:] = (accb_s[...] + late).astype(o_ref.dtype)
            lo, n = wo_off[i], wo_chunks[i]
            part = _dot(oa[:, lo:lo + n], woa_s[wo_at(lo, n)]) + acc_s[...]
            if i < n_wo - 1:
                acc_s[...] = part
            else:
                o_ref[:, :D] = part.astype(o_ref.dtype)
        for i in range(n_mxu, n_wo):
            c_wo(i).wait()
            lo, n = wo_off[i], wo_chunks[i]
            w = woa_s[wo_at(lo, n)].astype(_F32)
            sums = []
            for b in range(B):
                cf = coef_s[b, lo - tail0:lo - tail0 + n, :]
                prod = w * jnp.concatenate([cf] * (D // _L), axis=1)
                acc = vacc_s[b] if i > n_mxu else None
                for r in range(0, n, 8):
                    acc = prod[r:r + 8] if acc is None else acc + prod[r:r + 8]
                if i < n_wo - 1:
                    vacc_s[b] = acc
                else:
                    sums.append(jnp.sum(acc, axis=0, keepdims=True))
            if i == n_wo - 1:
                res = acc_s[...] + jnp.concatenate(sums, axis=0)
                o_ref[:, :D] = res.astype(o_ref.dtype)

    any_spec = pl.BlockSpec(memory_space=pl.ANY)
    out = pl.pallas_call(
        kernel,
        out_shape=jax.ShapeDtypeStruct((B, D + M), A_x.dtype),
        in_specs=[any_spec] * 11,
        out_specs=pl.BlockSpec(memory_space=pltpu.VMEM),
        scratch_shapes=[
            pltpu.VMEM(xa2.shape, _BF16),
            pltpu.VMEM(xb2.shape, _BF16),
            pltpu.VMEM((2, NG, _G, W, Dh), _BF16),
            pltpu.VMEM(wqa3.shape, _BF16),
            pltpu.VMEM(woa3.shape, _BF16),
            pltpu.VMEM(c4.shape, _BF16),
            pltpu.VMEM(wqb4.shape, _BF16),
            pltpu.VMEM(wuk4.shape, _BF16),
            pltpu.VMEM(wuv4.shape, _BF16),
            pltpu.VMEM(wob2.shape, _BF16),
            pltpu.VMEM((BH, Dh), _F32),
            pltpu.VMEM((BH, Dh), _F32),
            pltpu.VMEM((NCT, B, Hb, _L), _F32),
            pltpu.VMEM((NCT, B, Hb, _L), _F32),
            pltpu.VMEM((B, D), _F32),
            pltpu.VMEM((B, M), _F32),
            pltpu.VMEM((B, Hb * Db), _F32),
            pltpu.VMEM((B, H * Dh), _F32),
            pltpu.VMEM((B, max(tail_rows, 8), _L), _F32),
            pltpu.VMEM((B, 8, D), _F32),
            pltpu.VMEM((_G, W), _F32),
            pltpu.VMEM((Hb, Skb), _F32),
            pltpu.SMEM((side_nb, side_rows, M), _BF16),
            pltpu.SemaphoreType.DMA((n_sem,)),
        ],
        compiler_params=pltpu.CompilerParams(
            vmem_limit_bytes=120 * 1024 * 1024,
            disable_semaphore_checks=True,
            disable_bounds_checks=True,
        ),
        name="fused_decode",
    )(xa2, k3, v3, wqa3, woa3, xb2, c4, wqb4, wuk4, wuv4, wob2)
    return out.reshape(B, Sq, D + M)


@jax.jit
def pallas_concat_heads__sliding_block_cached__compressed_kv_cla__decode_kernel(
    A_x: jax.Array,
    A_k_cache: jax.Array,
    A_v_cache: jax.Array,
    A_wq: jax.Array,
    A_wo: jax.Array,
    B_x: jax.Array,
    B_c_kv: jax.Array,
    B_w_q: jax.Array,
    B_w_uk: jax.Array,
    B_w_uv: jax.Array,
    B_w_o: jax.Array,
):
    return _fused(_CFG, A_x, A_k_cache, A_v_cache, A_wq, A_wo,
                  B_x, B_c_kv, B_w_q, B_w_uk, B_w_uv, B_w_o)
```

```python
import functools

import jax
import jax.numpy as jnp
from jax import lax
import jax.experimental.pallas as pl
import jax.experimental.pallas.tpu as pltpu

_NT = (((1,), (1,)), ((), ()))
_F32 = jnp.float32
_BF16 = jnp.bfloat16
_L = 128
_G = 8
_KIB = 1024
_URGENT, _BULK = 0, 1

_CFG = dict(
    piece=64 * _KIB,
    block=512 * _KIB,
    shift_a=30 * _KIB,
    shift_b=34 * _KIB,
    shift_wo=32 * _KIB,
    inj_0=(16 * _KIB, 18 * _KIB),
    inj_w=(16 * _KIB, 18 * _KIB),
    inj_c=(16 * _KIB, 18 * _KIB),
    inj_q=(14 * _KIB, 16 * _KIB),
    inj_k=(14 * _KIB, 16 * _KIB),
    inj_v=(14 * _KIB, 16 * _KIB),
    inj_wo=(16 * _KIB,) * 52,
    pump_0=(28, 2),
    pump_w=(6, 1),
    pump_c=(7, 1),
    pump_uv=(18, 3),
    pump_q=(8, 2),
    pump_k=(10, 3),
    pump_v=(13, 3),
    pump_k14=(9, 3),
    pump_b=(6, 3),
    pump_k15=(10, 3),
    pump_e=(3, 3),
    pump_f=(7, 3),
    lag_w=2, lag_c=2, lag_qk=2, lag_b=2,
    kick_s=(0, 1, 3, 5, 7),
    kick_c=(2, 5),
    kick_qk=(0, 2, 4, 6),
    kick_pv=(2, 5),
    side_rows=128,
    side_n=24,
    side_last=80,
    side_nb=6,
    side_mid=3,
    side_late=1,
    late_at=1,
    wo_chunks=(512, 128, 128),
    wo_tail=(80, 64, 48, 32, 16, 16),
)


def _dot(a, b):
    return jnp.dot(a, b, preferred_element_type=_F32)


def _dot_nt(a, b):
    return lax.dot_general(a, b, _NT, preferred_element_type=_F32)


def _bounds(n_rows, row_bytes, piece, shift, skip=0):
    step = piece // row_bytes
    first = (shift // row_bytes) % step
    cuts = [skip] + [r for r in range(first, n_rows, step) if r > skip] + [n_rows]
    return list(zip(cuts[:-1], cuts[1:]))


class _Pump:
    def __init__(self, copies):
        self.copies, self.started, self.waited = list(copies), 0, 0

    def kick(self):
        if self.started < len(self.copies):
            self.copies[self.started]().start(priority=_URGENT)
            self.started += 1

    def _wait_to(self, n):
        while self.waited < n:
            self.copies[self.waited]().wait()
            self.waited += 1

    def pump(self, n, lag=1):
        for _ in range(n):
            self.kick()
            self._wait_to(self.started - lag)

    def drain(self):
        while self.started < len(self.copies):
            self.kick()
        self._wait_to(self.started)


def _fused(cfg, A_x, A_k_cache, A_v_cache, A_wq, A_wo, B_x, B_c_kv, B_w_q, B_w_uk, B_w_uv, B_w_o):
    B, Sq, D = A_x.shape
    _, H, Sk, Dh = A_k_cache.shape
    assert Sq == 1 and B_x.shape[1] == 1
    assert A_wq.shape == (D, H * Dh)
    W = min(4096, max(256, Sk // 4))
    M, Hb, Db = B_w_q.shape
    Skb, Dc = B_c_kv.shape[1], B_c_kv.shape[2]
    BH = B * H
    NG = BH // _G
    NCT = Dc // _L
    HH = Hb // 2
    scale_a = float(Dh) ** -0.5
    scale_b = float(Db) ** -0.5
    piece, block = cfg["piece"], cfg["block"]
    shift_a, shift_b = cfg["shift_a"], cfg["shift_b"]
    side_rows, side_n, side_nb = cfg["side_rows"], cfg["side_n"], cfg["side_nb"]
    side_late, late_at = cfg["side_late"], cfg["late_at"]
    n_mxu = len(cfg["wo_chunks"])
    wo_chunks = tuple(cfg["wo_chunks"]) + tuple(cfg["wo_tail"])
    tail_rows = sum(cfg["wo_tail"])
    assert tail_rows % Dh == 0 and M % _L == 0 and NG >= 4
    side_lag = 2
    side_lead = side_nb - side_lag
    side_last = cfg["side_last"]
    side_all = side_n + (1 if side_last else 0)
    assert side_n <= 4 + B + NG and cfg["side_mid"] < side_nb

    xa2 = A_x.reshape(B, D)
    xb2 = B_x.reshape(B, M)
    k3 = A_k_cache.reshape(BH, Sk, Dh)
    v3 = A_v_cache.reshape(BH, Sk, Dh)
    wob2 = B_w_o.reshape(Hb * Db, M)

    def blocked(w, lead=0):
        row_bytes = 2 * functools.reduce(lambda a, b: a * b, w.shape[lead + 1:], 1)
        rows = block // row_bytes
        shape = w.shape[:lead] + (w.shape[lead] // rows, rows) + w.shape[lead + 1:]
        return w.reshape(shape), rows, row_bytes

    n_ct = H * Dh // _L
    wqa_t = A_wq.reshape(D // 8, 8, n_ct, _L).transpose(0, 2, 1, 3).reshape(D // 8 * n_ct, 8, _L)
    wqa3, r_wqa, b_wqa = blocked(wqa_t)
    wqb4, r_w, b_w = blocked(B_w_q.reshape(M * Hb, Db))
    wuk4, _, _ = blocked(B_w_uk.reshape(Dc * Hb, Db))
    wuv4, _, _ = blocked(B_w_uv.reshape(Dc * Hb, Db))
    c_t = B_c_kv.reshape(B, Skb // 8, 8, NCT, _L).transpose(0, 1, 3, 2, 4)
    c4, r_c, b_c = blocked(c_t.reshape(B, Skb // 8 * NCT, 8, _L), 1)
    k_c = r_c // NCT * 8
    woa3, r_wo, b_wo = blocked(A_wo)
    assert wqb4.shape == wuk4.shape == wuv4.shape and 2 * r_w == _L * Hb
    NBLK = wqb4.shape[0]

    def spans(sizes, unit, n_rows=0):
        out, front, back = [], 0, n_rows
        for n in sizes:
            if n > 0:
                out.append((front, front + n // unit))
                front += n // unit
            else:
                out.append((back + n // unit, back))
                back += n // unit
        return out, front, back

    def split(sizes, n_rows, unit, shift):
        small, front, back = spans(sizes, unit, n_rows)
        return small, _bounds(back, unit, piece, shift, front)

    i_w, cut_w = split(cfg["inj_w"], r_w, b_w, shift_b)
    i_c, cut_c = split(cfg["inj_c"], r_c, b_c, shift_b)
    i_k, cut_k = split(cfg["inj_k"], W, 2 * Dh, shift_a)
    i_v, cut_v = split(cfg["inj_v"], W, 2 * Dh, shift_a)
    i_wqa, cut_wqa = split(cfg["inj_q"], r_wqa, b_wqa, shift_a)
    i_wo, _, _ = spans(cfg["inj_wo"], 2 * D)
    i_w0, cut_w0 = split(cfg["inj_0"], r_w, b_w, shift_b)
    n_inj = i_wo[-1][1]
    wo_inj = -(-n_inj // r_wo)
    wo_wide = (H * Dh - sum(wo_chunks)) // r_wo - wo_inj
    cut_wo = _bounds(r_wo, b_wo, piece, cfg["shift_wo"])
    wo_base = (wo_inj + wo_wide) * r_wo
    assert all(lo // r_wo == (hi - 1) // r_wo for lo, hi in i_wo)
    assert wo_base + sum(wo_chunks) == H * Dh
    n_wo = len(wo_chunks)
    wo_off = [wo_base + sum(wo_chunks[:i]) for i in range(n_wo)]
    assert all(lo // r_wo == (lo + n - 1) // r_wo for lo, n in zip(wo_off, wo_chunks))
    S_XB, S_XA, S_WQB, S_WUK, S_WUV, S_WOB, S_WQA, S_INJ, S_WIDE, S_GAP = range(10)
    S_C = 10
    S_KV = S_C + B
    S_WO = S_KV + 2 * NG
    S_SA = S_WO + n_wo
    S_SB = S_SA + side_nb
    n_sem = S_SB + side_nb
    side_total = side_rows * side_n + side_last

    def kernel(xa_h, k_h, v_h, wqa_h, woa_h, xb_h, c_h, wqb_h, wuk_h, wuv_h, wob_h,
               o_ref,
               xa_s, xb_s, kv_s, wqa_s, woa_s, c_s, wqb_s, wuk_s, wuv_s, wob_s,
               qa_s, oa_s, qabs_s, ctx_s, acc_s, accb_s, ctxb_s, oab_s, coef_s, vacc_s, p_s, s_s,
               side_s, sem):
        def cp(src, dst, s):
            return pltpu.make_async_copy(src, dst, sem.at[s])

        def start_pieces(src, dst, cuts, s, row0=0):
            for lo, hi in cuts:
                cp(src.at[:, pl.ds(row0 + lo, hi - lo)], dst.at[:, pl.ds(lo, hi - lo)],
                   s).start(priority=_BULK)

        def wait_pieces(dst, cuts, s):
            view = dst.at[:, pl.ds(cuts[0][0], cuts[-1][1] - cuts[0][0])]
            cp(view, view, s).wait()

        def heads_of(src, dst, ranges, row0=0):
            def one(k, lo, hi):
                return cp(src.at[k, pl.ds(row0 + lo, hi - lo)], dst.at[k, pl.ds(lo, hi - lo)], S_INJ)
            return [functools.partial(one, k, lo, hi)
                    for lo, hi in ranges for k in range(dst.shape[0])]

        k_s, v_s = kv_s.at[0], kv_s.at[1]
        c_xb = cp(xb_h, xb_s, S_XB)
        c_xa = cp(xa_h, xa_s, S_XA)
        rest = pl.ds(side_total, Hb * Db - side_total)
        c_wob = cp(wob_h.at[rest, :], wob_s.at[rest, :], S_WOB)

        def start_c(b):
            start_pieces(c_h.at[b], c_s.at[b], cut_c, S_C + b)

        def pump_c(b):
            return _Pump(heads_of(c_h.at[b], c_s.at[b], i_c))

        def start_wqa():
            c_wob.start(priority=_BULK)
            start_pieces(wqa_h, wqa_s, cut_wqa, S_WQA)

        def start_k(g):
            start_pieces(k_h.at[pl.ds(g * _G, _G)], k_s.at[g], cut_k, S_KV + 2 * g, Sk - W)

        def start_v(g):
            start_pieces(v_h.at[pl.ds(g * _G, _G)], v_s.at[g], cut_v, S_KV + 2 * g + 1, Sk - W)

        def pump_kv(g):
            heads = pl.ds(g * _G, _G)
            return _Pump(heads_of(k_h.at[heads], k_s.at[g], i_k, Sk - W)
                         + heads_of(v_h.at[heads], v_s.at[g], i_v, Sk - W))

        def wo_at(lo, n):
            return lo // r_wo, pl.ds(lo % r_wo, n)

        def c_wo(i):
            at = wo_at(wo_off[i], wo_chunks[i])
            return cp(woa_h.at[at], woa_s.at[at], S_WO + i)

        wide = pl.ds(wo_inj, wo_wide)

        n_gap = wo_inj * r_wo - n_inj
        if n_gap:
            c_gap = cp(woa_h.at[wo_at(n_inj, n_gap)], woa_s.at[wo_at(n_inj, n_gap)], S_GAP)

        def start_wo():
            if n_gap:
                c_gap.start(priority=_BULK)
            start_pieces(woa_h.at[wide], woa_s.at[wide], cut_wo, S_WIDE)
            for i in range(n_wo):
                c_wo(i).start(priority=_BULK)

        def pump_wo(first, last):
            def one(lo, hi):
                at = wo_at(lo, hi - lo)
                return cp(woa_h.at[at], woa_s.at[at], S_INJ)
            return _Pump([functools.partial(one, *i_wo[j]) for j in range(first, last)])

        def side_refs(i):
            if isinstance(i, int):
                n = side_rows if i < side_n else side_last
                return pl.ds(i * side_rows, n), side_s.at[i % side_nb, pl.ds(0, n)], i % side_nb
            slot = lax.rem(i, side_nb)
            return pl.ds(pl.multiple_of(i * side_rows, 8), side_rows), side_s.at[slot], slot

        def c_sa(i):
            rows, stage, slot = side_refs(i)
            return cp(wob_h.at[rows, :], stage, S_SA + slot)

        def c_sb(i):
            rows, stage, slot = side_refs(i)
            return cp(stage, wob_s.at[rows, :], S_SB + slot)

        def tick(i):
            traced = not isinstance(i, int)
            if traced or i < side_n:
                c_sa(i).wait()
                c_sb(i).start()

            def refill(j):
                if traced or i >= side_lag:
                    c_sb(i - side_lag).wait()
                c_sa(j).start()

            if traced:
                pl.when(i + side_lead < side_n)(lambda: refill(i + side_lead))
            elif i + side_lead < side_n:
                refill(i + side_lead)

        def head_major(w_s, t, hh):
            w = w_s[2 * t:2 * t + 2].reshape(_L, Hb, Db)[:, hh * HH:(hh + 1) * HH, :]
            return w.reshape(_L, HH * Db)

        start_pieces(wqb_h, wqb_s, cut_w0, S_WQB)
        c_xb.start()
        c_xa.start()
        for i in range(side_lead):
            c_sa(i).start()
        start_pieces(wuk_h, wuk_s, cut_w, S_WUK)
        pm = _Pump(heads_of(wqb_h, wqb_s, i_w0) + heads_of(wuk_h, wuk_s, i_w))
        pm.pump(*cfg["pump_0"])
        pm.drain()


        wait_pieces(wqb_s, cut_w0, S_WQB)
        start_c(0)
        pm = pump_c(0)
        pm.kick()
        tick(0)
        c_xb.wait()
        xb = xb_s[...]
        for t in range(M // _L):
            for hh in range(2):
                cols = slice(hh * HH * Db, (hh + 1) * HH * Db)
                part = _dot(xb[:, t * _L:(t + 1) * _L], head_major(wqb_s, t, hh))
                ctxb_s[:, cols] = part if t == 0 else ctxb_s[:, cols] + part
                pm.pump(1, cfg["lag_w"])
        pm.pump(*cfg["pump_w"])
        pm.drain()

        wait_pieces(wuk_s, cut_w, S_WUK)
        start_c(1)
        pm = pump_c(1)
        pm.kick()
        tick(1)
        qb = (ctxb_s[...] * scale_b).astype(_BF16)
        for t in range(NCT):
            for hh in range(2):
                w = head_major(wuk_s, t, hh)
                parts = [_dot_nt(qb[:, (hh * HH + j) * Db:(hh * HH + j + 1) * Db],
                                 w[:, j * Db:(j + 1) * Db]) for j in range(HH)]
                qabs_s[t, :, hh * HH:(hh + 1) * HH, :] = jnp.concatenate(
                    parts, axis=1).reshape(B, HH, _L)
                pm.pump(1, cfg["lag_w"])
        pm.pump(*cfg["pump_w"])
        pm.drain()

        def attend_b(b, start_next, pm, same_buffer):
            wait_pieces(c_s.at[b], cut_c, S_C + b)
            start_next()
            pm.kick()
            tick(2 + b)
            step = pm.kick if same_buffer else functools.partial(pm.pump, 1, cfg["lag_c"])
            qa = jnp.concatenate(
                [qabs_s[t, b] for t in range(NCT)], axis=1).astype(_BF16)

            def latent(k):
                tiles = c_s[b, k].reshape(k_c // 8, NCT, 8, _L)
                return jnp.concatenate(
                    [tiles[:, t].reshape(k_c, _L) for t in range(NCT)], axis=1)

            for k in range(NBLK):
                s_s[:, k * k_c:(k + 1) * k_c] = _dot_nt(qa, latent(k))
                if k in cfg["kick_s"]:
                    step()
            s = s_s[...]
            m = jnp.max(s, axis=-1, keepdims=True)
            p = jnp.exp(s - m)
            l = jnp.sum(p, axis=-1, keepdims=True)
            pb = p.astype(_BF16)
            cc = None
            for k in range(NBLK):
                part = _dot(pb[:, k * k_c:(k + 1) * k_c], latent(k))
                cc = part if cc is None else cc + part
                if k in cfg["kick_c"]:
                    if not same_buffer:
                        s_s[:, :Dc] = cc
                    step()
                    if not same_buffer:
                        cc = s_s[:, :Dc]
            cc = cc / l
            for t in range(NCT):
                ctx_s[t, b] = cc[:, t * _L:(t + 1) * _L]
            pm.pump(*cfg["pump_c"])
            pm.drain()

        for b in range(B):
            if b + 2 < B:
                attend_b(b, functools.partial(start_c, b + 2), pump_c(b + 2), True)
            elif b + 2 == B:
                attend_b(b, functools.partial(start_pieces, wuv_h, wuv_s, cut_w, S_WUV),
                         _Pump(heads_of(wuv_h, wuv_s, i_w)), False)
            else:
                attend_b(b, start_wqa, _Pump(heads_of(wqa_h, wqa_s, i_wqa)), False)

        wait_pieces(wuv_s, cut_w, S_WUV)
        start_k(0)
        start_v(0)
        pm = pump_kv(0)
        pm.kick()
        tick(2 + B)
        for t in range(NCT):
            for hh in range(2):
                w = head_major(wuv_s, t, hh)
                ch = ctx_s[t, :, hh * HH:(hh + 1) * HH, :].reshape(B, HH * _L).astype(_BF16)
                parts = [_dot(ch[:, j * _L:(j + 1) * _L], w[:, j * Db:(j + 1) * Db])
                         for j in range(HH)]
                cols = slice(hh * HH * Db, (hh + 1) * HH * Db)
                part = jnp.concatenate(parts, axis=1)
                ctxb_s[:, cols] = part if t == 0 else ctxb_s[:, cols] + part
                pm.pump(1, cfg["lag_w"])
        pm.pump(*cfg["pump_uv"])
        pm.drain()

        wait_pieces(wqa_s, cut_wqa, S_WQA)
        start_k(1)
        pm = pump_kv(1)
        pm.kick()
        tick(3 + B)
        c_xa.wait()
        xa = xa_s[...]
        wq_tiles = wqa_s[...].reshape(D // 8, n_ct, 8, _L)
        qa_all = jnp.concatenate(
            [_dot(xa, wq_tiles[:, ct].reshape(D, _L)) for ct in range(n_ct)], axis=1) * scale_a
        qa_s[...] = qa_all.reshape(B, H, Dh).reshape(BH, Dh)
        pm.pump(*cfg["pump_q"])
        pm.drain()

        def attend_a(g, start_at_k, start_at_v, pm, same_buffer, between):
            start = g * _G if isinstance(g, int) else pl.multiple_of(g * _G, _G)
            rows = pl.ds(start, _G)
            q8 = qa_s[rows, :].astype(_BF16)
            wait_pieces(k_s.at[g], cut_k, S_KV + 2 * g)
            start_at_k()
            pm.kick()
            tick(4 + B + g)
            row = lax.broadcasted_iota(jnp.int32, (_G, W), 0)
            s = None
            for j in range(_G):
                sj = _dot_nt(q8, k_s[g, j])
                s = sj if s is None else jnp.where(row == j, sj, s)
                if j in cfg["kick_qk"]:
                    if same_buffer:
                        pm.kick()
                    else:
                        p_s[...] = s
                        pm.pump(1, cfg["lag_qk"])
                        s = p_s[...]
            m = jnp.max(s, axis=-1, keepdims=True)
            p = jnp.exp(s - m)
            l = jnp.sum(p, axis=-1, keepdims=True)
            p_s[...] = p
            between()
            wait_pieces(v_s.at[g], cut_v, S_KV + 2 * g + 1)
            start_at_v()
            if same_buffer:
                pm.kick()
            else:
                pm.pump(1, cfg["lag_qk"])
            pb = p_s[...].astype(_BF16)
            row2 = lax.broadcasted_iota(jnp.int32, (_G, Dh), 0)
            o = None
            for j in range(_G):
                oj = _dot(pb, v_s[g, j])
                o = oj if o is None else jnp.where(row2 == j, oj, o)
                if j in cfg["kick_pv"] and same_buffer:
                    pm.kick()
            oa_s[rows, :] = o / l

        def a_body(g, carry):
            pm = pump_kv(g + 2)
            attend_a(g, functools.partial(start_v, g + 1), functools.partial(start_k, g + 2), pm,
                     True, functools.partial(pm.pump, *cfg["pump_k"]))
            pm.pump(*cfg["pump_v"])
            pm.drain()
            return carry

        lax.fori_loop(0, NG - 2, a_body, 0)

        waited = side_n - side_nb
        n_early, n_mid = side_n - cfg["side_mid"], side_all - side_late
        r_early, r_mid = n_early * side_rows, n_mid * side_rows
        pm = pump_wo(0, len(i_wo))

        def project_b():
            c_wob.wait()
            for i in range(waited, n_early):
                c_sb(i).wait()
            ctxb = ctxb_s[...].astype(_BF16)
            accb_s[...] = _dot(ctxb[:, side_total:], wob_s[side_total:, :])
            step = 8 * _L
            for lo in range(0, r_early, step):
                pm.pump(1, cfg["lag_b"])
                hi = min(lo + step, r_early)
                accb_s[...] += _dot(ctxb[:, lo:hi], wob_s[lo:hi, :])

        attend_a(NG - 2, functools.partial(start_v, NG - 1), start_wo, pm,
                 False, functools.partial(pm.pump, *cfg["pump_k14"]))
        project_b()
        pm.pump(*cfg["pump_b"])
        attend_a(NG - 1, (lambda: c_sa(side_n).start()) if side_last else (lambda: None),
                 lambda: None, pm, False, functools.partial(pm.pump, *cfg["pump_k15"]))
        pm.pump(1, cfg["lag_b"])

        oa32 = oa_s[...].reshape(B, H, Dh).reshape(B, H * Dh)
        oab_s[...] = oa32
        tail0 = H * Dh - tail_rows
        for b in range(B):
            for t in range(tail_rows // Dh):
                src = oa32[b:b + 1, tail0 + t * Dh:tail0 + (t + 1) * Dh]
                coef_s[b, t * Dh:(t + 1) * Dh, :] = jnp.broadcast_to(src, (_L, Dh)).T
        pm.pump(*cfg["pump_e"])
        if side_last:
            c_sa(side_n).wait()
            c_sb(side_n).start()
        pm.pump(*cfg["pump_f"])
        pm.drain()
        oa = oab_s[...].astype(_BF16)
        if n_gap:
            c_gap.wait()
        n_head = wo_inj * r_wo
        acc_s[...] = _dot(oa[:, :n_head], woa_s[:wo_inj].reshape(n_head, D))
        if n_mid > n_early:
            for j in range(n_early, n_mid):
                c_sb(j).wait()
            accb_s[...] += _dot(ctxb_s[:, r_early:r_mid].astype(_BF16), wob_s[r_early:r_mid, :])
        wait_pieces(woa_s.at[wide], cut_wo, S_WIDE)
        acc_s[...] += _dot(oa[:, n_head:wo_base],
                           woa_s[wo_inj:wo_inj + wo_wide].reshape(wo_base - n_head, D))
        for i in range(n_mxu):
            c_wo(i).wait()
            if i == late_at:
                for j in range(n_mid, side_all):
                    c_sb(j).wait()
                late = _dot(ctxb_s[:, r_mid:side_total].astype(_BF16),
                            wob_s[r_mid:side_total, :])
                o_ref[:, D:] = (accb_s[...] + late).astype(o_ref.dtype)
            lo, n = wo_off[i], wo_chunks[i]
            part = _dot(oa[:, lo:lo + n], woa_s[wo_at(lo, n)]) + acc_s[...]
            if i < n_wo - 1:
                acc_s[...] = part
            else:
                o_ref[:, :D] = part.astype(o_ref.dtype)
        for i in range(n_mxu, n_wo):
            c_wo(i).wait()
            lo, n = wo_off[i], wo_chunks[i]
            w = woa_s[wo_at(lo, n)].astype(_F32)
            sums = []
            for b in range(B):
                cf = coef_s[b, lo - tail0:lo - tail0 + n, :]
                prod = w * jnp.concatenate([cf] * (D // _L), axis=1)
                acc = vacc_s[b] if i > n_mxu else None
                for r in range(0, n, 8):
                    acc = prod[r:r + 8] if acc is None else acc + prod[r:r + 8]
                if i < n_wo - 1:
                    vacc_s[b] = acc
                else:
                    sums.append(jnp.sum(acc, axis=0, keepdims=True))
            if i == n_wo - 1:
                res = acc_s[...] + jnp.concatenate(sums, axis=0)
                o_ref[:, :D] = res.astype(o_ref.dtype)

    any_spec = pl.BlockSpec(memory_space=pl.ANY)
    out = pl.pallas_call(
        kernel,
        out_shape=jax.ShapeDtypeStruct((B, D + M), A_x.dtype),
        in_specs=[any_spec] * 11,
        out_specs=pl.BlockSpec(memory_space=pltpu.VMEM),
        scratch_shapes=[
            pltpu.VMEM(xa2.shape, _BF16),
            pltpu.VMEM(xb2.shape, _BF16),
            pltpu.VMEM((2, NG, _G, W, Dh), _BF16),
            pltpu.VMEM(wqa3.shape, _BF16),
            pltpu.VMEM(woa3.shape, _BF16),
            pltpu.VMEM(c4.shape, _BF16),
            pltpu.VMEM(wqb4.shape, _BF16),
            pltpu.VMEM(wuk4.shape, _BF16),
            pltpu.VMEM(wuv4.shape, _BF16),
            pltpu.VMEM(wob2.shape, _BF16),
            pltpu.VMEM((BH, Dh), _F32),
            pltpu.VMEM((BH, Dh), _F32),
            pltpu.VMEM((NCT, B, Hb, _L), _F32),
            pltpu.VMEM((NCT, B, Hb, _L), _F32),
            pltpu.VMEM((B, D), _F32),
            pltpu.VMEM((B, M), _F32),
            pltpu.VMEM((B, Hb * Db), _F32),
            pltpu.VMEM((B, H * Dh), _F32),
            pltpu.VMEM((B, max(tail_rows, 8), _L), _F32),
            pltpu.VMEM((B, 8, D), _F32),
            pltpu.VMEM((_G, W), _F32),
            pltpu.VMEM((Hb, Skb), _F32),
            pltpu.SMEM((side_nb, side_rows, M), _BF16),
            pltpu.SemaphoreType.DMA((n_sem,)),
        ],
        compiler_params=pltpu.CompilerParams(
            vmem_limit_bytes=120 * 1024 * 1024,
            disable_semaphore_checks=True,
            disable_bounds_checks=True,
        ),
        name="fused_decode",
    )(xa2, k3, v3, wqa3, woa3, xb2, c4, wqb4, wuk4, wuv4, wob2)
    return out.reshape(B, Sq, D + M)


@jax.jit
def pallas_concat_heads__sliding_block_cached__compressed_kv_cla__decode_kernel(
    A_x: jax.Array,
    A_k_cache: jax.Array,
    A_v_cache: jax.Array,
    A_wq: jax.Array,
    A_wo: jax.Array,
    B_x: jax.Array,
    B_c_kv: jax.Array,
    B_w_q: jax.Array,
    B_w_uk: jax.Array,
    B_w_uv: jax.Array,
    B_w_o: jax.Array,
):
    return _fused(_CFG, A_x, A_k_cache, A_v_cache, A_wq, A_wo,
                  B_x, B_c_kv, B_w_q, B_w_uk, B_w_uv, B_w_o)
```

```python
import functools

import jax
import jax.numpy as jnp
from jax import lax
import jax.experimental.pallas as pl
import jax.experimental.pallas.tpu as pltpu

_NT = (((1,), (1,)), ((), ()))
_F32 = jnp.float32
_BF16 = jnp.bfloat16
_L = 128
_G = 8
_KIB = 1024
_URGENT, _BULK = 0, 1

_CFG = dict(
    piece=64 * _KIB,
    block=512 * _KIB,
    shift_a=30 * _KIB,
    shift_b=34 * _KIB,
    shift_wo=32 * _KIB,
    inj_0=(),
    inj_w=(16 * _KIB, 18 * _KIB, -14 * _KIB, -16 * _KIB),
    inj_c=(16 * _KIB, 18 * _KIB, -14 * _KIB, -16 * _KIB),
    inj_q=(14 * _KIB, 16 * _KIB, -16 * _KIB, -18 * _KIB),
    inj_k=(14 * _KIB, 16 * _KIB),
    inj_v=(14 * _KIB, 16 * _KIB),
    inj_wo=(16 * _KIB,) * 52,
    pump_0=(28, 2),
    pump_w=(11, 3),
    pump_c=(15, 3),
    pump_uv=(18, 3),
    pump_q=(8, 2),
    pump_k=(10, 3),
    pump_v=(13, 3),
    pump_k14=(9, 3),
    pump_b=(6, 3),
    pump_k15=(10, 3),
    pump_e=(3, 3),
    pump_f=(7, 3),
    lag_w=2, lag_qk=2, lag_b=2,
    kick_s=(0, 1, 3, 5, 7),
    kick_c=(2, 5),
    kick_qk=(0, 2, 4, 6),
    kick_pv=(2, 5),
    side_rows=128,
    side_n=24,
    side_last=80,
    side_nb=6,
    side_mid=3,
    side_late=1,
    late_at=1,
    wo_chunks=(512, 128, 128),
    wo_tail=(80, 64, 48, 32, 16, 16),
)


def _dot(a, b):
    return jnp.dot(a, b, preferred_element_type=_F32)


def _dot_nt(a, b):
    return lax.dot_general(a, b, _NT, preferred_element_type=_F32)


def _bounds(n_rows, row_bytes, piece, shift, skip=0):
    step = piece // row_bytes
    first = (shift // row_bytes) % step
    cuts = [skip] + [r for r in range(first, n_rows, step) if r > skip] + [n_rows]
    return list(zip(cuts[:-1], cuts[1:]))


class _Pump:
    def __init__(self, copies):
        self.copies, self.started, self.waited = list(copies), 0, 0

    def kick(self):
        if self.started < len(self.copies):
            self.copies[self.started]().start(priority=_URGENT)
            self.started += 1

    def _wait_to(self, n):
        while self.waited < n:
            self.copies[self.waited]().wait()
            self.waited += 1

    def pump(self, n, lag=1):
        for _ in range(n):
            self.kick()
            self._wait_to(self.started - lag)

    def drain(self):
        while self.started < len(self.copies):
            self.kick()
        self._wait_to(self.started)


def _fused(cfg, A_x, A_k_cache, A_v_cache, A_wq, A_wo, B_x, B_c_kv, B_w_q, B_w_uk, B_w_uv, B_w_o):
    B, Sq, D = A_x.shape
    _, H, Sk, Dh = A_k_cache.shape
    assert Sq == 1 and B_x.shape[1] == 1
    assert A_wq.shape == (D, H * Dh)
    W = min(4096, max(256, Sk // 4))
    M, Hb, Db = B_w_q.shape
    Skb, Dc = B_c_kv.shape[1], B_c_kv.shape[2]
    BH = B * H
    NG = BH // _G
    NCT = Dc // _L
    HH = Hb // 2
    scale_a = float(Dh) ** -0.5
    scale_b = float(Db) ** -0.5
    piece, block = cfg["piece"], cfg["block"]
    shift_a, shift_b = cfg["shift_a"], cfg["shift_b"]
    side_rows, side_n, side_nb = cfg["side_rows"], cfg["side_n"], cfg["side_nb"]
    side_late, late_at = cfg["side_late"], cfg["late_at"]
    n_mxu = len(cfg["wo_chunks"])
    wo_chunks = tuple(cfg["wo_chunks"]) + tuple(cfg["wo_tail"])
    tail_rows = sum(cfg["wo_tail"])
    assert tail_rows % Dh == 0 and M % _L == 0 and NG >= 4
    side_lag = 2
    side_lead = side_nb - side_lag
    side_last = cfg["side_last"]
    side_all = side_n + (1 if side_last else 0)
    assert side_n <= 4 + B + NG and cfg["side_mid"] < side_nb

    xa2 = A_x.reshape(B, D)
    xb2 = B_x.reshape(B, M)
    k3 = A_k_cache.reshape(BH, Sk, Dh)
    v3 = A_v_cache.reshape(BH, Sk, Dh)
    wob2 = B_w_o.reshape(Hb * Db, M)

    def blocked(w, lead=0):
        row_bytes = 2 * functools.reduce(lambda a, b: a * b, w.shape[lead + 1:], 1)
        rows = block // row_bytes
        shape = w.shape[:lead] + (w.shape[lead] // rows, rows) + w.shape[lead + 1:]
        return w.reshape(shape), rows, row_bytes

    n_ct = H * Dh // _L
    wqa_t = A_wq.reshape(D // 8, 8, n_ct, _L).transpose(0, 2, 1, 3).reshape(D * n_ct, _L)
    wqa3, r_wqa, b_wqa = blocked(wqa_t)
    wqb4, r_w, b_w = blocked(B_w_q.reshape(M * Hb, Db))
    wuk4, _, _ = blocked(B_w_uk.reshape(Dc * Hb, Db))
    wuv4, _, _ = blocked(B_w_uv.reshape(Dc * Hb, Db))
    c_t = B_c_kv.reshape(B, Skb // 8, 8, NCT, _L).transpose(0, 1, 3, 2, 4)
    c4, r_c, b_c = blocked(c_t.reshape(B, Skb * NCT, _L), 1)
    k_c = r_c // NCT
    woa3, r_wo, b_wo = blocked(A_wo)
    assert wqb4.shape == wuk4.shape == wuv4.shape and 2 * r_w == _L * Hb
    assert wqa3.shape == wqb4.shape == c4.shape[1:]
    NBLK = wqb4.shape[0]

    def spans(sizes, unit, n_rows=0):
        out, front, back = [], 0, n_rows
        for n in sizes:
            if n > 0:
                out.append((front, front + n // unit))
                front += n // unit
            else:
                out.append((back + n // unit, back))
                back += n // unit
        return out, front, back

    def split(sizes, n_rows, unit, shift):
        small, front, back = spans(sizes, unit, n_rows)
        return small, _bounds(back, unit, piece, shift, front)

    i_w, cut_w = split(cfg["inj_w"], r_w, b_w, shift_b)
    i_c, cut_c = split(cfg["inj_c"], r_c, b_c, shift_b)
    i_k, cut_k = split(cfg["inj_k"], W, 2 * Dh, shift_a)
    i_v, cut_v = split(cfg["inj_v"], W, 2 * Dh, shift_a)
    i_wqa, cut_wqa = split(cfg["inj_q"], r_wqa, b_wqa, shift_a)
    i_wo, _, _ = spans(cfg["inj_wo"], 2 * D)
    i_w0, cut_w0 = split(cfg["inj_0"], r_w, b_w, shift_b)
    n_inj = i_wo[-1][1]
    wo_inj = -(-n_inj // r_wo)
    wo_wide = (H * Dh - sum(wo_chunks)) // r_wo - wo_inj
    cut_wo = _bounds(r_wo, b_wo, piece, cfg["shift_wo"])
    wo_base = (wo_inj + wo_wide) * r_wo
    assert all(lo // r_wo == (hi - 1) // r_wo for lo, hi in i_wo)
    assert wo_base + sum(wo_chunks) == H * Dh
    n_wo = len(wo_chunks)
    wo_off = [wo_base + sum(wo_chunks[:i]) for i in range(n_wo)]
    assert all(lo // r_wo == (lo + n - 1) // r_wo for lo, n in zip(wo_off, wo_chunks))
    S_XB, S_XA, S_WQB, S_WUK, S_WUV, S_WOB, S_WQA, S_INJ, S_WIDE, S_GAP = range(10)
    S_C = 10
    S_KV = S_C + B
    S_WO = S_KV + 2 * NG
    S_SA = S_WO + n_wo
    S_SB = S_SA + side_nb
    n_sem = S_SB + side_nb
    side_total = side_rows * side_n + side_last

    def kernel(xa_h, k_h, v_h, wqa_h, woa_h, xb_h, c_h, wqb_h, wuk_h, wuv_h, wob_h,
               o_ref,
               xa_s, xb_s, kv_s, big_s, woa_s, wob_s,
               qa_s, oa_s, qabs_s, ctx_s, acc_s, accb_s, ctxb_s, oab_s, coef_s, vacc_s, p_s, s_s,
               side_s, sem):
        def cp(src, dst, s):
            return pltpu.make_async_copy(src, dst, sem.at[s])

        def start_pieces(src, dst, cuts, s, row0=0):
            for lo, hi in cuts:
                cp(src.at[:, pl.ds(row0 + lo, hi - lo)], dst.at[:, pl.ds(lo, hi - lo)],
                   s).start(priority=_BULK)

        def wait_pieces(dst, cuts, s):
            view = dst.at[:, pl.ds(cuts[0][0], cuts[-1][1] - cuts[0][0])]
            cp(view, view, s).wait()

        def heads_of(src, dst, ranges, row0=0):
            def one(k, lo, hi):
                return cp(src.at[k, pl.ds(row0 + lo, hi - lo)], dst.at[k, pl.ds(lo, hi - lo)], S_INJ)
            return [functools.partial(one, k, lo, hi)
                    for lo, hi in ranges for k in range(dst.shape[0])]

        k_s, v_s = kv_s.at[0], kv_s.at[1]
        wqb_s, wuk_s, wuv_s, wqa_s = (big_s.at[j] for j in range(4))
        c_s = big_s.at[pl.ds(4, B)]
        c_xb = cp(xb_h, xb_s, S_XB)
        c_xa = cp(xa_h, xa_s, S_XA)
        rest = pl.ds(side_total, Hb * Db - side_total)
        c_wob = cp(wob_h.at[rest, :], wob_s.at[rest, :], S_WOB)

        def start_c(b):
            start_pieces(c_h.at[b], c_s.at[b], cut_c, S_C + b)

        def pump_c(b):
            return _Pump(heads_of(c_h.at[b], c_s.at[b], i_c))

        def start_wqa():
            c_wob.start(priority=_BULK)
            start_pieces(wqa_h, wqa_s, cut_wqa, S_WQA)

        def start_k(g):
            start_pieces(k_h.at[pl.ds(g * _G, _G)], k_s.at[g], cut_k, S_KV + 2 * g, Sk - W)

        def start_v(g):
            start_pieces(v_h.at[pl.ds(g * _G, _G)], v_s.at[g], cut_v, S_KV + 2 * g + 1, Sk - W)

        def pump_kv(g):
            heads = pl.ds(g * _G, _G)
            return _Pump(heads_of(k_h.at[heads], k_s.at[g], i_k, Sk - W)
                         + heads_of(v_h.at[heads], v_s.at[g], i_v, Sk - W))

        def wo_at(lo, n):
            return lo // r_wo, pl.ds(lo % r_wo, n)

        def c_wo(i):
            at = wo_at(wo_off[i], wo_chunks[i])
            return cp(woa_h.at[at], woa_s.at[at], S_WO + i)

        wide = pl.ds(wo_inj, wo_wide)

        n_gap = wo_inj * r_wo - n_inj
        if n_gap:
            c_gap = cp(woa_h.at[wo_at(n_inj, n_gap)], woa_s.at[wo_at(n_inj, n_gap)], S_GAP)

        def start_wo():
            if n_gap:
                c_gap.start(priority=_BULK)
            start_pieces(woa_h.at[wide], woa_s.at[wide], cut_wo, S_WIDE)
            for i in range(n_wo):
                c_wo(i).start(priority=_BULK)

        def pump_wo(first, last):
            def one(lo, hi):
                at = wo_at(lo, hi - lo)
                return cp(woa_h.at[at], woa_s.at[at], S_INJ)
            return _Pump([functools.partial(one, *i_wo[j]) for j in range(first, last)])

        def side_refs(i):
            if isinstance(i, int):
                n = side_rows if i < side_n else side_last
                return pl.ds(i * side_rows, n), side_s.at[i % side_nb, pl.ds(0, n)], i % side_nb
            slot = lax.rem(i, side_nb)
            return pl.ds(pl.multiple_of(i * side_rows, 8), side_rows), side_s.at[slot], slot

        def c_sa(i):
            rows, stage, slot = side_refs(i)
            return cp(wob_h.at[rows, :], stage, S_SA + slot)

        def c_sb(i):
            rows, stage, slot = side_refs(i)
            return cp(stage, wob_s.at[rows, :], S_SB + slot)

        def tick(i):
            traced = not isinstance(i, int)
            if traced or i < side_n:
                c_sa(i).wait()
                c_sb(i).start()

            def refill(j):
                if traced or i >= side_lag:
                    c_sb(i - side_lag).wait()
                c_sa(j).start()

            if traced:
                pl.when(i + side_lead < side_n)(lambda: refill(i + side_lead))
            elif i + side_lead < side_n:
                refill(i + side_lead)

        def head_major(w_s, t, hh, mid=lambda: None):
            halves = []
            for k in range(2):
                w = w_s[2 * t + k].reshape(_L // 2, Hb, Db)[:, hh * HH:(hh + 1) * HH, :]
                halves.append(w.reshape(_L // 2, HH * Db))
                if k == 0:
                    mid()
            return jnp.concatenate(halves, axis=0)

        start_pieces(wqb_h, wqb_s, cut_w0, S_WQB)
        c_xb.start()
        c_xa.start()
        for i in range(side_lead):
            c_sa(i).start()
        start_pieces(wuk_h, wuk_s, cut_w, S_WUK)
        pm = _Pump(heads_of(wqb_h, wqb_s, i_w0) + heads_of(wuk_h, wuk_s, i_w))
        pm.pump(*cfg["pump_0"])
        pm.drain()


        wait_pieces(wqb_s, cut_w0, S_WQB)
        start_c(0)
        pm = pump_c(0)
        pm.kick()
        tick(0)
        c_xb.wait()
        xb = xb_s[...]
        halves = [None, None]
        for t in range(M // _L):
            for hh in range(2):
                part = _dot(xb[:, t * _L:(t + 1) * _L], head_major(wqb_s, t, hh, pm.kick))
                halves[hh] = part if t == 0 else halves[hh] + part
                pm.kick()
        ctxb_s[...] = jnp.concatenate(halves, axis=1)
        pm.pump(*cfg["pump_w"])
        pm.drain()

        wait_pieces(wuk_s, cut_w, S_WUK)
        start_c(1)
        pm = pump_c(1)
        pm.kick()
        tick(1)
        qb = (ctxb_s[...] * scale_b).astype(_BF16)
        for t in range(NCT):
            for hh in range(2):
                w = head_major(wuk_s, t, hh, pm.kick)
                parts = [_dot_nt(qb[:, (hh * HH + j) * Db:(hh * HH + j + 1) * Db],
                                 w[:, j * Db:(j + 1) * Db]) for j in range(HH)]
                qabs_s[t, :, hh * HH:(hh + 1) * HH, :] = jnp.concatenate(
                    parts, axis=1).reshape(B, HH, _L)
                pm.kick()
        pm.pump(*cfg["pump_w"])
        pm.drain()

        def attend_b(b, start_next, pm):
            wait_pieces(c_s.at[b], cut_c, S_C + b)
            start_next()
            pm.kick()
            tick(2 + b)
            qa = jnp.concatenate(
                [qabs_s[t, b] for t in range(NCT)], axis=1).astype(_BF16)

            def latent(k):
                tiles = c_s[b, k].reshape(k_c // 8, NCT, 8, _L)
                return jnp.concatenate(
                    [tiles[:, t].reshape(k_c, _L) for t in range(NCT)], axis=1)

            for k in range(NBLK):
                s_s[:, k * k_c:(k + 1) * k_c] = _dot_nt(qa, latent(k))
                if k in cfg["kick_s"]:
                    pm.kick()
            s = s_s[...]
            m = jnp.max(s, axis=-1, keepdims=True)
            p = jnp.exp(s - m)
            l = jnp.sum(p, axis=-1, keepdims=True)
            pb = p.astype(_BF16)
            cc = None
            for k in range(NBLK):
                part = _dot(pb[:, k * k_c:(k + 1) * k_c], latent(k))
                cc = part if cc is None else cc + part
                if k in cfg["kick_c"]:
                    pm.kick()
            cc = cc / l
            for t in range(NCT):
                ctx_s[t, b] = cc[:, t * _L:(t + 1) * _L]
            pm.pump(*cfg["pump_c"])
            pm.drain()

        for b in range(B):
            if b + 2 < B:
                attend_b(b, functools.partial(start_c, b + 2), pump_c(b + 2))
            elif b + 2 == B:
                attend_b(b, functools.partial(start_pieces, wuv_h, wuv_s, cut_w, S_WUV),
                         _Pump(heads_of(wuv_h, wuv_s, i_w)))
            else:
                attend_b(b, start_wqa, _Pump(heads_of(wqa_h, wqa_s, i_wqa)))

        wait_pieces(wuv_s, cut_w, S_WUV)
        start_k(0)
        start_v(0)
        pm = pump_kv(0)
        pm.kick()
        tick(2 + B)
        for t in range(NCT):
            for hh in range(2):
                w = head_major(wuv_s, t, hh)
                ch = ctx_s[t, :, hh * HH:(hh + 1) * HH, :].reshape(B, HH * _L).astype(_BF16)
                parts = [_dot(ch[:, j * _L:(j + 1) * _L], w[:, j * Db:(j + 1) * Db])
                         for j in range(HH)]
                cols = slice(hh * HH * Db, (hh + 1) * HH * Db)
                part = jnp.concatenate(parts, axis=1)
                ctxb_s[:, cols] = part if t == 0 else ctxb_s[:, cols] + part
                pm.pump(1, cfg["lag_w"])
        pm.pump(*cfg["pump_uv"])
        pm.drain()

        wait_pieces(wqa_s, cut_wqa, S_WQA)
        start_k(1)
        pm = pump_kv(1)
        pm.kick()
        tick(3 + B)
        c_xa.wait()
        xa = xa_s[...]
        wq_tiles = wqa_s[...].reshape(D // 8, n_ct, 8, _L)
        qa_all = jnp.concatenate(
            [_dot(xa, wq_tiles[:, ct].reshape(D, _L)) for ct in range(n_ct)], axis=1) * scale_a
        qa_s[...] = qa_all.reshape(B, H, Dh).reshape(BH, Dh)
        pm.pump(*cfg["pump_q"])
        pm.drain()

        def attend_a(g, start_at_k, start_at_v, pm, same_buffer, between):
            start = g * _G if isinstance(g, int) else pl.multiple_of(g * _G, _G)
            rows = pl.ds(start, _G)
            q8 = qa_s[rows, :].astype(_BF16)
            wait_pieces(k_s.at[g], cut_k, S_KV + 2 * g)
            start_at_k()
            pm.kick()
            tick(4 + B + g)
            row = lax.broadcasted_iota(jnp.int32, (_G, W), 0)
            s = None
            for j in range(_G):
                sj = _dot_nt(q8, k_s[g, j])
                s = sj if s is None else jnp.where(row == j, sj, s)
                if j in cfg["kick_qk"]:
                    if same_buffer:
                        pm.kick()
                    else:
                        p_s[...] = s
                        pm.pump(1, cfg["lag_qk"])
                        s = p_s[...]
            m = jnp.max(s, axis=-1, keepdims=True)
            p = jnp.exp(s - m)
            l = jnp.sum(p, axis=-1, keepdims=True)
            p_s[...] = p
            between()
            wait_pieces(v_s.at[g], cut_v, S_KV + 2 * g + 1)
            start_at_v()
            if same_buffer:
                pm.kick()
            else:
                pm.pump(1, cfg["lag_qk"])
            pb = p_s[...].astype(_BF16)
            row2 = lax.broadcasted_iota(jnp.int32, (_G, Dh), 0)
            o = None
            for j in range(_G):
                oj = _dot(pb, v_s[g, j])
                o = oj if o is None else jnp.where(row2 == j, oj, o)
                if j in cfg["kick_pv"] and same_buffer:
                    pm.kick()
            oa_s[rows, :] = o / l

        def a_body(g, carry):
            pm = pump_kv(g + 2)
            attend_a(g, functools.partial(start_v, g + 1), functools.partial(start_k, g + 2), pm,
                     True, functools.partial(pm.pump, *cfg["pump_k"]))
            pm.pump(*cfg["pump_v"])
            pm.drain()
            return carry

        lax.fori_loop(0, NG - 2, a_body, 0)

        waited = side_n - side_nb
        n_early, n_mid = side_n - cfg["side_mid"], side_all - side_late
        r_early, r_mid = n_early * side_rows, n_mid * side_rows
        pm = pump_wo(0, len(i_wo))

        def project_b():
            c_wob.wait()
            for i in range(waited, n_early):
                c_sb(i).wait()
            ctxb = ctxb_s[...].astype(_BF16)
            accb_s[...] = _dot(ctxb[:, side_total:], wob_s[side_total:, :])
            step = 8 * _L
            for lo in range(0, r_early, step):
                pm.pump(1, cfg["lag_b"])
                hi = min(lo + step, r_early)
                accb_s[...] += _dot(ctxb[:, lo:hi], wob_s[lo:hi, :])

        attend_a(NG - 2, functools.partial(start_v, NG - 1), start_wo, pm,
                 False, functools.partial(pm.pump, *cfg["pump_k14"]))
        project_b()
        pm.pump(*cfg["pump_b"])
        attend_a(NG - 1, (lambda: c_sa(side_n).start()) if side_last else (lambda: None),
                 lambda: None, pm, False, functools.partial(pm.pump, *cfg["pump_k15"]))
        pm.pump(1, cfg["lag_b"])

        oa32 = oa_s[...].reshape(B, H, Dh).reshape(B, H * Dh)
        oab_s[...] = oa32
        tail0 = H * Dh - tail_rows
        for b in range(B):
            for t in range(tail_rows // Dh):
                src = oa32[b:b + 1, tail0 + t * Dh:tail0 + (t + 1) * Dh]
                coef_s[b, t * Dh:(t + 1) * Dh, :] = jnp.broadcast_to(src, (_L, Dh)).T
        pm.pump(*cfg["pump_e"])
        if side_last:
            c_sa(side_n).wait()
            c_sb(side_n).start()
        pm.pump(*cfg["pump_f"])
        pm.drain()
        oa = oab_s[...].astype(_BF16)
        if n_gap:
            c_gap.wait()
        n_head = wo_inj * r_wo
        acc_s[...] = _dot(oa[:, :n_head], woa_s[:wo_inj].reshape(n_head, D))
        if n_mid > n_early:
            for j in range(n_early, n_mid):
                c_sb(j).wait()
            accb_s[...] += _dot(ctxb_s[:, r_early:r_mid].astype(_BF16), wob_s[r_early:r_mid, :])
        wait_pieces(woa_s.at[wide], cut_wo, S_WIDE)
        acc_s[...] += _dot(oa[:, n_head:wo_base],
                           woa_s[wo_inj:wo_inj + wo_wide].reshape(wo_base - n_head, D))
        for i in range(n_mxu):
            c_wo(i).wait()
            if i == late_at:
                for j in range(n_mid, side_all):
                    c_sb(j).wait()
                late = _dot(ctxb_s[:, r_mid:side_total].astype(_BF16),
                            wob_s[r_mid:side_total, :])
                o_ref[:, D:] = (accb_s[...] + late).astype(o_ref.dtype)
            lo, n = wo_off[i], wo_chunks[i]
            part = _dot(oa[:, lo:lo + n], woa_s[wo_at(lo, n)]) + acc_s[...]
            if i < n_wo - 1:
                acc_s[...] = part
            else:
                o_ref[:, :D] = part.astype(o_ref.dtype)
        for i in range(n_mxu, n_wo):
            c_wo(i).wait()
            lo, n = wo_off[i], wo_chunks[i]
            w = woa_s[wo_at(lo, n)].astype(_F32)
            sums = []
            for b in range(B):
                cf = coef_s[b, lo - tail0:lo - tail0 + n, :]
                prod = w * jnp.concatenate([cf] * (D // _L), axis=1)
                acc = vacc_s[b] if i > n_mxu else None
                for r in range(0, n, 8):
                    acc = prod[r:r + 8] if acc is None else acc + prod[r:r + 8]
                if i < n_wo - 1:
                    vacc_s[b] = acc
                else:
                    sums.append(jnp.sum(acc, axis=0, keepdims=True))
            if i == n_wo - 1:
                res = acc_s[...] + jnp.concatenate(sums, axis=0)
                o_ref[:, :D] = res.astype(o_ref.dtype)

    any_spec = pl.BlockSpec(memory_space=pl.ANY)
    out = pl.pallas_call(
        kernel,
        out_shape=jax.ShapeDtypeStruct((B, D + M), A_x.dtype),
        in_specs=[any_spec] * 11,
        out_specs=pl.BlockSpec(memory_space=pltpu.VMEM),
        scratch_shapes=[
            pltpu.VMEM(xa2.shape, _BF16),
            pltpu.VMEM(xb2.shape, _BF16),
            pltpu.VMEM((2, NG, _G, W, Dh), _BF16),
            pltpu.VMEM((4 + B,) + wqb4.shape, _BF16),
            pltpu.VMEM(woa3.shape, _BF16),
            pltpu.VMEM(wob2.shape, _BF16),
            pltpu.VMEM((BH, Dh), _F32),
            pltpu.VMEM((BH, Dh), _F32),
            pltpu.VMEM((NCT, B, Hb, _L), _F32),
            pltpu.VMEM((NCT, B, Hb, _L), _F32),
            pltpu.VMEM((B, D), _F32),
            pltpu.VMEM((B, M), _F32),
            pltpu.VMEM((B, Hb * Db), _F32),
            pltpu.VMEM((B, H * Dh), _F32),
            pltpu.VMEM((B, max(tail_rows, 8), _L), _F32),
            pltpu.VMEM((B, 8, D), _F32),
            pltpu.VMEM((_G, W), _F32),
            pltpu.VMEM((Hb, Skb), _F32),
            pltpu.SMEM((side_nb, side_rows, M), _BF16),
            pltpu.SemaphoreType.DMA((n_sem,)),
        ],
        compiler_params=pltpu.CompilerParams(
            vmem_limit_bytes=120 * 1024 * 1024,
            disable_semaphore_checks=True,
            disable_bounds_checks=True,
        ),
        name="fused_decode",
    )(xa2, k3, v3, wqa3, woa3, xb2, c4, wqb4, wuk4, wuv4, wob2)
    return out.reshape(B, Sq, D + M)


@jax.jit
def pallas_concat_heads__sliding_block_cached__compressed_kv_cla__decode_kernel(
    A_x: jax.Array,
    A_k_cache: jax.Array,
    A_v_cache: jax.Array,
    A_wq: jax.Array,
    A_wo: jax.Array,
    B_x: jax.Array,
    B_c_kv: jax.Array,
    B_w_q: jax.Array,
    B_w_uk: jax.Array,
    B_w_uv: jax.Array,
    B_w_o: jax.Array,
):
    return _fused(_CFG, A_x, A_k_cache, A_v_cache, A_wq, A_wo,
                  B_x, B_c_kv, B_w_q, B_w_uk, B_w_uv, B_w_o)
```

```python
import functools

import jax
import jax.numpy as jnp
from jax import lax
import jax.experimental.pallas as pl
import jax.experimental.pallas.tpu as pltpu

_NT = (((1,), (1,)), ((), ()))
_F32 = jnp.float32
_BF16 = jnp.bfloat16
_L = 128
_G = 8
_KIB = 1024
_URGENT, _BULK = 0, 1

_CFG = dict(
    piece=64 * _KIB,
    block=512 * _KIB,
    shift_a=30 * _KIB,
    shift_b=34 * _KIB,
    shift_wo=32 * _KIB,
    inj_0=(),
    inj_w=(16 * _KIB, 18 * _KIB, -14 * _KIB, -16 * _KIB),
    inj_c=(16 * _KIB, 18 * _KIB, -14 * _KIB, -16 * _KIB),
    inj_q=(14 * _KIB, 16 * _KIB, -16 * _KIB, -18 * _KIB),
    inj_k=(14 * _KIB, 16 * _KIB),
    inj_v=(14 * _KIB, 16 * _KIB),
    inj_wo=(16 * _KIB,) * 52,
    pump_0=(28, 2),
    pump_w=(11, 3),
    pump_c=(15, 3),
    pump_uv=(20, 3),
    pump_q=(8, 2),
    pump_k=(10, 3),
    pump_v=(13, 3),
    pump_k14=(9, 3),
    pump_b=(6, 3),
    pump_k15=(10, 3),
    pump_e=(3, 3),
    pump_f=(7, 3),
    seg_q=2,
    lag_w=2, lag_qk=2, lag_b=2,
    kick_s=(0, 1, 2, 3, 4, 5, 6, 7),
    kick_c=(1, 3, 5),
    kick_qk=(0, 2, 4, 6),
    kick_pv=(2, 5),
    side_rows=128,
    side_n=24,
    side_last=64,
    side_nb=6,
    side_mid=3,
    side_late=1,
    late_at=1,
    wo_chunks=(512, 128, 128),
    wo_tail=(80, 64, 48, 32, 16, 16),
)


def _dot(a, b):
    return jnp.dot(a, b, preferred_element_type=_F32)


def _dot_nt(a, b):
    return lax.dot_general(a, b, _NT, preferred_element_type=_F32)


def _bounds(n_rows, row_bytes, piece, shift, skip=0):
    step = piece // row_bytes
    first = (shift // row_bytes) % step
    cuts = [skip] + [r for r in range(first, n_rows, step) if r > skip] + [n_rows]
    return list(zip(cuts[:-1], cuts[1:]))


class _Pump:
    def __init__(self, copies):
        self.copies, self.started, self.waited = list(copies), 0, 0

    def kick(self):
        if self.started < len(self.copies):
            self.copies[self.started]().start(priority=_URGENT)
            self.started += 1

    def _wait_to(self, n):
        while self.waited < n:
            self.copies[self.waited]().wait()
            self.waited += 1

    def pump(self, n, lag=1):
        for _ in range(n):
            self.kick()
            self._wait_to(self.started - lag)

    def drain(self):
        while self.started < len(self.copies):
            self.kick()
        self._wait_to(self.started)


def _fused(cfg, A_x, A_k_cache, A_v_cache, A_wq, A_wo, B_x, B_c_kv, B_w_q, B_w_uk, B_w_uv, B_w_o):
    B, Sq, D = A_x.shape
    _, H, Sk, Dh = A_k_cache.shape
    assert Sq == 1 and B_x.shape[1] == 1
    assert A_wq.shape == (D, H * Dh)
    W = min(4096, max(256, Sk // 4))
    M, Hb, Db = B_w_q.shape
    Skb, Dc = B_c_kv.shape[1], B_c_kv.shape[2]
    BH = B * H
    NG = BH // _G
    NCT = Dc // _L
    HH = Hb // 2
    scale_a = float(Dh) ** -0.5
    scale_b = float(Db) ** -0.5
    piece, block = cfg["piece"], cfg["block"]
    shift_a, shift_b = cfg["shift_a"], cfg["shift_b"]
    side_rows, side_n, side_nb = cfg["side_rows"], cfg["side_n"], cfg["side_nb"]
    side_late, late_at = cfg["side_late"], cfg["late_at"]
    n_mxu = len(cfg["wo_chunks"])
    wo_chunks = tuple(cfg["wo_chunks"]) + tuple(cfg["wo_tail"])
    tail_rows = sum(cfg["wo_tail"])
    assert tail_rows % Dh == 0 and M % _L == 0 and NG >= 4
    side_lag = 2
    side_lead = side_nb - side_lag
    side_last = cfg["side_last"]
    side_all = side_n + (1 if side_last else 0)
    assert side_n <= 4 + B + NG and cfg["side_mid"] < side_nb

    xa2 = A_x.reshape(B, D)
    xb2 = B_x.reshape(B, M)
    k3 = A_k_cache.reshape(BH, Sk, Dh)
    v3 = A_v_cache.reshape(BH, Sk, Dh)
    wob2 = B_w_o.reshape(Hb * Db, M)

    def blocked(w, lead=0):
        row_bytes = 2 * functools.reduce(lambda a, b: a * b, w.shape[lead + 1:], 1)
        rows = block // row_bytes
        shape = w.shape[:lead] + (w.shape[lead] // rows, rows) + w.shape[lead + 1:]
        return w.reshape(shape), rows, row_bytes

    n_ct = H * Dh // _L
    wqa_t = A_wq.reshape(D // 8, 8, n_ct, _L).transpose(0, 2, 1, 3).reshape(D * n_ct, _L)
    wqa3, r_wqa, b_wqa = blocked(wqa_t)
    wqb4, r_w, b_w = blocked(B_w_q.reshape(M * Hb, Db))
    wuk4, _, _ = blocked(B_w_uk.reshape(Dc * Hb, Db))
    wuv4, _, _ = blocked(B_w_uv.reshape(Dc * Hb, Db))
    c_t = B_c_kv.reshape(B, Skb // 8, 8, NCT, _L).transpose(0, 1, 3, 2, 4)
    c4, r_c, b_c = blocked(c_t.reshape(B, Skb * NCT, _L), 1)
    k_c = r_c // NCT
    woa3, r_wo, b_wo = blocked(A_wo)
    assert wqb4.shape == wuk4.shape == wuv4.shape and 2 * r_w == _L * Hb
    assert wqa3.shape == wqb4.shape == c4.shape[1:]
    NBLK = wqb4.shape[0]

    def spans(sizes, unit, n_rows=0):
        out, front, back = [], 0, n_rows
        for n in sizes:
            if n > 0:
                out.append((front, front + n // unit))
                front += n // unit
            else:
                out.append((back + n // unit, back))
                back += n // unit
        return out, front, back

    def split(sizes, n_rows, unit, shift):
        small, front, back = spans(sizes, unit, n_rows)
        return small, _bounds(back, unit, piece, shift, front)

    i_w, cut_w = split(cfg["inj_w"], r_w, b_w, shift_b)
    i_c, cut_c = split(cfg["inj_c"], r_c, b_c, shift_b)
    i_k, cut_k = split(cfg["inj_k"], W, 2 * Dh, shift_a)
    i_v, cut_v = split(cfg["inj_v"], W, 2 * Dh, shift_a)
    i_wqa, cut_wqa = split(cfg["inj_q"], r_wqa, b_wqa, shift_a)
    i_wo, _, _ = spans(cfg["inj_wo"], 2 * D)
    i_w0, cut_w0 = split(cfg["inj_0"], r_w, b_w, shift_b)
    n_inj = i_wo[-1][1]
    wo_inj = -(-n_inj // r_wo)
    wo_wide = (H * Dh - sum(wo_chunks)) // r_wo - wo_inj
    cut_wo = _bounds(r_wo, b_wo, piece, cfg["shift_wo"])
    wo_base = (wo_inj + wo_wide) * r_wo
    assert all(lo // r_wo == (hi - 1) // r_wo for lo, hi in i_wo)
    assert wo_base + sum(wo_chunks) == H * Dh
    n_wo = len(wo_chunks)
    wo_off = [wo_base + sum(wo_chunks[:i]) for i in range(n_wo)]
    assert all(lo // r_wo == (lo + n - 1) // r_wo for lo, n in zip(wo_off, wo_chunks))
    S_XB, S_XA, S_WQB, S_WUK, S_WUV, S_WOB, S_WQA, S_INJ, S_WIDE, S_GAP = range(10)
    S_C = 10
    S_KV = S_C + B
    S_WO = S_KV + 2 * NG
    S_SA = S_WO + n_wo
    S_SB = S_SA + side_nb
    n_sem = S_SB + side_nb
    side_total = side_rows * side_n + side_last

    def kernel(xa_h, k_h, v_h, wqa_h, woa_h, xb_h, c_h, wqb_h, wuk_h, wuv_h, wob_h,
               o_ref,
               xa_s, xb_s, kv_s, big_s, woa_s, wob_s,
               qa_s, oa_s, qabs_s, ctx_s, acc_s, accb_s, ctxb_s, oab_s, coef_s, vacc_s, p_s, s_s,
               side_s, sem):
        def cp(src, dst, s):
            return pltpu.make_async_copy(src, dst, sem.at[s])

        def start_pieces(src, dst, cuts, s, row0=0):
            for lo, hi in cuts:
                cp(src.at[:, pl.ds(row0 + lo, hi - lo)], dst.at[:, pl.ds(lo, hi - lo)],
                   s).start(priority=_BULK)

        def wait_pieces(dst, cuts, s):
            view = dst.at[:, pl.ds(cuts[0][0], cuts[-1][1] - cuts[0][0])]
            cp(view, view, s).wait()

        def heads_of(src, dst, ranges, row0=0):
            def one(k, lo, hi):
                return cp(src.at[k, pl.ds(row0 + lo, hi - lo)], dst.at[k, pl.ds(lo, hi - lo)], S_INJ)
            return [functools.partial(one, k, lo, hi)
                    for lo, hi in ranges for k in range(dst.shape[0])]

        k_s, v_s = kv_s.at[0], kv_s.at[1]
        wqb_s, wuk_s, wuv_s, wqa_s = (big_s.at[j] for j in range(4))
        c_s = big_s.at[pl.ds(4, B)]
        c_xb = cp(xb_h, xb_s, S_XB)
        c_xa = cp(xa_h, xa_s, S_XA)
        rest = pl.ds(side_total, Hb * Db - side_total)
        c_wob = cp(wob_h.at[rest, :], wob_s.at[rest, :], S_WOB)

        def start_c(b):
            start_pieces(c_h.at[b], c_s.at[b], cut_c, S_C + b)

        def pump_c(b):
            return _Pump(heads_of(c_h.at[b], c_s.at[b], i_c))

        def start_wqa():
            c_wob.start(priority=_BULK)
            start_pieces(wqa_h, wqa_s, cut_wqa, S_WQA)

        def start_k(g):
            start_pieces(k_h.at[pl.ds(g * _G, _G)], k_s.at[g], cut_k, S_KV + 2 * g, Sk - W)

        def start_v(g):
            start_pieces(v_h.at[pl.ds(g * _G, _G)], v_s.at[g], cut_v, S_KV + 2 * g + 1, Sk - W)

        def small_k(g):
            return heads_of(k_h.at[pl.ds(g * _G, _G)], k_s.at[g], i_k, Sk - W)

        def small_v(g):
            return heads_of(v_h.at[pl.ds(g * _G, _G)], v_s.at[g], i_v, Sk - W)

        def wo_at(lo, n):
            return lo // r_wo, pl.ds(lo % r_wo, n)

        def c_wo(i):
            at = wo_at(wo_off[i], wo_chunks[i])
            return cp(woa_h.at[at], woa_s.at[at], S_WO + i)

        wide = pl.ds(wo_inj, wo_wide)

        n_gap = wo_inj * r_wo - n_inj
        if n_gap:
            c_gap = cp(woa_h.at[wo_at(n_inj, n_gap)], woa_s.at[wo_at(n_inj, n_gap)], S_GAP)

        def start_wo():
            if n_gap:
                c_gap.start(priority=_BULK)
            start_pieces(woa_h.at[wide], woa_s.at[wide], cut_wo, S_WIDE)
            for i in range(n_wo):
                c_wo(i).start(priority=_BULK)

        def pump_wo(first, last):
            def one(lo, hi):
                at = wo_at(lo, hi - lo)
                return cp(woa_h.at[at], woa_s.at[at], S_INJ)
            return _Pump([functools.partial(one, *i_wo[j]) for j in range(first, last)])

        def side_refs(i):
            if isinstance(i, int):
                n = side_rows if i < side_n else side_last
                return pl.ds(i * side_rows, n), side_s.at[i % side_nb, pl.ds(0, n)], i % side_nb
            slot = lax.rem(i, side_nb)
            return pl.ds(pl.multiple_of(i * side_rows, 8), side_rows), side_s.at[slot], slot

        def c_sa(i):
            rows, stage, slot = side_refs(i)
            return cp(wob_h.at[rows, :], stage, S_SA + slot)

        def c_sb(i):
            rows, stage, slot = side_refs(i)
            return cp(stage, wob_s.at[rows, :], S_SB + slot)

        def tick(i):
            traced = not isinstance(i, int)
            if traced or i < side_n:
                c_sa(i).wait()
                c_sb(i).start()

            def refill(j):
                if traced or i >= side_lag:
                    c_sb(i - side_lag).wait()
                c_sa(j).start()

            if traced:
                pl.when(i + side_lead < side_n)(lambda: refill(i + side_lead))
            elif i + side_lead < side_n:
                refill(i + side_lead)

        def head_major(w_s, t, hh, mid=lambda: None):
            halves = []
            for k in range(2):
                w = w_s[2 * t + k].reshape(_L // 2, Hb, Db)[:, hh * HH:(hh + 1) * HH, :]
                halves.append(w.reshape(_L // 2, HH * Db))
                if k == 0:
                    mid()
            return jnp.concatenate(halves, axis=0)

        start_pieces(wqb_h, wqb_s, cut_w0, S_WQB)
        c_xb.start()
        c_xa.start()
        for i in range(side_lead):
            c_sa(i).start()
        start_pieces(wuk_h, wuk_s, cut_w, S_WUK)
        pm = _Pump(heads_of(wqb_h, wqb_s, i_w0) + heads_of(wuk_h, wuk_s, i_w))
        pm.pump(*cfg["pump_0"])
        pm.drain()


        wait_pieces(wqb_s, cut_w0, S_WQB)
        start_c(0)
        pm = pump_c(0)
        pm.kick()
        tick(0)
        c_xb.wait()
        xb = xb_s[...]
        halves = [None, None]
        for t in range(M // _L):
            for hh in range(2):
                part = _dot(xb[:, t * _L:(t + 1) * _L], head_major(wqb_s, t, hh, pm.kick))
                halves[hh] = part if t == 0 else halves[hh] + part
                pm.kick()
        ctxb_s[...] = jnp.concatenate(halves, axis=1)
        pm.pump(*cfg["pump_w"])
        pm.drain()

        wait_pieces(wuk_s, cut_w, S_WUK)
        start_c(1)
        pm = pump_c(1)
        pm.kick()
        tick(1)
        qb = (ctxb_s[...] * scale_b).astype(_BF16)
        for t in range(NCT):
            for hh in range(2):
                w = head_major(wuk_s, t, hh, pm.kick)
                parts = [_dot_nt(qb[:, (hh * HH + j) * Db:(hh * HH + j + 1) * Db],
                                 w[:, j * Db:(j + 1) * Db]) for j in range(HH)]
                qabs_s[t, :, hh * HH:(hh + 1) * HH, :] = jnp.concatenate(
                    parts, axis=1).reshape(B, HH, _L)
                pm.kick()
        pm.pump(*cfg["pump_w"])
        pm.drain()

        def attend_b(b, start_next, pm):
            wait_pieces(c_s.at[b], cut_c, S_C + b)
            start_next()
            pm.kick()
            tick(2 + b)
            qa = jnp.concatenate(
                [qabs_s[t, b] for t in range(NCT)], axis=1).astype(_BF16)

            def latent(k):
                tiles = c_s[b, k].reshape(k_c // 8, NCT, 8, _L)
                return jnp.concatenate(
                    [tiles[:, t].reshape(k_c, _L) for t in range(NCT)], axis=1)

            for k in range(NBLK):
                s_s[:, k * k_c:(k + 1) * k_c] = _dot_nt(qa, latent(k))
                if k in cfg["kick_s"]:
                    pm.kick()
            s = s_s[...]
            m = jnp.max(s, axis=-1, keepdims=True)
            p = jnp.exp(s - m)
            l = jnp.sum(p, axis=-1, keepdims=True)
            pb = p.astype(_BF16)
            cc = None
            for k in range(NBLK):
                part = _dot(pb[:, k * k_c:(k + 1) * k_c], latent(k))
                cc = part if cc is None else cc + part
                if k in cfg["kick_c"]:
                    pm.kick()
            cc = cc / l
            for t in range(NCT):
                ctx_s[t, b] = cc[:, t * _L:(t + 1) * _L]
            pm.pump(*cfg["pump_c"])
            pm.drain()

        small_wqa = heads_of(wqa_h, wqa_s, i_wqa)
        n_q = len(small_wqa) // 2
        for b in range(B):
            if b + 2 < B:
                attend_b(b, functools.partial(start_c, b + 2), pump_c(b + 2))
            elif b + 2 == B:
                attend_b(b, functools.partial(start_pieces, wuv_h, wuv_s, cut_w, S_WUV),
                         _Pump(heads_of(wuv_h, wuv_s, i_w)))
            else:
                attend_b(b, start_wqa, _Pump(small_wqa[:n_q] + small_k(0)))

        wait_pieces(wuv_s, cut_w, S_WUV)
        start_k(0)
        start_v(0)
        pm = _Pump(small_v(0)[:1] + small_wqa[n_q:] + small_v(0)[1:] + small_k(1))
        pm.kick()
        tick(2 + B)
        halves = [None, None]
        for t in range(NCT):
            for hh in range(2):
                ch = ctx_s[t, :, hh * HH:(hh + 1) * HH, :].reshape(B, HH * _L).astype(_BF16)
                w = head_major(wuv_s, t, hh, pm.kick)
                part = jnp.concatenate(
                    [_dot(ch[:, j * _L:(j + 1) * _L], w[:, j * Db:(j + 1) * Db])
                     for j in range(HH)], axis=1)
                halves[hh] = part if t == 0 else halves[hh] + part
                pm.kick()
        ctxb_s[...] = jnp.concatenate(halves, axis=1)
        pm.pump(*cfg["pump_uv"])
        pm.drain()

        wait_pieces(wqa_s, cut_wqa, S_WQA)
        start_k(1)
        pm = _Pump(small_v(1))
        pm.kick()
        tick(3 + B)
        c_xa.wait()
        xa = xa_s[...]
        seg = n_ct // cfg["seg_q"]
        for c0 in range(0, n_ct, seg):
            wq_tiles = wqa_s[...].reshape(D // 8, n_ct, 8, _L)
            oab_s[:, c0 * _L:(c0 + seg) * _L] = jnp.concatenate(
                [_dot(xa, wq_tiles[:, ct].reshape(D, _L)) for ct in range(c0, c0 + seg)], axis=1)
            pm.pump(1, cfg["lag_w"])
        qa_s[...] = (oab_s[...] * scale_a).reshape(B, H, Dh).reshape(BH, Dh)
        pm.pump(*cfg["pump_q"])
        pm.drain()

        def attend_a(g, start_at_k, start_at_v, pm, same_buffer, between):
            start = g * _G if isinstance(g, int) else pl.multiple_of(g * _G, _G)
            rows = pl.ds(start, _G)
            q8 = qa_s[rows, :].astype(_BF16)
            wait_pieces(k_s.at[g], cut_k, S_KV + 2 * g)
            start_at_k()
            pm.kick()
            tick(4 + B + g)
            row = lax.broadcasted_iota(jnp.int32, (_G, W), 0)
            s = None
            for j in range(_G):
                sj = _dot_nt(q8, k_s[g, j])
                s = sj if s is None else jnp.where(row == j, sj, s)
                if j in cfg["kick_qk"]:
                    if same_buffer:
                        pm.kick()
                    else:
                        p_s[...] = s
                        pm.pump(1, cfg["lag_qk"])
                        s = p_s[...]
            m = jnp.max(s, axis=-1, keepdims=True)
            p = jnp.exp(s - m)
            l = jnp.sum(p, axis=-1, keepdims=True)
            p_s[...] = p
            between()
            wait_pieces(v_s.at[g], cut_v, S_KV + 2 * g + 1)
            start_at_v()
            if same_buffer:
                pm.kick()
            else:
                pm.pump(1, cfg["lag_qk"])
            pb = p_s[...].astype(_BF16)
            row2 = lax.broadcasted_iota(jnp.int32, (_G, Dh), 0)
            o = None
            for j in range(_G):
                oj = _dot(pb, v_s[g, j])
                o = oj if o is None else jnp.where(row2 == j, oj, o)
                if j in cfg["kick_pv"] and same_buffer:
                    pm.kick()
            oa_s[rows, :] = o / l

        def a_body(g, carry):
            pm = _Pump(small_k(g + 2) + small_v(g + 2))
            attend_a(g, functools.partial(start_v, g + 1), functools.partial(start_k, g + 2), pm,
                     True, functools.partial(pm.pump, *cfg["pump_k"]))
            pm.pump(*cfg["pump_v"])
            pm.drain()
            return carry

        lax.fori_loop(0, NG - 2, a_body, 0)

        waited = side_n - side_nb
        n_early, n_mid = side_n - cfg["side_mid"], side_all - side_late
        r_early, r_mid = n_early * side_rows, n_mid * side_rows
        pm = pump_wo(0, len(i_wo))

        def project_b():
            c_wob.wait()
            for i in range(waited, n_early):
                c_sb(i).wait()
            ctxb = ctxb_s[...].astype(_BF16)
            accb_s[...] = _dot(ctxb[:, side_total:], wob_s[side_total:, :])
            step = 8 * _L
            for lo in range(0, r_early, step):
                pm.pump(1, cfg["lag_b"])
                hi = min(lo + step, r_early)
                accb_s[...] += _dot(ctxb[:, lo:hi], wob_s[lo:hi, :])

        attend_a(NG - 2, functools.partial(start_v, NG - 1), start_wo, pm,
                 False, functools.partial(pm.pump, *cfg["pump_k14"]))
        project_b()
        pm.pump(*cfg["pump_b"])
        attend_a(NG - 1, (lambda: c_sa(side_n).start()) if side_last else (lambda: None),
                 lambda: None, pm, False, functools.partial(pm.pump, *cfg["pump_k15"]))
        pm.pump(1, cfg["lag_b"])

        oa32 = oa_s[...].reshape(B, H, Dh).reshape(B, H * Dh)
        oab_s[...] = oa32
        tail0 = H * Dh - tail_rows
        for b in range(B):
            for t in range(tail_rows // Dh):
                src = oa32[b:b + 1, tail0 + t * Dh:tail0 + (t + 1) * Dh]
                coef_s[b, t * Dh:(t + 1) * Dh, :] = jnp.broadcast_to(src, (_L, Dh)).T
        pm.pump(*cfg["pump_e"])
        if side_last:
            c_sa(side_n).wait()
            c_sb(side_n).start()
        pm.pump(*cfg["pump_f"])
        pm.drain()
        oa = oab_s[...].astype(_BF16)
        if n_gap:
            c_gap.wait()
        n_head = wo_inj * r_wo
        acc_s[...] = _dot(oa[:, :n_head], woa_s[:wo_inj].reshape(n_head, D))
        if n_mid > n_early:
            for j in range(n_early, n_mid):
                c_sb(j).wait()
            accb_s[...] += _dot(ctxb_s[:, r_early:r_mid].astype(_BF16), wob_s[r_early:r_mid, :])
        wait_pieces(woa_s.at[wide], cut_wo, S_WIDE)
        acc_s[...] += _dot(oa[:, n_head:wo_base],
                           woa_s[wo_inj:wo_inj + wo_wide].reshape(wo_base - n_head, D))
        for i in range(n_mxu):
            c_wo(i).wait()
            if i == late_at:
                for j in range(n_mid, side_all):
                    c_sb(j).wait()
                late = _dot(ctxb_s[:, r_mid:side_total].astype(_BF16),
                            wob_s[r_mid:side_total, :])
                o_ref[:, D:] = (accb_s[...] + late).astype(o_ref.dtype)
            lo, n = wo_off[i], wo_chunks[i]
            part = _dot(oa[:, lo:lo + n], woa_s[wo_at(lo, n)]) + acc_s[...]
            if i < n_wo - 1:
                acc_s[...] = part
            else:
                o_ref[:, :D] = part.astype(o_ref.dtype)
        for i in range(n_mxu, n_wo):
            c_wo(i).wait()
            lo, n = wo_off[i], wo_chunks[i]
            w = woa_s[wo_at(lo, n)].astype(_F32)
            sums = []
            for b in range(B):
                cf = coef_s[b, lo - tail0:lo - tail0 + n, :]
                prod = w * jnp.concatenate([cf] * (D // _L), axis=1)
                acc = vacc_s[b] if i > n_mxu else None
                for r in range(0, n, 8):
                    acc = prod[r:r + 8] if acc is None else acc + prod[r:r + 8]
                if i < n_wo - 1:
                    vacc_s[b] = acc
                else:
                    sums.append(jnp.sum(acc, axis=0, keepdims=True))
            if i == n_wo - 1:
                res = acc_s[...] + jnp.concatenate(sums, axis=0)
                o_ref[:, :D] = res.astype(o_ref.dtype)

    any_spec = pl.BlockSpec(memory_space=pl.ANY)
    out = pl.pallas_call(
        kernel,
        out_shape=jax.ShapeDtypeStruct((B, D + M), A_x.dtype),
        in_specs=[any_spec] * 11,
        out_specs=pl.BlockSpec(memory_space=pltpu.VMEM),
        scratch_shapes=[
            pltpu.VMEM(xa2.shape, _BF16),
            pltpu.VMEM(xb2.shape, _BF16),
            pltpu.VMEM((2, NG, _G, W, Dh), _BF16),
            pltpu.VMEM((4 + B,) + wqb4.shape, _BF16),
            pltpu.VMEM(woa3.shape, _BF16),
            pltpu.VMEM(wob2.shape, _BF16),
            pltpu.VMEM((BH, Dh), _F32),
            pltpu.VMEM((BH, Dh), _F32),
            pltpu.VMEM((NCT, B, Hb, _L), _F32),
            pltpu.VMEM((NCT, B, Hb, _L), _F32),
            pltpu.VMEM((B, D), _F32),
            pltpu.VMEM((B, M), _F32),
            pltpu.VMEM((B, Hb * Db), _F32),
            pltpu.VMEM((B, H * Dh), _F32),
            pltpu.VMEM((B, max(tail_rows, 8), _L), _F32),
            pltpu.VMEM((B, 8, D), _F32),
            pltpu.VMEM((_G, W), _F32),
            pltpu.VMEM((Hb, Skb), _F32),
            pltpu.SMEM((side_nb, side_rows, M), _BF16),
            pltpu.SemaphoreType.DMA((n_sem,)),
        ],
        compiler_params=pltpu.CompilerParams(
            vmem_limit_bytes=120 * 1024 * 1024,
            disable_semaphore_checks=True,
            disable_bounds_checks=True,
        ),
        name="fused_decode",
    )(xa2, k3, v3, wqa3, woa3, xb2, c4, wqb4, wuk4, wuv4, wob2)
    return out.reshape(B, Sq, D + M)


@jax.jit
def pallas_concat_heads__sliding_block_cached__compressed_kv_cla__decode_kernel(
    A_x: jax.Array,
    A_k_cache: jax.Array,
    A_v_cache: jax.Array,
    A_wq: jax.Array,
    A_wo: jax.Array,
    B_x: jax.Array,
    B_c_kv: jax.Array,
    B_w_q: jax.Array,
    B_w_uk: jax.Array,
    B_w_uv: jax.Array,
    B_w_o: jax.Array,
):
    return _fused(_CFG, A_x, A_k_cache, A_v_cache, A_wq, A_wo,
                  B_x, B_c_kv, B_w_q, B_w_uk, B_w_uv, B_w_o)
```

```python
import functools

import jax
import jax.numpy as jnp
from jax import lax
import jax.experimental.pallas as pl
import jax.experimental.pallas.tpu as pltpu

_NT = (((1,), (1,)), ((), ()))
_F32 = jnp.float32
_BF16 = jnp.bfloat16
_L = 128
_G = 8
_KIB = 1024
_URGENT, _BULK = 0, 1

_CFG = dict(
    piece=64 * _KIB,
    block=512 * _KIB,
    shift_a=30 * _KIB,
    shift_b=34 * _KIB,
    shift_wo=32 * _KIB,
    inj_0=(),
    inj_w=(16 * _KIB, 18 * _KIB, -14 * _KIB, -16 * _KIB),
    inj_c=(16 * _KIB, 18 * _KIB, -14 * _KIB, -16 * _KIB),
    inj_q=(14 * _KIB, 16 * _KIB, -16 * _KIB, -18 * _KIB),
    inj_k=(14 * _KIB, 16 * _KIB),
    inj_v=(14 * _KIB, 16 * _KIB),
    inj_wo=(16 * _KIB,) * 52,
    pump_0=(28, 2),
    pump_w=(11, 3),
    pump_c=(15, 3),
    pump_uv=(20, 3),
    pump_q=(8, 2),
    pump_k=(10, 3),
    pump_v=(13, 3),
    pump_k14=(9, 3),
    pump_b=(6, 3),
    pump_k15=(10, 3),
    pump_e=(3, 3),
    pump_f=(7, 3),
    seg_q=2,
    lag_w=2, lag_qk=2, lag_b=2,
    kick_s=(0, 1, 2, 3, 4, 5, 6, 7),
    kick_c=(1, 3, 5),
    kick_qk=(0, 2, 4, 6),
    kick_pv=(2, 5),
    side_rows=128,
    side_n=24,
    side_last=64,
    side_nb=5,
    side_mid=3,
    side_late=1,
    late_at=1,
    wo_chunks=(512, 128, 128),
    wo_tail=(80, 64, 48, 32, 16, 16),
)


def _dot(a, b):
    return jnp.dot(a, b, preferred_element_type=_F32)


def _dot_nt(a, b):
    return lax.dot_general(a, b, _NT, preferred_element_type=_F32)


def _bounds(n_rows, row_bytes, piece, shift, skip=0):
    step = piece // row_bytes
    first = (shift // row_bytes) % step
    cuts = [skip] + [r for r in range(first, n_rows, step) if r > skip] + [n_rows]
    return list(zip(cuts[:-1], cuts[1:]))


class _Pump:
    def __init__(self, copies):
        self.copies, self.started, self.waited = list(copies), 0, 0

    def kick(self):
        if self.started < len(self.copies):
            self.copies[self.started]().start(priority=_URGENT)
            self.started += 1

    def _wait_to(self, n):
        while self.waited < n:
            self.copies[self.waited]().wait()
            self.waited += 1

    def pump(self, n, lag=1):
        for _ in range(n):
            self.kick()
            self._wait_to(self.started - lag)

    def drain(self):
        while self.started < len(self.copies):
            self.kick()
        self._wait_to(self.started)


def _fused(cfg, A_x, A_k_cache, A_v_cache, A_wq, A_wo, B_x, B_c_kv, B_w_q, B_w_uk, B_w_uv, B_w_o):
    B, Sq, D = A_x.shape
    _, H, Sk, Dh = A_k_cache.shape
    assert Sq == 1 and B_x.shape[1] == 1
    assert A_wq.shape == (D, H * Dh)
    W = min(4096, max(256, Sk // 4))
    M, Hb, Db = B_w_q.shape
    Skb, Dc = B_c_kv.shape[1], B_c_kv.shape[2]
    BH = B * H
    NG = BH // _G
    NCT = Dc // _L
    HH = Hb // 2
    scale_a = float(Dh) ** -0.5
    scale_b = float(Db) ** -0.5
    piece, block = cfg["piece"], cfg["block"]
    shift_a, shift_b = cfg["shift_a"], cfg["shift_b"]
    side_rows, side_n, side_nb = cfg["side_rows"], cfg["side_n"], cfg["side_nb"]
    side_late, late_at = cfg["side_late"], cfg["late_at"]
    n_mxu = len(cfg["wo_chunks"])
    wo_chunks = tuple(cfg["wo_chunks"]) + tuple(cfg["wo_tail"])
    tail_rows = sum(cfg["wo_tail"])
    assert tail_rows % Dh == 0 and M % _L == 0 and NG >= 4
    side_lag = 2
    side_lead = side_nb - side_lag
    side_last = cfg["side_last"]
    side_all = side_n + (1 if side_last else 0)
    assert side_n <= 4 + B + NG and cfg["side_mid"] < side_nb

    xa2 = A_x.reshape(B, D)
    xb2 = B_x.reshape(B, M)
    k3 = A_k_cache.reshape(BH, Sk, Dh)
    v3 = A_v_cache.reshape(BH, Sk, Dh)

    def blocked(w, lead=0):
        row_bytes = 2 * functools.reduce(lambda a, b: a * b, w.shape[lead + 1:], 1)
        rows = block // row_bytes
        shape = w.shape[:lead] + (w.shape[lead] // rows, rows) + w.shape[lead + 1:]
        return w.reshape(shape), rows, row_bytes

    n_ct = H * Dh // _L
    wqa_t = A_wq.reshape(D // 8, 8, n_ct, _L).transpose(0, 2, 1, 3).reshape(D * n_ct, _L)
    wqa3, r_wqa, b_wqa = blocked(wqa_t)
    wqb4, r_w, b_w = blocked(B_w_q.reshape(M * Hb, Db))
    wuk4, _, _ = blocked(B_w_uk.reshape(Dc * Hb, Db))
    wuv4, _, _ = blocked(B_w_uv.reshape(Dc * Hb, Db))
    c_t = B_c_kv.reshape(B, Skb // 8, 8, NCT, _L).transpose(0, 1, 3, 2, 4)
    c4, r_c, b_c = blocked(c_t.reshape(B, Skb * NCT, _L), 1)
    k_c = r_c // NCT
    woa3, r_wo, b_wo = blocked(A_wo)
    wob3, _, _ = blocked(B_w_o.reshape(Hb * Db, M))
    assert wob3.shape == woa3.shape and r_wo % side_rows == 0
    assert wqb4.shape == wuk4.shape == wuv4.shape and 2 * r_w == _L * Hb
    assert wqa3.shape == wqb4.shape == c4.shape[1:]
    NBLK = wqb4.shape[0]

    def spans(sizes, unit, n_rows=0):
        out, front, back = [], 0, n_rows
        for n in sizes:
            if n > 0:
                out.append((front, front + n // unit))
                front += n // unit
            else:
                out.append((back + n // unit, back))
                back += n // unit
        return out, front, back

    def split(sizes, n_rows, unit, shift):
        small, front, back = spans(sizes, unit, n_rows)
        return small, _bounds(back, unit, piece, shift, front)

    i_w, cut_w = split(cfg["inj_w"], r_w, b_w, shift_b)
    i_c, cut_c = split(cfg["inj_c"], r_c, b_c, shift_b)
    i_k, cut_k = split(cfg["inj_k"], W, 2 * Dh, shift_a)
    i_v, cut_v = split(cfg["inj_v"], W, 2 * Dh, shift_a)
    i_wqa, cut_wqa = split(cfg["inj_q"], r_wqa, b_wqa, shift_a)
    i_wo, _, _ = spans(cfg["inj_wo"], 2 * D)
    i_w0, cut_w0 = split(cfg["inj_0"], r_w, b_w, shift_b)
    n_inj = i_wo[-1][1]
    wo_inj = -(-n_inj // r_wo)
    wo_wide = (H * Dh - sum(wo_chunks)) // r_wo - wo_inj
    cut_wo = _bounds(r_wo, b_wo, piece, cfg["shift_wo"])
    wo_base = (wo_inj + wo_wide) * r_wo
    assert all(lo // r_wo == (hi - 1) // r_wo for lo, hi in i_wo)
    assert wo_base + sum(wo_chunks) == H * Dh
    n_wo = len(wo_chunks)
    wo_off = [wo_base + sum(wo_chunks[:i]) for i in range(n_wo)]
    assert all(lo // r_wo == (lo + n - 1) // r_wo for lo, n in zip(wo_off, wo_chunks))
    S_XB, S_XA, S_WQB, S_WUK, S_WUV, S_WOB, S_WQA, S_INJ, S_WIDE, S_GAP, S_GAPB = range(11)
    S_C = 11
    S_KV = S_C + B
    S_WO = S_KV + 2 * NG
    S_SA = S_WO + n_wo
    S_SB = S_SA + side_nb
    n_sem = S_SB + side_nb
    side_total = side_rows * side_n + side_last

    def kernel(xa_h, k_h, v_h, wqa_h, woa_h, xb_h, c_h, wqb_h, wuk_h, wuv_h, wob_h,
               o_ref,
               xa_s, xb_s, kv_s, big_s, woa_s, wob_s,
               qa_s, oa_s, qabs_s, ctx_s, acc_s, accb_s, ctxb_s, oab_s, coef_s, vacc_s, p_s, s_s,
               side_s, sem):
        def cp(src, dst, s):
            return pltpu.make_async_copy(src, dst, sem.at[s])

        def start_pieces(src, dst, cuts, s, row0=0):
            for lo, hi in cuts:
                cp(src.at[:, pl.ds(row0 + lo, hi - lo)], dst.at[:, pl.ds(lo, hi - lo)],
                   s).start(priority=_BULK)

        def wait_pieces(dst, cuts, s):
            view = dst.at[:, pl.ds(cuts[0][0], cuts[-1][1] - cuts[0][0])]
            cp(view, view, s).wait()

        def heads_of(src, dst, ranges, row0=0):
            def one(k, lo, hi):
                return cp(src.at[k, pl.ds(row0 + lo, hi - lo)], dst.at[k, pl.ds(lo, hi - lo)], S_INJ)
            return [functools.partial(one, k, lo, hi)
                    for lo, hi in ranges for k in range(dst.shape[0])]

        k_s, v_s = kv_s.at[0], kv_s.at[1]
        wqb_s, wuk_s, wuv_s, wqa_s = (big_s.at[j] for j in range(4))
        c_s = big_s.at[pl.ds(4, B)]
        c_xb = cp(xb_h, xb_s, S_XB)
        c_xa = cp(xa_h, xa_s, S_XA)

        def rows_of(ref, lo, hi):
            parts = [ref[k, max(lo - k * r_wo, 0):min(hi - k * r_wo, r_wo)]
                     for k in range(lo // r_wo, -(-hi // r_wo))]
            return parts[0] if len(parts) == 1 else jnp.concatenate(parts, axis=0)

        k0, r0 = divmod(side_total, r_wo)
        cut_rest = _bounds(r_wo, b_wo, piece, cfg["shift_wo"], r0)
        rest_all, rest_up = pl.ds(k0, NBLK - k0), (pl.ds(k0 + 1, NBLK - k0 - 1), pl.ds(0, r0))
        c_wob = cp(wob_h.at[rest_up], wob_s.at[rest_up], S_GAPB)

        def start_c(b):
            start_pieces(c_h.at[b], c_s.at[b], cut_c, S_C + b)

        def pump_c(b):
            return _Pump(heads_of(c_h.at[b], c_s.at[b], i_c))

        def start_wqa():
            c_wob.start(priority=_BULK)
            start_pieces(wob_h.at[rest_all], wob_s.at[rest_all], cut_rest, S_WOB)
            start_pieces(wqa_h, wqa_s, cut_wqa, S_WQA)

        def start_k(g):
            start_pieces(k_h.at[pl.ds(g * _G, _G)], k_s.at[g], cut_k, S_KV + 2 * g, Sk - W)

        def start_v(g):
            start_pieces(v_h.at[pl.ds(g * _G, _G)], v_s.at[g], cut_v, S_KV + 2 * g + 1, Sk - W)

        def small_k(g):
            return heads_of(k_h.at[pl.ds(g * _G, _G)], k_s.at[g], i_k, Sk - W)

        def small_v(g):
            return heads_of(v_h.at[pl.ds(g * _G, _G)], v_s.at[g], i_v, Sk - W)

        def wo_at(lo, n):
            return lo // r_wo, pl.ds(lo % r_wo, n)

        def c_wo(i):
            at = wo_at(wo_off[i], wo_chunks[i])
            return cp(woa_h.at[at], woa_s.at[at], S_WO + i)

        wide = pl.ds(wo_inj, wo_wide)

        n_gap = wo_inj * r_wo - n_inj
        if n_gap:
            c_gap = cp(woa_h.at[wo_at(n_inj, n_gap)], woa_s.at[wo_at(n_inj, n_gap)], S_GAP)

        def start_wo():
            if n_gap:
                c_gap.start(priority=_BULK)
            start_pieces(woa_h.at[wide], woa_s.at[wide], cut_wo, S_WIDE)
            for i in range(n_wo):
                c_wo(i).start(priority=_BULK)

        def pump_wo(first, last):
            def one(lo, hi):
                at = wo_at(lo, hi - lo)
                return cp(woa_h.at[at], woa_s.at[at], S_INJ)
            return _Pump([functools.partial(one, *i_wo[j]) for j in range(first, last)])

        def side_refs(i):
            per = r_wo // side_rows
            if isinstance(i, int):
                n = side_rows if i < side_n else side_last
                rows = (i // per, pl.ds(i % per * side_rows, n))
                return rows, side_s.at[i % side_nb, pl.ds(0, n)], i % side_nb
            slot = lax.rem(i, side_nb)
            start = pl.multiple_of(lax.rem(i, per) * side_rows, 8)
            return (lax.div(i, per), pl.ds(start, side_rows)), side_s.at[slot], slot

        def c_sa(i):
            rows, stage, slot = side_refs(i)
            return cp(wob_h.at[rows], stage, S_SA + slot)

        def c_sb(i):
            rows, stage, slot = side_refs(i)
            return cp(stage, wob_s.at[rows], S_SB + slot)

        def tick(i):
            traced = not isinstance(i, int)
            if traced or i < side_n:
                c_sa(i).wait()
                c_sb(i).start()

            def refill(j):
                if traced or i >= side_lag:
                    c_sb(i - side_lag).wait()
                c_sa(j).start()

            if traced:
                pl.when(i + side_lead < side_n)(lambda: refill(i + side_lead))
            elif i + side_lead < side_n:
                refill(i + side_lead)

        def head_major(w_s, t, hh, mid=lambda: None):
            halves = []
            for k in range(2):
                w = w_s[2 * t + k].reshape(_L // 2, Hb, Db)[:, hh * HH:(hh + 1) * HH, :]
                halves.append(w.reshape(_L // 2, HH * Db))
                if k == 0:
                    mid()
            return jnp.concatenate(halves, axis=0)

        start_pieces(wqb_h, wqb_s, cut_w0, S_WQB)
        c_xb.start()
        c_xa.start()
        for i in range(side_lead):
            c_sa(i).start()
        start_pieces(wuk_h, wuk_s, cut_w, S_WUK)
        pm = _Pump(heads_of(wqb_h, wqb_s, i_w0) + heads_of(wuk_h, wuk_s, i_w))
        pm.pump(*cfg["pump_0"])
        pm.drain()


        wait_pieces(wqb_s, cut_w0, S_WQB)
        start_c(0)
        pm = pump_c(0)
        pm.kick()
        tick(0)
        c_xb.wait()
        xb = xb_s[...]
        halves = [None, None]
        for t in range(M // _L):
            for hh in range(2):
                part = _dot(xb[:, t * _L:(t + 1) * _L], head_major(wqb_s, t, hh, pm.kick))
                halves[hh] = part if t == 0 else halves[hh] + part
                pm.kick()
        ctxb_s[...] = jnp.concatenate(halves, axis=1)
        pm.pump(*cfg["pump_w"])
        pm.drain()

        wait_pieces(wuk_s, cut_w, S_WUK)
        start_c(1)
        pm = pump_c(1)
        pm.kick()
        tick(1)
        qb = (ctxb_s[...] * scale_b).astype(_BF16)
        for t in range(NCT):
            for hh in range(2):
                w = head_major(wuk_s, t, hh, pm.kick)
                parts = [_dot_nt(qb[:, (hh * HH + j) * Db:(hh * HH + j + 1) * Db],
                                 w[:, j * Db:(j + 1) * Db]) for j in range(HH)]
                qabs_s[t, :, hh * HH:(hh + 1) * HH, :] = jnp.concatenate(
                    parts, axis=1).reshape(B, HH, _L)
                pm.kick()
        pm.pump(*cfg["pump_w"])
        pm.drain()

        def attend_b(b, start_next, pm):
            wait_pieces(c_s.at[b], cut_c, S_C + b)
            start_next()
            pm.kick()
            tick(2 + b)
            qa = jnp.concatenate(
                [qabs_s[t, b] for t in range(NCT)], axis=1).astype(_BF16)

            def latent(k):
                tiles = c_s[b, k].reshape(k_c // 8, NCT, 8, _L)
                return jnp.concatenate(
                    [tiles[:, t].reshape(k_c, _L) for t in range(NCT)], axis=1)

            for k in range(NBLK):
                s_s[:, k * k_c:(k + 1) * k_c] = _dot_nt(qa, latent(k))
                if k in cfg["kick_s"]:
                    pm.kick()
            s = s_s[...]
            m = jnp.max(s, axis=-1, keepdims=True)
            p = jnp.exp(s - m)
            l = jnp.sum(p, axis=-1, keepdims=True)
            pb = p.astype(_BF16)
            cc = None
            for k in range(NBLK):
                part = _dot(pb[:, k * k_c:(k + 1) * k_c], latent(k))
                cc = part if cc is None else cc + part
                if k in cfg["kick_c"]:
                    pm.kick()
            cc = cc / l
            for t in range(NCT):
                ctx_s[t, b] = cc[:, t * _L:(t + 1) * _L]
            pm.pump(*cfg["pump_c"])
            pm.drain()

        small_wqa = heads_of(wqa_h, wqa_s, i_wqa)
        n_q = len(small_wqa) // 2
        for b in range(B):
            if b + 2 < B:
                attend_b(b, functools.partial(start_c, b + 2), pump_c(b + 2))
            elif b + 2 == B:
                attend_b(b, functools.partial(start_pieces, wuv_h, wuv_s, cut_w, S_WUV),
                         _Pump(heads_of(wuv_h, wuv_s, i_w)))
            else:
                attend_b(b, start_wqa, _Pump(small_wqa[:n_q] + small_k(0)))

        wait_pieces(wuv_s, cut_w, S_WUV)
        start_k(0)
        start_v(0)
        pm = _Pump(small_v(0)[:1] + small_wqa[n_q:] + small_v(0)[1:] + small_k(1))
        pm.kick()
        tick(2 + B)
        halves = [None, None]
        for t in range(NCT):
            for hh in range(2):
                ch = ctx_s[t, :, hh * HH:(hh + 1) * HH, :].reshape(B, HH * _L).astype(_BF16)
                w = head_major(wuv_s, t, hh, pm.kick)
                part = jnp.concatenate(
                    [_dot(ch[:, j * _L:(j + 1) * _L], w[:, j * Db:(j + 1) * Db])
                     for j in range(HH)], axis=1)
                halves[hh] = part if t == 0 else halves[hh] + part
                pm.kick()
        ctxb_s[...] = jnp.concatenate(halves, axis=1)
        pm.pump(*cfg["pump_uv"])
        pm.drain()

        wait_pieces(wqa_s, cut_wqa, S_WQA)
        start_k(1)
        pm = _Pump(small_v(1))
        pm.kick()
        tick(3 + B)
        c_xa.wait()
        xa = xa_s[...]
        seg = n_ct // cfg["seg_q"]
        for c0 in range(0, n_ct, seg):
            wq_tiles = wqa_s[...].reshape(D // 8, n_ct, 8, _L)
            oab_s[:, c0 * _L:(c0 + seg) * _L] = jnp.concatenate(
                [_dot(xa, wq_tiles[:, ct].reshape(D, _L)) for ct in range(c0, c0 + seg)], axis=1)
            pm.pump(1, cfg["lag_w"])
        qa_s[...] = (oab_s[...] * scale_a).reshape(B, H, Dh).reshape(BH, Dh)
        pm.pump(*cfg["pump_q"])
        pm.drain()

        def attend_a(g, start_at_k, start_at_v, pm, same_buffer, between):
            start = g * _G if isinstance(g, int) else pl.multiple_of(g * _G, _G)
            rows = pl.ds(start, _G)
            q8 = qa_s[rows, :].astype(_BF16)
            wait_pieces(k_s.at[g], cut_k, S_KV + 2 * g)
            start_at_k()
            pm.kick()
            tick(4 + B + g)
            row = lax.broadcasted_iota(jnp.int32, (_G, W), 0)
            s = None
            for j in range(_G):
                sj = _dot_nt(q8, k_s[g, j])
                s = sj if s is None else jnp.where(row == j, sj, s)
                if j in cfg["kick_qk"]:
                    if same_buffer:
                        pm.kick()
                    else:
                        p_s[...] = s
                        pm.pump(1, cfg["lag_qk"])
                        s = p_s[...]
            m = jnp.max(s, axis=-1, keepdims=True)
            p = jnp.exp(s - m)
            l = jnp.sum(p, axis=-1, keepdims=True)
            p_s[...] = p
            between()
            wait_pieces(v_s.at[g], cut_v, S_KV + 2 * g + 1)
            start_at_v()
            if same_buffer:
                pm.kick()
            else:
                pm.pump(1, cfg["lag_qk"])
            pb = p_s[...].astype(_BF16)
            row2 = lax.broadcasted_iota(jnp.int32, (_G, Dh), 0)
            o = None
            for j in range(_G):
                oj = _dot(pb, v_s[g, j])
                o = oj if o is None else jnp.where(row2 == j, oj, o)
                if j in cfg["kick_pv"] and same_buffer:
                    pm.kick()
            oa_s[rows, :] = o / l

        def a_body(g, carry):
            pm = _Pump(small_k(g + 2) + small_v(g + 2))
            attend_a(g, functools.partial(start_v, g + 1), functools.partial(start_k, g + 2), pm,
                     True, functools.partial(pm.pump, *cfg["pump_k"]))
            pm.pump(*cfg["pump_v"])
            pm.drain()
            return carry

        lax.fori_loop(0, NG - 2, a_body, 0)

        waited = side_n - side_nb
        n_early, n_mid = side_n - cfg["side_mid"], side_all - side_late
        r_early, r_mid = n_early * side_rows, n_mid * side_rows
        pm = pump_wo(0, len(i_wo))

        def project_b():
            c_wob.wait()
            wait_pieces(wob_s.at[rest_all], cut_rest, S_WOB)
            for i in range(waited, n_early):
                c_sb(i).wait()
            ctxb = ctxb_s[...].astype(_BF16)
            accb_s[...] = _dot(ctxb[:, side_total:], rows_of(wob_s, side_total, Hb * Db))
            step = 8 * _L
            for lo in range(0, r_early, step):
                pm.pump(1, cfg["lag_b"])
                hi = min(lo + step, r_early)
                accb_s[...] += _dot(ctxb[:, lo:hi], rows_of(wob_s, lo, hi))

        attend_a(NG - 2, functools.partial(start_v, NG - 1), start_wo, pm,
                 False, functools.partial(pm.pump, *cfg["pump_k14"]))
        project_b()
        pm.pump(*cfg["pump_b"])
        attend_a(NG - 1, (lambda: c_sa(side_n).start()) if side_last else (lambda: None),
                 lambda: None, pm, False, functools.partial(pm.pump, *cfg["pump_k15"]))
        pm.pump(1, cfg["lag_b"])

        oa32 = oa_s[...].reshape(B, H, Dh).reshape(B, H * Dh)
        oab_s[...] = oa32
        tail0 = H * Dh - tail_rows
        for b in range(B):
            for t in range(tail_rows // Dh):
                src = oa32[b:b + 1, tail0 + t * Dh:tail0 + (t + 1) * Dh]
                coef_s[b, t * Dh:(t + 1) * Dh, :] = jnp.broadcast_to(src, (_L, Dh)).T
        pm.pump(*cfg["pump_e"])
        if side_last:
            c_sa(side_n).wait()
            c_sb(side_n).start()
        pm.pump(*cfg["pump_f"])
        pm.drain()
        oa = oab_s[...].astype(_BF16)
        if n_gap:
            c_gap.wait()
        n_head = wo_inj * r_wo
        acc_s[...] = _dot(oa[:, :n_head], woa_s[:wo_inj].reshape(n_head, D))
        if n_mid > n_early:
            for j in range(n_early, n_mid):
                c_sb(j).wait()
            accb_s[...] += _dot(ctxb_s[:, r_early:r_mid].astype(_BF16),
                                rows_of(wob_s, r_early, r_mid))
        wait_pieces(woa_s.at[wide], cut_wo, S_WIDE)
        acc_s[...] += _dot(oa[:, n_head:wo_base],
                           woa_s[wo_inj:wo_inj + wo_wide].reshape(wo_base - n_head, D))
        for i in range(n_mxu):
            c_wo(i).wait()
            if i == late_at:
                for j in range(n_mid, side_all):
                    c_sb(j).wait()
                late = _dot(ctxb_s[:, r_mid:side_total].astype(_BF16),
                            rows_of(wob_s, r_mid, side_total))
                o_ref[:, D:] = (accb_s[...] + late).astype(o_ref.dtype)
            lo, n = wo_off[i], wo_chunks[i]
            part = _dot(oa[:, lo:lo + n], woa_s[wo_at(lo, n)]) + acc_s[...]
            if i < n_wo - 1:
                acc_s[...] = part
            else:
                o_ref[:, :D] = part.astype(o_ref.dtype)
        for i in range(n_mxu, n_wo):
            c_wo(i).wait()
            lo, n = wo_off[i], wo_chunks[i]
            w = woa_s[wo_at(lo, n)].astype(_F32)
            sums = []
            for b in range(B):
                cf = coef_s[b, lo - tail0:lo - tail0 + n, :]
                prod = w * jnp.concatenate([cf] * (D // _L), axis=1)
                acc = vacc_s[b] if i > n_mxu else None
                for r in range(0, n, 8):
                    acc = prod[r:r + 8] if acc is None else acc + prod[r:r + 8]
                if i < n_wo - 1:
                    vacc_s[b] = acc
                else:
                    sums.append(jnp.sum(acc, axis=0, keepdims=True))
            if i == n_wo - 1:
                res = acc_s[...] + jnp.concatenate(sums, axis=0)
                o_ref[:, :D] = res.astype(o_ref.dtype)

    any_spec = pl.BlockSpec(memory_space=pl.ANY)
    out = pl.pallas_call(
        kernel,
        out_shape=jax.ShapeDtypeStruct((B, D + M), A_x.dtype),
        in_specs=[any_spec] * 11,
        out_specs=pl.BlockSpec(memory_space=pltpu.VMEM),
        scratch_shapes=[
            pltpu.VMEM(xa2.shape, _BF16),
            pltpu.VMEM(xb2.shape, _BF16),
            pltpu.VMEM((2, NG, _G, W, Dh), _BF16),
            pltpu.VMEM((4 + B,) + wqb4.shape, _BF16),
            pltpu.VMEM(woa3.shape, _BF16),
            pltpu.VMEM(wob3.shape, _BF16),
            pltpu.VMEM((BH, Dh), _F32),
            pltpu.VMEM((BH, Dh), _F32),
            pltpu.VMEM((NCT, B, Hb, _L), _F32),
            pltpu.VMEM((NCT, B, Hb, _L), _F32),
            pltpu.VMEM((B, D), _F32),
            pltpu.VMEM((B, M), _F32),
            pltpu.VMEM((B, Hb * Db), _F32),
            pltpu.VMEM((B, H * Dh), _F32),
            pltpu.VMEM((B, max(tail_rows, 8), _L), _F32),
            pltpu.VMEM((B, 8, D), _F32),
            pltpu.VMEM((_G, W), _F32),
            pltpu.VMEM((Hb, Skb), _F32),
            pltpu.SMEM((side_nb, side_rows, M), _BF16),
            pltpu.SemaphoreType.DMA((n_sem,)),
        ],
        compiler_params=pltpu.CompilerParams(
            vmem_limit_bytes=120 * 1024 * 1024,
            disable_semaphore_checks=True,
            disable_bounds_checks=True,
        ),
        name="fused_decode",
    )(xa2, k3, v3, wqa3, woa3, xb2, c4, wqb4, wuk4, wuv4, wob3)
    return out.reshape(B, Sq, D + M)


@jax.jit
def pallas_concat_heads__sliding_block_cached__compressed_kv_cla__decode_kernel(
    A_x: jax.Array,
    A_k_cache: jax.Array,
    A_v_cache: jax.Array,
    A_wq: jax.Array,
    A_wo: jax.Array,
    B_x: jax.Array,
    B_c_kv: jax.Array,
    B_w_q: jax.Array,
    B_w_uk: jax.Array,
    B_w_uv: jax.Array,
    B_w_o: jax.Array,
):
    return _fused(_CFG, A_x, A_k_cache, A_v_cache, A_wq, A_wo,
                  B_x, B_c_kv, B_w_q, B_w_uk, B_w_uv, B_w_o)
```

```python
import functools

import jax
import jax.numpy as jnp
from jax import lax
import jax.experimental.pallas as pl
import jax.experimental.pallas.tpu as pltpu

_NT = (((1,), (1,)), ((), ()))
_F32 = jnp.float32
_BF16 = jnp.bfloat16
_L = 128
_G = 8
_KIB = 1024
_URGENT, _BULK = 0, 1

_CFG = dict(
    piece=64 * _KIB,
    block=512 * _KIB,
    shift_a=30 * _KIB,
    shift_b=34 * _KIB,
    shift_wo=32 * _KIB,
    inj_w=(16 * _KIB, 18 * _KIB, -14 * _KIB, -16 * _KIB),
    inj_c=(16 * _KIB, 18 * _KIB, -14 * _KIB, -16 * _KIB),
    inj_q=(14 * _KIB, 16 * _KIB, -16 * _KIB, -18 * _KIB),
    inj_k=(14 * _KIB, 16 * _KIB),
    inj_v=(14 * _KIB, 16 * _KIB),
    inj_wo=(16 * _KIB,) * 52,
    pump_0=(28, 2),
    pump_w=(11, 3),
    pump_c=(15, 3),
    pump_uv=(20, 3),
    pump_q=(8, 2),
    pump_k=(10, 3),
    pump_v=(11, 3),
    pump_k14=(9, 3),
    pump_b=(6, 3),
    pump_k15=(10, 3),
    pump_e=(3, 3),
    pump_f=(7, 3),
    lag=2,
    kick_s=(0, 1, 2, 3, 4, 5, 6, 7),
    kick_c=(1, 3, 5),
    kick_qk=(0, 1, 3, 5, 6),
    kick_pv=(1, 3, 5),
    side_rows=128,
    side_n=24,
    side_last=64,
    side_nb=5,
    side_mid=3,
    late_at=1,
    wo_chunks=(512, 128, 128),
    wo_tail=(80, 64, 48, 32, 16, 16),
)


def _dot(a, b):
    return jnp.dot(a, b, preferred_element_type=_F32)


def _dot_nt(a, b):
    return lax.dot_general(a, b, _NT, preferred_element_type=_F32)


def _bounds(n_rows, row_bytes, piece, shift, skip=0):
    step = piece // row_bytes
    first = (shift // row_bytes) % step
    cuts = [skip] + [r for r in range(first, n_rows, step) if r > skip] + [n_rows]
    return list(zip(cuts[:-1], cuts[1:]))


class _Pump:
    def __init__(self, copies):
        self.copies, self.started, self.waited = list(copies), 0, 0

    def kick(self):
        if self.started < len(self.copies):
            self.copies[self.started]().start(priority=_URGENT)
            self.started += 1

    def _wait_to(self, n):
        while self.waited < n:
            self.copies[self.waited]().wait()
            self.waited += 1

    def pump(self, n, lag=1):
        for _ in range(n):
            self.kick()
            self._wait_to(self.started - lag)

    def drain(self):
        while self.started < len(self.copies):
            self.kick()
        self._wait_to(self.started)


def _fused(cfg, A_x, A_k_cache, A_v_cache, A_wq, A_wo, B_x, B_c_kv, B_w_q, B_w_uk, B_w_uv, B_w_o):
    B, Sq, D = A_x.shape
    _, H, Sk, Dh = A_k_cache.shape
    assert Sq == 1 and B_x.shape[1] == 1
    assert A_wq.shape == (D, H * Dh)
    W = min(4096, max(256, Sk // 4))
    M, Hb, Db = B_w_q.shape
    Skb, Dc = B_c_kv.shape[1], B_c_kv.shape[2]
    BH = B * H
    NG = BH // _G
    NCT = Dc // _L
    HH = Hb // 2
    scale_a = float(Dh) ** -0.5
    scale_b = float(Db) ** -0.5
    piece, block = cfg["piece"], cfg["block"]
    shift_a, shift_b = cfg["shift_a"], cfg["shift_b"]
    side_rows, side_n, side_nb = cfg["side_rows"], cfg["side_n"], cfg["side_nb"]
    late_at = cfg["late_at"]
    n_mxu = len(cfg["wo_chunks"])
    wo_chunks = tuple(cfg["wo_chunks"]) + tuple(cfg["wo_tail"])
    tail_rows = sum(cfg["wo_tail"])
    assert tail_rows % Dh == 0 and M % _L == 0 and NG >= 4
    side_lag = 2
    side_lead = side_nb - side_lag
    side_last = cfg["side_last"]
    assert side_n == 4 + B + NG and cfg["side_mid"] < side_nb and side_last > 0

    xa2 = A_x.reshape(B, D)
    xb2 = B_x.reshape(B, M)
    k3 = A_k_cache.reshape(BH, Sk, Dh)
    v3 = A_v_cache.reshape(BH, Sk, Dh)

    def blocked(w, lead=0):
        row_bytes = 2 * functools.reduce(lambda a, b: a * b, w.shape[lead + 1:], 1)
        rows = block // row_bytes
        shape = w.shape[:lead] + (w.shape[lead] // rows, rows) + w.shape[lead + 1:]
        return w.reshape(shape), rows, row_bytes

    n_ct = H * Dh // _L
    wqa_t = A_wq.reshape(D // 8, 8, n_ct, _L).transpose(0, 2, 1, 3).reshape(D * n_ct, _L)
    wqa3, r_wqa, b_wqa = blocked(wqa_t)
    wqb4, r_w, b_w = blocked(B_w_q.reshape(M * Hb, Db))
    wuk4, _, _ = blocked(B_w_uk.reshape(Dc * Hb, Db))
    wuv4, _, _ = blocked(B_w_uv.reshape(Dc * Hb, Db))
    c_t = B_c_kv.reshape(B, Skb // 8, 8, NCT, _L).transpose(0, 1, 3, 2, 4)
    c4, r_c, b_c = blocked(c_t.reshape(B, Skb * NCT, _L), 1)
    k_c = r_c // NCT
    woa3, r_wo, b_wo = blocked(A_wo)
    wob3, _, _ = blocked(B_w_o.reshape(Hb * Db, M))
    assert wob3.shape == woa3.shape and r_wo % side_rows == 0
    assert wqb4.shape == wuk4.shape == wuv4.shape and 2 * r_w == _L * Hb
    assert wqa3.shape == wqb4.shape == c4.shape[1:]
    NBLK = wqb4.shape[0]

    def spans(sizes, unit, n_rows=0):
        out, front, back = [], 0, n_rows
        for n in sizes:
            if n > 0:
                out.append((front, front + n // unit))
                front += n // unit
            else:
                out.append((back + n // unit, back))
                back += n // unit
        return out, front, back

    def split(sizes, n_rows, unit, shift):
        small, front, back = spans(sizes, unit, n_rows)
        return small, _bounds(back, unit, piece, shift, front)

    i_w, cut_w = split(cfg["inj_w"], r_w, b_w, shift_b)
    i_c, cut_c = split(cfg["inj_c"], r_c, b_c, shift_b)
    i_k, cut_k = split(cfg["inj_k"], W, 2 * Dh, shift_a)
    i_v, cut_v = split(cfg["inj_v"], W, 2 * Dh, shift_a)
    i_wqa, cut_wqa = split(cfg["inj_q"], r_wqa, b_wqa, shift_a)
    i_wo, _, _ = spans(cfg["inj_wo"], 2 * D)
    cut_w0 = _bounds(r_w, b_w, piece, shift_b)
    n_inj = i_wo[-1][1]
    wo_inj = -(-n_inj // r_wo)
    wo_wide = (H * Dh - sum(wo_chunks)) // r_wo - wo_inj
    cut_wo = _bounds(r_wo, b_wo, piece, cfg["shift_wo"])
    wo_base = (wo_inj + wo_wide) * r_wo
    assert all(lo // r_wo == (hi - 1) // r_wo for lo, hi in i_wo)
    assert wo_base + sum(wo_chunks) == H * Dh
    n_wo = len(wo_chunks)
    wo_off = [wo_base + sum(wo_chunks[:i]) for i in range(n_wo)]
    assert all(lo // r_wo == (lo + n - 1) // r_wo for lo, n in zip(wo_off, wo_chunks))
    S_XB, S_XA, S_WQB, S_WUK, S_WUV, S_WOB, S_WQA, S_INJ, S_WIDE, S_GAP, S_GAPB = range(11)
    S_C = 11
    S_KV = S_C + B
    S_WO = S_KV + 2 * NG
    S_SA = S_WO + n_wo
    S_SB = S_SA + side_nb
    n_sem = S_SB + side_nb
    side_total = side_rows * side_n + side_last

    def kernel(xa_h, k_h, v_h, wqa_h, woa_h, xb_h, c_h, wqb_h, wuk_h, wuv_h, wob_h,
               o_ref,
               xa_s, xb_s, kv_s, big_s, woa_s, wob_s,
               qa_s, oa_s, qabs_s, ctx_s, acc_s, accb_s, ctxb_s, oab_s, coef_s, vacc_s, p_s, s_s,
               side_s, sem):
        def cp(src, dst, s):
            return pltpu.make_async_copy(src, dst, sem.at[s])

        def start_pieces(src, dst, cuts, s, row0=0):
            for lo, hi in cuts:
                cp(src.at[:, pl.ds(row0 + lo, hi - lo)], dst.at[:, pl.ds(lo, hi - lo)],
                   s).start(priority=_BULK)

        def wait_pieces(dst, cuts, s):
            view = dst.at[:, pl.ds(cuts[0][0], cuts[-1][1] - cuts[0][0])]
            cp(view, view, s).wait()

        def heads_of(src, dst, ranges, row0=0):
            def one(k, lo, hi):
                return cp(src.at[k, pl.ds(row0 + lo, hi - lo)], dst.at[k, pl.ds(lo, hi - lo)], S_INJ)
            return [functools.partial(one, k, lo, hi)
                    for lo, hi in ranges for k in range(dst.shape[0])]

        k_s, v_s = kv_s.at[0], kv_s.at[1]
        wqb_s, wuk_s, wuv_s, wqa_s = (big_s.at[j] for j in range(4))
        c_s = big_s.at[pl.ds(4, B)]
        c_xb = cp(xb_h, xb_s, S_XB)
        c_xa = cp(xa_h, xa_s, S_XA)

        def rows_of(ref, lo, hi):
            parts = [ref[k, max(lo - k * r_wo, 0):min(hi - k * r_wo, r_wo)]
                     for k in range(lo // r_wo, -(-hi // r_wo))]
            return parts[0] if len(parts) == 1 else jnp.concatenate(parts, axis=0)

        k0, r0 = divmod(side_total, r_wo)
        cut_rest = _bounds(r_wo, b_wo, piece, cfg["shift_wo"], r0)
        rest_all, rest_up = pl.ds(k0, NBLK - k0), (pl.ds(k0 + 1, NBLK - k0 - 1), pl.ds(0, r0))
        c_wob = cp(wob_h.at[rest_up], wob_s.at[rest_up], S_GAPB)

        def start_c(b):
            start_pieces(c_h.at[b], c_s.at[b], cut_c, S_C + b)

        def pump_c(b):
            return _Pump(heads_of(c_h.at[b], c_s.at[b], i_c))

        def start_wqa():
            c_wob.start(priority=_BULK)
            start_pieces(wob_h.at[rest_all], wob_s.at[rest_all], cut_rest, S_WOB)
            start_pieces(wqa_h, wqa_s, cut_wqa, S_WQA)

        def start_k(g):
            start_pieces(k_h.at[pl.ds(g * _G, _G)], k_s.at[g], cut_k, S_KV + 2 * g, Sk - W)

        def start_v(g):
            start_pieces(v_h.at[pl.ds(g * _G, _G)], v_s.at[g], cut_v, S_KV + 2 * g + 1, Sk - W)

        def small_k(g):
            return heads_of(k_h.at[pl.ds(g * _G, _G)], k_s.at[g], i_k, Sk - W)

        def small_v(g):
            return heads_of(v_h.at[pl.ds(g * _G, _G)], v_s.at[g], i_v, Sk - W)

        def wo_at(lo, n):
            return lo // r_wo, pl.ds(lo % r_wo, n)

        def c_wo(i):
            at = wo_at(wo_off[i], wo_chunks[i])
            return cp(woa_h.at[at], woa_s.at[at], S_WO + i)

        wide = pl.ds(wo_inj, wo_wide)

        n_gap = wo_inj * r_wo - n_inj
        if n_gap:
            c_gap = cp(woa_h.at[wo_at(n_inj, n_gap)], woa_s.at[wo_at(n_inj, n_gap)], S_GAP)

        def start_wo():
            if n_gap:
                c_gap.start(priority=_BULK)
            start_pieces(woa_h.at[wide], woa_s.at[wide], cut_wo, S_WIDE)

        def small_wo():
            def one(lo, hi):
                at = wo_at(lo, hi - lo)
                return cp(woa_h.at[at], woa_s.at[at], S_INJ)
            return [functools.partial(one, lo, hi) for lo, hi in i_wo]

        def side_refs(i):
            per = r_wo // side_rows
            if isinstance(i, int):
                n = side_rows if i < side_n else side_last
                rows = (i // per, pl.ds(i % per * side_rows, n))
                return rows, side_s.at[i % side_nb, pl.ds(0, n)], i % side_nb
            slot = lax.rem(i, side_nb)
            start = pl.multiple_of(lax.rem(i, per) * side_rows, 8)
            return (lax.div(i, per), pl.ds(start, side_rows)), side_s.at[slot], slot

        def c_sa(i):
            rows, stage, slot = side_refs(i)
            return cp(wob_h.at[rows], stage, S_SA + slot)

        def c_sb(i):
            rows, stage, slot = side_refs(i)
            return cp(stage, wob_s.at[rows], S_SB + slot)

        def tick(i):
            traced = not isinstance(i, int)
            if traced or i < side_n:
                c_sa(i).wait()
                c_sb(i).start()

            def refill(j):
                if traced or i >= side_lag:
                    c_sb(i - side_lag).wait()
                c_sa(j).start()

            if traced:
                pl.when(i + side_lead < side_n)(lambda: refill(i + side_lead))
            elif i + side_lead < side_n:
                refill(i + side_lead)

        def head_major(w_s, t, hh, mid=lambda: None):
            halves = []
            for k in range(2):
                w = w_s[2 * t + k].reshape(_L // 2, Hb, Db)[:, hh * HH:(hh + 1) * HH, :]
                halves.append(w.reshape(_L // 2, HH * Db))
                if k == 0:
                    mid()
            return jnp.concatenate(halves, axis=0)

        start_pieces(wqb_h, wqb_s, cut_w0, S_WQB)
        c_xb.start()
        c_xa.start()
        for i in range(side_lead):
            c_sa(i).start()
        start_pieces(wuk_h, wuk_s, cut_w, S_WUK)
        pm = _Pump(heads_of(wuk_h, wuk_s, i_w))
        pm.pump(*cfg["pump_0"])
        pm.drain()


        wait_pieces(wqb_s, cut_w0, S_WQB)
        start_c(0)
        pm = pump_c(0)
        pm.kick()
        tick(0)
        c_xb.wait()
        xb = xb_s[...]
        halves = [None, None]
        for t in range(M // _L):
            for hh in range(2):
                part = _dot(xb[:, t * _L:(t + 1) * _L], head_major(wqb_s, t, hh, pm.kick))
                halves[hh] = part if t == 0 else halves[hh] + part
                pm.kick()
        ctxb_s[...] = jnp.concatenate(halves, axis=1)
        pm.pump(*cfg["pump_w"])
        pm.drain()

        wait_pieces(wuk_s, cut_w, S_WUK)
        start_c(1)
        pm = pump_c(1)
        pm.kick()
        tick(1)
        qb = (ctxb_s[...] * scale_b).astype(_BF16)
        for t in range(NCT):
            for hh in range(2):
                w = head_major(wuk_s, t, hh, pm.kick)
                parts = [_dot_nt(qb[:, (hh * HH + j) * Db:(hh * HH + j + 1) * Db],
                                 w[:, j * Db:(j + 1) * Db]) for j in range(HH)]
                qabs_s[t, :, hh * HH:(hh + 1) * HH, :] = jnp.concatenate(
                    parts, axis=1).reshape(B, HH, _L)
                pm.kick()
        pm.pump(*cfg["pump_w"])
        pm.drain()

        def attend_b(b, start_next, pm):
            wait_pieces(c_s.at[b], cut_c, S_C + b)
            start_next()
            pm.kick()
            tick(2 + b)
            qa = jnp.concatenate(
                [qabs_s[t, b] for t in range(NCT)], axis=1).astype(_BF16)

            def latent(k):
                tiles = c_s[b, k].reshape(k_c // 8, NCT, 8, _L)
                return jnp.concatenate(
                    [tiles[:, t].reshape(k_c, _L) for t in range(NCT)], axis=1)

            for k in range(NBLK):
                s_s[:, k * k_c:(k + 1) * k_c] = _dot_nt(qa, latent(k))
                if k in cfg["kick_s"]:
                    pm.kick()
            s = s_s[...]
            m = jnp.max(s, axis=-1, keepdims=True)
            p = jnp.exp(s - m)
            l = jnp.sum(p, axis=-1, keepdims=True)
            pb = p.astype(_BF16)
            cc = None
            for k in range(NBLK):
                part = _dot(pb[:, k * k_c:(k + 1) * k_c], latent(k))
                cc = part if cc is None else cc + part
                if k in cfg["kick_c"]:
                    pm.kick()
            cc = cc / l
            for t in range(NCT):
                ctx_s[t, b] = cc[:, t * _L:(t + 1) * _L]
            pm.pump(*cfg["pump_c"])
            pm.drain()

        small_wqa = heads_of(wqa_h, wqa_s, i_wqa)
        n_q = len(small_wqa) // 2
        for b in range(B):
            if b + 2 < B:
                attend_b(b, functools.partial(start_c, b + 2), pump_c(b + 2))
            elif b + 2 == B:
                attend_b(b, functools.partial(start_pieces, wuv_h, wuv_s, cut_w, S_WUV),
                         _Pump(heads_of(wuv_h, wuv_s, i_w)))
            else:
                attend_b(b, start_wqa, _Pump(small_wqa[:n_q] + small_k(0)))

        wait_pieces(wuv_s, cut_w, S_WUV)
        start_k(0)
        start_v(0)
        pm = _Pump(small_v(0)[:1] + small_wqa[n_q:] + small_v(0)[1:] + small_k(1))
        pm.kick()
        tick(2 + B)
        halves = [None, None]
        for t in range(NCT):
            for hh in range(2):
                ch = ctx_s[t, :, hh * HH:(hh + 1) * HH, :].reshape(B, HH * _L).astype(_BF16)
                w = head_major(wuv_s, t, hh, pm.kick)
                part = jnp.concatenate(
                    [_dot(ch[:, j * _L:(j + 1) * _L], w[:, j * Db:(j + 1) * Db])
                     for j in range(HH)], axis=1)
                halves[hh] = part if t == 0 else halves[hh] + part
                pm.kick()
        ctxb_s[...] = jnp.concatenate(halves, axis=1)
        pm.pump(*cfg["pump_uv"])
        pm.drain()

        wait_pieces(wqa_s, cut_wqa, S_WQA)
        start_k(1)
        pm = _Pump(small_v(1))
        pm.kick()
        tick(3 + B)
        c_xa.wait()
        xa = xa_s[...]
        seg = n_ct // 2
        for c0 in range(0, n_ct, seg):
            wq_tiles = wqa_s[...].reshape(D // 8, n_ct, 8, _L)
            oab_s[:, c0 * _L:(c0 + seg) * _L] = jnp.concatenate(
                [_dot(xa, wq_tiles[:, ct].reshape(D, _L)) for ct in range(c0, c0 + seg)], axis=1)
            pm.pump(1, cfg["lag"])
        qa_s[...] = (oab_s[...] * scale_a).reshape(B, H, Dh).reshape(BH, Dh)
        pm.pump(*cfg["pump_q"])
        pm.drain()

        def attend_a(g, start_at_k, start_at_v, pm, same_buffer, between):
            start = g * _G if isinstance(g, int) else pl.multiple_of(g * _G, _G)
            rows = pl.ds(start, _G)
            q8 = qa_s[rows, :].astype(_BF16)
            wait_pieces(k_s.at[g], cut_k, S_KV + 2 * g)
            start_at_k()
            pm.kick()
            tick(4 + B + g)
            row = lax.broadcasted_iota(jnp.int32, (_G, W), 0)
            s = None
            for j in range(_G):
                sj = _dot_nt(q8, k_s[g, j])
                s = sj if s is None else jnp.where(row == j, sj, s)
                if j in cfg["kick_qk"]:
                    if same_buffer:
                        pm.kick()
                    else:
                        p_s[...] = s
                        pm.pump(1, cfg["lag"])
                        s = p_s[...]
            m = jnp.max(s, axis=-1, keepdims=True)
            p = jnp.exp(s - m)
            l = jnp.sum(p, axis=-1, keepdims=True)
            p_s[...] = p
            between()
            wait_pieces(v_s.at[g], cut_v, S_KV + 2 * g + 1)
            start_at_v()
            if same_buffer:
                pm.kick()
            else:
                pm.pump(1, cfg["lag"])
            pb = p_s[...].astype(_BF16)
            row2 = lax.broadcasted_iota(jnp.int32, (_G, Dh), 0)
            o = None
            for j in range(_G):
                oj = _dot(pb, v_s[g, j])
                o = oj if o is None else jnp.where(row2 == j, oj, o)
                if j in cfg["kick_pv"] and same_buffer:
                    pm.kick()
            oa_s[rows, :] = o / l

        def a_body(g, carry):
            pm = _Pump(small_k(g + 2) + small_v(g + 2))
            attend_a(g, functools.partial(start_v, g + 1), functools.partial(start_k, g + 2), pm,
                     True, functools.partial(pm.pump, *cfg["pump_k"]))
            pm.pump(*cfg["pump_v"])
            pm.drain()
            return carry

        lax.fori_loop(0, NG - 2, a_body, 0)

        waited = side_n - side_nb
        n_early = side_n - cfg["side_mid"]
        r_early, r_mid = n_early * side_rows, side_n * side_rows
        pm = _Pump(small_wo())

        def project_b():
            c_wob.wait()
            wait_pieces(wob_s.at[rest_all], cut_rest, S_WOB)
            for i in range(waited, n_early):
                c_sb(i).wait()
            ctxb = ctxb_s[...].astype(_BF16)
            accb_s[...] = _dot(ctxb[:, side_total:], rows_of(wob_s, side_total, Hb * Db))
            step = 8 * _L
            for lo in range(0, r_early, step):
                pm.pump(1, cfg["lag"])
                hi = min(lo + step, r_early)
                accb_s[...] += _dot(ctxb[:, lo:hi], rows_of(wob_s, lo, hi))

        attend_a(NG - 2, functools.partial(start_v, NG - 1), start_wo, pm,
                 False, functools.partial(pm.pump, *cfg["pump_k14"]))
        project_b()
        pm.pump(*cfg["pump_b"])

        def start_last():
            for i in range(n_wo):
                c_wo(i).start(priority=_BULK)
            c_sa(side_n).start()

        attend_a(NG - 1, start_last, lambda: None, pm,
                 False, functools.partial(pm.pump, *cfg["pump_k15"]))
        pm.pump(1, cfg["lag"])

        oa32 = oa_s[...].reshape(B, H, Dh).reshape(B, H * Dh)
        oab_s[...] = oa32
        tail0 = H * Dh - tail_rows
        for b in range(B):
            for t in range(tail_rows // Dh):
                src = oa32[b:b + 1, tail0 + t * Dh:tail0 + (t + 1) * Dh]
                coef_s[b, t * Dh:(t + 1) * Dh, :] = jnp.broadcast_to(src, (_L, Dh)).T
        pm.pump(*cfg["pump_e"])
        c_sa(side_n).wait()
        c_sb(side_n).start()
        pm.pump(*cfg["pump_f"])
        pm.drain()
        oa = oab_s[...].astype(_BF16)
        if n_gap:
            c_gap.wait()
        n_head = wo_inj * r_wo
        acc_s[...] = _dot(oa[:, :n_head], woa_s[:wo_inj].reshape(n_head, D))
        for j in range(n_early, side_n):
            c_sb(j).wait()
        accb_s[...] += _dot(ctxb_s[:, r_early:r_mid].astype(_BF16), rows_of(wob_s, r_early, r_mid))
        wait_pieces(woa_s.at[wide], cut_wo, S_WIDE)
        acc_s[...] += _dot(oa[:, n_head:wo_base],
                           woa_s[wo_inj:wo_inj + wo_wide].reshape(wo_base - n_head, D))
        for i in range(n_mxu):
            c_wo(i).wait()
            if i == late_at:
                c_sb(side_n).wait()
                late = _dot(ctxb_s[:, r_mid:side_total].astype(_BF16),
                            rows_of(wob_s, r_mid, side_total))
                o_ref[:, D:] = (accb_s[...] + late).astype(o_ref.dtype)
            lo, n = wo_off[i], wo_chunks[i]
            part = _dot(oa[:, lo:lo + n], woa_s[wo_at(lo, n)]) + acc_s[...]
            if i < n_wo - 1:
                acc_s[...] = part
            else:
                o_ref[:, :D] = part.astype(o_ref.dtype)
        for i in range(n_mxu, n_wo):
            c_wo(i).wait()
            lo, n = wo_off[i], wo_chunks[i]
            w = woa_s[wo_at(lo, n)].astype(_F32)
            sums = []
            for b in range(B):
                cf = coef_s[b, lo - tail0:lo - tail0 + n, :]
                prod = w * jnp.concatenate([cf] * (D // _L), axis=1)
                acc = vacc_s[b] if i > n_mxu else None
                for r in range(0, n, 8):
                    acc = prod[r:r + 8] if acc is None else acc + prod[r:r + 8]
                if i < n_wo - 1:
                    vacc_s[b] = acc
                else:
                    sums.append(jnp.sum(acc, axis=0, keepdims=True))
            if i == n_wo - 1:
                res = acc_s[...] + jnp.concatenate(sums, axis=0)
                o_ref[:, :D] = res.astype(o_ref.dtype)

    any_spec = pl.BlockSpec(memory_space=pl.ANY)
    out = pl.pallas_call(
        kernel,
        out_shape=jax.ShapeDtypeStruct((B, D + M), A_x.dtype),
        in_specs=[any_spec] * 11,
        out_specs=pl.BlockSpec(memory_space=pltpu.VMEM),
        scratch_shapes=[
            pltpu.VMEM(xa2.shape, _BF16),
            pltpu.VMEM(xb2.shape, _BF16),
            pltpu.VMEM((2, NG, _G, W, Dh), _BF16),
            pltpu.VMEM((4 + B,) + wqb4.shape, _BF16),
            pltpu.VMEM(woa3.shape, _BF16),
            pltpu.VMEM(wob3.shape, _BF16),
            pltpu.VMEM((BH, Dh), _F32),
            pltpu.VMEM((BH, Dh), _F32),
            pltpu.VMEM((NCT, B, Hb, _L), _F32),
            pltpu.VMEM((NCT, B, Hb, _L), _F32),
            pltpu.VMEM((B, D), _F32),
            pltpu.VMEM((B, M), _F32),
            pltpu.VMEM((B, Hb * Db), _F32),
            pltpu.VMEM((B, H * Dh), _F32),
            pltpu.VMEM((B, max(tail_rows, 8), _L), _F32),
            pltpu.VMEM((B, 8, D), _F32),
            pltpu.VMEM((_G, W), _F32),
            pltpu.VMEM((Hb, Skb), _F32),
            pltpu.SMEM((side_nb, side_rows, M), _BF16),
            pltpu.SemaphoreType.DMA((n_sem,)),
        ],
        compiler_params=pltpu.CompilerParams(
            vmem_limit_bytes=120 * 1024 * 1024,
            disable_semaphore_checks=True,
            disable_bounds_checks=True,
        ),
        name="fused_decode",
    )(xa2, k3, v3, wqa3, woa3, xb2, c4, wqb4, wuk4, wuv4, wob3)
    return out.reshape(B, Sq, D + M)


@jax.jit
def pallas_concat_heads__sliding_block_cached__compressed_kv_cla__decode_kernel(
    A_x: jax.Array,
    A_k_cache: jax.Array,
    A_v_cache: jax.Array,
    A_wq: jax.Array,
    A_wo: jax.Array,
    B_x: jax.Array,
    B_c_kv: jax.Array,
    B_w_q: jax.Array,
    B_w_uk: jax.Array,
    B_w_uv: jax.Array,
    B_w_o: jax.Array,
):
    return _fused(_CFG, A_x, A_k_cache, A_v_cache, A_wq, A_wo,
                  B_x, B_c_kv, B_w_q, B_w_uk, B_w_uv, B_w_o)
```

```python
import functools

import jax
import jax.numpy as jnp
from jax import lax
import jax.experimental.pallas as pl
import jax.experimental.pallas.tpu as pltpu

_NT = (((1,), (1,)), ((), ()))
_F32 = jnp.float32
_BF16 = jnp.bfloat16
_L = 128
_G = 8
_KIB = 1024
_URGENT, _BULK = 0, 1

_CFG = dict(
    piece=64 * _KIB,
    block=512 * _KIB,
    shift_a=30 * _KIB,
    shift_b=34 * _KIB,
    shift_wo=32 * _KIB,
    inj_w=(18 * _KIB, 16 * _KIB, -14 * _KIB, -16 * _KIB),
    inj_c=(18 * _KIB, 16 * _KIB, -14 * _KIB, -16 * _KIB),
    inj_q=(14 * _KIB, 16 * _KIB, -18 * _KIB, -16 * _KIB),
    inj_k=(14 * _KIB, 16 * _KIB),
    inj_v=(-18 * _KIB, -16 * _KIB),
    inj_wo=(16 * _KIB,) * 52,
    pump_0=(28, 2),
    pump_w=(11, 3),
    pump_c=(15, 3),
    pump_uv=(20, 3),
    pump_q=(8, 2),
    pump_k=(10, 3),
    pump_v=(11, 3),
    pump_k14=(9, 3),
    pump_b=(6, 3),
    pump_k15=(10, 3),
    pump_e=(3, 3),
    pump_f=(7, 3),
    lag=2,
    kick_s=(0, 1, 2, 3, 4, 5, 6, 7),
    kick_c=(1, 3, 5),
    kick_qk=(0, 1, 3, 5, 6),
    kick_pv=(1, 3, 5),
    side_rows=128,
    side_n=24,
    side_last=64,
    side_nb=5,
    side_mid=3,
    late_at=1,
    wo_chunks=(512, 128, 128),
    wo_tail=(80, 64, 48, 32, 16, 16),
)


def _dot(a, b):
    return jnp.dot(a, b, preferred_element_type=_F32)


def _dot_nt(a, b):
    return lax.dot_general(a, b, _NT, preferred_element_type=_F32)


def _bounds(n_rows, row_bytes, piece, shift, skip=0):
    step = piece // row_bytes
    first = (shift // row_bytes) % step
    cuts = [skip] + [r for r in range(first, n_rows, step) if r > skip] + [n_rows]
    return list(zip(cuts[:-1], cuts[1:]))


class _Pump:
    def __init__(self, copies):
        self.copies, self.started, self.waited = list(copies), 0, 0

    def kick(self):
        if self.started < len(self.copies):
            self.copies[self.started]().start(priority=_URGENT)
            self.started += 1

    def _wait_to(self, n):
        while self.waited < n:
            self.copies[self.waited]().wait()
            self.waited += 1

    def pump(self, n, lag=1):
        for _ in range(n):
            self.kick()
            self._wait_to(self.started - lag)

    def drain(self):
        while self.started < len(self.copies):
            self.kick()
        self._wait_to(self.started)


def _fused(cfg, A_x, A_k_cache, A_v_cache, A_wq, A_wo, B_x, B_c_kv, B_w_q, B_w_uk, B_w_uv, B_w_o):
    B, Sq, D = A_x.shape
    _, H, Sk, Dh = A_k_cache.shape
    assert Sq == 1 and B_x.shape[1] == 1
    assert A_wq.shape == (D, H * Dh)
    W = min(4096, max(256, Sk // 4))
    M, Hb, Db = B_w_q.shape
    Skb, Dc = B_c_kv.shape[1], B_c_kv.shape[2]
    BH = B * H
    NG = BH // _G
    NCT = Dc // _L
    HH = Hb // 2
    scale_a = float(Dh) ** -0.5
    scale_b = float(Db) ** -0.5
    piece, block = cfg["piece"], cfg["block"]
    shift_a, shift_b = cfg["shift_a"], cfg["shift_b"]
    side_rows, side_n, side_nb = cfg["side_rows"], cfg["side_n"], cfg["side_nb"]
    late_at = cfg["late_at"]
    n_mxu = len(cfg["wo_chunks"])
    wo_chunks = tuple(cfg["wo_chunks"]) + tuple(cfg["wo_tail"])
    tail_rows = sum(cfg["wo_tail"])
    assert tail_rows % Dh == 0 and M % _L == 0 and NG >= 4
    side_lag = 2
    side_lead = side_nb - side_lag
    side_last = cfg["side_last"]
    assert side_n == 4 + B + NG and cfg["side_mid"] < side_nb and side_last > 0

    xa2 = A_x.reshape(B, D)
    xb2 = B_x.reshape(B, M)
    k3 = A_k_cache.reshape(BH, Sk, Dh)
    v3 = A_v_cache.reshape(BH, Sk, Dh)

    def blocked(w, lead=0):
        row_bytes = 2 * functools.reduce(lambda a, b: a * b, w.shape[lead + 1:], 1)
        rows = block // row_bytes
        shape = w.shape[:lead] + (w.shape[lead] // rows, rows) + w.shape[lead + 1:]
        return w.reshape(shape), rows, row_bytes

    n_ct = H * Dh // _L
    wqa_t = A_wq.reshape(D // 8, 8, n_ct, _L).transpose(0, 2, 1, 3).reshape(D * n_ct, _L)
    wqa3, r_wqa, b_wqa = blocked(wqa_t)
    wqb4, r_w, b_w = blocked(B_w_q.reshape(M * Hb, Db))
    wuk4, _, _ = blocked(B_w_uk.reshape(Dc * Hb, Db))
    wuv4, _, _ = blocked(B_w_uv.reshape(Dc * Hb, Db))
    c_t = B_c_kv.reshape(B, Skb // 8, 8, NCT, _L).transpose(0, 1, 3, 2, 4)
    c4, r_c, b_c = blocked(c_t.reshape(B, Skb * NCT, _L), 1)
    k_c = r_c // NCT
    woa3, r_wo, b_wo = blocked(A_wo)
    wob3, _, _ = blocked(B_w_o.reshape(Hb * Db, M))
    assert wob3.shape == woa3.shape and r_wo % side_rows == 0
    assert wqb4.shape == wuk4.shape == wuv4.shape and 2 * r_w == _L * Hb
    assert wqa3.shape == wqb4.shape == c4.shape[1:]
    NBLK = wqb4.shape[0]

    def spans(sizes, unit, n_rows=0):
        out, front, back = [], 0, n_rows
        for n in sizes:
            if n > 0:
                out.append((front, front + n // unit))
                front += n // unit
            else:
                out.append((back + n // unit, back))
                back += n // unit
        return out, front, back

    def split(sizes, n_rows, unit, shift):
        small, front, back = spans(sizes, unit, n_rows)
        return small, _bounds(back, unit, piece, shift, front)

    i_w, cut_w = split(cfg["inj_w"], r_w, b_w, shift_b)
    i_c, cut_c = split(cfg["inj_c"], r_c, b_c, shift_b)
    i_k, cut_k = split(cfg["inj_k"], W, 2 * Dh, shift_a)
    i_v, cut_v = split(cfg["inj_v"], W, 2 * Dh, shift_a)
    i_wqa, cut_wqa = split(cfg["inj_q"], r_wqa, b_wqa, shift_a)
    i_wo, _, _ = spans(cfg["inj_wo"], 2 * D)
    cut_w0 = _bounds(r_w, b_w, piece, shift_b)
    n_inj = i_wo[-1][1]
    wo_inj = -(-n_inj // r_wo)
    wo_wide = (H * Dh - sum(wo_chunks)) // r_wo - wo_inj
    cut_wo = _bounds(r_wo, b_wo, piece, cfg["shift_wo"])
    wo_base = (wo_inj + wo_wide) * r_wo
    assert all(lo // r_wo == (hi - 1) // r_wo for lo, hi in i_wo)
    assert wo_base + sum(wo_chunks) == H * Dh
    n_wo = len(wo_chunks)
    wo_off = [wo_base + sum(wo_chunks[:i]) for i in range(n_wo)]
    assert all(lo // r_wo == (lo + n - 1) // r_wo for lo, n in zip(wo_off, wo_chunks))
    S_XB, S_XA, S_WQB, S_WUK, S_WUV, S_WOB, S_WQA, S_INJ, S_WIDE, S_GAP, S_GAPB = range(11)
    S_C = 11
    S_KV = S_C + B
    S_WO = S_KV + 2 * NG
    S_SA = S_WO + n_wo
    S_SB = S_SA + side_nb
    n_sem = S_SB + side_nb
    side_total = side_rows * side_n + side_last

    def kernel(xa_h, k_h, v_h, wqa_h, woa_h, xb_h, c_h, wqb_h, wuk_h, wuv_h, wob_h,
               o_ref,
               xa_s, xb_s, kv_s, big_s, woa_s, wob_s,
               qa_s, oa_s, qabs_s, ctx_s, acc_s, accb_s, ctxb_s, oab_s, coef_s, vacc_s, p_s, s_s,
               side_s, sem):
        def cp(src, dst, s):
            return pltpu.make_async_copy(src, dst, sem.at[s])

        def start_pieces(src, dst, cuts, s, row0=0):
            for lo, hi in cuts:
                cp(src.at[:, pl.ds(row0 + lo, hi - lo)], dst.at[:, pl.ds(lo, hi - lo)],
                   s).start(priority=_BULK)

        def wait_pieces(dst, cuts, s):
            view = dst.at[:, pl.ds(cuts[0][0], cuts[-1][1] - cuts[0][0])]
            cp(view, view, s).wait()

        def heads_of(src, dst, ranges, row0=0):
            def one(k, lo, hi):
                return cp(src.at[k, pl.ds(row0 + lo, hi - lo)], dst.at[k, pl.ds(lo, hi - lo)], S_INJ)
            return [functools.partial(one, k, lo, hi)
                    for k in range(dst.shape[0]) for lo, hi in sorted(ranges)]

        k_s, v_s = kv_s.at[0], kv_s.at[1]
        wqb_s, wuk_s, wuv_s, wqa_s = (big_s.at[j] for j in range(4))
        c_s = big_s.at[pl.ds(4, B)]
        c_xb = cp(xb_h, xb_s, S_XB)
        c_xa = cp(xa_h, xa_s, S_XA)

        def rows_of(ref, lo, hi):
            parts = [ref[k, max(lo - k * r_wo, 0):min(hi - k * r_wo, r_wo)]
                     for k in range(lo // r_wo, -(-hi // r_wo))]
            return parts[0] if len(parts) == 1 else jnp.concatenate(parts, axis=0)

        k0, r0 = divmod(side_total, r_wo)
        cut_rest = _bounds(r_wo, b_wo, piece, cfg["shift_wo"], r0)
        rest_all, rest_up = pl.ds(k0, NBLK - k0), (pl.ds(k0 + 1, NBLK - k0 - 1), pl.ds(0, r0))
        c_wob = cp(wob_h.at[rest_up], wob_s.at[rest_up], S_GAPB)

        def start_c(b):
            start_pieces(c_h.at[b], c_s.at[b], cut_c, S_C + b)

        def pump_c(b):
            return _Pump(heads_of(c_h.at[b], c_s.at[b], i_c))

        def start_wqa():
            c_wob.start(priority=_BULK)
            start_pieces(wob_h.at[rest_all], wob_s.at[rest_all], cut_rest, S_WOB)
            start_pieces(wqa_h, wqa_s, cut_wqa, S_WQA)

        def start_k(g):
            start_pieces(k_h.at[pl.ds(g * _G, _G)], k_s.at[g], cut_k, S_KV + 2 * g, Sk - W)

        def start_v(g):
            start_pieces(v_h.at[pl.ds(g * _G, _G)], v_s.at[g], cut_v, S_KV + 2 * g + 1, Sk - W)

        def small_k(g):
            return heads_of(k_h.at[pl.ds(g * _G, _G)], k_s.at[g], i_k, Sk - W)

        def small_v(g):
            return heads_of(v_h.at[pl.ds(g * _G, _G)], v_s.at[g], i_v, Sk - W)

        def wo_at(lo, n):
            return lo // r_wo, pl.ds(lo % r_wo, n)

        def c_wo(i):
            at = wo_at(wo_off[i], wo_chunks[i])
            return cp(woa_h.at[at], woa_s.at[at], S_WO + i)

        wide = pl.ds(wo_inj, wo_wide)

        n_gap = wo_inj * r_wo - n_inj
        if n_gap:
            c_gap = cp(woa_h.at[wo_at(n_inj, n_gap)], woa_s.at[wo_at(n_inj, n_gap)], S_GAP)

        def start_wo():
            if n_gap:
                c_gap.start(priority=_BULK)
            start_pieces(woa_h.at[wide], woa_s.at[wide], cut_wo, S_WIDE)

        def small_wo():
            def one(lo, hi):
                at = wo_at(lo, hi - lo)
                return cp(woa_h.at[at], woa_s.at[at], S_INJ)
            return [functools.partial(one, lo, hi) for lo, hi in i_wo]

        def side_refs(i):
            per = r_wo // side_rows
            if isinstance(i, int):
                n = side_rows if i < side_n else side_last
                rows = (i // per, pl.ds(i % per * side_rows, n))
                return rows, side_s.at[i % side_nb, pl.ds(0, n)], i % side_nb
            slot = lax.rem(i, side_nb)
            start = pl.multiple_of(lax.rem(i, per) * side_rows, 8)
            return (lax.div(i, per), pl.ds(start, side_rows)), side_s.at[slot], slot

        def c_sa(i):
            rows, stage, slot = side_refs(i)
            return cp(wob_h.at[rows], stage, S_SA + slot)

        def c_sb(i):
            rows, stage, slot = side_refs(i)
            return cp(stage, wob_s.at[rows], S_SB + slot)

        def tick(i):
            traced = not isinstance(i, int)
            if traced or i < side_n:
                c_sa(i).wait()
                c_sb(i).start()

            def refill(j):
                if traced or i >= side_lag:
                    c_sb(i - side_lag).wait()
                c_sa(j).start()

            if traced:
                pl.when(i + side_lead < side_n)(lambda: refill(i + side_lead))
            elif i + side_lead < side_n:
                refill(i + side_lead)

        def head_major(w_s, t, hh, mid=lambda: None):
            halves = []
            for k in range(2):
                w = w_s[2 * t + k].reshape(_L // 2, Hb, Db)[:, hh * HH:(hh + 1) * HH, :]
                halves.append(w.reshape(_L // 2, HH * Db))
                if k == 0:
                    mid()
            return jnp.concatenate(halves, axis=0)

        start_pieces(wqb_h, wqb_s, cut_w0, S_WQB)
        c_xb.start()
        c_xa.start()
        for i in range(side_lead):
            c_sa(i).start()
        start_pieces(wuk_h, wuk_s, cut_w, S_WUK)
        pm = _Pump(heads_of(wuk_h, wuk_s, i_w))
        pm.pump(*cfg["pump_0"])
        pm.drain()


        wait_pieces(wqb_s, cut_w0, S_WQB)
        start_c(0)
        pm = pump_c(0)
        pm.kick()
        tick(0)
        c_xb.wait()
        xb = xb_s[...]
        halves = [None, None]
        for t in range(M // _L):
            for hh in range(2):
                part = _dot(xb[:, t * _L:(t + 1) * _L], head_major(wqb_s, t, hh, pm.kick))
                halves[hh] = part if t == 0 else halves[hh] + part
                pm.kick()
        ctxb_s[...] = jnp.concatenate(halves, axis=1)
        pm.pump(*cfg["pump_w"])
        pm.drain()

        wait_pieces(wuk_s, cut_w, S_WUK)
        start_c(1)
        pm = pump_c(1)
        pm.kick()
        tick(1)
        qb = (ctxb_s[...] * scale_b).astype(_BF16)
        for t in range(NCT):
            for hh in range(2):
                w = head_major(wuk_s, t, hh, pm.kick)
                parts = [_dot_nt(qb[:, (hh * HH + j) * Db:(hh * HH + j + 1) * Db],
                                 w[:, j * Db:(j + 1) * Db]) for j in range(HH)]
                qabs_s[t, :, hh * HH:(hh + 1) * HH, :] = jnp.concatenate(
                    parts, axis=1).reshape(B, HH, _L)
                pm.kick()
        pm.pump(*cfg["pump_w"])
        pm.drain()

        def attend_b(b, start_next, pm):
            wait_pieces(c_s.at[b], cut_c, S_C + b)
            start_next()
            pm.kick()
            tick(2 + b)
            qa = jnp.concatenate(
                [qabs_s[t, b] for t in range(NCT)], axis=1).astype(_BF16)

            def latent(k):
                tiles = c_s[b, k].reshape(k_c // 8, NCT, 8, _L)
                return jnp.concatenate(
                    [tiles[:, t].reshape(k_c, _L) for t in range(NCT)], axis=1)

            for k in range(NBLK):
                s_s[:, k * k_c:(k + 1) * k_c] = _dot_nt(qa, latent(k))
                if k in cfg["kick_s"]:
                    pm.kick()
            s = s_s[...]
            m = jnp.max(s, axis=-1, keepdims=True)
            p = jnp.exp(s - m)
            l = jnp.sum(p, axis=-1, keepdims=True)
            pb = p.astype(_BF16)
            cc = None
            for k in range(NBLK):
                part = _dot(pb[:, k * k_c:(k + 1) * k_c], latent(k))
                cc = part if cc is None else cc + part
                if k in cfg["kick_c"]:
                    pm.kick()
            cc = cc / l
            for t in range(NCT):
                ctx_s[t, b] = cc[:, t * _L:(t + 1) * _L]
            pm.pump(*cfg["pump_c"])
            pm.drain()

        small_wqa = heads_of(wqa_h, wqa_s, i_wqa)
        n_q = len(small_wqa) // 2
        for b in range(B):
            if b + 2 < B:
                attend_b(b, functools.partial(start_c, b + 2), pump_c(b + 2))
            elif b + 2 == B:
                attend_b(b, functools.partial(start_pieces, wuv_h, wuv_s, cut_w, S_WUV),
                         _Pump(heads_of(wuv_h, wuv_s, i_w)))
            else:
                attend_b(b, start_wqa, _Pump(small_wqa[:n_q] + small_k(0)))

        wait_pieces(wuv_s, cut_w, S_WUV)
        start_k(0)
        start_v(0)
        pm = _Pump(small_v(0)[:1] + small_wqa[n_q:] + small_v(0)[1:] + small_k(1))
        pm.kick()
        tick(2 + B)
        halves = [None, None]
        for t in range(NCT):
            for hh in range(2):
                ch = ctx_s[t, :, hh * HH:(hh + 1) * HH, :].reshape(B, HH * _L).astype(_BF16)
                w = head_major(wuv_s, t, hh, pm.kick)
                part = jnp.concatenate(
                    [_dot(ch[:, j * _L:(j + 1) * _L], w[:, j * Db:(j + 1) * Db])
                     for j in range(HH)], axis=1)
                halves[hh] = part if t == 0 else halves[hh] + part
                pm.kick()
        ctxb_s[...] = jnp.concatenate(halves, axis=1)
        pm.pump(*cfg["pump_uv"])
        pm.drain()

        wait_pieces(wqa_s, cut_wqa, S_WQA)
        start_k(1)
        pm = _Pump(small_v(1))
        pm.kick()
        tick(3 + B)
        c_xa.wait()
        xa = xa_s[...]
        seg = n_ct // 2
        for c0 in range(0, n_ct, seg):
            wq_tiles = wqa_s[...].reshape(D // 8, n_ct, 8, _L)
            oab_s[:, c0 * _L:(c0 + seg) * _L] = jnp.concatenate(
                [_dot(xa, wq_tiles[:, ct].reshape(D, _L)) for ct in range(c0, c0 + seg)], axis=1)
            pm.pump(1, cfg["lag"])
        qa_s[...] = (oab_s[...] * scale_a).reshape(B, H, Dh).reshape(BH, Dh)
        pm.pump(*cfg["pump_q"])
        pm.drain()

        def attend_a(g, start_at_k, start_at_v, pm, same_buffer, between):
            start = g * _G if isinstance(g, int) else pl.multiple_of(g * _G, _G)
            rows = pl.ds(start, _G)
            q8 = qa_s[rows, :].astype(_BF16)
            wait_pieces(k_s.at[g], cut_k, S_KV + 2 * g)
            start_at_k()
            pm.kick()
            tick(4 + B + g)
            row = lax.broadcasted_iota(jnp.int32, (_G, W), 0)
            s = None
            for j in range(_G):
                sj = _dot_nt(q8, k_s[g, j])
                s = sj if s is None else jnp.where(row == j, sj, s)
                if j in cfg["kick_qk"]:
                    if same_buffer:
                        pm.kick()
                    else:
                        p_s[...] = s
                        pm.pump(1, cfg["lag"])
                        s = p_s[...]
            m = jnp.max(s, axis=-1, keepdims=True)
            p = jnp.exp(s - m)
            l = jnp.sum(p, axis=-1, keepdims=True)
            p_s[...] = p
            between()
            wait_pieces(v_s.at[g], cut_v, S_KV + 2 * g + 1)
            start_at_v()
            if same_buffer:
                pm.kick()
            else:
                pm.pump(1, cfg["lag"])
            pb = p_s[...].astype(_BF16)
            row2 = lax.broadcasted_iota(jnp.int32, (_G, Dh), 0)
            o = None
            for j in range(_G):
                oj = _dot(pb, v_s[g, j])
                o = oj if o is None else jnp.where(row2 == j, oj, o)
                if j in cfg["kick_pv"] and same_buffer:
                    pm.kick()
            oa_s[rows, :] = o / l

        def a_body(g, carry):
            pm = _Pump(small_k(g + 2) + small_v(g + 2))
            attend_a(g, functools.partial(start_v, g + 1), functools.partial(start_k, g + 2), pm,
                     True, functools.partial(pm.pump, *cfg["pump_k"]))
            pm.pump(*cfg["pump_v"])
            pm.drain()
            return carry

        lax.fori_loop(0, NG - 2, a_body, 0)

        waited = side_n - side_nb
        n_early = side_n - cfg["side_mid"]
        r_early, r_mid = n_early * side_rows, side_n * side_rows
        pm = _Pump(small_wo())

        def project_b():
            c_wob.wait()
            wait_pieces(wob_s.at[rest_all], cut_rest, S_WOB)
            for i in range(waited, n_early):
                c_sb(i).wait()
            ctxb = ctxb_s[...].astype(_BF16)
            accb_s[...] = _dot(ctxb[:, side_total:], rows_of(wob_s, side_total, Hb * Db))
            step = 8 * _L
            for lo in range(0, r_early, step):
                pm.pump(1, cfg["lag"])
                hi = min(lo + step, r_early)
                accb_s[...] += _dot(ctxb[:, lo:hi], rows_of(wob_s, lo, hi))

        attend_a(NG - 2, functools.partial(start_v, NG - 1), start_wo, pm,
                 False, functools.partial(pm.pump, *cfg["pump_k14"]))
        project_b()
        pm.pump(*cfg["pump_b"])

        def start_last():
            for i in range(n_wo):
                c_wo(i).start(priority=_BULK)
            c_sa(side_n).start()

        attend_a(NG - 1, start_last, lambda: None, pm,
                 False, functools.partial(pm.pump, *cfg["pump_k15"]))
        pm.pump(1, cfg["lag"])

        oa32 = oa_s[...].reshape(B, H, Dh).reshape(B, H * Dh)
        oab_s[...] = oa32
        tail0 = H * Dh - tail_rows
        for b in range(B):
            for t in range(tail_rows // Dh):
                src = oa32[b:b + 1, tail0 + t * Dh:tail0 + (t + 1) * Dh]
                coef_s[b, t * Dh:(t + 1) * Dh, :] = jnp.broadcast_to(src, (_L, Dh)).T
        pm.pump(*cfg["pump_e"])
        c_sa(side_n).wait()
        c_sb(side_n).start()
        pm.pump(*cfg["pump_f"])
        pm.drain()
        oa = oab_s[...].astype(_BF16)
        if n_gap:
            c_gap.wait()
        n_head = wo_inj * r_wo
        acc_s[...] = _dot(oa[:, :n_head], woa_s[:wo_inj].reshape(n_head, D))
        for j in range(n_early, side_n):
            c_sb(j).wait()
        accb_s[...] += _dot(ctxb_s[:, r_early:r_mid].astype(_BF16), rows_of(wob_s, r_early, r_mid))
        wait_pieces(woa_s.at[wide], cut_wo, S_WIDE)
        acc_s[...] += _dot(oa[:, n_head:wo_base],
                           woa_s[wo_inj:wo_inj + wo_wide].reshape(wo_base - n_head, D))
        for i in range(n_mxu):
            c_wo(i).wait()
            if i == late_at:
                c_sb(side_n).wait()
                late = _dot(ctxb_s[:, r_mid:side_total].astype(_BF16),
                            rows_of(wob_s, r_mid, side_total))
                o_ref[:, D:] = (accb_s[...] + late).astype(o_ref.dtype)
            lo, n = wo_off[i], wo_chunks[i]
            part = _dot(oa[:, lo:lo + n], woa_s[wo_at(lo, n)]) + acc_s[...]
            if i < n_wo - 1:
                acc_s[...] = part
            else:
                o_ref[:, :D] = part.astype(o_ref.dtype)
        for i in range(n_mxu, n_wo):
            c_wo(i).wait()
            lo, n = wo_off[i], wo_chunks[i]
            w = woa_s[wo_at(lo, n)].astype(_F32)
            sums = []
            for b in range(B):
                cf = coef_s[b, lo - tail0:lo - tail0 + n, :]
                prod = w * jnp.concatenate([cf] * (D // _L), axis=1)
                acc = vacc_s[b] if i > n_mxu else None
                for r in range(0, n, 8):
                    acc = prod[r:r + 8] if acc is None else acc + prod[r:r + 8]
                if i < n_wo - 1:
                    vacc_s[b] = acc
                else:
                    sums.append(jnp.sum(acc, axis=0, keepdims=True))
            if i == n_wo - 1:
                res = acc_s[...] + jnp.concatenate(sums, axis=0)
                o_ref[:, :D] = res.astype(o_ref.dtype)

    any_spec = pl.BlockSpec(memory_space=pl.ANY)
    out = pl.pallas_call(
        kernel,
        out_shape=jax.ShapeDtypeStruct((B, D + M), A_x.dtype),
        in_specs=[any_spec] * 11,
        out_specs=pl.BlockSpec(memory_space=pltpu.VMEM),
        scratch_shapes=[
            pltpu.VMEM(xa2.shape, _BF16),
            pltpu.VMEM(xb2.shape, _BF16),
            pltpu.VMEM((2, NG, _G, W, Dh), _BF16),
            pltpu.VMEM((4 + B,) + wqb4.shape, _BF16),
            pltpu.VMEM(woa3.shape, _BF16),
            pltpu.VMEM(wob3.shape, _BF16),
            pltpu.VMEM((BH, Dh), _F32),
            pltpu.VMEM((BH, Dh), _F32),
            pltpu.VMEM((NCT, B, Hb, _L), _F32),
            pltpu.VMEM((NCT, B, Hb, _L), _F32),
            pltpu.VMEM((B, D), _F32),
            pltpu.VMEM((B, M), _F32),
            pltpu.VMEM((B, Hb * Db), _F32),
            pltpu.VMEM((B, H * Dh), _F32),
            pltpu.VMEM((B, max(tail_rows, 8), _L), _F32),
            pltpu.VMEM((B, 8, D), _F32),
            pltpu.VMEM((_G, W), _F32),
            pltpu.VMEM((Hb, Skb), _F32),
            pltpu.SMEM((side_nb, side_rows, M), _BF16),
            pltpu.SemaphoreType.DMA((n_sem,)),
        ],
        compiler_params=pltpu.CompilerParams(
            vmem_limit_bytes=120 * 1024 * 1024,
            disable_semaphore_checks=True,
            disable_bounds_checks=True,
        ),
        name="fused_decode",
    )(xa2, k3, v3, wqa3, woa3, xb2, c4, wqb4, wuk4, wuv4, wob3)
    return out.reshape(B, Sq, D + M)


@jax.jit
def pallas_concat_heads__sliding_block_cached__compressed_kv_cla__decode_kernel(
    A_x: jax.Array,
    A_k_cache: jax.Array,
    A_v_cache: jax.Array,
    A_wq: jax.Array,
    A_wo: jax.Array,
    B_x: jax.Array,
    B_c_kv: jax.Array,
    B_w_q: jax.Array,
    B_w_uk: jax.Array,
    B_w_uv: jax.Array,
    B_w_o: jax.Array,
):
    return _fused(_CFG, A_x, A_k_cache, A_v_cache, A_wq, A_wo,
                  B_x, B_c_kv, B_w_q, B_w_uk, B_w_uv, B_w_o)
```

```python
import functools

import jax
import jax.numpy as jnp
from jax import lax
import jax.experimental.pallas as pl
import jax.experimental.pallas.tpu as pltpu

_NT = (((1,), (1,)), ((), ()))
_F32 = jnp.float32
_BF16 = jnp.bfloat16
_L = 128
_G = 8
_KIB = 1024
_URGENT, _BULK = 0, 1

_CFG = dict(
    piece=64 * _KIB,
    block=512 * _KIB,
    shift_a=30 * _KIB,
    shift_b=34 * _KIB,
    shift_wo=32 * _KIB,
    inj_w=(18 * _KIB, 16 * _KIB, -14 * _KIB, -16 * _KIB),
    inj_c=(18 * _KIB, 16 * _KIB, -14 * _KIB, -16 * _KIB),
    inj_q=(14 * _KIB, 16 * _KIB, -18 * _KIB, -16 * _KIB),
    inj_k=(14 * _KIB, 16 * _KIB),
    inj_v=(-18 * _KIB, -16 * _KIB),
    inj_vl=(14 * _KIB, 16 * _KIB),
    inj_wo=(16 * _KIB,) * 44,
    pump_0=(28, 2),
    pump_w=(11, 3),
    pump_c=(15, 3),
    pump_uv=(20, 3),
    pump_q=(8, 2),
    pump_k=(10, 3),
    pump_v=(11, 3),
    pump_k14=(9, 3),
    pump_b=(6, 3),
    pump_k15=(10, 3),
    pump_e=(3, 3),
    pump_f=(7, 3),
    seg_b=512,
    lag=2,
    kick_s=(0, 1, 2, 3, 4, 5, 6, 7),
    kick_c=(1, 3, 5),
    kick_qk=(0, 1, 3, 5, 6),
    kick_pv=(1, 3, 5),
    side_rows=128,
    side_n=24,
    side_last=64,
    side_nb=5,
    side_mid=3,
    late_at=1,
    wo_chunks=(512, 128, 128),
    wo_tail=(80, 64, 48, 32, 16, 16),
)


def _dot(a, b):
    return jnp.dot(a, b, preferred_element_type=_F32)


def _dot_nt(a, b):
    return lax.dot_general(a, b, _NT, preferred_element_type=_F32)


def _bounds(n_rows, row_bytes, piece, shift, skip=0):
    step = piece // row_bytes
    first = (shift // row_bytes) % step
    cuts = [skip] + [r for r in range(first, n_rows, step) if r > skip] + [n_rows]
    return list(zip(cuts[:-1], cuts[1:]))


class _Pump:
    def __init__(self, copies):
        self.copies, self.started, self.waited = list(copies), 0, 0

    def kick(self):
        if self.started < len(self.copies):
            self.copies[self.started]().start(priority=_URGENT)
            self.started += 1

    def _wait_to(self, n):
        while self.waited < n:
            self.copies[self.waited]().wait()
            self.waited += 1

    def pump(self, n, lag=1):
        for _ in range(n):
            self.kick()
            self._wait_to(self.started - lag)

    def drain(self):
        while self.started < len(self.copies):
            self.kick()
        self._wait_to(self.started)


def _fused(cfg, A_x, A_k_cache, A_v_cache, A_wq, A_wo, B_x, B_c_kv, B_w_q, B_w_uk, B_w_uv, B_w_o):
    B, Sq, D = A_x.shape
    _, H, Sk, Dh = A_k_cache.shape
    assert Sq == 1 and B_x.shape[1] == 1
    assert A_wq.shape == (D, H * Dh)
    W = min(4096, max(256, Sk // 4))
    M, Hb, Db = B_w_q.shape
    Skb, Dc = B_c_kv.shape[1], B_c_kv.shape[2]
    BH = B * H
    NG = BH // _G
    NCT = Dc // _L
    HH = Hb // 2
    scale_a = float(Dh) ** -0.5
    scale_b = float(Db) ** -0.5
    piece, block = cfg["piece"], cfg["block"]
    shift_a, shift_b = cfg["shift_a"], cfg["shift_b"]
    side_rows, side_n, side_nb = cfg["side_rows"], cfg["side_n"], cfg["side_nb"]
    late_at = cfg["late_at"]
    n_mxu = len(cfg["wo_chunks"])
    wo_chunks = tuple(cfg["wo_chunks"]) + tuple(cfg["wo_tail"])
    tail_rows = sum(cfg["wo_tail"])
    assert tail_rows % Dh == 0 and M % _L == 0 and NG >= 4
    side_lag = 2
    side_lead = side_nb - side_lag
    side_last = cfg["side_last"]
    assert side_n == 4 + B + NG and cfg["side_mid"] < side_nb and side_last > 0

    xa2 = A_x.reshape(B, D)
    xb2 = B_x.reshape(B, M)
    k3 = A_k_cache.reshape(BH, Sk, Dh)
    v3 = A_v_cache.reshape(BH, Sk, Dh)

    def blocked(w, lead=0):
        row_bytes = 2 * functools.reduce(lambda a, b: a * b, w.shape[lead + 1:], 1)
        rows = block // row_bytes
        shape = w.shape[:lead] + (w.shape[lead] // rows, rows) + w.shape[lead + 1:]
        return w.reshape(shape), rows, row_bytes

    n_ct = H * Dh // _L
    wqa_t = A_wq.reshape(D // 8, 8, n_ct, _L).transpose(0, 2, 1, 3).reshape(D * n_ct, _L)
    wqa3, r_wqa, b_wqa = blocked(wqa_t)
    wqb4, r_w, b_w = blocked(B_w_q.reshape(M * Hb, Db))
    wuk4, _, _ = blocked(B_w_uk.reshape(Dc * Hb, Db))
    wuv4, _, _ = blocked(B_w_uv.reshape(Dc * Hb, Db))
    c_t = B_c_kv.reshape(B, Skb // 8, 8, NCT, _L).transpose(0, 1, 3, 2, 4)
    c4, r_c, b_c = blocked(c_t.reshape(B, Skb * NCT, _L), 1)
    k_c = r_c // NCT
    woa3, r_wo, b_wo = blocked(A_wo)
    wob3, _, _ = blocked(B_w_o.reshape(Hb * Db, M))
    assert wob3.shape == woa3.shape and r_wo % side_rows == 0
    assert wqb4.shape == wuk4.shape == wuv4.shape and 2 * r_w == _L * Hb
    assert wqa3.shape == wqb4.shape == c4.shape[1:]
    NBLK = wqb4.shape[0]

    def spans(sizes, unit, n_rows=0):
        out, front, back = [], 0, n_rows
        for n in sizes:
            if n > 0:
                out.append((front, front + n // unit))
                front += n // unit
            else:
                out.append((back + n // unit, back))
                back += n // unit
        return out, front, back

    def split(sizes, n_rows, unit, shift):
        small, front, back = spans(sizes, unit, n_rows)
        return small, _bounds(back, unit, piece, shift, front)

    i_w, cut_w = split(cfg["inj_w"], r_w, b_w, shift_b)
    i_c, cut_c = split(cfg["inj_c"], r_c, b_c, shift_b)
    i_k, cut_k = split(cfg["inj_k"], W, 2 * Dh, shift_a)
    i_v, cut_v = split(cfg["inj_v"], W, 2 * Dh, shift_a)
    i_vl, cut_vl = split(cfg["inj_v"] + cfg["inj_vl"], W, 2 * Dh, shift_a)
    i_vl = i_vl[len(i_v):]
    i_wqa, cut_wqa = split(cfg["inj_q"], r_wqa, b_wqa, shift_a)
    i_wo, _, _ = spans(cfg["inj_wo"], 2 * D)
    cut_w0 = _bounds(r_w, b_w, piece, shift_b)
    n_inj = i_wo[-1][1]
    wo_inj = -(-n_inj // r_wo)
    wo_wide = (H * Dh - sum(wo_chunks)) // r_wo - wo_inj
    cut_wo = _bounds(r_wo, b_wo, piece, cfg["shift_wo"])
    wo_base = (wo_inj + wo_wide) * r_wo
    assert all(lo // r_wo == (hi - 1) // r_wo for lo, hi in i_wo)
    assert wo_base + sum(wo_chunks) == H * Dh
    n_wo = len(wo_chunks)
    wo_off = [wo_base + sum(wo_chunks[:i]) for i in range(n_wo)]
    assert all(lo // r_wo == (lo + n - 1) // r_wo for lo, n in zip(wo_off, wo_chunks))
    S_XB, S_XA, S_WQB, S_WUK, S_WUV, S_WOB, S_WQA, S_INJ, S_WIDE, S_GAP, S_GAPB, S_INJ2 = range(12)
    S_C = 12
    S_KV = S_C + B
    S_WO = S_KV + 2 * NG
    S_SA = S_WO + n_wo
    S_SB = S_SA + side_nb
    n_sem = S_SB + side_nb
    side_total = side_rows * side_n + side_last

    def kernel(xa_h, k_h, v_h, wqa_h, woa_h, xb_h, c_h, wqb_h, wuk_h, wuv_h, wob_h,
               o_ref,
               xa_s, xb_s, kv_s, big_s, wo_s,
               qa_s, oa_s, qabs_s, ctx_s, acc_s, accb_s, ctxb_s, oab_s, coef_s, vacc_s, p_s, s_s,
               side_s, sem):
        def cp(src, dst, s):
            return pltpu.make_async_copy(src, dst, sem.at[s])

        def start_pieces(src, dst, cuts, s, row0=0):
            for lo, hi in cuts:
                cp(src.at[:, pl.ds(row0 + lo, hi - lo)], dst.at[:, pl.ds(lo, hi - lo)],
                   s).start(priority=_BULK)

        def wait_pieces(dst, cuts, s):
            view = dst.at[:, pl.ds(cuts[0][0], cuts[-1][1] - cuts[0][0])]
            cp(view, view, s).wait()

        def heads_of(src, dst, ranges, row0=0, s=S_INJ):
            def one(k, lo, hi):
                return cp(src.at[k, pl.ds(row0 + lo, hi - lo)], dst.at[k, pl.ds(lo, hi - lo)], s)
            return [functools.partial(one, k, lo, hi)
                    for k in range(dst.shape[0]) for lo, hi in sorted(ranges)]

        k_s, v_s = kv_s.at[0], kv_s.at[1]
        wqb_s, wuk_s, wuv_s, wqa_s = (big_s.at[j] for j in range(4))
        c_s = big_s.at[pl.ds(4, B)]
        woa_s, wob_s = wo_s.at[0], wo_s.at[1]
        c_xb = cp(xb_h, xb_s, S_XB)
        c_xa = cp(xa_h, xa_s, S_XA)

        def rows_of(ref, lo, hi):
            parts = [ref[k, max(lo - k * r_wo, 0):min(hi - k * r_wo, r_wo)]
                     for k in range(lo // r_wo, -(-hi // r_wo))]
            return parts[0] if len(parts) == 1 else jnp.concatenate(parts, axis=0)

        k0, r0 = divmod(side_total, r_wo)
        cut_rest = _bounds(r_wo, b_wo, piece, cfg["shift_wo"], r0)
        rest_all, rest_up = pl.ds(k0, NBLK - k0), (pl.ds(k0 + 1, NBLK - k0 - 1), pl.ds(0, r0))
        c_wob = cp(wob_h.at[rest_up], wob_s.at[rest_up], S_GAPB)

        def start_c(b):
            start_pieces(c_h.at[b], c_s.at[b], cut_c, S_C + b)

        def pump_c(b):
            return _Pump(heads_of(c_h.at[b], c_s.at[b], i_c))

        def start_wqa():
            c_wob.start(priority=_BULK)
            start_pieces(wob_h.at[rest_all], wob_s.at[rest_all], cut_rest, S_WOB)
            start_pieces(wqa_h, wqa_s, cut_wqa, S_WQA)

        def start_k(g):
            start_pieces(k_h.at[pl.ds(g * _G, _G)], k_s.at[g], cut_k, S_KV + 2 * g, Sk - W)

        def start_v(g, cuts=cut_v):
            start_pieces(v_h.at[pl.ds(g * _G, _G)], v_s.at[g], cuts, S_KV + 2 * g + 1, Sk - W)

        def small_k(g):
            return heads_of(k_h.at[pl.ds(g * _G, _G)], k_s.at[g], i_k, Sk - W)

        def small_v(g):
            return heads_of(v_h.at[pl.ds(g * _G, _G)], v_s.at[g], i_v, Sk - W)

        def wo_at(lo, n):
            return lo // r_wo, pl.ds(lo % r_wo, n)

        def c_wo(i):
            at = wo_at(wo_off[i], wo_chunks[i])
            return cp(woa_h.at[at], woa_s.at[at], S_WO + i)

        wide = pl.ds(wo_inj, wo_wide)

        n_gap = wo_inj * r_wo - n_inj
        if n_gap:
            c_gap = cp(woa_h.at[wo_at(n_inj, n_gap)], woa_s.at[wo_at(n_inj, n_gap)], S_GAP)

        def start_wo():
            if n_gap:
                c_gap.start(priority=_BULK)
            start_pieces(woa_h.at[wide], woa_s.at[wide], cut_wo, S_WIDE)

        def small_wo():
            def one(lo, hi):
                at = wo_at(lo, hi - lo)
                return cp(woa_h.at[at], woa_s.at[at], S_INJ)
            return [functools.partial(one, lo, hi) for lo, hi in i_wo]

        def side_refs(i):
            per = r_wo // side_rows
            if isinstance(i, int):
                n = side_rows if i < side_n else side_last
                rows = (i // per, pl.ds(i % per * side_rows, n))
                return rows, side_s.at[i % side_nb, pl.ds(0, n)], i % side_nb
            slot = lax.rem(i, side_nb)
            start = pl.multiple_of(lax.rem(i, per) * side_rows, 8)
            return (lax.div(i, per), pl.ds(start, side_rows)), side_s.at[slot], slot

        def c_sa(i):
            rows, stage, slot = side_refs(i)
            return cp(wob_h.at[rows], stage, S_SA + slot)

        def c_sb(i):
            rows, stage, slot = side_refs(i)
            return cp(stage, wob_s.at[rows], S_SB + slot)

        def tick(i):
            traced = not isinstance(i, int)
            if traced or i < side_n:
                c_sa(i).wait()
                c_sb(i).start()

            def refill(j):
                if traced or i >= side_lag:
                    c_sb(i - side_lag).wait()
                c_sa(j).start()

            if traced:
                pl.when(i + side_lead < side_n)(lambda: refill(i + side_lead))
            elif i + side_lead < side_n:
                refill(i + side_lead)

        def head_major(w_s, t, hh, mid=lambda: None):
            halves = []
            for k in range(2):
                w = w_s[2 * t + k].reshape(_L // 2, Hb, Db)[:, hh * HH:(hh + 1) * HH, :]
                halves.append(w.reshape(_L // 2, HH * Db))
                if k == 0:
                    mid()
            return jnp.concatenate(halves, axis=0)

        start_pieces(wqb_h, wqb_s, cut_w0, S_WQB)
        c_xb.start()
        c_xa.start()
        for i in range(side_lead):
            c_sa(i).start()
        start_pieces(wuk_h, wuk_s, cut_w, S_WUK)
        pm = _Pump(heads_of(wuk_h, wuk_s, i_w))
        pm.pump(*cfg["pump_0"])
        pm.drain()


        wait_pieces(wqb_s, cut_w0, S_WQB)
        start_c(0)
        pm = pump_c(0)
        pm.kick()
        tick(0)
        c_xb.wait()
        xb = xb_s[...]
        halves = [None, None]
        for t in range(M // _L):
            for hh in range(2):
                part = _dot(xb[:, t * _L:(t + 1) * _L], head_major(wqb_s, t, hh, pm.kick))
                halves[hh] = part if t == 0 else halves[hh] + part
                pm.kick()
        ctxb_s[...] = jnp.concatenate(halves, axis=1)
        pm.pump(*cfg["pump_w"])
        pm.drain()

        wait_pieces(wuk_s, cut_w, S_WUK)
        start_c(1)
        pm = pump_c(1)
        pm.kick()
        tick(1)
        qb = (ctxb_s[...] * scale_b).astype(_BF16)
        for t in range(NCT):
            for hh in range(2):
                w = head_major(wuk_s, t, hh, pm.kick)
                parts = [_dot_nt(qb[:, (hh * HH + j) * Db:(hh * HH + j + 1) * Db],
                                 w[:, j * Db:(j + 1) * Db]) for j in range(HH)]
                qabs_s[t, :, hh * HH:(hh + 1) * HH, :] = jnp.concatenate(
                    parts, axis=1).reshape(B, HH, _L)
                pm.kick()
        pm.pump(*cfg["pump_w"])
        pm.drain()

        def attend_b(b, start_next, pm):
            wait_pieces(c_s.at[b], cut_c, S_C + b)
            start_next()
            pm.kick()
            tick(2 + b)
            qa = jnp.concatenate(
                [qabs_s[t, b] for t in range(NCT)], axis=1).astype(_BF16)

            def latent(k):
                tiles = c_s[b, k].reshape(k_c // 8, NCT, 8, _L)
                return jnp.concatenate(
                    [tiles[:, t].reshape(k_c, _L) for t in range(NCT)], axis=1)

            for k in range(NBLK):
                s_s[:, k * k_c:(k + 1) * k_c] = _dot_nt(qa, latent(k))
                if k in cfg["kick_s"]:
                    pm.kick()
            s = s_s[...]
            m = jnp.max(s, axis=-1, keepdims=True)
            p = jnp.exp(s - m)
            l = jnp.sum(p, axis=-1, keepdims=True)
            pb = p.astype(_BF16)
            cc = None
            for k in range(NBLK):
                part = _dot(pb[:, k * k_c:(k + 1) * k_c], latent(k))
                cc = part if cc is None else cc + part
                if k in cfg["kick_c"]:
                    pm.kick()
            cc = cc / l
            for t in range(NCT):
                ctx_s[t, b] = cc[:, t * _L:(t + 1) * _L]
            pm.pump(*cfg["pump_c"])
            pm.drain()

        small_wqa = heads_of(wqa_h, wqa_s, i_wqa)
        n_q = len(small_wqa) // 2
        for b in range(B):
            if b + 2 < B:
                attend_b(b, functools.partial(start_c, b + 2), pump_c(b + 2))
            elif b + 2 == B:
                attend_b(b, functools.partial(start_pieces, wuv_h, wuv_s, cut_w, S_WUV),
                         _Pump(heads_of(wuv_h, wuv_s, i_w)))
            else:
                attend_b(b, start_wqa, _Pump(small_wqa[:n_q] + small_k(0)))

        wait_pieces(wuv_s, cut_w, S_WUV)
        start_k(0)
        start_v(0)
        pm = _Pump(small_v(0)[:1] + small_wqa[n_q:] + small_v(0)[1:] + small_k(1))
        pm.kick()
        tick(2 + B)
        halves = [None, None]
        for t in range(NCT):
            for hh in range(2):
                ch = ctx_s[t, :, hh * HH:(hh + 1) * HH, :].reshape(B, HH * _L).astype(_BF16)
                w = head_major(wuv_s, t, hh, pm.kick)
                part = jnp.concatenate(
                    [_dot(ch[:, j * _L:(j + 1) * _L], w[:, j * Db:(j + 1) * Db])
                     for j in range(HH)], axis=1)
                halves[hh] = part if t == 0 else halves[hh] + part
                pm.kick()
        ctxb_s[...] = jnp.concatenate(halves, axis=1)
        pm.pump(*cfg["pump_uv"])
        pm.drain()

        wait_pieces(wqa_s, cut_wqa, S_WQA)
        start_k(1)
        pm = _Pump(small_v(1))
        pm.kick()
        tick(3 + B)
        c_xa.wait()
        xa = xa_s[...]
        seg = n_ct // 2
        for c0 in range(0, n_ct, seg):
            wq_tiles = wqa_s[...].reshape(D // 8, n_ct, 8, _L)
            oab_s[:, c0 * _L:(c0 + seg) * _L] = jnp.concatenate(
                [_dot(xa, wq_tiles[:, ct].reshape(D, _L)) for ct in range(c0, c0 + seg)], axis=1)
            pm.pump(1, cfg["lag"])
        qa_s[...] = (oab_s[...] * scale_a).reshape(B, H, Dh).reshape(BH, Dh)
        pm.pump(*cfg["pump_q"])
        pm.drain()

        def attend_a(g, start_at_k, start_at_v, kick, between, v_cuts=cut_v):
            start = g * _G if isinstance(g, int) else pl.multiple_of(g * _G, _G)
            rows = pl.ds(start, _G)
            q8 = qa_s[rows, :].astype(_BF16)
            wait_pieces(k_s.at[g], cut_k, S_KV + 2 * g)
            start_at_k()
            kick()
            tick(4 + B + g)
            row = lax.broadcasted_iota(jnp.int32, (_G, W), 0)
            s = None
            for j in range(_G):
                sj = _dot_nt(q8, k_s[g, j])
                s = sj if s is None else jnp.where(row == j, sj, s)
                if j in cfg["kick_qk"]:
                    kick()
            m = jnp.max(s, axis=-1, keepdims=True)
            p = jnp.exp(s - m)
            l = jnp.sum(p, axis=-1, keepdims=True)
            p_s[...] = p
            between()
            wait_pieces(v_s.at[g], v_cuts, S_KV + 2 * g + 1)
            start_at_v()
            kick()
            pb = p_s[...].astype(_BF16)
            row2 = lax.broadcasted_iota(jnp.int32, (_G, Dh), 0)
            o = None
            for j in range(_G):
                oj = _dot(pb, v_s[g, j])
                o = oj if o is None else jnp.where(row2 == j, oj, o)
                if j in cfg["kick_pv"]:
                    kick()
            oa_s[rows, :] = o / l

        def a_body(g, carry):
            pm = _Pump(small_k(g + 2) + small_v(g + 2))
            attend_a(g, functools.partial(start_v, g + 1), functools.partial(start_k, g + 2),
                     pm.kick, functools.partial(pm.pump, *cfg["pump_k"]))
            pm.pump(*cfg["pump_v"])
            pm.drain()
            return carry

        lax.fori_loop(0, NG - 2, a_body, 0)

        waited = side_n - side_nb
        n_early = side_n - cfg["side_mid"]
        r_early, r_mid = n_early * side_rows, side_n * side_rows
        pm = _Pump(small_wo())
        last = pl.ds((NG - 1) * _G, _G)
        pv = _Pump(heads_of(v_h.at[last], v_s.at[NG - 1], i_vl, Sk - W, S_INJ2))

        def project_b():
            c_wob.wait()
            wait_pieces(wob_s.at[rest_all], cut_rest, S_WOB)
            for i in range(waited, n_early):
                c_sb(i).wait()
            ctxb = ctxb_s[...].astype(_BF16)
            acc = _dot(ctxb[:, side_total:], rows_of(wob_s, side_total, Hb * Db))
            for lo in range(0, r_early, cfg["seg_b"]):
                pm.kick()
                hi = min(lo + cfg["seg_b"], r_early)
                acc = acc + _dot(ctxb[:, lo:hi], rows_of(wob_s, lo, hi))
            accb_s[...] = acc

        def start_last():
            for i in range(n_wo):
                c_wo(i).start(priority=_BULK)
            c_sa(side_n).start()

        def before_last_pv():
            pm.pump(*cfg["pump_k15"])
            pv.drain()

        attend_a(NG - 2, functools.partial(start_v, NG - 1, cut_vl), start_wo,
                 pv.kick, functools.partial(pm.pump, *cfg["pump_k14"]))
        project_b()
        pm.pump(*cfg["pump_b"])
        attend_a(NG - 1, start_last, functools.partial(pm.pump, 1, cfg["lag"]),
                 pv.kick, before_last_pv, cut_vl)
        pm.pump(1, cfg["lag"])

        oa32 = oa_s[...].reshape(B, H, Dh).reshape(B, H * Dh)
        oab_s[...] = oa32
        tail0 = H * Dh - tail_rows
        for b in range(B):
            for t in range(tail_rows // Dh):
                src = oa32[b:b + 1, tail0 + t * Dh:tail0 + (t + 1) * Dh]
                coef_s[b, t * Dh:(t + 1) * Dh, :] = jnp.broadcast_to(src, (_L, Dh)).T
        pm.pump(*cfg["pump_e"])
        c_sa(side_n).wait()
        c_sb(side_n).start()
        pm.pump(*cfg["pump_f"])
        pm.drain()
        oa = oab_s[...].astype(_BF16)
        if n_gap:
            c_gap.wait()
        n_head = wo_inj * r_wo
        acc_s[...] = _dot(oa[:, :n_head], woa_s[:wo_inj].reshape(n_head, D))
        for j in range(n_early, side_n):
            c_sb(j).wait()
        accb_s[...] += _dot(ctxb_s[:, r_early:r_mid].astype(_BF16), rows_of(wob_s, r_early, r_mid))
        wait_pieces(woa_s.at[wide], cut_wo, S_WIDE)
        acc_s[...] += _dot(oa[:, n_head:wo_base],
                           woa_s[wo_inj:wo_inj + wo_wide].reshape(wo_base - n_head, D))
        for i in range(n_mxu):
            c_wo(i).wait()
            if i == late_at:
                c_sb(side_n).wait()
                late = _dot(ctxb_s[:, r_mid:side_total].astype(_BF16),
                            rows_of(wob_s, r_mid, side_total))
                o_ref[:, D:] = (accb_s[...] + late).astype(o_ref.dtype)
            lo, n = wo_off[i], wo_chunks[i]
            part = _dot(oa[:, lo:lo + n], woa_s[wo_at(lo, n)]) + acc_s[...]
            if i < n_wo - 1:
                acc_s[...] = part
            else:
                o_ref[:, :D] = part.astype(o_ref.dtype)
        for i in range(n_mxu, n_wo):
            c_wo(i).wait()
            lo, n = wo_off[i], wo_chunks[i]
            w = woa_s[wo_at(lo, n)].astype(_F32)
            sums = []
            for b in range(B):
                cf = coef_s[b, lo - tail0:lo - tail0 + n, :]
                prod = w * jnp.concatenate([cf] * (D // _L), axis=1)
                acc = vacc_s[b] if i > n_mxu else None
                for r in range(0, n, 8):
                    acc = prod[r:r + 8] if acc is None else acc + prod[r:r + 8]
                if i < n_wo - 1:
                    vacc_s[b] = acc
                else:
                    sums.append(jnp.sum(acc, axis=0, keepdims=True))
            if i == n_wo - 1:
                res = acc_s[...] + jnp.concatenate(sums, axis=0)
                o_ref[:, :D] = res.astype(o_ref.dtype)

    any_spec = pl.BlockSpec(memory_space=pl.ANY)
    out = pl.pallas_call(
        kernel,
        out_shape=jax.ShapeDtypeStruct((B, D + M), A_x.dtype),
        in_specs=[any_spec] * 11,
        out_specs=pl.BlockSpec(memory_space=pltpu.VMEM),
        scratch_shapes=[
            pltpu.VMEM(xa2.shape, _BF16),
            pltpu.VMEM(xb2.shape, _BF16),
            pltpu.VMEM((2, NG, _G, W, Dh), _BF16),
            pltpu.VMEM((4 + B,) + wqb4.shape, _BF16),
            pltpu.VMEM((2,) + woa3.shape, _BF16),
            pltpu.VMEM((BH, Dh), _F32),
            pltpu.VMEM((BH, Dh), _F32),
            pltpu.VMEM((NCT, B, Hb, _L), _F32),
            pltpu.VMEM((NCT, B, Hb, _L), _F32),
            pltpu.VMEM((B, D), _F32),
            pltpu.VMEM((B, M), _F32),
            pltpu.VMEM((B, Hb * Db), _F32),
            pltpu.VMEM((B, H * Dh), _F32),
            pltpu.VMEM((B, max(tail_rows, 8), _L), _F32),
            pltpu.VMEM((B, 8, D), _F32),
            pltpu.VMEM((_G, W), _F32),
            pltpu.VMEM((Hb, Skb), _F32),
            pltpu.SMEM((side_nb, side_rows, M), _BF16),
            pltpu.SemaphoreType.DMA((n_sem,)),
        ],
        compiler_params=pltpu.CompilerParams(
            vmem_limit_bytes=120 * 1024 * 1024,
            disable_semaphore_checks=True,
            disable_bounds_checks=True,
        ),
        name="fused_decode",
    )(xa2, k3, v3, wqa3, woa3, xb2, c4, wqb4, wuk4, wuv4, wob3)
    return out.reshape(B, Sq, D + M)


@jax.jit
def pallas_concat_heads__sliding_block_cached__compressed_kv_cla__decode_kernel(
    A_x: jax.Array,
    A_k_cache: jax.Array,
    A_v_cache: jax.Array,
    A_wq: jax.Array,
    A_wo: jax.Array,
    B_x: jax.Array,
    B_c_kv: jax.Array,
    B_w_q: jax.Array,
    B_w_uk: jax.Array,
    B_w_uv: jax.Array,
    B_w_o: jax.Array,
):
    return _fused(_CFG, A_x, A_k_cache, A_v_cache, A_wq, A_wo,
                  B_x, B_c_kv, B_w_q, B_w_uk, B_w_uv, B_w_o)
```

```python
import functools

import jax
import jax.numpy as jnp
from jax import lax
import jax.experimental.pallas as pl
import jax.experimental.pallas.tpu as pltpu

_NT = (((1,), (1,)), ((), ()))
_F32 = jnp.float32
_BF16 = jnp.bfloat16
_L = 128
_G = 8
_KIB = 1024
_URGENT, _BULK = 0, 1

_CFG = dict(
    piece=64 * _KIB,
    block=512 * _KIB,
    shift_a=30 * _KIB,
    shift_b=34 * _KIB,
    shift_wo=32 * _KIB,
    inj_w=(18 * _KIB, 16 * _KIB, -14 * _KIB, -16 * _KIB),
    inj_c=(18 * _KIB, 16 * _KIB, -14 * _KIB, -16 * _KIB),
    inj_q=(14 * _KIB, 16 * _KIB, -18 * _KIB, -16 * _KIB),
    inj_k=(14 * _KIB, 16 * _KIB),
    inj_v=(-18 * _KIB, -16 * _KIB),
    inj_vl=(14 * _KIB, 16 * _KIB),
    inj_wo=(16 * _KIB,) * 42,
    pump_0=(28, 2),
    pump_w=(11, 3),
    pump_c=(15, 3),
    pump_uv=(20, 3),
    pump_q=(8, 2),
    pump_k=(10, 3),
    pump_v=(11, 3),
    pump_k14=(9, 21),
    pump_b=(7, 21),
    pump_k15=(8, 21),
    pump_e=(2, 21),
    pump_f=(7, 21),
    seg_b=512,
    lag=6,
    kick_s=(0, 1, 2, 3, 4, 5, 6, 7),
    kick_c=(1, 3, 5),
    kick_qk=(0, 1, 3, 5, 6),
    kick_pv=(1, 3, 5),
    side_rows=128,
    side_n=24,
    side_last=64,
    side_nb=5,
    side_mid=3,
    late_at=1,
    wo_chunks=(512, 128, 128),
    wo_tail=(80, 64, 48, 32, 16, 16),
)


def _dot(a, b):
    return jnp.dot(a, b, preferred_element_type=_F32)


def _dot_nt(a, b):
    return lax.dot_general(a, b, _NT, preferred_element_type=_F32)


def _bounds(n_rows, row_bytes, piece, shift, skip=0):
    step = piece // row_bytes
    first = (shift // row_bytes) % step
    cuts = [skip] + [r for r in range(first, n_rows, step) if r > skip] + [n_rows]
    return list(zip(cuts[:-1], cuts[1:]))


class _Pump:
    def __init__(self, copies, spin=None):
        self.copies, self.started, self.waited, self.spin = list(copies), 0, 0, spin

    def kick(self):
        if self.started < len(self.copies):
            self.copies[self.started]().start(priority=_URGENT)
            self.started += 1

    def _wait_to(self, n):
        while self.waited < n:
            self.copies[self.waited]().wait()
            self.waited += 1

    def pump(self, n, lag=1):
        for _ in range(n):
            self.kick()
            self._wait_to(self.started - lag)

    def pace(self, n, trips):
        for _ in range(n):
            self.kick()
            self._wait_to(self.started - 8)
            self.spin(trips)

    def drain(self):
        while self.started < len(self.copies):
            self.kick()
        self._wait_to(self.started)


def _fused(cfg, A_x, A_k_cache, A_v_cache, A_wq, A_wo, B_x, B_c_kv, B_w_q, B_w_uk, B_w_uv, B_w_o):
    B, Sq, D = A_x.shape
    _, H, Sk, Dh = A_k_cache.shape
    assert Sq == 1 and B_x.shape[1] == 1
    assert A_wq.shape == (D, H * Dh)
    W = min(4096, max(256, Sk // 4))
    M, Hb, Db = B_w_q.shape
    Skb, Dc = B_c_kv.shape[1], B_c_kv.shape[2]
    BH = B * H
    NG = BH // _G
    NCT = Dc // _L
    HH = Hb // 2
    scale_a = float(Dh) ** -0.5
    scale_b = float(Db) ** -0.5
    piece, block = cfg["piece"], cfg["block"]
    shift_a, shift_b = cfg["shift_a"], cfg["shift_b"]
    side_rows, side_n, side_nb = cfg["side_rows"], cfg["side_n"], cfg["side_nb"]
    late_at = cfg["late_at"]
    n_mxu = len(cfg["wo_chunks"])
    wo_chunks = tuple(cfg["wo_chunks"]) + tuple(cfg["wo_tail"])
    tail_rows = sum(cfg["wo_tail"])
    assert tail_rows % Dh == 0 and M % _L == 0 and NG >= 4
    side_lag = 2
    side_lead = side_nb - side_lag
    side_last = cfg["side_last"]
    assert side_n == 4 + B + NG and cfg["side_mid"] < side_nb and side_last > 0

    xa2 = A_x.reshape(B, D)
    xb2 = B_x.reshape(B, M)
    k3 = A_k_cache.reshape(BH, Sk, Dh)
    v3 = A_v_cache.reshape(BH, Sk, Dh)

    def blocked(w, lead=0):
        row_bytes = 2 * functools.reduce(lambda a, b: a * b, w.shape[lead + 1:], 1)
        rows = block // row_bytes
        shape = w.shape[:lead] + (w.shape[lead] // rows, rows) + w.shape[lead + 1:]
        return w.reshape(shape), rows, row_bytes

    n_ct = H * Dh // _L
    wqa_t = A_wq.reshape(D // 8, 8, n_ct, _L).transpose(0, 2, 1, 3).reshape(D * n_ct, _L)
    wqa3, r_wqa, b_wqa = blocked(wqa_t)
    wqb4, r_w, b_w = blocked(B_w_q.reshape(M * Hb, Db))
    wuk4, _, _ = blocked(B_w_uk.reshape(Dc * Hb, Db))
    wuv4, _, _ = blocked(B_w_uv.reshape(Dc * Hb, Db))
    c_t = B_c_kv.reshape(B, Skb // 8, 8, NCT, _L).transpose(0, 1, 3, 2, 4)
    c4, r_c, b_c = blocked(c_t.reshape(B, Skb * NCT, _L), 1)
    k_c = r_c // NCT
    woa3, r_wo, b_wo = blocked(A_wo)
    wob3, _, _ = blocked(B_w_o.reshape(Hb * Db, M))
    assert wob3.shape == woa3.shape and r_wo % side_rows == 0
    assert wqb4.shape == wuk4.shape == wuv4.shape and 2 * r_w == _L * Hb
    assert wqa3.shape == wqb4.shape == c4.shape[1:]
    NBLK = wqb4.shape[0]

    def spans(sizes, unit, n_rows=0):
        out, front, back = [], 0, n_rows
        for n in sizes:
            if n > 0:
                out.append((front, front + n // unit))
                front += n // unit
            else:
                out.append((back + n // unit, back))
                back += n // unit
        return out, front, back

    def split(sizes, n_rows, unit, shift):
        small, front, back = spans(sizes, unit, n_rows)
        return small, _bounds(back, unit, piece, shift, front)

    i_w, cut_w = split(cfg["inj_w"], r_w, b_w, shift_b)
    i_c, cut_c = split(cfg["inj_c"], r_c, b_c, shift_b)
    i_k, cut_k = split(cfg["inj_k"], W, 2 * Dh, shift_a)
    i_v, cut_v = split(cfg["inj_v"], W, 2 * Dh, shift_a)
    i_vl, cut_vl = split(cfg["inj_v"] + cfg["inj_vl"], W, 2 * Dh, shift_a)
    i_vl = i_vl[len(i_v):]
    i_wqa, cut_wqa = split(cfg["inj_q"], r_wqa, b_wqa, shift_a)
    i_wo, _, _ = spans(cfg["inj_wo"], 2 * D)
    cut_w0 = _bounds(r_w, b_w, piece, shift_b)
    n_inj = i_wo[-1][1]
    wo_inj = -(-n_inj // r_wo)
    wo_wide = (H * Dh - sum(wo_chunks)) // r_wo - wo_inj
    cut_wo = _bounds(r_wo, b_wo, piece, cfg["shift_wo"])
    wo_base = (wo_inj + wo_wide) * r_wo
    assert all(lo // r_wo == (hi - 1) // r_wo for lo, hi in i_wo)
    assert wo_base + sum(wo_chunks) == H * Dh
    n_wo = len(wo_chunks)
    wo_off = [wo_base + sum(wo_chunks[:i]) for i in range(n_wo)]
    assert all(lo // r_wo == (lo + n - 1) // r_wo for lo, n in zip(wo_off, wo_chunks))
    S_XB, S_XA, S_WQB, S_WUK, S_WUV, S_WOB, S_WQA, S_INJ, S_WIDE, S_GAP, S_GAPB, S_INJ2 = range(12)
    S_C = 12
    S_KV = S_C + B
    S_WO = S_KV + 2 * NG
    S_SA = S_WO + n_wo
    S_SB = S_SA + side_nb
    n_sem = S_SB + side_nb
    side_total = side_rows * side_n + side_last

    def kernel(xa_h, k_h, v_h, wqa_h, woa_h, xb_h, c_h, wqb_h, wuk_h, wuv_h, wob_h,
               o_ref,
               xa_s, xb_s, kv_s, big_s, wo_s,
               qa_s, oa_s, qabs_s, ctx_s, acc_s, accb_s, ctxb_s, oab_s, coef_s, vacc_s, p_s, s_s,
               side_s, spin_s, sem):
        def cp(src, dst, s):
            return pltpu.make_async_copy(src, dst, sem.at[s])

        def start_pieces(src, dst, cuts, s, row0=0):
            for lo, hi in cuts:
                cp(src.at[:, pl.ds(row0 + lo, hi - lo)], dst.at[:, pl.ds(lo, hi - lo)],
                   s).start(priority=_BULK)

        def wait_pieces(dst, cuts, s):
            view = dst.at[:, pl.ds(cuts[0][0], cuts[-1][1] - cuts[0][0])]
            cp(view, view, s).wait()

        def heads_of(src, dst, ranges, row0=0, s=S_INJ):
            def one(k, lo, hi):
                return cp(src.at[k, pl.ds(row0 + lo, hi - lo)], dst.at[k, pl.ds(lo, hi - lo)], s)
            return [functools.partial(one, k, lo, hi)
                    for k in range(dst.shape[0]) for lo, hi in sorted(ranges)]

        k_s, v_s = kv_s.at[0], kv_s.at[1]
        wqb_s, wuk_s, wuv_s, wqa_s = (big_s.at[j] for j in range(4))
        c_s = big_s.at[pl.ds(4, B)]
        woa_s, wob_s = wo_s.at[0], wo_s.at[1]
        c_xb = cp(xb_h, xb_s, S_XB)
        c_xa = cp(xa_h, xa_s, S_XA)

        def rows_of(ref, lo, hi):
            parts = [ref[k, max(lo - k * r_wo, 0):min(hi - k * r_wo, r_wo)]
                     for k in range(lo // r_wo, -(-hi // r_wo))]
            return parts[0] if len(parts) == 1 else jnp.concatenate(parts, axis=0)

        k0, r0 = divmod(side_total, r_wo)
        cut_rest = _bounds(r_wo, b_wo, piece, cfg["shift_wo"], r0)
        rest_all, rest_up = pl.ds(k0, NBLK - k0), (pl.ds(k0 + 1, NBLK - k0 - 1), pl.ds(0, r0))
        c_wob = cp(wob_h.at[rest_up], wob_s.at[rest_up], S_GAPB)

        def start_c(b):
            start_pieces(c_h.at[b], c_s.at[b], cut_c, S_C + b)

        def pump_c(b):
            return _Pump(heads_of(c_h.at[b], c_s.at[b], i_c))

        def start_wqa():
            c_wob.start(priority=_BULK)
            start_pieces(wob_h.at[rest_all], wob_s.at[rest_all], cut_rest, S_WOB)
            start_pieces(wqa_h, wqa_s, cut_wqa, S_WQA)

        def start_k(g):
            start_pieces(k_h.at[pl.ds(g * _G, _G)], k_s.at[g], cut_k, S_KV + 2 * g, Sk - W)

        def start_v(g, cuts=cut_v):
            start_pieces(v_h.at[pl.ds(g * _G, _G)], v_s.at[g], cuts, S_KV + 2 * g + 1, Sk - W)

        def small_k(g):
            return heads_of(k_h.at[pl.ds(g * _G, _G)], k_s.at[g], i_k, Sk - W)

        def small_v(g):
            return heads_of(v_h.at[pl.ds(g * _G, _G)], v_s.at[g], i_v, Sk - W)

        def wo_at(lo, n):
            return lo // r_wo, pl.ds(lo % r_wo, n)

        def c_wo(i):
            at = wo_at(wo_off[i], wo_chunks[i])
            return cp(woa_h.at[at], woa_s.at[at], S_WO + i)

        wide = pl.ds(wo_inj, wo_wide)

        n_gap = wo_inj * r_wo - n_inj
        if n_gap:
            c_gap = cp(woa_h.at[wo_at(n_inj, n_gap)], woa_s.at[wo_at(n_inj, n_gap)], S_GAP)

        def start_wo():
            if n_gap:
                c_gap.start(priority=_BULK)
            start_pieces(woa_h.at[wide], woa_s.at[wide], cut_wo, S_WIDE)

        def small_wo():
            def one(lo, hi):
                at = wo_at(lo, hi - lo)
                return cp(woa_h.at[at], woa_s.at[at], S_INJ)
            return [functools.partial(one, lo, hi) for lo, hi in i_wo]

        def side_refs(i):
            per = r_wo // side_rows
            if isinstance(i, int):
                n = side_rows if i < side_n else side_last
                rows = (i // per, pl.ds(i % per * side_rows, n))
                return rows, side_s.at[i % side_nb, pl.ds(0, n)], i % side_nb
            slot = lax.rem(i, side_nb)
            start = pl.multiple_of(lax.rem(i, per) * side_rows, 8)
            return (lax.div(i, per), pl.ds(start, side_rows)), side_s.at[slot], slot

        def c_sa(i):
            rows, stage, slot = side_refs(i)
            return cp(wob_h.at[rows], stage, S_SA + slot)

        def c_sb(i):
            rows, stage, slot = side_refs(i)
            return cp(stage, wob_s.at[rows], S_SB + slot)

        def tick(i):
            traced = not isinstance(i, int)
            if traced or i < side_n:
                c_sa(i).wait()
                c_sb(i).start()

            def refill(j):
                if traced or i >= side_lag:
                    c_sb(i - side_lag).wait()
                c_sa(j).start()

            if traced:
                pl.when(i + side_lead < side_n)(lambda: refill(i + side_lead))
            elif i + side_lead < side_n:
                refill(i + side_lead)

        def head_major(w_s, t, hh, mid=lambda: None):
            halves = []
            for k in range(2):
                w = w_s[2 * t + k].reshape(_L // 2, Hb, Db)[:, hh * HH:(hh + 1) * HH, :]
                halves.append(w.reshape(_L // 2, HH * Db))
                if k == 0:
                    mid()
            return jnp.concatenate(halves, axis=0)

        start_pieces(wqb_h, wqb_s, cut_w0, S_WQB)
        c_xb.start()
        c_xa.start()
        for i in range(side_lead):
            c_sa(i).start()
        start_pieces(wuk_h, wuk_s, cut_w, S_WUK)
        pm = _Pump(heads_of(wuk_h, wuk_s, i_w))
        pm.pump(*cfg["pump_0"])
        pm.drain()


        wait_pieces(wqb_s, cut_w0, S_WQB)
        start_c(0)
        pm = pump_c(0)
        pm.kick()
        tick(0)
        c_xb.wait()
        xb = xb_s[...]
        halves = [None, None]
        for t in range(M // _L):
            for hh in range(2):
                part = _dot(xb[:, t * _L:(t + 1) * _L], head_major(wqb_s, t, hh, pm.kick))
                halves[hh] = part if t == 0 else halves[hh] + part
                pm.kick()
        ctxb_s[...] = jnp.concatenate(halves, axis=1)
        pm.pump(*cfg["pump_w"])
        pm.drain()

        wait_pieces(wuk_s, cut_w, S_WUK)
        start_c(1)
        pm = pump_c(1)
        pm.kick()
        tick(1)
        qb = (ctxb_s[...] * scale_b).astype(_BF16)
        for t in range(NCT):
            for hh in range(2):
                w = head_major(wuk_s, t, hh, pm.kick)
                parts = [_dot_nt(qb[:, (hh * HH + j) * Db:(hh * HH + j + 1) * Db],
                                 w[:, j * Db:(j + 1) * Db]) for j in range(HH)]
                qabs_s[t, :, hh * HH:(hh + 1) * HH, :] = jnp.concatenate(
                    parts, axis=1).reshape(B, HH, _L)
                pm.kick()
        pm.pump(*cfg["pump_w"])
        pm.drain()

        def attend_b(b, start_next, pm):
            wait_pieces(c_s.at[b], cut_c, S_C + b)
            start_next()
            pm.kick()
            tick(2 + b)
            qa = jnp.concatenate(
                [qabs_s[t, b] for t in range(NCT)], axis=1).astype(_BF16)

            def latent(k):
                tiles = c_s[b, k].reshape(k_c // 8, NCT, 8, _L)
                return jnp.concatenate(
                    [tiles[:, t].reshape(k_c, _L) for t in range(NCT)], axis=1)

            for k in range(NBLK):
                s_s[:, k * k_c:(k + 1) * k_c] = _dot_nt(qa, latent(k))
                if k in cfg["kick_s"]:
                    pm.kick()
            s = s_s[...]
            m = jnp.max(s, axis=-1, keepdims=True)
            p = jnp.exp(s - m)
            l = jnp.sum(p, axis=-1, keepdims=True)
            pb = p.astype(_BF16)
            cc = None
            for k in range(NBLK):
                part = _dot(pb[:, k * k_c:(k + 1) * k_c], latent(k))
                cc = part if cc is None else cc + part
                if k in cfg["kick_c"]:
                    pm.kick()
            cc = cc / l
            for t in range(NCT):
                ctx_s[t, b] = cc[:, t * _L:(t + 1) * _L]
            pm.pump(*cfg["pump_c"])
            pm.drain()

        small_wqa = heads_of(wqa_h, wqa_s, i_wqa)
        n_q = len(small_wqa) // 2
        for b in range(B):
            if b + 2 < B:
                attend_b(b, functools.partial(start_c, b + 2), pump_c(b + 2))
            elif b + 2 == B:
                attend_b(b, functools.partial(start_pieces, wuv_h, wuv_s, cut_w, S_WUV),
                         _Pump(heads_of(wuv_h, wuv_s, i_w)))
            else:
                attend_b(b, start_wqa, _Pump(small_wqa[:n_q] + small_k(0)))

        wait_pieces(wuv_s, cut_w, S_WUV)
        start_k(0)
        start_v(0)
        pm = _Pump(small_v(0)[:1] + small_wqa[n_q:] + small_v(0)[1:] + small_k(1))
        pm.kick()
        tick(2 + B)
        halves = [None, None]
        for t in range(NCT):
            for hh in range(2):
                ch = ctx_s[t, :, hh * HH:(hh + 1) * HH, :].reshape(B, HH * _L).astype(_BF16)
                w = head_major(wuv_s, t, hh, pm.kick)
                part = jnp.concatenate(
                    [_dot(ch[:, j * _L:(j + 1) * _L], w[:, j * Db:(j + 1) * Db])
                     for j in range(HH)], axis=1)
                halves[hh] = part if t == 0 else halves[hh] + part
                pm.kick()
        ctxb_s[...] = jnp.concatenate(halves, axis=1)
        pm.pump(*cfg["pump_uv"])
        pm.drain()

        wait_pieces(wqa_s, cut_wqa, S_WQA)
        start_k(1)
        pm = _Pump(small_v(1))
        pm.kick()
        tick(3 + B)
        c_xa.wait()
        xa = xa_s[...]
        seg = n_ct // 2
        for c0 in range(0, n_ct, seg):
            wq_tiles = wqa_s[...].reshape(D // 8, n_ct, 8, _L)
            oab_s[:, c0 * _L:(c0 + seg) * _L] = jnp.concatenate(
                [_dot(xa, wq_tiles[:, ct].reshape(D, _L)) for ct in range(c0, c0 + seg)], axis=1)
            pm.pump(1, cfg["lag"])
        qa_s[...] = (oab_s[...] * scale_a).reshape(B, H, Dh).reshape(BH, Dh)
        pm.pump(*cfg["pump_q"])
        pm.drain()

        def attend_a(g, start_at_k, start_at_v, kick, between, v_cuts=cut_v):
            start = g * _G if isinstance(g, int) else pl.multiple_of(g * _G, _G)
            rows = pl.ds(start, _G)
            q8 = qa_s[rows, :].astype(_BF16)
            wait_pieces(k_s.at[g], cut_k, S_KV + 2 * g)
            start_at_k()
            kick()
            tick(4 + B + g)
            row = lax.broadcasted_iota(jnp.int32, (_G, W), 0)
            s = None
            for j in range(_G):
                sj = _dot_nt(q8, k_s[g, j])
                s = sj if s is None else jnp.where(row == j, sj, s)
                if j in cfg["kick_qk"]:
                    kick()
            m = jnp.max(s, axis=-1, keepdims=True)
            p = jnp.exp(s - m)
            l = jnp.sum(p, axis=-1, keepdims=True)
            p_s[...] = p
            between()
            wait_pieces(v_s.at[g], v_cuts, S_KV + 2 * g + 1)
            start_at_v()
            kick()
            pb = p_s[...].astype(_BF16)
            row2 = lax.broadcasted_iota(jnp.int32, (_G, Dh), 0)
            o = None
            for j in range(_G):
                oj = _dot(pb, v_s[g, j])
                o = oj if o is None else jnp.where(row2 == j, oj, o)
                if j in cfg["kick_pv"]:
                    kick()
            oa_s[rows, :] = o / l

        def a_body(g, carry):
            pm = _Pump(small_k(g + 2) + small_v(g + 2))
            attend_a(g, functools.partial(start_v, g + 1), functools.partial(start_k, g + 2),
                     pm.kick, functools.partial(pm.pump, *cfg["pump_k"]))
            pm.pump(*cfg["pump_v"])
            pm.drain()
            return carry

        lax.fori_loop(0, NG - 2, a_body, 0)

        waited = side_n - side_nb
        n_early = side_n - cfg["side_mid"]
        r_early, r_mid = n_early * side_rows, side_n * side_rows

        def spin(trips):
            spin_s[0] = lax.fori_loop(0, trips, lambda i, c: c * 3 + i, spin_s[0])

        spin_s[0] = 0
        pm = _Pump(small_wo(), spin)
        last = pl.ds((NG - 1) * _G, _G)
        pv = _Pump(heads_of(v_h.at[last], v_s.at[NG - 1], i_vl, Sk - W, S_INJ2))

        def project_b():
            c_wob.wait()
            wait_pieces(wob_s.at[rest_all], cut_rest, S_WOB)
            for i in range(waited, n_early):
                c_sb(i).wait()
            ctxb = ctxb_s[...].astype(_BF16)
            acc = _dot(ctxb[:, side_total:], rows_of(wob_s, side_total, Hb * Db))
            for lo in range(0, r_early, cfg["seg_b"]):
                pm.kick()
                hi = min(lo + cfg["seg_b"], r_early)
                acc = acc + _dot(ctxb[:, lo:hi], rows_of(wob_s, lo, hi))
            accb_s[...] = acc

        def start_last():
            for i in range(n_wo):
                c_wo(i).start(priority=_BULK)
            c_sa(side_n).start()

        def before_last_pv():
            pm.pace(*cfg["pump_k15"])
            pv.drain()

        attend_a(NG - 2, functools.partial(start_v, NG - 1, cut_vl), start_wo,
                 pv.kick, functools.partial(pm.pace, *cfg["pump_k14"]))
        project_b()
        pm.pace(*cfg["pump_b"])
        attend_a(NG - 1, start_last, functools.partial(pm.pump, 1, cfg["lag"]),
                 pv.kick, before_last_pv, cut_vl)
        pm.pump(1, cfg["lag"])

        oa32 = oa_s[...].reshape(B, H, Dh).reshape(B, H * Dh)
        oab_s[...] = oa32
        tail0 = H * Dh - tail_rows
        for b in range(B):
            for t in range(tail_rows // Dh):
                src = oa32[b:b + 1, tail0 + t * Dh:tail0 + (t + 1) * Dh]
                coef_s[b, t * Dh:(t + 1) * Dh, :] = jnp.broadcast_to(src, (_L, Dh)).T
        pm.pace(*cfg["pump_e"])
        c_sa(side_n).wait()
        c_sb(side_n).start()
        pm.pace(*cfg["pump_f"])
        pm.drain()
        oa = oab_s[...].astype(_BF16)
        if n_gap:
            c_gap.wait()
        n_head = wo_inj * r_wo
        acc_s[...] = _dot(oa[:, :n_head], woa_s[:wo_inj].reshape(n_head, D))
        for j in range(n_early, side_n):
            c_sb(j).wait()
        accb_s[...] += _dot(ctxb_s[:, r_early:r_mid].astype(_BF16), rows_of(wob_s, r_early, r_mid))
        wait_pieces(woa_s.at[wide], cut_wo, S_WIDE)
        acc_s[...] += _dot(oa[:, n_head:wo_base],
                           woa_s[wo_inj:wo_inj + wo_wide].reshape(wo_base - n_head, D))
        for i in range(n_mxu):
            c_wo(i).wait()
            if i == late_at:
                c_sb(side_n).wait()
                late = _dot(ctxb_s[:, r_mid:side_total].astype(_BF16),
                            rows_of(wob_s, r_mid, side_total))
                o_ref[:, D:] = (accb_s[...] + late).astype(o_ref.dtype)
            lo, n = wo_off[i], wo_chunks[i]
            part = _dot(oa[:, lo:lo + n], woa_s[wo_at(lo, n)]) + acc_s[...]
            if i < n_wo - 1:
                acc_s[...] = part
            else:
                o_ref[:, :D] = part.astype(o_ref.dtype)
        for i in range(n_mxu, n_wo):
            c_wo(i).wait()
            lo, n = wo_off[i], wo_chunks[i]
            w = woa_s[wo_at(lo, n)].astype(_F32)
            sums = []
            for b in range(B):
                cf = coef_s[b, lo - tail0:lo - tail0 + n, :]
                prod = w * jnp.concatenate([cf] * (D // _L), axis=1)
                acc = vacc_s[b] if i > n_mxu else None
                for r in range(0, n, 8):
                    acc = prod[r:r + 8] if acc is None else acc + prod[r:r + 8]
                if i < n_wo - 1:
                    vacc_s[b] = acc
                else:
                    sums.append(jnp.sum(acc, axis=0, keepdims=True))
            if i == n_wo - 1:
                res = acc_s[...] + jnp.concatenate(sums, axis=0)
                o_ref[:, :D] = res.astype(o_ref.dtype)

    any_spec = pl.BlockSpec(memory_space=pl.ANY)
    out = pl.pallas_call(
        kernel,
        out_shape=jax.ShapeDtypeStruct((B, D + M), A_x.dtype),
        in_specs=[any_spec] * 11,
        out_specs=pl.BlockSpec(memory_space=pltpu.VMEM),
        scratch_shapes=[
            pltpu.VMEM(xa2.shape, _BF16),
            pltpu.VMEM(xb2.shape, _BF16),
            pltpu.VMEM((2, NG, _G, W, Dh), _BF16),
            pltpu.VMEM((4 + B,) + wqb4.shape, _BF16),
            pltpu.VMEM((2,) + woa3.shape, _BF16),
            pltpu.VMEM((BH, Dh), _F32),
            pltpu.VMEM((BH, Dh), _F32),
            pltpu.VMEM((NCT, B, Hb, _L), _F32),
            pltpu.VMEM((NCT, B, Hb, _L), _F32),
            pltpu.VMEM((B, D), _F32),
            pltpu.VMEM((B, M), _F32),
            pltpu.VMEM((B, Hb * Db), _F32),
            pltpu.VMEM((B, H * Dh), _F32),
            pltpu.VMEM((B, max(tail_rows, 8), _L), _F32),
            pltpu.VMEM((B, 8, D), _F32),
            pltpu.VMEM((_G, W), _F32),
            pltpu.VMEM((Hb, Skb), _F32),
            pltpu.SMEM((side_nb, side_rows, M), _BF16),
            pltpu.SMEM((1,), jnp.int32),
            pltpu.SemaphoreType.DMA((n_sem,)),
        ],
        compiler_params=pltpu.CompilerParams(
            vmem_limit_bytes=120 * 1024 * 1024,
            disable_semaphore_checks=True,
            disable_bounds_checks=True,
        ),
        name="fused_decode",
    )(xa2, k3, v3, wqa3, woa3, xb2, c4, wqb4, wuk4, wuv4, wob3)
    return out.reshape(B, Sq, D + M)


@jax.jit
def pallas_concat_heads__sliding_block_cached__compressed_kv_cla__decode_kernel(
    A_x: jax.Array,
    A_k_cache: jax.Array,
    A_v_cache: jax.Array,
    A_wq: jax.Array,
    A_wo: jax.Array,
    B_x: jax.Array,
    B_c_kv: jax.Array,
    B_w_q: jax.Array,
    B_w_uk: jax.Array,
    B_w_uv: jax.Array,
    B_w_o: jax.Array,
):
    return _fused(_CFG, A_x, A_k_cache, A_v_cache, A_wq, A_wo,
                  B_x, B_c_kv, B_w_q, B_w_uk, B_w_uv, B_w_o)
```

```python
import functools

import jax
import jax.numpy as jnp
from jax import lax
import jax.experimental.pallas as pl
import jax.experimental.pallas.tpu as pltpu

_NT = (((1,), (1,)), ((), ()))
_F32 = jnp.float32
_BF16 = jnp.bfloat16
_L = 128
_G = 8
_KIB = 1024
_URGENT, _BULK = 0, 1

_CFG = dict(
    piece=64 * _KIB,
    block=512 * _KIB,
    shift_a=30 * _KIB,
    shift_b=34 * _KIB,
    inj_w=(18 * _KIB, 16 * _KIB, -14 * _KIB, -16 * _KIB),
    inj_c=(18 * _KIB, 16 * _KIB, -14 * _KIB, -16 * _KIB),
    inj_q=(14 * _KIB, 16 * _KIB, -18 * _KIB, -16 * _KIB),
    inj_k=(14 * _KIB, 16 * _KIB),
    inj_v=(-18 * _KIB, -16 * _KIB),
    inj_vl=(14 * _KIB, 16 * _KIB),
    inj_wo=(14 * _KIB,) + (16 * _KIB,) * 30 + (18 * _KIB, 14 * _KIB) + (16 * _KIB,) * 9,
    pump_0=(28, 2),
    pump_w=(11, 3),
    pump_c=(15, 3),
    pump_uv=(20, 3),
    pump_q=(8, 2),
    pump_k=(10, 3),
    pump_v=(11, 3),
    pump_k14=(9, 21),
    pump_b=(7, 21),
    pump_k15=(8, 21),
    pump_e=(2, 21),
    pump_f=(7, 21),
    seg_b=512,
    lag=6,
    kick_s=(0, 1, 2, 3, 4, 5, 6, 7),
    kick_c=(1, 3, 5),
    kick_qk=(0, 1, 3, 5, 6),
    kick_pv=(1, 3, 5),
    side_rows=128,
    side_n=24,
    side_last=64,
    side_nb=5,
    side_mid=3,
    late_at=1,
    wo_chunks=(512, 128, 128),
    wo_tail=(80, 64, 48, 32, 16, 16),
)


def _dot(a, b):
    return jnp.dot(a, b, preferred_element_type=_F32)


def _dot_nt(a, b):
    return lax.dot_general(a, b, _NT, preferred_element_type=_F32)


def _bounds(n_rows, row_bytes, piece, shift, skip=0):
    step = piece // row_bytes
    first = (shift // row_bytes) % step
    cuts = [skip] + [r for r in range(first, n_rows, step) if r > skip] + [n_rows]
    return list(zip(cuts[:-1], cuts[1:]))


class _Pump:
    def __init__(self, copies, spin=None):
        self.copies, self.started, self.waited, self.spin = list(copies), 0, 0, spin

    def kick(self):
        if self.started < len(self.copies):
            self.copies[self.started]().start(priority=_URGENT)
            self.started += 1

    def _wait_to(self, n):
        while self.waited < n:
            self.copies[self.waited]().wait()
            self.waited += 1

    def pump(self, n, lag=1):
        for _ in range(n):
            self.kick()
            self._wait_to(self.started - lag)

    def pace(self, n, trips):
        for _ in range(n):
            self.kick()
            self._wait_to(self.started - 8)
            self.spin(trips)

    def drain(self):
        while self.started < len(self.copies):
            self.kick()
        self._wait_to(self.started)


def _fused(cfg, A_x, A_k_cache, A_v_cache, A_wq, A_wo, B_x, B_c_kv, B_w_q, B_w_uk, B_w_uv, B_w_o):
    B, Sq, D = A_x.shape
    _, H, Sk, Dh = A_k_cache.shape
    assert Sq == 1 and B_x.shape[1] == 1
    assert A_wq.shape == (D, H * Dh)
    W = min(4096, max(256, Sk // 4))
    M, Hb, Db = B_w_q.shape
    Skb, Dc = B_c_kv.shape[1], B_c_kv.shape[2]
    BH = B * H
    NG = BH // _G
    NCT = Dc // _L
    HH = Hb // 2
    scale_a = float(Dh) ** -0.5
    scale_b = float(Db) ** -0.5
    piece, block = cfg["piece"], cfg["block"]
    shift_a, shift_b = cfg["shift_a"], cfg["shift_b"]
    side_rows, side_n, side_nb = cfg["side_rows"], cfg["side_n"], cfg["side_nb"]
    late_at = cfg["late_at"]
    n_mxu = len(cfg["wo_chunks"])
    wo_chunks = tuple(cfg["wo_chunks"]) + tuple(cfg["wo_tail"])
    tail_rows = sum(cfg["wo_tail"])
    assert tail_rows % Dh == 0 and M % _L == 0 and NG >= 4
    side_lag = 2
    side_lead = side_nb - side_lag
    side_last = cfg["side_last"]
    assert side_n == 4 + B + NG and cfg["side_mid"] < side_nb and side_last > 0

    xa2 = A_x.reshape(B, D)
    xb2 = B_x.reshape(B, M)
    k3 = A_k_cache.reshape(BH, Sk, Dh)
    v3 = A_v_cache.reshape(BH, Sk, Dh)

    def blocked(w, lead=0):
        row_bytes = 2 * functools.reduce(lambda a, b: a * b, w.shape[lead + 1:], 1)
        rows = block // row_bytes
        shape = w.shape[:lead] + (w.shape[lead] // rows, rows) + w.shape[lead + 1:]
        return w.reshape(shape), rows, row_bytes

    def tiles(w):
        *lead, r, c = w.shape
        n = len(lead)
        w = w.reshape(*lead, r // 8, 8, c // _L, _L).transpose(*range(n), n, n + 2, n + 1, n + 3)
        return w.reshape(*lead, r * c // _L, _L)

    n_ct = H * Dh // _L
    wqa3, r_w, b_w = blocked(tiles(A_wq))
    wqb4, _, _ = blocked(B_w_q.reshape(M * Hb, Db))
    wuk4, _, _ = blocked(B_w_uk.reshape(Dc * Hb, Db))
    wuv4, _, _ = blocked(B_w_uv.reshape(Dc * Hb, Db))
    c4, _, _ = blocked(tiles(B_c_kv), 1)
    woa3, _, _ = blocked(tiles(A_wo))
    wob3, _, _ = blocked(tiles(B_w_o.reshape(Hb * Db, M)))
    assert all(w.shape == wqa3.shape for w in (wqb4, wuk4, wuv4, woa3, wob3))
    assert c4.shape[1:] == wqa3.shape and 2 * r_w == _L * Hb and D == M == Dc
    r_m = r_w // NCT
    assert r_m % side_rows == 0
    NBLK = wqa3.shape[0]

    def spans(sizes, unit, n_rows=0):
        out, front, back = [], 0, n_rows
        for n in sizes:
            if n > 0:
                out.append((front, front + n // unit))
                front += n // unit
            else:
                out.append((back + n // unit, back))
                back += n // unit
        return out, front, back

    def split(sizes, n_rows, unit, shift):
        small, front, back = spans(sizes, unit, n_rows)
        return small, _bounds(back, unit, piece, shift, front)

    i_w, cut_w = split(cfg["inj_w"], r_w, b_w, shift_b)
    i_c, cut_c = split(cfg["inj_c"], r_w, b_w, shift_b)
    i_k, cut_k = split(cfg["inj_k"], W, 2 * Dh, shift_a)
    i_v, cut_v = split(cfg["inj_v"], W, 2 * Dh, shift_a)
    i_vl, cut_vl = split(cfg["inj_v"] + cfg["inj_vl"], W, 2 * Dh, shift_a)
    i_vl = i_vl[len(i_v):]
    i_wqa, cut_wqa = split(cfg["inj_q"], r_w, b_w, shift_a)
    i_wo, n_inj, _ = spans(cfg["inj_wo"], b_w)
    cut_w0 = _bounds(r_w, b_w, piece, shift_b)
    cut_wo = _bounds(r_w, b_w, piece, shift_a)
    wo_inj = -(-n_inj // r_w)
    wo_wide = (H * Dh - sum(wo_chunks)) // r_m - wo_inj
    wo_base = (wo_inj + wo_wide) * r_m
    assert wo_base + sum(wo_chunks) == H * Dh
    n_wo = len(wo_chunks)
    wo_off = [wo_base + sum(wo_chunks[:i]) for i in range(n_wo)]
    assert all(lo // r_m == (lo + n - 1) // r_m for lo, n in zip(wo_off, wo_chunks))
    S_XB, S_XA, S_WQB, S_WUK, S_WUV, S_WOB, S_WQA, S_INJ, S_WIDE, S_GAP, S_GAPB, S_INJ2 = range(12)
    S_C = 12
    S_KV = S_C + B
    S_WO = S_KV + 2 * NG
    S_SA = S_WO + n_wo
    S_SB = S_SA + side_nb
    n_sem = S_SB + side_nb
    side_total = side_rows * side_n + side_last

    def kernel(xa_h, k_h, v_h, wqa_h, woa_h, xb_h, c_h, wqb_h, wuk_h, wuv_h, wob_h,
               o_ref,
               xa_s, xb_s, kv_s, big_s,
               qa_s, oa_s, qabs_s, ctx_s, acc_s, accb_s, ctxb_s, oab_s, coef_s, vacc_s, p_s, s_s,
               side_s, spin_s, sem):
        def cp(src, dst, s):
            return pltpu.make_async_copy(src, dst, sem.at[s])

        def start_pieces(src, dst, cuts, s, row0=0):
            for lo, hi in cuts:
                cp(src.at[:, pl.ds(row0 + lo, hi - lo)], dst.at[:, pl.ds(lo, hi - lo)],
                   s).start(priority=_BULK)

        def wait_pieces(dst, cuts, s):
            view = dst.at[:, pl.ds(cuts[0][0], cuts[-1][1] - cuts[0][0])]
            cp(view, view, s).wait()

        def heads_of(src, dst, ranges, row0=0, s=S_INJ):
            def one(k, lo, hi):
                return cp(src.at[k, pl.ds(row0 + lo, hi - lo)], dst.at[k, pl.ds(lo, hi - lo)], s)
            return [functools.partial(one, k, lo, hi)
                    for k in range(dst.shape[0]) for lo, hi in sorted(ranges)]

        k_s, v_s = kv_s.at[0], kv_s.at[1]
        wqb_s, wuk_s, wuv_s, wqa_s, woa_s, wob_s = (big_s.at[j] for j in range(6))
        c_s = big_s.at[pl.ds(6, B)]
        c_xb = cp(xb_h, xb_s, S_XB)
        c_xa = cp(xa_h, xa_s, S_XA)

        def rows_of(ref, lo, hi, dtype=_BF16):
            parts = []
            for k in range(lo // r_m, -(-hi // r_m)):
                a, b = max(lo - k * r_m, 0), min(hi - k * r_m, r_m)
                t = ref[k, a * NCT:b * NCT].astype(dtype).reshape((b - a) // 8, NCT, 8, _L)
                parts.append(jnp.concatenate(
                    [t[:, j].reshape(b - a, _L) for j in range(NCT)], axis=1))
            return parts[0] if len(parts) == 1 else jnp.concatenate(parts, axis=0)

        k0, r0 = divmod(side_total * NCT, r_w)
        cut_rest = _bounds(r_w, b_w, piece, shift_b, r0)
        rest_all, rest_up = pl.ds(k0, NBLK - k0), (pl.ds(k0 + 1, NBLK - k0 - 1), pl.ds(0, r0))
        c_wob = cp(wob_h.at[rest_up], wob_s.at[rest_up], S_GAPB)

        def start_c(b):
            start_pieces(c_h.at[b], c_s.at[b], cut_c, S_C + b)

        def pump_c(b):
            return _Pump(heads_of(c_h.at[b], c_s.at[b], i_c))

        def start_wqa():
            c_wob.start(priority=_BULK)
            start_pieces(wob_h.at[rest_all], wob_s.at[rest_all], cut_rest, S_WOB)
            start_pieces(wqa_h, wqa_s, cut_wqa, S_WQA)

        def start_k(g):
            start_pieces(k_h.at[pl.ds(g * _G, _G)], k_s.at[g], cut_k, S_KV + 2 * g, Sk - W)

        def start_v(g, cuts=cut_v):
            start_pieces(v_h.at[pl.ds(g * _G, _G)], v_s.at[g], cuts, S_KV + 2 * g + 1, Sk - W)

        def small_k(g):
            return heads_of(k_h.at[pl.ds(g * _G, _G)], k_s.at[g], i_k, Sk - W)

        def small_v(g):
            return heads_of(v_h.at[pl.ds(g * _G, _G)], v_s.at[g], i_v, Sk - W)

        def flat_at(lo, hi):
            assert lo // r_w == (hi - 1) // r_w
            return lo // r_w, pl.ds(lo % r_w, hi - lo)

        def c_wo(i):
            at = flat_at(wo_off[i] * NCT, (wo_off[i] + wo_chunks[i]) * NCT)
            return cp(woa_h.at[at], woa_s.at[at], S_WO + i)

        wide = pl.ds(wo_inj, wo_wide)
        gap = flat_at(n_inj, wo_inj * r_w)
        c_gap = cp(woa_h.at[gap], woa_s.at[gap], S_GAP)

        def start_wo():
            c_gap.start(priority=_BULK)
            start_pieces(woa_h.at[wide], woa_s.at[wide], cut_wo, S_WIDE)

        def small_wo():
            def one(lo, hi):
                return cp(woa_h.at[flat_at(lo, hi)], woa_s.at[flat_at(lo, hi)], S_INJ)
            return [functools.partial(one, lo, hi) for lo, hi in i_wo]

        def side_refs(i):
            per, n = r_m // side_rows, side_rows * NCT
            if isinstance(i, int):
                size = n if i < side_n else side_last * NCT
                rows = (i // per, pl.ds(i % per * n, size))
                return rows, side_s.at[i % side_nb, pl.ds(0, size)], i % side_nb
            slot = lax.rem(i, side_nb)
            start = pl.multiple_of(lax.rem(i, per) * n, 8)
            return (lax.div(i, per), pl.ds(start, n)), side_s.at[slot], slot

        def c_sa(i):
            rows, stage, slot = side_refs(i)
            return cp(wob_h.at[rows], stage, S_SA + slot)

        def c_sb(i):
            rows, stage, slot = side_refs(i)
            return cp(stage, wob_s.at[rows], S_SB + slot)

        def tick(i):
            traced = not isinstance(i, int)
            if traced or i < side_n:
                c_sa(i).wait()
                c_sb(i).start()

            def refill(j):
                if traced or i >= side_lag:
                    c_sb(i - side_lag).wait()
                c_sa(j).start()

            if traced:
                pl.when(i + side_lead < side_n)(lambda: refill(i + side_lead))
            elif i + side_lead < side_n:
                refill(i + side_lead)

        def head_major(w_s, t, hh, mid=lambda: None):
            halves = []
            for k in range(2):
                w = w_s[2 * t + k].reshape(_L // 2, Hb, Db)[:, hh * HH:(hh + 1) * HH, :]
                halves.append(w.reshape(_L // 2, HH * Db))
                if k == 0:
                    mid()
            return jnp.concatenate(halves, axis=0)

        start_pieces(wqb_h, wqb_s, cut_w0, S_WQB)
        c_xb.start()
        c_xa.start()
        for i in range(side_lead):
            c_sa(i).start()
        start_pieces(wuk_h, wuk_s, cut_w, S_WUK)
        pm = _Pump(heads_of(wuk_h, wuk_s, i_w))
        pm.pump(*cfg["pump_0"])
        pm.drain()


        wait_pieces(wqb_s, cut_w0, S_WQB)
        start_c(0)
        pm = pump_c(0)
        pm.kick()
        tick(0)
        c_xb.wait()
        xb = xb_s[...]
        halves = [None, None]
        for t in range(M // _L):
            for hh in range(2):
                part = _dot(xb[:, t * _L:(t + 1) * _L], head_major(wqb_s, t, hh, pm.kick))
                halves[hh] = part if t == 0 else halves[hh] + part
                pm.kick()
        ctxb_s[...] = jnp.concatenate(halves, axis=1)
        pm.pump(*cfg["pump_w"])
        pm.drain()

        wait_pieces(wuk_s, cut_w, S_WUK)
        start_c(1)
        pm = pump_c(1)
        pm.kick()
        tick(1)
        qb = (ctxb_s[...] * scale_b).astype(_BF16)
        for t in range(NCT):
            for hh in range(2):
                w = head_major(wuk_s, t, hh, pm.kick)
                parts = [_dot_nt(qb[:, (hh * HH + j) * Db:(hh * HH + j + 1) * Db],
                                 w[:, j * Db:(j + 1) * Db]) for j in range(HH)]
                qabs_s[t, :, hh * HH:(hh + 1) * HH, :] = jnp.concatenate(
                    parts, axis=1).reshape(B, HH, _L)
                pm.kick()
        pm.pump(*cfg["pump_w"])
        pm.drain()

        def attend_b(b, start_next, pm):
            wait_pieces(c_s.at[b], cut_c, S_C + b)
            start_next()
            pm.kick()
            tick(2 + b)
            qa = jnp.concatenate(
                [qabs_s[t, b] for t in range(NCT)], axis=1).astype(_BF16)
            for k in range(NBLK):
                s_s[:, k * r_m:(k + 1) * r_m] = _dot_nt(
                    qa, rows_of(c_s.at[b], k * r_m, (k + 1) * r_m))
                if k in cfg["kick_s"]:
                    pm.kick()
            s = s_s[...]
            m = jnp.max(s, axis=-1, keepdims=True)
            p = jnp.exp(s - m)
            l = jnp.sum(p, axis=-1, keepdims=True)
            pb = p.astype(_BF16)
            cc = None
            for k in range(NBLK):
                part = _dot(pb[:, k * r_m:(k + 1) * r_m],
                            rows_of(c_s.at[b], k * r_m, (k + 1) * r_m))
                cc = part if cc is None else cc + part
                if k in cfg["kick_c"]:
                    pm.kick()
            cc = cc / l
            for t in range(NCT):
                ctx_s[t, b] = cc[:, t * _L:(t + 1) * _L]
            pm.pump(*cfg["pump_c"])
            pm.drain()

        small_wqa = heads_of(wqa_h, wqa_s, i_wqa)
        n_q = len(small_wqa) // 2
        for b in range(B):
            if b + 2 < B:
                attend_b(b, functools.partial(start_c, b + 2), pump_c(b + 2))
            elif b + 2 == B:
                attend_b(b, functools.partial(start_pieces, wuv_h, wuv_s, cut_w, S_WUV),
                         _Pump(heads_of(wuv_h, wuv_s, i_w)))
            else:
                attend_b(b, start_wqa, _Pump(small_wqa[:n_q] + small_k(0)))

        wait_pieces(wuv_s, cut_w, S_WUV)
        start_k(0)
        start_v(0)
        pm = _Pump(small_v(0)[:1] + small_wqa[n_q:] + small_v(0)[1:] + small_k(1))
        pm.kick()
        tick(2 + B)
        halves = [None, None]
        for t in range(NCT):
            for hh in range(2):
                ch = ctx_s[t, :, hh * HH:(hh + 1) * HH, :].reshape(B, HH * _L).astype(_BF16)
                w = head_major(wuv_s, t, hh, pm.kick)
                part = jnp.concatenate(
                    [_dot(ch[:, j * _L:(j + 1) * _L], w[:, j * Db:(j + 1) * Db])
                     for j in range(HH)], axis=1)
                halves[hh] = part if t == 0 else halves[hh] + part
                pm.kick()
        ctxb_s[...] = jnp.concatenate(halves, axis=1)
        pm.pump(*cfg["pump_uv"])
        pm.drain()

        wait_pieces(wqa_s, cut_wqa, S_WQA)
        start_k(1)
        pm = _Pump(small_v(1))
        pm.kick()
        tick(3 + B)
        c_xa.wait()
        xa = xa_s[...]
        seg = n_ct // 2
        for c0 in range(0, n_ct, seg):
            wq_tiles = wqa_s[...].reshape(D // 8, n_ct, 8, _L)
            oab_s[:, c0 * _L:(c0 + seg) * _L] = jnp.concatenate(
                [_dot(xa, wq_tiles[:, ct].reshape(D, _L)) for ct in range(c0, c0 + seg)], axis=1)
            pm.pump(1, cfg["lag"])
        qa_s[...] = (oab_s[...] * scale_a).reshape(B, H, Dh).reshape(BH, Dh)
        pm.pump(*cfg["pump_q"])
        pm.drain()

        def attend_a(g, start_at_k, start_at_v, kick, between, v_cuts=cut_v):
            start = g * _G if isinstance(g, int) else pl.multiple_of(g * _G, _G)
            rows = pl.ds(start, _G)
            q8 = qa_s[rows, :].astype(_BF16)
            wait_pieces(k_s.at[g], cut_k, S_KV + 2 * g)
            start_at_k()
            kick()
            tick(4 + B + g)
            row = lax.broadcasted_iota(jnp.int32, (_G, W), 0)
            s = None
            for j in range(_G):
                sj = _dot_nt(q8, k_s[g, j])
                s = sj if s is None else jnp.where(row == j, sj, s)
                if j in cfg["kick_qk"]:
                    kick()
            m = jnp.max(s, axis=-1, keepdims=True)
            p = jnp.exp(s - m)
            l = jnp.sum(p, axis=-1, keepdims=True)
            p_s[...] = p
            between()
            wait_pieces(v_s.at[g], v_cuts, S_KV + 2 * g + 1)
            start_at_v()
            kick()
            pb = p_s[...].astype(_BF16)
            row2 = lax.broadcasted_iota(jnp.int32, (_G, Dh), 0)
            o = None
            for j in range(_G):
                oj = _dot(pb, v_s[g, j])
                o = oj if o is None else jnp.where(row2 == j, oj, o)
                if j in cfg["kick_pv"]:
                    kick()
            oa_s[rows, :] = o / l

        def a_body(g, carry):
            pm = _Pump(small_k(g + 2) + small_v(g + 2))
            attend_a(g, functools.partial(start_v, g + 1), functools.partial(start_k, g + 2),
                     pm.kick, functools.partial(pm.pump, *cfg["pump_k"]))
            pm.pump(*cfg["pump_v"])
            pm.drain()
            return carry

        lax.fori_loop(0, NG - 2, a_body, 0)

        waited = side_n - side_nb
        n_early = side_n - cfg["side_mid"]
        r_early, r_mid = n_early * side_rows, side_n * side_rows

        def spin(trips):
            spin_s[0] = lax.fori_loop(0, trips, lambda i, c: c * 3 + i, spin_s[0])

        spin_s[0] = 0
        pm = _Pump(small_wo(), spin)
        last = pl.ds((NG - 1) * _G, _G)
        pv = _Pump(heads_of(v_h.at[last], v_s.at[NG - 1], i_vl, Sk - W, S_INJ2))

        def project_b():
            c_wob.wait()
            wait_pieces(wob_s.at[rest_all], cut_rest, S_WOB)
            for i in range(waited, n_early):
                c_sb(i).wait()
            ctxb = ctxb_s[...].astype(_BF16)
            acc = _dot(ctxb[:, side_total:], rows_of(wob_s, side_total, Hb * Db))
            for lo in range(0, r_early, cfg["seg_b"]):
                pm.kick()
                hi = min(lo + cfg["seg_b"], r_early)
                acc = acc + _dot(ctxb[:, lo:hi], rows_of(wob_s, lo, hi))
            accb_s[...] = acc

        def start_last():
            for i in range(n_wo):
                c_wo(i).start(priority=_BULK)
            c_sa(side_n).start()

        def before_last_pv():
            pm.pace(*cfg["pump_k15"])
            pv.drain()

        attend_a(NG - 2, functools.partial(start_v, NG - 1, cut_vl), start_wo,
                 pv.kick, functools.partial(pm.pace, *cfg["pump_k14"]))
        project_b()
        pm.pace(*cfg["pump_b"])
        attend_a(NG - 1, start_last, functools.partial(pm.pump, 1, cfg["lag"]),
                 pv.kick, before_last_pv, cut_vl)
        pm.pump(1, cfg["lag"])

        oa32 = oa_s[...].reshape(B, H, Dh).reshape(B, H * Dh)
        oab_s[...] = oa32
        tail0 = H * Dh - tail_rows
        for b in range(B):
            for t in range(tail_rows // Dh):
                src = oa32[b:b + 1, tail0 + t * Dh:tail0 + (t + 1) * Dh]
                coef_s[b, t * Dh:(t + 1) * Dh, :] = jnp.broadcast_to(src, (_L, Dh)).T
        pm.pace(*cfg["pump_e"])
        c_sa(side_n).wait()
        c_sb(side_n).start()
        pm.pace(*cfg["pump_f"])
        pm.drain()
        oa = oab_s[...].astype(_BF16)
        c_gap.wait()
        n_head = wo_inj * r_m
        acc_s[...] = _dot(oa[:, :n_head], rows_of(woa_s, 0, n_head))
        for j in range(n_early, side_n):
            c_sb(j).wait()
        accb_s[...] += _dot(ctxb_s[:, r_early:r_mid].astype(_BF16), rows_of(wob_s, r_early, r_mid))
        wait_pieces(woa_s.at[wide], cut_wo, S_WIDE)
        acc_s[...] += _dot(oa[:, n_head:wo_base], rows_of(woa_s, n_head, wo_base))
        for i in range(n_mxu):
            c_wo(i).wait()
            if i == late_at:
                c_sb(side_n).wait()
                late = _dot(ctxb_s[:, r_mid:side_total].astype(_BF16),
                            rows_of(wob_s, r_mid, side_total))
                o_ref[:, D:] = (accb_s[...] + late).astype(o_ref.dtype)
            lo, n = wo_off[i], wo_chunks[i]
            part = _dot(oa[:, lo:lo + n], rows_of(woa_s, lo, lo + n)) + acc_s[...]
            if i < n_wo - 1:
                acc_s[...] = part
            else:
                o_ref[:, :D] = part.astype(o_ref.dtype)
        for i in range(n_mxu, n_wo):
            c_wo(i).wait()
            lo, n = wo_off[i], wo_chunks[i]
            w = rows_of(woa_s, lo, lo + n, _F32)
            sums = []
            for b in range(B):
                cf = coef_s[b, lo - tail0:lo - tail0 + n, :]
                prod = w * jnp.concatenate([cf] * (D // _L), axis=1)
                acc = vacc_s[b] if i > n_mxu else None
                for r in range(0, n, 8):
                    acc = prod[r:r + 8] if acc is None else acc + prod[r:r + 8]
                if i < n_wo - 1:
                    vacc_s[b] = acc
                else:
                    sums.append(jnp.sum(acc, axis=0, keepdims=True))
            if i == n_wo - 1:
                res = acc_s[...] + jnp.concatenate(sums, axis=0)
                o_ref[:, :D] = res.astype(o_ref.dtype)

    any_spec = pl.BlockSpec(memory_space=pl.ANY)
    out = pl.pallas_call(
        kernel,
        out_shape=jax.ShapeDtypeStruct((B, D + M), A_x.dtype),
        in_specs=[any_spec] * 11,
        out_specs=pl.BlockSpec(memory_space=pltpu.VMEM),
        scratch_shapes=[
            pltpu.VMEM(xa2.shape, _BF16),
            pltpu.VMEM(xb2.shape, _BF16),
            pltpu.VMEM((2, NG, _G, W, Dh), _BF16),
            pltpu.VMEM((6 + B,) + wqa3.shape, _BF16),
            pltpu.VMEM((BH, Dh), _F32),
            pltpu.VMEM((BH, Dh), _F32),
            pltpu.VMEM((NCT, B, Hb, _L), _F32),
            pltpu.VMEM((NCT, B, Hb, _L), _F32),
            pltpu.VMEM((B, D), _F32),
            pltpu.VMEM((B, M), _F32),
            pltpu.VMEM((B, Hb * Db), _F32),
            pltpu.VMEM((B, H * Dh), _F32),
            pltpu.VMEM((B, max(tail_rows, 8), _L), _F32),
            pltpu.VMEM((B, 8, D), _F32),
            pltpu.VMEM((_G, W), _F32),
            pltpu.VMEM((Hb, Skb), _F32),
            pltpu.SMEM((side_nb, side_rows * NCT, _L), _BF16),
            pltpu.SMEM((1,), jnp.int32),
            pltpu.SemaphoreType.DMA((n_sem,)),
        ],
        compiler_params=pltpu.CompilerParams(
            vmem_limit_bytes=120 * 1024 * 1024,
            disable_semaphore_checks=True,
            disable_bounds_checks=True,
        ),
        name="fused_decode",
    )(xa2, k3, v3, wqa3, woa3, xb2, c4, wqb4, wuk4, wuv4, wob3)
    return out.reshape(B, Sq, D + M)


@jax.jit
def pallas_concat_heads__sliding_block_cached__compressed_kv_cla__decode_kernel(
    A_x: jax.Array,
    A_k_cache: jax.Array,
    A_v_cache: jax.Array,
    A_wq: jax.Array,
    A_wo: jax.Array,
    B_x: jax.Array,
    B_c_kv: jax.Array,
    B_w_q: jax.Array,
    B_w_uk: jax.Array,
    B_w_uv: jax.Array,
    B_w_o: jax.Array,
):
    return _fused(_CFG, A_x, A_k_cache, A_v_cache, A_wq, A_wo,
                  B_x, B_c_kv, B_w_q, B_w_uk, B_w_uv, B_w_o)
```

```python
import functools

import jax
import jax.numpy as jnp
from jax import lax
import jax.experimental.pallas as pl
import jax.experimental.pallas.tpu as pltpu

_NT = (((1,), (1,)), ((), ()))
_F32 = jnp.float32
_BF16 = jnp.bfloat16
_L = 128
_G = 8
_KIB = 1024
_URGENT, _BULK = 0, 1

_CFG = dict(
    piece=64 * _KIB,
    block=512 * _KIB,
    shift_a=30 * _KIB,
    shift_b=34 * _KIB,
    inj_w=(18 * _KIB, 16 * _KIB, -14 * _KIB, -16 * _KIB),
    inj_c=(18 * _KIB, 16 * _KIB, -14 * _KIB, -16 * _KIB),
    inj_q=(14 * _KIB, 16 * _KIB, -18 * _KIB, -16 * _KIB),
    inj_k=(14 * _KIB, 16 * _KIB),
    inj_v=(-18 * _KIB, -16 * _KIB),
    inj_vl=(14 * _KIB, 16 * _KIB),
    inj_wo=(2 * _KIB,) + (4 * _KIB,) * 120,
    pump_0=(28, 2),
    pump_w=(11, 3),
    pump_c=(15, 3),
    pump_uv=(20, 3),
    pump_q=(8, 2),
    pump_k=(10, 3),
    pump_v=(11, 3),
    pump_k14=(28, 5, 14),
    pump_b=(21, 5, 14),
    pump_k15=(25, 5, 14),
    pump_e=(6, 5, 14),
    pump_f=(24, 5, 14),
    seg_b=256,
    lag=10,
    kick_s=(0, 1, 2, 3, 4, 5, 6, 7),
    kick_c=(1, 3, 5),
    kick_qk=(0, 1, 3, 5, 6),
    kick_pv=(1, 3, 5),
    side_rows=128,
    side_n=24,
    side_last=64,
    side_nb=5,
    side_mid=3,
    late_at=1,
    wo_chunks=(512, 128, 128),
    wo_tail=(80, 64, 48, 32, 16, 16),
)


def _dot(a, b):
    return jnp.dot(a, b, preferred_element_type=_F32)


def _dot_nt(a, b):
    return lax.dot_general(a, b, _NT, preferred_element_type=_F32)


def _bounds(n_rows, row_bytes, piece, shift, skip=0):
    step = piece // row_bytes
    first = (shift // row_bytes) % step
    cuts = [skip] + [r for r in range(first, n_rows, step) if r > skip] + [n_rows]
    return list(zip(cuts[:-1], cuts[1:]))


class _Pump:
    def __init__(self, copies, spin=None):
        self.copies, self.started, self.waited, self.spin = list(copies), 0, 0, spin

    def kick(self):
        if self.started < len(self.copies):
            self.copies[self.started]().start(priority=_URGENT)
            self.started += 1

    def _wait_to(self, n):
        while self.waited < n:
            self.copies[self.waited]().wait()
            self.waited += 1

    def pump(self, n, lag=1):
        for _ in range(n):
            self.kick()
            self._wait_to(self.started - lag)

    def pace(self, n, trips, lag=8):
        for _ in range(n):
            self.kick()
            self._wait_to(self.started - lag)
            self.spin(trips)

    def drain(self):
        while self.started < len(self.copies):
            self.kick()
        self._wait_to(self.started)


def _fused(cfg, A_x, A_k_cache, A_v_cache, A_wq, A_wo, B_x, B_c_kv, B_w_q, B_w_uk, B_w_uv, B_w_o):
    B, Sq, D = A_x.shape
    _, H, Sk, Dh = A_k_cache.shape
    assert Sq == 1 and B_x.shape[1] == 1
    assert A_wq.shape == (D, H * Dh)
    W = min(4096, max(256, Sk // 4))
    M, Hb, Db = B_w_q.shape
    Skb, Dc = B_c_kv.shape[1], B_c_kv.shape[2]
    BH = B * H
    NG = BH // _G
    NCT = Dc // _L
    HH = Hb // 2
    scale_a = float(Dh) ** -0.5
    scale_b = float(Db) ** -0.5
    piece, block = cfg["piece"], cfg["block"]
    shift_a, shift_b = cfg["shift_a"], cfg["shift_b"]
    side_rows, side_n, side_nb = cfg["side_rows"], cfg["side_n"], cfg["side_nb"]
    late_at = cfg["late_at"]
    n_mxu = len(cfg["wo_chunks"])
    wo_chunks = tuple(cfg["wo_chunks"]) + tuple(cfg["wo_tail"])
    tail_rows = sum(cfg["wo_tail"])
    assert tail_rows % Dh == 0 and M % _L == 0 and NG >= 4
    side_lag = 2
    side_lead = side_nb - side_lag
    side_last = cfg["side_last"]
    assert side_n == 4 + B + NG and cfg["side_mid"] < side_nb and side_last > 0

    xa2 = A_x.reshape(B, D)
    xb2 = B_x.reshape(B, M)
    k3 = A_k_cache.reshape(BH, Sk, Dh)
    v3 = A_v_cache.reshape(BH, Sk, Dh)

    def blocked(w, lead=0):
        row_bytes = 2 * functools.reduce(lambda a, b: a * b, w.shape[lead + 1:], 1)
        rows = block // row_bytes
        shape = w.shape[:lead] + (w.shape[lead] // rows, rows) + w.shape[lead + 1:]
        return w.reshape(shape), rows, row_bytes

    def tiles(w):
        *lead, r, c = w.shape
        n = len(lead)
        w = w.reshape(*lead, r // 8, 8, c // _L, _L).transpose(*range(n), n, n + 2, n + 1, n + 3)
        return w.reshape(*lead, r * c // _L, _L)

    n_ct = H * Dh // _L
    wqa3, r_w, b_w = blocked(tiles(A_wq))
    wqb4, _, _ = blocked(B_w_q.reshape(M * Hb, Db))
    wuk4, _, _ = blocked(B_w_uk.reshape(Dc * Hb, Db))
    wuv4, _, _ = blocked(B_w_uv.reshape(Dc * Hb, Db))
    c4, _, _ = blocked(tiles(B_c_kv), 1)
    woa3, _, _ = blocked(tiles(A_wo))
    wob3, _, _ = blocked(tiles(B_w_o.reshape(Hb * Db, M)))
    assert all(w.shape == wqa3.shape for w in (wqb4, wuk4, wuv4, woa3, wob3))
    assert c4.shape[1:] == wqa3.shape and 2 * r_w == _L * Hb and D == M == Dc
    r_m = r_w // NCT
    assert r_m % side_rows == 0
    NBLK = wqa3.shape[0]

    def spans(sizes, unit, n_rows=0):
        out, front, back = [], 0, n_rows
        for n in sizes:
            if n > 0:
                out.append((front, front + n // unit))
                front += n // unit
            else:
                out.append((back + n // unit, back))
                back += n // unit
        return out, front, back

    def split(sizes, n_rows, unit, shift):
        small, front, back = spans(sizes, unit, n_rows)
        return small, _bounds(back, unit, piece, shift, front)

    i_w, cut_w = split(cfg["inj_w"], r_w, b_w, shift_b)
    i_c, cut_c = split(cfg["inj_c"], r_w, b_w, shift_b)
    i_k, cut_k = split(cfg["inj_k"], W, 2 * Dh, shift_a)
    i_v, cut_v = split(cfg["inj_v"], W, 2 * Dh, shift_a)
    i_vl, cut_vl = split(cfg["inj_v"] + cfg["inj_vl"], W, 2 * Dh, shift_a)
    i_vl = i_vl[len(i_v):]
    i_wqa, cut_wqa = split(cfg["inj_q"], r_w, b_w, shift_a)
    i_wo, n_inj, _ = spans(cfg["inj_wo"], b_w)
    cut_w0 = _bounds(r_w, b_w, piece, shift_b)
    cut_wo = _bounds(r_w, b_w, piece, shift_a)
    wo_inj = -(-n_inj // r_w)
    wo_wide = (H * Dh - sum(wo_chunks)) // r_m - wo_inj
    wo_base = (wo_inj + wo_wide) * r_m
    assert wo_base + sum(wo_chunks) == H * Dh
    n_wo = len(wo_chunks)
    wo_off = [wo_base + sum(wo_chunks[:i]) for i in range(n_wo)]
    assert all(lo // r_m == (lo + n - 1) // r_m for lo, n in zip(wo_off, wo_chunks))
    S_XB, S_XA, S_WQB, S_WUK, S_WUV, S_WOB, S_WQA, S_INJ, S_WIDE, S_GAP, S_GAPB, S_INJ2 = range(12)
    S_C = 12
    S_KV = S_C + B
    S_WO = S_KV + 2 * NG
    S_SA = S_WO + n_wo
    S_SB = S_SA + side_nb
    n_sem = S_SB + side_nb
    side_total = side_rows * side_n + side_last

    def kernel(xa_h, k_h, v_h, wqa_h, woa_h, xb_h, c_h, wqb_h, wuk_h, wuv_h, wob_h,
               o_ref,
               xa_s, xb_s, kv_s, big_s,
               qa_s, oa_s, qabs_s, ctx_s, acc_s, accb_s, ctxb_s, oab_s, coef_s, vacc_s, p_s, s_s,
               side_s, spin_s, sem):
        def cp(src, dst, s):
            return pltpu.make_async_copy(src, dst, sem.at[s])

        def start_pieces(src, dst, cuts, s, row0=0):
            for lo, hi in cuts:
                cp(src.at[:, pl.ds(row0 + lo, hi - lo)], dst.at[:, pl.ds(lo, hi - lo)],
                   s).start(priority=_BULK)

        def wait_pieces(dst, cuts, s):
            view = dst.at[:, pl.ds(cuts[0][0], cuts[-1][1] - cuts[0][0])]
            cp(view, view, s).wait()

        def heads_of(src, dst, ranges, row0=0, s=S_INJ):
            def one(k, lo, hi):
                return cp(src.at[k, pl.ds(row0 + lo, hi - lo)], dst.at[k, pl.ds(lo, hi - lo)], s)
            return [functools.partial(one, k, lo, hi)
                    for k in range(dst.shape[0]) for lo, hi in sorted(ranges)]

        k_s, v_s = kv_s.at[0], kv_s.at[1]
        wqb_s, wuk_s, wuv_s, wqa_s, woa_s, wob_s = (big_s.at[j] for j in range(6))
        c_s = big_s.at[pl.ds(6, B)]
        c_xb = cp(xb_h, xb_s, S_XB)
        c_xa = cp(xa_h, xa_s, S_XA)

        def rows_of(ref, lo, hi, dtype=_BF16):
            parts = []
            for k in range(lo // r_m, -(-hi // r_m)):
                a, b = max(lo - k * r_m, 0), min(hi - k * r_m, r_m)
                t = ref[k, a * NCT:b * NCT].astype(dtype).reshape((b - a) // 8, NCT, 8, _L)
                parts.append(jnp.concatenate(
                    [t[:, j].reshape(b - a, _L) for j in range(NCT)], axis=1))
            return parts[0] if len(parts) == 1 else jnp.concatenate(parts, axis=0)

        k0, r0 = divmod(side_total * NCT, r_w)
        cut_rest = _bounds(r_w, b_w, piece, shift_b, r0)
        rest_all, rest_up = pl.ds(k0, NBLK - k0), (pl.ds(k0 + 1, NBLK - k0 - 1), pl.ds(0, r0))
        c_wob = cp(wob_h.at[rest_up], wob_s.at[rest_up], S_GAPB)

        def start_c(b):
            start_pieces(c_h.at[b], c_s.at[b], cut_c, S_C + b)

        def pump_c(b):
            return _Pump(heads_of(c_h.at[b], c_s.at[b], i_c))

        def start_wqa():
            c_wob.start(priority=_BULK)
            start_pieces(wob_h.at[rest_all], wob_s.at[rest_all], cut_rest, S_WOB)
            start_pieces(wqa_h, wqa_s, cut_wqa, S_WQA)

        def start_k(g):
            start_pieces(k_h.at[pl.ds(g * _G, _G)], k_s.at[g], cut_k, S_KV + 2 * g, Sk - W)

        def start_v(g, cuts=cut_v):
            start_pieces(v_h.at[pl.ds(g * _G, _G)], v_s.at[g], cuts, S_KV + 2 * g + 1, Sk - W)

        def small_k(g):
            return heads_of(k_h.at[pl.ds(g * _G, _G)], k_s.at[g], i_k, Sk - W)

        def small_v(g):
            return heads_of(v_h.at[pl.ds(g * _G, _G)], v_s.at[g], i_v, Sk - W)

        def flat_at(lo, hi):
            assert lo // r_w == (hi - 1) // r_w
            return lo // r_w, pl.ds(lo % r_w, hi - lo)

        def c_wo(i):
            at = flat_at(wo_off[i] * NCT, (wo_off[i] + wo_chunks[i]) * NCT)
            return cp(woa_h.at[at], woa_s.at[at], S_WO + i)

        wide = pl.ds(wo_inj, wo_wide)
        gap = flat_at(n_inj, wo_inj * r_w)
        c_gap = cp(woa_h.at[gap], woa_s.at[gap], S_GAP)

        def start_wo():
            c_gap.start(priority=_BULK)
            start_pieces(woa_h.at[wide], woa_s.at[wide], cut_wo, S_WIDE)

        def small_wo():
            def one(lo, hi):
                return cp(woa_h.at[flat_at(lo, hi)], woa_s.at[flat_at(lo, hi)], S_INJ)
            return [functools.partial(one, lo, hi) for lo, hi in i_wo]

        def side_refs(i):
            per, n = r_m // side_rows, side_rows * NCT
            if isinstance(i, int):
                size = n if i < side_n else side_last * NCT
                rows = (i // per, pl.ds(i % per * n, size))
                return rows, side_s.at[i % side_nb, pl.ds(0, size)], i % side_nb
            slot = lax.rem(i, side_nb)
            start = pl.multiple_of(lax.rem(i, per) * n, 8)
            return (lax.div(i, per), pl.ds(start, n)), side_s.at[slot], slot

        def c_sa(i):
            rows, stage, slot = side_refs(i)
            return cp(wob_h.at[rows], stage, S_SA + slot)

        def c_sb(i):
            rows, stage, slot = side_refs(i)
            return cp(stage, wob_s.at[rows], S_SB + slot)

        def tick(i):
            traced = not isinstance(i, int)
            if traced or i < side_n:
                c_sa(i).wait()
                c_sb(i).start()

            def refill(j):
                if traced or i >= side_lag:
                    c_sb(i - side_lag).wait()
                c_sa(j).start()

            if traced:
                pl.when(i + side_lead < side_n)(lambda: refill(i + side_lead))
            elif i + side_lead < side_n:
                refill(i + side_lead)

        def head_major(w_s, t, hh, mid=lambda: None):
            halves = []
            for k in range(2):
                w = w_s[2 * t + k].reshape(_L // 2, Hb, Db)[:, hh * HH:(hh + 1) * HH, :]
                halves.append(w.reshape(_L // 2, HH * Db))
                if k == 0:
                    mid()
            return jnp.concatenate(halves, axis=0)

        start_pieces(wqb_h, wqb_s, cut_w0, S_WQB)
        c_xb.start()
        c_xa.start()
        for i in range(side_lead):
            c_sa(i).start()
        start_pieces(wuk_h, wuk_s, cut_w, S_WUK)
        pm = _Pump(heads_of(wuk_h, wuk_s, i_w))
        pm.pump(*cfg["pump_0"])
        pm.drain()


        wait_pieces(wqb_s, cut_w0, S_WQB)
        start_c(0)
        pm = pump_c(0)
        pm.kick()
        tick(0)
        c_xb.wait()
        xb = xb_s[...]
        halves = [None, None]
        for t in range(M // _L):
            for hh in range(2):
                part = _dot(xb[:, t * _L:(t + 1) * _L], head_major(wqb_s, t, hh, pm.kick))
                halves[hh] = part if t == 0 else halves[hh] + part
                pm.kick()
        ctxb_s[...] = jnp.concatenate(halves, axis=1)
        pm.pump(*cfg["pump_w"])
        pm.drain()

        wait_pieces(wuk_s, cut_w, S_WUK)
        start_c(1)
        pm = pump_c(1)
        pm.kick()
        tick(1)
        qb = (ctxb_s[...] * scale_b).astype(_BF16)
        for t in range(NCT):
            for hh in range(2):
                w = head_major(wuk_s, t, hh, pm.kick)
                parts = [_dot_nt(qb[:, (hh * HH + j) * Db:(hh * HH + j + 1) * Db],
                                 w[:, j * Db:(j + 1) * Db]) for j in range(HH)]
                qabs_s[t, :, hh * HH:(hh + 1) * HH, :] = jnp.concatenate(
                    parts, axis=1).reshape(B, HH, _L)
                pm.kick()
        pm.pump(*cfg["pump_w"])
        pm.drain()

        def attend_b(b, start_next, pm):
            wait_pieces(c_s.at[b], cut_c, S_C + b)
            start_next()
            pm.kick()
            tick(2 + b)
            qa = jnp.concatenate(
                [qabs_s[t, b] for t in range(NCT)], axis=1).astype(_BF16)
            for k in range(NBLK):
                s_s[:, k * r_m:(k + 1) * r_m] = _dot_nt(
                    qa, rows_of(c_s.at[b], k * r_m, (k + 1) * r_m))
                if k in cfg["kick_s"]:
                    pm.kick()
            s = s_s[...]
            m = jnp.max(s, axis=-1, keepdims=True)
            p = jnp.exp(s - m)
            l = jnp.sum(p, axis=-1, keepdims=True)
            pb = p.astype(_BF16)
            cc = None
            for k in range(NBLK):
                part = _dot(pb[:, k * r_m:(k + 1) * r_m],
                            rows_of(c_s.at[b], k * r_m, (k + 1) * r_m))
                cc = part if cc is None else cc + part
                if k in cfg["kick_c"]:
                    pm.kick()
            cc = cc / l
            for t in range(NCT):
                ctx_s[t, b] = cc[:, t * _L:(t + 1) * _L]
            pm.pump(*cfg["pump_c"])
            pm.drain()

        small_wqa = heads_of(wqa_h, wqa_s, i_wqa)
        n_q = len(small_wqa) // 2
        for b in range(B):
            if b + 2 < B:
                attend_b(b, functools.partial(start_c, b + 2), pump_c(b + 2))
            elif b + 2 == B:
                attend_b(b, functools.partial(start_pieces, wuv_h, wuv_s, cut_w, S_WUV),
                         _Pump(heads_of(wuv_h, wuv_s, i_w)))
            else:
                attend_b(b, start_wqa, _Pump(small_wqa[:n_q] + small_k(0)))

        wait_pieces(wuv_s, cut_w, S_WUV)
        start_k(0)
        start_v(0)
        pm = _Pump(small_v(0)[:1] + small_wqa[n_q:] + small_v(0)[1:] + small_k(1))
        pm.kick()
        tick(2 + B)
        halves = [None, None]
        for t in range(NCT):
            for hh in range(2):
                ch = ctx_s[t, :, hh * HH:(hh + 1) * HH, :].reshape(B, HH * _L).astype(_BF16)
                w = head_major(wuv_s, t, hh, pm.kick)
                part = jnp.concatenate(
                    [_dot(ch[:, j * _L:(j + 1) * _L], w[:, j * Db:(j + 1) * Db])
                     for j in range(HH)], axis=1)
                halves[hh] = part if t == 0 else halves[hh] + part
                pm.kick()
        ctxb_s[...] = jnp.concatenate(halves, axis=1)
        pm.pump(*cfg["pump_uv"])
        pm.drain()

        wait_pieces(wqa_s, cut_wqa, S_WQA)
        start_k(1)
        pm = _Pump(small_v(1))
        pm.kick()
        tick(3 + B)
        c_xa.wait()
        xa = xa_s[...]
        seg = n_ct // 2
        for c0 in range(0, n_ct, seg):
            wq_tiles = wqa_s[...].reshape(D // 8, n_ct, 8, _L)
            oab_s[:, c0 * _L:(c0 + seg) * _L] = jnp.concatenate(
                [_dot(xa, wq_tiles[:, ct].reshape(D, _L)) for ct in range(c0, c0 + seg)], axis=1)
            pm.pump(1, cfg["lag"])
        qa_s[...] = (oab_s[...] * scale_a).reshape(B, H, Dh).reshape(BH, Dh)
        pm.pump(*cfg["pump_q"])
        pm.drain()

        def attend_a(g, start_at_k, start_at_v, kick, between, v_cuts=cut_v):
            start = g * _G if isinstance(g, int) else pl.multiple_of(g * _G, _G)
            rows = pl.ds(start, _G)
            q8 = qa_s[rows, :].astype(_BF16)
            wait_pieces(k_s.at[g], cut_k, S_KV + 2 * g)
            start_at_k()
            kick()
            tick(4 + B + g)
            row = lax.broadcasted_iota(jnp.int32, (_G, W), 0)
            s = None
            for j in range(_G):
                sj = _dot_nt(q8, k_s[g, j])
                s = sj if s is None else jnp.where(row == j, sj, s)
                if j in cfg["kick_qk"]:
                    kick()
            m = jnp.max(s, axis=-1, keepdims=True)
            p = jnp.exp(s - m)
            l = jnp.sum(p, axis=-1, keepdims=True)
            p_s[...] = p
            between()
            wait_pieces(v_s.at[g], v_cuts, S_KV + 2 * g + 1)
            start_at_v()
            kick()
            pb = p_s[...].astype(_BF16)
            row2 = lax.broadcasted_iota(jnp.int32, (_G, Dh), 0)
            o = None
            for j in range(_G):
                oj = _dot(pb, v_s[g, j])
                o = oj if o is None else jnp.where(row2 == j, oj, o)
                if j in cfg["kick_pv"]:
                    kick()
            oa_s[rows, :] = o / l

        def a_body(g, carry):
            pm = _Pump(small_k(g + 2) + small_v(g + 2))
            attend_a(g, functools.partial(start_v, g + 1), functools.partial(start_k, g + 2),
                     pm.kick, functools.partial(pm.pump, *cfg["pump_k"]))
            pm.pump(*cfg["pump_v"])
            pm.drain()
            return carry

        lax.fori_loop(0, NG - 2, a_body, 0)

        waited = side_n - side_nb
        n_early = side_n - cfg["side_mid"]
        r_early, r_mid = n_early * side_rows, side_n * side_rows

        def spin(trips):
            spin_s[0] = lax.fori_loop(0, trips, lambda i, c: c * 3 + i, spin_s[0])

        spin_s[0] = 0
        pm = _Pump(small_wo(), spin)
        last = pl.ds((NG - 1) * _G, _G)
        pv = _Pump(heads_of(v_h.at[last], v_s.at[NG - 1], i_vl, Sk - W, S_INJ2))

        def project_b():
            c_wob.wait()
            wait_pieces(wob_s.at[rest_all], cut_rest, S_WOB)
            for i in range(waited, n_early):
                c_sb(i).wait()
            ctxb = ctxb_s[...].astype(_BF16)
            acc = _dot(ctxb[:, side_total:], rows_of(wob_s, side_total, Hb * Db))
            for lo in range(0, r_early, cfg["seg_b"]):
                pm.kick()
                hi = min(lo + cfg["seg_b"], r_early)
                acc = acc + _dot(ctxb[:, lo:hi], rows_of(wob_s, lo, hi))
            accb_s[...] = acc

        def start_tail():
            for i in range(n_wo):
                c_wo(i).start(priority=_BULK)
            pm.pump(1, cfg["lag"])

        def before_last_pv():
            pm.pace(*cfg["pump_k15"])
            pv.drain()

        attend_a(NG - 2, functools.partial(start_v, NG - 1, cut_vl), start_wo,
                 pv.kick, functools.partial(pm.pace, *cfg["pump_k14"]))
        project_b()
        pm.pace(*cfg["pump_b"])
        attend_a(NG - 1, lambda: c_sa(side_n).start(), start_tail, pv.kick, before_last_pv, cut_vl)
        pm.pump(1, cfg["lag"])

        oa32 = oa_s[...].reshape(B, H, Dh).reshape(B, H * Dh)
        oab_s[...] = oa32
        tail0 = H * Dh - tail_rows
        for b in range(B):
            for t in range(tail_rows // Dh):
                src = oa32[b:b + 1, tail0 + t * Dh:tail0 + (t + 1) * Dh]
                coef_s[b, t * Dh:(t + 1) * Dh, :] = jnp.broadcast_to(src, (_L, Dh)).T
        pm.pace(*cfg["pump_e"])
        c_sa(side_n).wait()
        c_sb(side_n).start()
        pm.pace(*cfg["pump_f"])
        pm.drain()
        oa = oab_s[...].astype(_BF16)
        c_gap.wait()
        n_head = wo_inj * r_m
        acc_s[...] = _dot(oa[:, :n_head], rows_of(woa_s, 0, n_head))
        for j in range(n_early, side_n):
            c_sb(j).wait()
        accb_s[...] += _dot(ctxb_s[:, r_early:r_mid].astype(_BF16), rows_of(wob_s, r_early, r_mid))
        wait_pieces(woa_s.at[wide], cut_wo, S_WIDE)
        acc_s[...] += _dot(oa[:, n_head:wo_base], rows_of(woa_s, n_head, wo_base))
        for i in range(n_mxu):
            c_wo(i).wait()
            if i == late_at:
                c_sb(side_n).wait()
                late = _dot(ctxb_s[:, r_mid:side_total].astype(_BF16),
                            rows_of(wob_s, r_mid, side_total))
                o_ref[:, D:] = (accb_s[...] + late).astype(o_ref.dtype)
            lo, n = wo_off[i], wo_chunks[i]
            part = _dot(oa[:, lo:lo + n], rows_of(woa_s, lo, lo + n)) + acc_s[...]
            if i < n_wo - 1:
                acc_s[...] = part
            else:
                o_ref[:, :D] = part.astype(o_ref.dtype)
        for i in range(n_mxu, n_wo):
            c_wo(i).wait()
            lo, n = wo_off[i], wo_chunks[i]
            w = rows_of(woa_s, lo, lo + n, _F32)
            sums = []
            for b in range(B):
                cf = coef_s[b, lo - tail0:lo - tail0 + n, :]
                prod = w * jnp.concatenate([cf] * (D // _L), axis=1)
                acc = vacc_s[b] if i > n_mxu else None
                for r in range(0, n, 8):
                    acc = prod[r:r + 8] if acc is None else acc + prod[r:r + 8]
                if i < n_wo - 1:
                    vacc_s[b] = acc
                else:
                    sums.append(jnp.sum(acc, axis=0, keepdims=True))
            if i == n_wo - 1:
                res = acc_s[...] + jnp.concatenate(sums, axis=0)
                o_ref[:, :D] = res.astype(o_ref.dtype)

    any_spec = pl.BlockSpec(memory_space=pl.ANY)
    out = pl.pallas_call(
        kernel,
        out_shape=jax.ShapeDtypeStruct((B, D + M), A_x.dtype),
        in_specs=[any_spec] * 11,
        out_specs=pl.BlockSpec(memory_space=pltpu.VMEM),
        scratch_shapes=[
            pltpu.VMEM(xa2.shape, _BF16),
            pltpu.VMEM(xb2.shape, _BF16),
            pltpu.VMEM((2, NG, _G, W, Dh), _BF16),
            pltpu.VMEM((6 + B,) + wqa3.shape, _BF16),
            pltpu.VMEM((BH, Dh), _F32),
            pltpu.VMEM((BH, Dh), _F32),
            pltpu.VMEM((NCT, B, Hb, _L), _F32),
            pltpu.VMEM((NCT, B, Hb, _L), _F32),
            pltpu.VMEM((B, D), _F32),
            pltpu.VMEM((B, M), _F32),
            pltpu.VMEM((B, Hb * Db), _F32),
            pltpu.VMEM((B, H * Dh), _F32),
            pltpu.VMEM((B, max(tail_rows, 8), _L), _F32),
            pltpu.VMEM((B, 8, D), _F32),
            pltpu.VMEM((_G, W), _F32),
            pltpu.VMEM((Hb, Skb), _F32),
            pltpu.SMEM((side_nb, side_rows * NCT, _L), _BF16),
            pltpu.SMEM((1,), jnp.int32),
            pltpu.SemaphoreType.DMA((n_sem,)),
        ],
        compiler_params=pltpu.CompilerParams(
            vmem_limit_bytes=120 * 1024 * 1024,
            disable_semaphore_checks=True,
            disable_bounds_checks=True,
        ),
        name="fused_decode",
    )(xa2, k3, v3, wqa3, woa3, xb2, c4, wqb4, wuk4, wuv4, wob3)
    return out.reshape(B, Sq, D + M)


@jax.jit
def pallas_concat_heads__sliding_block_cached__compressed_kv_cla__decode_kernel(
    A_x: jax.Array,
    A_k_cache: jax.Array,
    A_v_cache: jax.Array,
    A_wq: jax.Array,
    A_wo: jax.Array,
    B_x: jax.Array,
    B_c_kv: jax.Array,
    B_w_q: jax.Array,
    B_w_uk: jax.Array,
    B_w_uv: jax.Array,
    B_w_o: jax.Array,
):
    return _fused(_CFG, A_x, A_k_cache, A_v_cache, A_wq, A_wo,
                  B_x, B_c_kv, B_w_q, B_w_uk, B_w_uv, B_w_o)
```

```python
import functools

import jax
import jax.numpy as jnp
from jax import lax
import jax.experimental.pallas as pl
import jax.experimental.pallas.tpu as pltpu

_NT = (((1,), (1,)), ((), ()))
_F32 = jnp.float32
_BF16 = jnp.bfloat16
_L = 128
_G = 8
_KIB = 1024
_URGENT, _BULK = 0, 1

_CFG = dict(
    piece=64 * _KIB,
    block=512 * _KIB,
    shift_a=30 * _KIB,
    shift_b=34 * _KIB,
    inj_w=(18 * _KIB, 16 * _KIB, -14 * _KIB, -16 * _KIB),
    inj_c=(18 * _KIB, 16 * _KIB, -14 * _KIB, -16 * _KIB),
    inj_q=(14 * _KIB, 16 * _KIB, -18 * _KIB, -16 * _KIB),
    inj_k=(14 * _KIB, 16 * _KIB),
    inj_v=(-18 * _KIB, -16 * _KIB),
    inj_vl=(14 * _KIB, 16 * _KIB),
    inj_wo=(2 * _KIB,) + (4 * _KIB,) * 120,
    pump_0=(28, 2),
    pump_w=(11, 3),
    pump_c=(15, 3),
    pump_uv=(20, 3),
    pump_q=(10, 3),
    pump_k=(10, 3),
    pump_v=(11, 3),
    pump_k14=(28, 5, 14),
    pump_b=(21, 5, 14),
    pump_k15=(25, 5, 14),
    pump_e=(6, 5, 14),
    pump_f=(24, 5, 14),
    seg_b=256,
    lag=10,
    kick_s=(0, 1, 2, 3, 4, 5, 6, 7),
    kick_c=(1, 3, 5),
    kick_qk=(0, 1, 3, 5, 6),
    kick_pv=(1, 3, 5),
    side_rows=128,
    side_n=24,
    side_last=64,
    side_nb=5,
    side_mid=3,
    late_at=1,
    wo_chunks=(512, 128, 128),
    wo_tail=(80, 64, 48, 32, 16, 16),
)


def _dot(a, b):
    return jnp.dot(a, b, preferred_element_type=_F32)


def _dot_nt(a, b):
    return lax.dot_general(a, b, _NT, preferred_element_type=_F32)


def _bounds(n_rows, row_bytes, piece, shift, skip=0):
    step = piece // row_bytes
    first = (shift // row_bytes) % step
    cuts = [skip] + [r for r in range(first, n_rows, step) if r > skip] + [n_rows]
    return list(zip(cuts[:-1], cuts[1:]))


class _Pump:
    def __init__(self, copies, spin=None):
        self.copies, self.started, self.waited, self.spin = list(copies), 0, 0, spin

    def kick(self):
        if self.started < len(self.copies):
            self.copies[self.started]().start(priority=_URGENT)
            self.started += 1

    def _wait_to(self, n):
        while self.waited < n:
            self.copies[self.waited]().wait()
            self.waited += 1

    def pump(self, n, lag=1):
        for _ in range(n):
            self.kick()
            self._wait_to(self.started - lag)

    def pace(self, n, trips, lag=8):
        for _ in range(n):
            self.kick()
            self._wait_to(self.started - lag)
            self.spin(trips)

    def drain(self):
        while self.started < len(self.copies):
            self.kick()
        self._wait_to(self.started)


def _fused(cfg, A_x, A_k_cache, A_v_cache, A_wq, A_wo, B_x, B_c_kv, B_w_q, B_w_uk, B_w_uv, B_w_o):
    B, Sq, D = A_x.shape
    _, H, Sk, Dh = A_k_cache.shape
    assert Sq == 1 and B_x.shape[1] == 1
    assert A_wq.shape == (D, H * Dh)
    W = min(4096, max(256, Sk // 4))
    M, Hb, Db = B_w_q.shape
    Skb, Dc = B_c_kv.shape[1], B_c_kv.shape[2]
    BH = B * H
    NG = BH // _G
    NCT = Dc // _L
    HH = Hb // 2
    scale_a = float(Dh) ** -0.5
    scale_b = float(Db) ** -0.5
    piece, block = cfg["piece"], cfg["block"]
    shift_a, shift_b = cfg["shift_a"], cfg["shift_b"]
    side_rows, side_n, side_nb = cfg["side_rows"], cfg["side_n"], cfg["side_nb"]
    late_at = cfg["late_at"]
    n_mxu = len(cfg["wo_chunks"])
    wo_chunks = tuple(cfg["wo_chunks"]) + tuple(cfg["wo_tail"])
    tail_rows = sum(cfg["wo_tail"])
    assert tail_rows % Dh == 0 and M % _L == 0 and NG >= 4
    side_lag = 2
    side_lead = side_nb - side_lag
    side_last = cfg["side_last"]
    assert side_n == 4 + B + NG and cfg["side_mid"] < side_nb and side_last > 0

    xa2 = A_x.reshape(B, D)
    xb2 = B_x.reshape(B, M)
    k3 = A_k_cache.reshape(BH, Sk, Dh)
    v3 = A_v_cache.reshape(BH, Sk, Dh)

    def blocked(w, lead=0):
        row_bytes = 2 * functools.reduce(lambda a, b: a * b, w.shape[lead + 1:], 1)
        rows = block // row_bytes
        shape = w.shape[:lead] + (w.shape[lead] // rows, rows) + w.shape[lead + 1:]
        return w.reshape(shape), rows, row_bytes

    def tiles(w):
        *lead, r, c = w.shape
        n = len(lead)
        w = w.reshape(*lead, r // 8, 8, c // _L, _L).transpose(*range(n), n, n + 2, n + 1, n + 3)
        return w.reshape(*lead, r * c // _L, _L)

    n_ct = H * Dh // _L
    wqa3, r_w, b_w = blocked(tiles(A_wq))
    wqb4, _, _ = blocked(B_w_q.reshape(M * Hb, Db))
    wuk4, _, _ = blocked(B_w_uk.reshape(Dc * Hb, Db))
    wuv4, _, _ = blocked(B_w_uv.reshape(Dc * Hb, Db))
    c4, _, _ = blocked(tiles(B_c_kv), 1)
    woa3, _, _ = blocked(tiles(A_wo))
    wob3, _, _ = blocked(tiles(B_w_o.reshape(Hb * Db, M)))
    assert all(w.shape == wqa3.shape for w in (wqb4, wuk4, wuv4, woa3, wob3))
    assert c4.shape[1:] == wqa3.shape and 2 * r_w == _L * Hb and D == M == Dc
    r_m = r_w // NCT
    assert r_m % side_rows == 0
    NBLK = wqa3.shape[0]

    def spans(sizes, unit, n_rows=0):
        out, front, back = [], 0, n_rows
        for n in sizes:
            if n > 0:
                out.append((front, front + n // unit))
                front += n // unit
            else:
                out.append((back + n // unit, back))
                back += n // unit
        return out, front, back

    def split(sizes, n_rows, unit, shift):
        small, front, back = spans(sizes, unit, n_rows)
        return small, _bounds(back, unit, piece, shift, front)

    i_w, cut_w = split(cfg["inj_w"], r_w, b_w, shift_b)
    i_c, cut_c = split(cfg["inj_c"], r_w, b_w, shift_b)
    i_k, cut_k = split(cfg["inj_k"], W, 2 * Dh, shift_a)
    i_v, cut_v = split(cfg["inj_v"], W, 2 * Dh, shift_a)
    i_vl, cut_vl = split(cfg["inj_v"] + cfg["inj_vl"], W, 2 * Dh, shift_a)
    i_vl = i_vl[len(i_v):]
    i_wqa, cut_wqa = split(cfg["inj_q"], r_w, b_w, shift_a)
    i_wo, n_inj, _ = spans(cfg["inj_wo"], b_w)
    cut_w0 = _bounds(r_w, b_w, piece, shift_b)
    cut_wo = _bounds(r_w, b_w, piece, shift_a)
    wo_inj = -(-n_inj // r_w)
    wo_wide = (H * Dh - sum(wo_chunks)) // r_m - wo_inj
    wo_base = (wo_inj + wo_wide) * r_m
    assert wo_base + sum(wo_chunks) == H * Dh
    n_wo = len(wo_chunks)
    wo_off = [wo_base + sum(wo_chunks[:i]) for i in range(n_wo)]
    assert all(lo // r_m == (lo + n - 1) // r_m for lo, n in zip(wo_off, wo_chunks))
    S_XB, S_XA, S_WQB, S_WUK, S_WUV, S_WOB, S_WQA, S_INJ, S_WIDE, S_GAP, S_GAPB, S_INJ2 = range(12)
    S_C = 12
    S_KV = S_C + B
    S_WO = S_KV + 2 * NG
    S_SA = S_WO + n_wo
    S_SB = S_SA + side_nb
    n_sem = S_SB + side_nb
    side_total = side_rows * side_n + side_last

    def kernel(xa_h, k_h, v_h, wqa_h, woa_h, xb_h, c_h, wqb_h, wuk_h, wuv_h, wob_h,
               o_ref,
               xa_s, xb_s, kv_s, big_s,
               qa_s, oa_s, qabs_s, ctx_s, acc_s, accb_s, ctxb_s, oab_s, coef_s, vacc_s, p_s, s_s,
               side_s, spin_s, sem):
        def cp(src, dst, s):
            return pltpu.make_async_copy(src, dst, sem.at[s])

        def start_pieces(src, dst, cuts, s, row0=0):
            for lo, hi in cuts:
                cp(src.at[:, pl.ds(row0 + lo, hi - lo)], dst.at[:, pl.ds(lo, hi - lo)],
                   s).start(priority=_BULK)

        def wait_pieces(dst, cuts, s):
            view = dst.at[:, pl.ds(cuts[0][0], cuts[-1][1] - cuts[0][0])]
            cp(view, view, s).wait()

        def heads_of(src, dst, ranges, row0=0, s=S_INJ):
            def one(k, lo, hi):
                return cp(src.at[k, pl.ds(row0 + lo, hi - lo)], dst.at[k, pl.ds(lo, hi - lo)], s)
            return [functools.partial(one, k, lo, hi)
                    for k in range(dst.shape[0]) for lo, hi in sorted(ranges)]

        k_s, v_s = kv_s.at[0], kv_s.at[1]
        wqb_s, wuk_s, wuv_s, wqa_s, woa_s, wob_s = (big_s.at[j] for j in range(6))
        c_s = big_s.at[pl.ds(6, B)]
        c_xb = cp(xb_h, xb_s, S_XB)
        c_xa = cp(xa_h, xa_s, S_XA)

        def rows_of(ref, lo, hi, dtype=_BF16):
            parts = []
            for k in range(lo // r_m, -(-hi // r_m)):
                a, b = max(lo - k * r_m, 0), min(hi - k * r_m, r_m)
                t = ref[k, a * NCT:b * NCT].astype(dtype).reshape((b - a) // 8, NCT, 8, _L)
                parts.append(jnp.concatenate(
                    [t[:, j].reshape(b - a, _L) for j in range(NCT)], axis=1))
            return parts[0] if len(parts) == 1 else jnp.concatenate(parts, axis=0)

        k0, r0 = divmod(side_total * NCT, r_w)
        cut_rest = _bounds(r_w, b_w, piece, shift_b, r0)
        rest_all, rest_up = pl.ds(k0, NBLK - k0), (pl.ds(k0 + 1, NBLK - k0 - 1), pl.ds(0, r0))
        c_wob = cp(wob_h.at[rest_up], wob_s.at[rest_up], S_GAPB)

        def start_c(b):
            start_pieces(c_h.at[b], c_s.at[b], cut_c, S_C + b)

        def pump_c(b):
            return _Pump(heads_of(c_h.at[b], c_s.at[b], i_c))

        def start_wqa():
            c_wob.start(priority=_BULK)
            start_pieces(wob_h.at[rest_all], wob_s.at[rest_all], cut_rest, S_WOB)
            start_pieces(wqa_h, wqa_s, cut_wqa, S_WQA)

        def start_k(g):
            start_pieces(k_h.at[pl.ds(g * _G, _G)], k_s.at[g], cut_k, S_KV + 2 * g, Sk - W)

        def start_v(g, cuts=cut_v):
            start_pieces(v_h.at[pl.ds(g * _G, _G)], v_s.at[g], cuts, S_KV + 2 * g + 1, Sk - W)

        def small_k(g):
            return heads_of(k_h.at[pl.ds(g * _G, _G)], k_s.at[g], i_k, Sk - W)

        def small_v(g):
            return heads_of(v_h.at[pl.ds(g * _G, _G)], v_s.at[g], i_v, Sk - W)

        def flat_at(lo, hi):
            assert lo // r_w == (hi - 1) // r_w
            return lo // r_w, pl.ds(lo % r_w, hi - lo)

        def c_wo(i):
            at = flat_at(wo_off[i] * NCT, (wo_off[i] + wo_chunks[i]) * NCT)
            return cp(woa_h.at[at], woa_s.at[at], S_WO + i)

        wide = pl.ds(wo_inj, wo_wide)
        gap = flat_at(n_inj, wo_inj * r_w)
        c_gap = cp(woa_h.at[gap], woa_s.at[gap], S_GAP)

        def start_wo():
            c_gap.start(priority=_BULK)
            start_pieces(woa_h.at[wide], woa_s.at[wide], cut_wo, S_WIDE)

        def small_wo():
            def one(lo, hi):
                return cp(woa_h.at[flat_at(lo, hi)], woa_s.at[flat_at(lo, hi)], S_INJ)
            return [functools.partial(one, lo, hi) for lo, hi in i_wo]

        def side_refs(i):
            per, n = r_m // side_rows, side_rows * NCT
            if isinstance(i, int):
                size = n if i < side_n else side_last * NCT
                rows = (i // per, pl.ds(i % per * n, size))
                return rows, side_s.at[i % side_nb, pl.ds(0, size)], i % side_nb
            slot = lax.rem(i, side_nb)
            start = pl.multiple_of(lax.rem(i, per) * n, 8)
            return (lax.div(i, per), pl.ds(start, n)), side_s.at[slot], slot

        def c_sa(i):
            rows, stage, slot = side_refs(i)
            return cp(wob_h.at[rows], stage, S_SA + slot)

        def c_sb(i):
            rows, stage, slot = side_refs(i)
            return cp(stage, wob_s.at[rows], S_SB + slot)

        def tick(i):
            traced = not isinstance(i, int)
            if traced or i < side_n:
                c_sa(i).wait()
                c_sb(i).start()

            def refill(j):
                if traced or i >= side_lag:
                    c_sb(i - side_lag).wait()
                c_sa(j).start()

            if traced:
                pl.when(i + side_lead < side_n)(lambda: refill(i + side_lead))
            elif i + side_lead < side_n:
                refill(i + side_lead)

        def head_major(w_s, t, hh, mid=lambda: None):
            halves = []
            for k in range(2):
                w = w_s[2 * t + k].reshape(_L // 2, Hb, Db)[:, hh * HH:(hh + 1) * HH, :]
                halves.append(w.reshape(_L // 2, HH * Db))
                if k == 0:
                    mid()
            return jnp.concatenate(halves, axis=0)

        start_pieces(wqb_h, wqb_s, cut_w0, S_WQB)
        c_xb.start()
        c_xa.start()
        for i in range(side_lead):
            c_sa(i).start()
        start_pieces(wuk_h, wuk_s, cut_w, S_WUK)
        pm = _Pump(heads_of(wuk_h, wuk_s, i_w))
        pm.pump(*cfg["pump_0"])
        pm.drain()


        wait_pieces(wqb_s, cut_w0, S_WQB)
        start_c(0)
        pm = pump_c(0)
        pm.kick()
        tick(0)
        c_xb.wait()
        xb = xb_s[...]
        halves = [None, None]
        for t in range(M // _L):
            for hh in range(2):
                part = _dot(xb[:, t * _L:(t + 1) * _L], head_major(wqb_s, t, hh, pm.kick))
                halves[hh] = part if t == 0 else halves[hh] + part
                pm.kick()
        ctxb_s[...] = jnp.concatenate(halves, axis=1)
        pm.pump(*cfg["pump_w"])
        pm.drain()

        wait_pieces(wuk_s, cut_w, S_WUK)
        start_c(1)
        pm = pump_c(1)
        pm.kick()
        tick(1)
        qb = (ctxb_s[...] * scale_b).astype(_BF16)
        for t in range(NCT):
            for hh in range(2):
                w = head_major(wuk_s, t, hh, pm.kick)
                parts = [_dot_nt(qb[:, (hh * HH + j) * Db:(hh * HH + j + 1) * Db],
                                 w[:, j * Db:(j + 1) * Db]) for j in range(HH)]
                qabs_s[t, :, hh * HH:(hh + 1) * HH, :] = jnp.concatenate(
                    parts, axis=1).reshape(B, HH, _L)
                pm.kick()
        pm.pump(*cfg["pump_w"])
        pm.drain()

        def attend_b(b, start_next, pm):
            wait_pieces(c_s.at[b], cut_c, S_C + b)
            start_next()
            pm.kick()
            tick(2 + b)
            qa = jnp.concatenate(
                [qabs_s[t, b] for t in range(NCT)], axis=1).astype(_BF16)
            for k in range(NBLK):
                s_s[:, k * r_m:(k + 1) * r_m] = _dot_nt(
                    qa, rows_of(c_s.at[b], k * r_m, (k + 1) * r_m))
                if k in cfg["kick_s"]:
                    pm.kick()
            s = s_s[...]
            m = jnp.max(s, axis=-1, keepdims=True)
            p = jnp.exp(s - m)
            l = jnp.sum(p, axis=-1, keepdims=True)
            pb = p.astype(_BF16)
            cc = None
            for k in range(NBLK):
                part = _dot(pb[:, k * r_m:(k + 1) * r_m],
                            rows_of(c_s.at[b], k * r_m, (k + 1) * r_m))
                cc = part if cc is None else cc + part
                if k in cfg["kick_c"]:
                    pm.kick()
            cc = cc / l
            for t in range(NCT):
                ctx_s[t, b] = cc[:, t * _L:(t + 1) * _L]
            pm.pump(*cfg["pump_c"])
            pm.drain()

        small_wqa = heads_of(wqa_h, wqa_s, i_wqa)
        n_q = len(small_wqa) // 2
        for b in range(B):
            if b + 2 < B:
                attend_b(b, functools.partial(start_c, b + 2), pump_c(b + 2))
            elif b + 2 == B:
                attend_b(b, functools.partial(start_pieces, wuv_h, wuv_s, cut_w, S_WUV),
                         _Pump(heads_of(wuv_h, wuv_s, i_w)))
            else:
                attend_b(b, start_wqa, _Pump(small_wqa[:n_q] + small_k(0)))

        wait_pieces(wuv_s, cut_w, S_WUV)
        start_k(0)
        start_v(0)
        pm = _Pump(small_v(0)[:1] + small_wqa[n_q:] + small_v(0)[1:] + small_k(1))
        pm.kick()
        tick(2 + B)
        halves = [None, None]
        for t in range(NCT):
            for hh in range(2):
                ch = ctx_s[t, :, hh * HH:(hh + 1) * HH, :].reshape(B, HH * _L).astype(_BF16)
                w = head_major(wuv_s, t, hh, pm.kick)
                part = jnp.concatenate(
                    [_dot(ch[:, j * _L:(j + 1) * _L], w[:, j * Db:(j + 1) * Db])
                     for j in range(HH)], axis=1)
                halves[hh] = part if t == 0 else halves[hh] + part
                pm.kick()
        ctxb_s[...] = jnp.concatenate(halves, axis=1)
        pm.pump(*cfg["pump_uv"])
        pm.drain()

        wait_pieces(wqa_s, cut_wqa, S_WQA)
        start_k(1)
        pm = _Pump(small_v(1))
        pm.kick()
        tick(3 + B)
        c_xa.wait()
        xa = xa_s[...]
        wq_tiles = wqa_s[...].reshape(D // 8, n_ct, 8, _L)
        qa_all = jnp.concatenate(
            [_dot(xa, wq_tiles[:, ct].reshape(D, _L)) for ct in range(n_ct)], axis=1) * scale_a
        qa_s[...] = qa_all.reshape(B, H, Dh).reshape(BH, Dh)
        pm.pump(*cfg["pump_q"])
        pm.drain()

        def attend_a(g, start_at_k, start_at_v, kick, between, v_cuts=cut_v):
            start = g * _G if isinstance(g, int) else pl.multiple_of(g * _G, _G)
            rows = pl.ds(start, _G)
            q8 = qa_s[rows, :].astype(_BF16)
            wait_pieces(k_s.at[g], cut_k, S_KV + 2 * g)
            start_at_k()
            kick()
            tick(4 + B + g)
            row = lax.broadcasted_iota(jnp.int32, (_G, W), 0)
            s = None
            for j in range(_G):
                sj = _dot_nt(q8, k_s[g, j])
                s = sj if s is None else jnp.where(row == j, sj, s)
                if j in cfg["kick_qk"]:
                    kick()
            m = jnp.max(s, axis=-1, keepdims=True)
            p = jnp.exp(s - m)
            l = jnp.sum(p, axis=-1, keepdims=True)
            p_s[...] = p
            between()
            wait_pieces(v_s.at[g], v_cuts, S_KV + 2 * g + 1)
            start_at_v()
            kick()
            pb = p_s[...].astype(_BF16)
            row2 = lax.broadcasted_iota(jnp.int32, (_G, Dh), 0)
            o = None
            for j in range(_G):
                oj = _dot(pb, v_s[g, j])
                o = oj if o is None else jnp.where(row2 == j, oj, o)
                if j in cfg["kick_pv"]:
                    kick()
            oa_s[rows, :] = o / l

        def a_body(g, carry):
            pm = _Pump(small_k(g + 2) + small_v(g + 2))
            attend_a(g, functools.partial(start_v, g + 1), functools.partial(start_k, g + 2),
                     pm.kick, functools.partial(pm.pump, *cfg["pump_k"]))
            pm.pump(*cfg["pump_v"])
            pm.drain()
            return carry

        lax.fori_loop(0, NG - 2, a_body, 0)

        waited = side_n - side_nb
        n_early = side_n - cfg["side_mid"]
        r_early, r_mid = n_early * side_rows, side_n * side_rows

        def spin(trips):
            spin_s[0] = lax.fori_loop(0, trips, lambda i, c: c * 3 + i, spin_s[0])

        spin_s[0] = 0
        pm = _Pump(small_wo(), spin)
        last = pl.ds((NG - 1) * _G, _G)
        pv = _Pump(heads_of(v_h.at[last], v_s.at[NG - 1], i_vl, Sk - W, S_INJ2))

        def project_b():
            c_wob.wait()
            wait_pieces(wob_s.at[rest_all], cut_rest, S_WOB)
            for i in range(waited, n_early):
                c_sb(i).wait()
            ctxb = ctxb_s[...].astype(_BF16)
            acc = _dot(ctxb[:, side_total:], rows_of(wob_s, side_total, Hb * Db))
            for lo in range(0, r_early, cfg["seg_b"]):
                pm.kick()
                hi = min(lo + cfg["seg_b"], r_early)
                acc = acc + _dot(ctxb[:, lo:hi], rows_of(wob_s, lo, hi))
            accb_s[...] = acc

        def start_tail():
            for i in range(n_wo):
                c_wo(i).start(priority=_BULK)
            pm.pump(1, cfg["lag"])

        def before_last_pv():
            pm.pace(*cfg["pump_k15"])
            pv.drain()

        attend_a(NG - 2, functools.partial(start_v, NG - 1, cut_vl), start_wo,
                 pv.kick, functools.partial(pm.pace, *cfg["pump_k14"]))
        project_b()
        pm.pace(*cfg["pump_b"])
        attend_a(NG - 1, lambda: c_sa(side_n).start(), start_tail, pv.kick, before_last_pv, cut_vl)
        pm.pump(1, cfg["lag"])

        oa32 = oa_s[...].reshape(B, H, Dh).reshape(B, H * Dh)
        oab_s[...] = oa32
        tail0 = H * Dh - tail_rows
        for b in range(B):
            for t in range(tail_rows // Dh):
                src = oa32[b:b + 1, tail0 + t * Dh:tail0 + (t + 1) * Dh]
                coef_s[b, t * Dh:(t + 1) * Dh, :] = jnp.broadcast_to(src, (_L, Dh)).T
        pm.pace(*cfg["pump_e"])
        c_sa(side_n).wait()
        c_sb(side_n).start()
        pm.pace(*cfg["pump_f"])
        pm.drain()
        oa = oab_s[...].astype(_BF16)
        c_gap.wait()
        n_head = wo_inj * r_m
        acc_s[...] = _dot(oa[:, :n_head], rows_of(woa_s, 0, n_head))
        for j in range(n_early, side_n):
            c_sb(j).wait()
        accb_s[...] += _dot(ctxb_s[:, r_early:r_mid].astype(_BF16), rows_of(wob_s, r_early, r_mid))
        wait_pieces(woa_s.at[wide], cut_wo, S_WIDE)
        acc_s[...] += _dot(oa[:, n_head:wo_base], rows_of(woa_s, n_head, wo_base))
        for i in range(n_mxu):
            c_wo(i).wait()
            if i == late_at:
                c_sb(side_n).wait()
                late = _dot(ctxb_s[:, r_mid:side_total].astype(_BF16),
                            rows_of(wob_s, r_mid, side_total))
                o_ref[:, D:] = (accb_s[...] + late).astype(o_ref.dtype)
            lo, n = wo_off[i], wo_chunks[i]
            part = _dot(oa[:, lo:lo + n], rows_of(woa_s, lo, lo + n)) + acc_s[...]
            if i < n_wo - 1:
                acc_s[...] = part
            else:
                o_ref[:, :D] = part.astype(o_ref.dtype)
        for i in range(n_mxu, n_wo):
            c_wo(i).wait()
            lo, n = wo_off[i], wo_chunks[i]
            w = rows_of(woa_s, lo, lo + n, _F32)
            sums = []
            for b in range(B):
                cf = coef_s[b, lo - tail0:lo - tail0 + n, :]
                prod = w * jnp.concatenate([cf] * (D // _L), axis=1)
                acc = vacc_s[b] if i > n_mxu else None
                for r in range(0, n, 8):
                    acc = prod[r:r + 8] if acc is None else acc + prod[r:r + 8]
                if i < n_wo - 1:
                    vacc_s[b] = acc
                else:
                    sums.append(jnp.sum(acc, axis=0, keepdims=True))
            if i == n_wo - 1:
                res = acc_s[...] + jnp.concatenate(sums, axis=0)
                o_ref[:, :D] = res.astype(o_ref.dtype)

    any_spec = pl.BlockSpec(memory_space=pl.ANY)
    out = pl.pallas_call(
        kernel,
        out_shape=jax.ShapeDtypeStruct((B, D + M), A_x.dtype),
        in_specs=[any_spec] * 11,
        out_specs=pl.BlockSpec(memory_space=pltpu.VMEM),
        scratch_shapes=[
            pltpu.VMEM(xa2.shape, _BF16),
            pltpu.VMEM(xb2.shape, _BF16),
            pltpu.VMEM((2, NG, _G, W, Dh), _BF16),
            pltpu.VMEM((6 + B,) + wqa3.shape, _BF16),
            pltpu.VMEM((BH, Dh), _F32),
            pltpu.VMEM((BH, Dh), _F32),
            pltpu.VMEM((NCT, B, Hb, _L), _F32),
            pltpu.VMEM((NCT, B, Hb, _L), _F32),
            pltpu.VMEM((B, D), _F32),
            pltpu.VMEM((B, M), _F32),
            pltpu.VMEM((B, Hb * Db), _F32),
            pltpu.VMEM((B, H * Dh), _F32),
            pltpu.VMEM((B, max(tail_rows, 8), _L), _F32),
            pltpu.VMEM((B, 8, D), _F32),
            pltpu.VMEM((_G, W), _F32),
            pltpu.VMEM((Hb, Skb), _F32),
            pltpu.SMEM((side_nb, side_rows * NCT, _L), _BF16),
            pltpu.SMEM((1,), jnp.int32),
            pltpu.SemaphoreType.DMA((n_sem,)),
        ],
        compiler_params=pltpu.CompilerParams(
            vmem_limit_bytes=120 * 1024 * 1024,
            disable_semaphore_checks=True,
            disable_bounds_checks=True,
        ),
        name="fused_decode",
    )(xa2, k3, v3, wqa3, woa3, xb2, c4, wqb4, wuk4, wuv4, wob3)
    return out.reshape(B, Sq, D + M)


@jax.jit
def pallas_concat_heads__sliding_block_cached__compressed_kv_cla__decode_kernel(
    A_x: jax.Array,
    A_k_cache: jax.Array,
    A_v_cache: jax.Array,
    A_wq: jax.Array,
    A_wo: jax.Array,
    B_x: jax.Array,
    B_c_kv: jax.Array,
    B_w_q: jax.Array,
    B_w_uk: jax.Array,
    B_w_uv: jax.Array,
    B_w_o: jax.Array,
):
    return _fused(_CFG, A_x, A_k_cache, A_v_cache, A_wq, A_wo,
                  B_x, B_c_kv, B_w_q, B_w_uk, B_w_uv, B_w_o)
```

```python
import functools

import jax
import jax.numpy as jnp
from jax import lax
import jax.experimental.pallas as pl
import jax.experimental.pallas.tpu as pltpu

_NT = (((1,), (1,)), ((), ()))
_F32 = jnp.float32
_BF16 = jnp.bfloat16
_L = 128
_G = 8
_KIB = 1024
_URGENT, _BULK = 0, 1

_CFG = dict(
    piece=64 * _KIB,
    block=512 * _KIB,
    shift_a=30 * _KIB,
    shift_b=34 * _KIB,
    inj_w=(18 * _KIB, 16 * _KIB, -14 * _KIB, -16 * _KIB),
    inj_c=(18 * _KIB, 16 * _KIB, -14 * _KIB, -16 * _KIB),
    inj_q=(14 * _KIB, 16 * _KIB, -18 * _KIB, -16 * _KIB),
    inj_k=(14 * _KIB, 16 * _KIB),
    inj_v=(-18 * _KIB, -16 * _KIB),
    inj_vl=(14 * _KIB, 16 * _KIB),
    inj_wo=(2 * _KIB,) + (4 * _KIB,) * 120,
    pump_0=(28, 2),
    pump_w=(11, 3),
    pump_c=(15, 3),
    pump_uv=(20, 3),
    pump_q=(10, 3),
    pump_k=(10, 3),
    pump_v=(11, 3),
    pump_k14=(28, 5, 14),
    pump_b=(21, 5, 14),
    pump_k15=(25, 5, 14),
    pump_e=(6, 5, 14),
    pump_f=(24, 5, 14),
    seg_b=256,
    lag=10,
    kick_s=(0, 1, 2, 3, 4, 5, 6, 7),
    kick_c=(1, 3, 5),
    kick_qk=(0, 1, 3, 5, 6),
    kick_pv=(1, 3, 5),
    side_rows=128,
    side_n=24,
    side_last=64,
    side_nb=5,
    side_mid=3,
    late_at=1,
    wo_chunks=(512, 128, 128),
    wo_tail=(80, 64, 48, 32, 16, 16),
)


def _dot(a, b):
    return jnp.dot(a, b, preferred_element_type=_F32)


def _dot_nt(a, b):
    return lax.dot_general(a, b, _NT, preferred_element_type=_F32)


def _bounds(n_rows, row_bytes, piece, shift, skip=0):
    step = piece // row_bytes
    first = (shift // row_bytes) % step
    cuts = [skip] + [r for r in range(first, n_rows, step) if r > skip] + [n_rows]
    return list(zip(cuts[:-1], cuts[1:]))


class _Pump:
    def __init__(self, copies, spin=None):
        self.copies, self.started, self.waited, self.spin = list(copies), 0, 0, spin

    def kick(self):
        if self.started < len(self.copies):
            self.copies[self.started]().start(priority=_URGENT)
            self.started += 1

    def _wait_to(self, n):
        while self.waited < n:
            self.copies[self.waited]().wait()
            self.waited += 1

    def pump(self, n, lag=1):
        for _ in range(n):
            self.kick()
            self._wait_to(self.started - lag)

    def pace(self, n, trips, lag=8):
        for _ in range(n):
            self.kick()
            self._wait_to(self.started - lag)
            self.spin(trips)

    def drain(self):
        while self.started < len(self.copies):
            self.kick()
        self._wait_to(self.started)


def _fused(cfg, A_x, A_k_cache, A_v_cache, A_wq, A_wo, B_x, B_c_kv, B_w_q, B_w_uk, B_w_uv, B_w_o):
    B, Sq, D = A_x.shape
    _, H, Sk, Dh = A_k_cache.shape
    assert Sq == 1 and B_x.shape[1] == 1
    assert A_wq.shape == (D, H * Dh)
    W = min(4096, max(256, Sk // 4))
    M, Hb, Db = B_w_q.shape
    Skb, Dc = B_c_kv.shape[1], B_c_kv.shape[2]
    BH = B * H
    NG = BH // _G
    NCT = Dc // _L
    HH = Hb // 2
    scale_a = float(Dh) ** -0.5
    scale_b = float(Db) ** -0.5
    piece, block = cfg["piece"], cfg["block"]
    shift_a, shift_b = cfg["shift_a"], cfg["shift_b"]
    side_rows, side_n, side_nb = cfg["side_rows"], cfg["side_n"], cfg["side_nb"]
    late_at = cfg["late_at"]
    n_mxu = len(cfg["wo_chunks"])
    wo_chunks = tuple(cfg["wo_chunks"]) + tuple(cfg["wo_tail"])
    tail_rows = sum(cfg["wo_tail"])
    assert 0 < tail_rows and tail_rows % Dh == 0 and M % _L == 0 and NG >= 4
    side_lag = 2
    side_lead = side_nb - side_lag
    side_last = cfg["side_last"]
    assert side_n == 4 + B + NG and cfg["side_mid"] < side_nb and side_last > 0

    xa2 = A_x.reshape(B, D)
    xb2 = B_x.reshape(B, M)
    k3 = A_k_cache.reshape(BH, Sk, Dh)
    v3 = A_v_cache.reshape(BH, Sk, Dh)

    def blocked(w, lead=0):
        row_bytes = 2 * functools.reduce(lambda a, b: a * b, w.shape[lead + 1:], 1)
        rows = block // row_bytes
        shape = w.shape[:lead] + (w.shape[lead] // rows, rows) + w.shape[lead + 1:]
        return w.reshape(shape), rows, row_bytes

    def tiles(w):
        *lead, r, c = w.shape
        n = len(lead)
        w = w.reshape(*lead, r // 8, 8, c // _L, _L).transpose(*range(n), n, n + 2, n + 1, n + 3)
        return w.reshape(*lead, r * c // _L, _L)

    n_ct = H * Dh // _L
    wqa3, r_w, b_w = blocked(tiles(A_wq))
    wqb4, _, _ = blocked(B_w_q.reshape(M * Hb, Db))
    wuk4, _, _ = blocked(B_w_uk.reshape(Dc * Hb, Db))
    wuv4, _, _ = blocked(B_w_uv.reshape(Dc * Hb, Db))
    c4, _, _ = blocked(tiles(B_c_kv), 1)
    woa3, _, _ = blocked(tiles(A_wo))
    wob3, _, _ = blocked(tiles(B_w_o.reshape(Hb * Db, M)))
    assert all(w.shape == wqa3.shape for w in (wqb4, wuk4, wuv4, woa3, wob3))
    assert c4.shape[1:] == wqa3.shape and 2 * r_w == _L * Hb and D == M == Dc
    r_m = r_w // NCT
    assert r_m % side_rows == 0
    NBLK = wqa3.shape[0]

    def spans(sizes, unit, n_rows=0):
        out, front, back = [], 0, n_rows
        for n in sizes:
            if n > 0:
                out.append((front, front + n // unit))
                front += n // unit
            else:
                out.append((back + n // unit, back))
                back += n // unit
        return out, front, back

    def split(sizes, n_rows, unit, shift):
        small, front, back = spans(sizes, unit, n_rows)
        return small, _bounds(back, unit, piece, shift, front)

    i_w, cut_w = split(cfg["inj_w"], r_w, b_w, shift_b)
    i_c, cut_c = split(cfg["inj_c"], r_w, b_w, shift_b)
    i_k, cut_k = split(cfg["inj_k"], W, 2 * Dh, shift_a)
    i_v, cut_v = split(cfg["inj_v"], W, 2 * Dh, shift_a)
    i_vl, cut_vl = split(cfg["inj_v"] + cfg["inj_vl"], W, 2 * Dh, shift_a)
    i_vl = i_vl[len(i_v):]
    i_wqa, cut_wqa = split(cfg["inj_q"], r_w, b_w, shift_a)
    i_wo, n_inj, _ = spans(cfg["inj_wo"], b_w)
    cut_w0 = _bounds(r_w, b_w, piece, shift_b)
    cut_wo = _bounds(r_w, b_w, piece, shift_a)
    wo_inj = -(-n_inj // r_w)
    wo_wide = (H * Dh - sum(wo_chunks)) // r_m - wo_inj
    wo_base = (wo_inj + wo_wide) * r_m
    assert wo_base + sum(wo_chunks) == H * Dh
    n_wo = len(wo_chunks)
    wo_off = [wo_base + sum(wo_chunks[:i]) for i in range(n_wo)]
    assert all(lo // r_m == (lo + n - 1) // r_m for lo, n in zip(wo_off, wo_chunks))
    S_XB, S_XA, S_WQB, S_WUK, S_WUV, S_WOB, S_WQA, S_INJ, S_WIDE, S_GAP, S_GAPB, S_INJ2 = range(12)
    S_C = 12
    S_KV = S_C + B
    S_WO = S_KV + 2 * NG
    S_SA = S_WO + n_wo
    S_SB = S_SA + side_nb
    n_sem = S_SB + side_nb
    side_total = side_rows * side_n + side_last

    def kernel(xa_h, k_h, v_h, wqa_h, woa_h, xb_h, c_h, wqb_h, wuk_h, wuv_h, wob_h,
               o_ref,
               xa_s, xb_s, kv_s, big_s,
               qa_s, oa_s, qabs_s, ctx_s, acc_s, accb_s, ctxb_s, oab_s, coef_s, vacc_s, p_s, s_s,
               side_s, spin_s, sem):
        def cp(src, dst, s):
            return pltpu.make_async_copy(src, dst, sem.at[s])

        def start_pieces(src, dst, cuts, s, row0=0):
            for lo, hi in cuts:
                cp(src.at[:, pl.ds(row0 + lo, hi - lo)], dst.at[:, pl.ds(lo, hi - lo)],
                   s).start(priority=_BULK)

        def wait_pieces(dst, cuts, s):
            view = dst.at[:, pl.ds(cuts[0][0], cuts[-1][1] - cuts[0][0])]
            cp(view, view, s).wait()

        def heads_of(src, dst, ranges, row0=0, s=S_INJ):
            def one(k, lo, hi):
                return cp(src.at[k, pl.ds(row0 + lo, hi - lo)], dst.at[k, pl.ds(lo, hi - lo)], s)
            return [functools.partial(one, k, lo, hi)
                    for k in range(dst.shape[0]) for lo, hi in sorted(ranges)]

        k_s, v_s = kv_s.at[0], kv_s.at[1]
        wqb_s, wuk_s, wuv_s, wqa_s, woa_s, wob_s = (big_s.at[j] for j in range(6))
        c_s = big_s.at[pl.ds(6, B)]
        c_xb = cp(xb_h, xb_s, S_XB)
        c_xa = cp(xa_h, xa_s, S_XA)

        def rows_of(ref, lo, hi, dtype=_BF16):
            parts = []
            for k in range(lo // r_m, -(-hi // r_m)):
                a, b = max(lo - k * r_m, 0), min(hi - k * r_m, r_m)
                t = ref[k, a * NCT:b * NCT].astype(dtype).reshape((b - a) // 8, NCT, 8, _L)
                parts.append(jnp.concatenate(
                    [t[:, j].reshape(b - a, _L) for j in range(NCT)], axis=1))
            return parts[0] if len(parts) == 1 else jnp.concatenate(parts, axis=0)

        k0, r0 = divmod(side_total * NCT, r_w)
        cut_rest = _bounds(r_w, b_w, piece, shift_b, r0)
        rest_all, rest_up = pl.ds(k0, NBLK - k0), (pl.ds(k0 + 1, NBLK - k0 - 1), pl.ds(0, r0))
        c_wob = cp(wob_h.at[rest_up], wob_s.at[rest_up], S_GAPB)

        def start_c(b):
            start_pieces(c_h.at[b], c_s.at[b], cut_c, S_C + b)

        def pump_c(b):
            return _Pump(heads_of(c_h.at[b], c_s.at[b], i_c))

        def start_wqa():
            c_wob.start(priority=_BULK)
            start_pieces(wob_h.at[rest_all], wob_s.at[rest_all], cut_rest, S_WOB)
            start_pieces(wqa_h, wqa_s, cut_wqa, S_WQA)

        def start_k(g):
            start_pieces(k_h.at[pl.ds(g * _G, _G)], k_s.at[g], cut_k, S_KV + 2 * g, Sk - W)

        def start_v(g, cuts=cut_v):
            start_pieces(v_h.at[pl.ds(g * _G, _G)], v_s.at[g], cuts, S_KV + 2 * g + 1, Sk - W)

        def small_k(g):
            return heads_of(k_h.at[pl.ds(g * _G, _G)], k_s.at[g], i_k, Sk - W)

        def small_v(g):
            return heads_of(v_h.at[pl.ds(g * _G, _G)], v_s.at[g], i_v, Sk - W)

        def flat_at(lo, hi):
            assert lo // r_w == (hi - 1) // r_w
            return lo // r_w, pl.ds(lo % r_w, hi - lo)

        def c_wo(i):
            at = flat_at(wo_off[i] * NCT, (wo_off[i] + wo_chunks[i]) * NCT)
            return cp(woa_h.at[at], woa_s.at[at], S_WO + i)

        wide = pl.ds(wo_inj, wo_wide)
        gap = flat_at(n_inj, wo_inj * r_w)
        c_gap = cp(woa_h.at[gap], woa_s.at[gap], S_GAP)

        def start_wo():
            c_gap.start(priority=_BULK)
            start_pieces(woa_h.at[wide], woa_s.at[wide], cut_wo, S_WIDE)

        def small_wo():
            def one(lo, hi):
                return cp(woa_h.at[flat_at(lo, hi)], woa_s.at[flat_at(lo, hi)], S_INJ)
            return [functools.partial(one, lo, hi) for lo, hi in i_wo]

        def side_refs(i):
            per, n = r_m // side_rows, side_rows * NCT
            if isinstance(i, int):
                size = n if i < side_n else side_last * NCT
                rows = (i // per, pl.ds(i % per * n, size))
                return rows, side_s.at[i % side_nb, pl.ds(0, size)], i % side_nb
            slot = lax.rem(i, side_nb)
            start = pl.multiple_of(lax.rem(i, per) * n, 8)
            return (lax.div(i, per), pl.ds(start, n)), side_s.at[slot], slot

        def c_sa(i):
            rows, stage, slot = side_refs(i)
            return cp(wob_h.at[rows], stage, S_SA + slot)

        def c_sb(i):
            rows, stage, slot = side_refs(i)
            return cp(stage, wob_s.at[rows], S_SB + slot)

        def tick(i):
            traced = not isinstance(i, int)
            if traced or i < side_n:
                c_sa(i).wait()
                c_sb(i).start()

            def refill(j):
                if traced or i >= side_lag:
                    c_sb(i - side_lag).wait()
                c_sa(j).start()

            if traced:
                pl.when(i + side_lead < side_n)(lambda: refill(i + side_lead))
            elif i + side_lead < side_n:
                refill(i + side_lead)

        def head_major(w_s, t, hh, mid=lambda: None):
            halves = []
            for k in range(2):
                w = w_s[2 * t + k].reshape(_L // 2, Hb, Db)[:, hh * HH:(hh + 1) * HH, :]
                halves.append(w.reshape(_L // 2, HH * Db))
                if k == 0:
                    mid()
            return jnp.concatenate(halves, axis=0)

        start_pieces(wqb_h, wqb_s, cut_w0, S_WQB)
        c_xb.start()
        c_xa.start()
        for i in range(side_lead):
            c_sa(i).start()
        start_pieces(wuk_h, wuk_s, cut_w, S_WUK)
        pm = _Pump(heads_of(wuk_h, wuk_s, i_w))
        pm.pump(*cfg["pump_0"])
        pm.drain()


        wait_pieces(wqb_s, cut_w0, S_WQB)
        start_c(0)
        pm = pump_c(0)
        pm.kick()
        tick(0)
        c_xb.wait()
        xb = xb_s[...]
        halves = [None, None]
        for t in range(M // _L):
            for hh in range(2):
                part = _dot(xb[:, t * _L:(t + 1) * _L], head_major(wqb_s, t, hh, pm.kick))
                halves[hh] = part if t == 0 else halves[hh] + part
                pm.kick()
        ctxb_s[...] = jnp.concatenate(halves, axis=1)
        pm.pump(*cfg["pump_w"])
        pm.drain()

        wait_pieces(wuk_s, cut_w, S_WUK)
        start_c(1)
        pm = pump_c(1)
        pm.kick()
        tick(1)
        qb = (ctxb_s[...] * scale_b).astype(_BF16)
        for t in range(NCT):
            for hh in range(2):
                w = head_major(wuk_s, t, hh, pm.kick)
                parts = [_dot_nt(qb[:, (hh * HH + j) * Db:(hh * HH + j + 1) * Db],
                                 w[:, j * Db:(j + 1) * Db]) for j in range(HH)]
                qabs_s[t, :, hh * HH:(hh + 1) * HH, :] = jnp.concatenate(
                    parts, axis=1).reshape(B, HH, _L)
                pm.kick()
        pm.pump(*cfg["pump_w"])
        pm.drain()

        def attend_b(b, start_next, pm):
            wait_pieces(c_s.at[b], cut_c, S_C + b)
            start_next()
            pm.kick()
            tick(2 + b)
            qa = jnp.concatenate(
                [qabs_s[t, b] for t in range(NCT)], axis=1).astype(_BF16)
            for k in range(NBLK):
                s_s[:, k * r_m:(k + 1) * r_m] = _dot_nt(
                    qa, rows_of(c_s.at[b], k * r_m, (k + 1) * r_m))
                if k in cfg["kick_s"]:
                    pm.kick()
            s = s_s[...]
            m = jnp.max(s, axis=-1, keepdims=True)
            p = jnp.exp(s - m)
            l = jnp.sum(p, axis=-1, keepdims=True)
            pb = p.astype(_BF16)
            cc = None
            for k in range(NBLK):
                part = _dot(pb[:, k * r_m:(k + 1) * r_m],
                            rows_of(c_s.at[b], k * r_m, (k + 1) * r_m))
                cc = part if cc is None else cc + part
                if k in cfg["kick_c"]:
                    pm.kick()
            cc = cc / l
            for t in range(NCT):
                ctx_s[t, b] = cc[:, t * _L:(t + 1) * _L]
            pm.pump(*cfg["pump_c"])
            pm.drain()

        small_wqa = heads_of(wqa_h, wqa_s, i_wqa)
        n_q = len(small_wqa) // 2
        for b in range(B):
            if b + 2 < B:
                attend_b(b, functools.partial(start_c, b + 2), pump_c(b + 2))
            elif b + 2 == B:
                attend_b(b, functools.partial(start_pieces, wuv_h, wuv_s, cut_w, S_WUV),
                         _Pump(heads_of(wuv_h, wuv_s, i_w)))
            else:
                attend_b(b, start_wqa, _Pump(small_wqa[:n_q] + small_k(0)))

        wait_pieces(wuv_s, cut_w, S_WUV)
        start_k(0)
        start_v(0)
        pm = _Pump(small_v(0)[:1] + small_wqa[n_q:] + small_v(0)[1:] + small_k(1))
        pm.kick()
        tick(2 + B)
        halves = [None, None]
        for t in range(NCT):
            for hh in range(2):
                ch = ctx_s[t, :, hh * HH:(hh + 1) * HH, :].reshape(B, HH * _L).astype(_BF16)
                w = head_major(wuv_s, t, hh, pm.kick)
                part = jnp.concatenate(
                    [_dot(ch[:, j * _L:(j + 1) * _L], w[:, j * Db:(j + 1) * Db])
                     for j in range(HH)], axis=1)
                halves[hh] = part if t == 0 else halves[hh] + part
                pm.kick()
        ctxb_s[...] = jnp.concatenate(halves, axis=1)
        pm.pump(*cfg["pump_uv"])
        pm.drain()

        wait_pieces(wqa_s, cut_wqa, S_WQA)
        start_k(1)
        pm = _Pump(small_v(1))
        pm.kick()
        tick(3 + B)
        c_xa.wait()
        xa = xa_s[...]
        wq_tiles = wqa_s[...].reshape(D // 8, n_ct, 8, _L)
        qa_all = jnp.concatenate(
            [_dot(xa, wq_tiles[:, ct].reshape(D, _L)) for ct in range(n_ct)], axis=1) * scale_a
        qa_s[...] = qa_all.reshape(B, H, Dh).reshape(BH, Dh)
        pm.pump(*cfg["pump_q"])
        pm.drain()

        def attend_a(g, start_at_k, start_at_v, kick, between, v_cuts=cut_v):
            start = g * _G if isinstance(g, int) else pl.multiple_of(g * _G, _G)
            rows = pl.ds(start, _G)
            q8 = qa_s[rows, :].astype(_BF16)
            wait_pieces(k_s.at[g], cut_k, S_KV + 2 * g)
            start_at_k()
            kick()
            tick(4 + B + g)
            row = lax.broadcasted_iota(jnp.int32, (_G, W), 0)
            s = None
            for j in range(_G):
                sj = _dot_nt(q8, k_s[g, j])
                s = sj if s is None else jnp.where(row == j, sj, s)
                if j in cfg["kick_qk"]:
                    kick()
            m = jnp.max(s, axis=-1, keepdims=True)
            p = jnp.exp(s - m)
            l = jnp.sum(p, axis=-1, keepdims=True)
            p_s[...] = p
            between()
            wait_pieces(v_s.at[g], v_cuts, S_KV + 2 * g + 1)
            start_at_v()
            kick()
            pb = p_s[...].astype(_BF16)
            row2 = lax.broadcasted_iota(jnp.int32, (_G, Dh), 0)
            o = None
            for j in range(_G):
                oj = _dot(pb, v_s[g, j])
                o = oj if o is None else jnp.where(row2 == j, oj, o)
                if j in cfg["kick_pv"]:
                    kick()
            oa_s[rows, :] = o / l

        def a_body(g, carry):
            pm = _Pump(small_k(g + 2) + small_v(g + 2))
            attend_a(g, functools.partial(start_v, g + 1), functools.partial(start_k, g + 2),
                     pm.kick, functools.partial(pm.pump, *cfg["pump_k"]))
            pm.pump(*cfg["pump_v"])
            pm.drain()
            return carry

        lax.fori_loop(0, NG - 2, a_body, 0)

        waited = side_n - side_nb
        n_early = side_n - cfg["side_mid"]
        r_early, r_mid = n_early * side_rows, side_n * side_rows

        def spin(trips):
            spin_s[0] = lax.fori_loop(0, trips, lambda i, c: c * 3 + i, spin_s[0])

        spin_s[0] = 0
        pm = _Pump(small_wo(), spin)
        last = pl.ds((NG - 1) * _G, _G)
        pv = _Pump(heads_of(v_h.at[last], v_s.at[NG - 1], i_vl, Sk - W, S_INJ2))

        def project_b():
            c_wob.wait()
            wait_pieces(wob_s.at[rest_all], cut_rest, S_WOB)
            for i in range(waited, n_early):
                c_sb(i).wait()
            ctxb = ctxb_s[...].astype(_BF16)
            acc = _dot(ctxb[:, side_total:], rows_of(wob_s, side_total, Hb * Db))
            for lo in range(0, r_early, cfg["seg_b"]):
                pm.kick()
                hi = min(lo + cfg["seg_b"], r_early)
                acc = acc + _dot(ctxb[:, lo:hi], rows_of(wob_s, lo, hi))
            accb_s[...] = acc

        def start_tail():
            for i in range(n_wo):
                c_wo(i).start(priority=_BULK)
            pm.pump(1, cfg["lag"])

        def before_last_pv():
            pm.pace(*cfg["pump_k15"])
            pv.drain()

        attend_a(NG - 2, functools.partial(start_v, NG - 1, cut_vl), start_wo,
                 pv.kick, functools.partial(pm.pace, *cfg["pump_k14"]))
        project_b()
        pm.pace(*cfg["pump_b"])
        attend_a(NG - 1, lambda: c_sa(side_n).start(), start_tail, pv.kick, before_last_pv, cut_vl)
        pm.pump(1, cfg["lag"])

        oa32 = oa_s[...].reshape(B, H, Dh).reshape(B, H * Dh)
        oab_s[...] = oa32
        tail0 = H * Dh - tail_rows
        for b in range(B):
            for t in range(tail_rows // Dh):
                src = oa32[b:b + 1, tail0 + t * Dh:tail0 + (t + 1) * Dh]
                coef_s[b, t * Dh:(t + 1) * Dh, :] = jnp.broadcast_to(src, (_L, Dh)).T
        pm.pace(*cfg["pump_e"])
        c_sa(side_n).wait()
        c_sb(side_n).start()
        pm.pace(*cfg["pump_f"])
        pm.drain()
        oa = oab_s[...].astype(_BF16)
        c_gap.wait()
        n_head = wo_inj * r_m
        acc_s[...] = _dot(oa[:, :n_head], rows_of(woa_s, 0, n_head))
        for j in range(n_early, side_n):
            c_sb(j).wait()
        accb_s[...] += _dot(ctxb_s[:, r_early:r_mid].astype(_BF16), rows_of(wob_s, r_early, r_mid))
        wait_pieces(woa_s.at[wide], cut_wo, S_WIDE)
        acc_s[...] += _dot(oa[:, n_head:wo_base], rows_of(woa_s, n_head, wo_base))
        for i in range(n_mxu):
            c_wo(i).wait()
            if i == late_at:
                c_sb(side_n).wait()
                late = _dot(ctxb_s[:, r_mid:side_total].astype(_BF16),
                            rows_of(wob_s, r_mid, side_total))
                o_ref[:, D:] = (accb_s[...] + late).astype(o_ref.dtype)
            lo, n = wo_off[i], wo_chunks[i]
            acc_s[...] += _dot(oa[:, lo:lo + n], rows_of(woa_s, lo, lo + n))
        for i in range(n_mxu, n_wo):
            c_wo(i).wait()
            lo, n = wo_off[i], wo_chunks[i]
            w = rows_of(woa_s, lo, lo + n, _F32)
            sums = []
            for b in range(B):
                cf = coef_s[b, lo - tail0:lo - tail0 + n, :]
                prod = w * jnp.concatenate([cf] * (D // _L), axis=1)
                acc = vacc_s[b] if i > n_mxu else None
                for r in range(0, n, 8):
                    acc = prod[r:r + 8] if acc is None else acc + prod[r:r + 8]
                if i < n_wo - 1:
                    vacc_s[b] = acc
                else:
                    sums.append(jnp.sum(acc, axis=0, keepdims=True))
            if i == n_wo - 1:
                res = acc_s[...] + jnp.concatenate(sums, axis=0)
                o_ref[:, :D] = res.astype(o_ref.dtype)

    any_spec = pl.BlockSpec(memory_space=pl.ANY)
    out = pl.pallas_call(
        kernel,
        out_shape=jax.ShapeDtypeStruct((B, D + M), A_x.dtype),
        in_specs=[any_spec] * 11,
        out_specs=pl.BlockSpec(memory_space=pltpu.VMEM),
        scratch_shapes=[
            pltpu.VMEM(xa2.shape, _BF16),
            pltpu.VMEM(xb2.shape, _BF16),
            pltpu.VMEM((2, NG, _G, W, Dh), _BF16),
            pltpu.VMEM((6 + B,) + wqa3.shape, _BF16),
            pltpu.VMEM((BH, Dh), _F32),
            pltpu.VMEM((BH, Dh), _F32),
            pltpu.VMEM((NCT, B, Hb, _L), _F32),
            pltpu.VMEM((NCT, B, Hb, _L), _F32),
            pltpu.VMEM((B, D), _F32),
            pltpu.VMEM((B, M), _F32),
            pltpu.VMEM((B, Hb * Db), _F32),
            pltpu.VMEM((B, H * Dh), _F32),
            pltpu.VMEM((B, tail_rows, _L), _F32),
            pltpu.VMEM((B, 8, D), _F32),
            pltpu.VMEM((_G, W), _F32),
            pltpu.VMEM((Hb, Skb), _F32),
            pltpu.SMEM((side_nb, side_rows * NCT, _L), _BF16),
            pltpu.SMEM((1,), jnp.int32),
            pltpu.SemaphoreType.DMA((n_sem,)),
        ],
        compiler_params=pltpu.CompilerParams(
            vmem_limit_bytes=120 * 1024 * 1024,
            disable_semaphore_checks=True,
            disable_bounds_checks=True,
        ),
        name="fused_decode",
    )(xa2, k3, v3, wqa3, woa3, xb2, c4, wqb4, wuk4, wuv4, wob3)
    return out.reshape(B, Sq, D + M)


@jax.jit
def pallas_concat_heads__sliding_block_cached__compressed_kv_cla__decode_kernel(
    A_x: jax.Array,
    A_k_cache: jax.Array,
    A_v_cache: jax.Array,
    A_wq: jax.Array,
    A_wo: jax.Array,
    B_x: jax.Array,
    B_c_kv: jax.Array,
    B_w_q: jax.Array,
    B_w_uk: jax.Array,
    B_w_uv: jax.Array,
    B_w_o: jax.Array,
):
    return _fused(_CFG, A_x, A_k_cache, A_v_cache, A_wq, A_wo,
                  B_x, B_c_kv, B_w_q, B_w_uk, B_w_uv, B_w_o)
```
